```python
import jax
import jax.numpy as jnp

def _softmax(x, axis=-1):
    return jax.nn.softmax(x, axis=axis)
def _gelu(x):
    return jax.nn.gelu(x, approximate=True)
def _silu(x):
    return jax.nn.silu(x)
def _sigmoid(x):
    return jax.nn.sigmoid(x)
def _layernorm(x, axis=-1, eps=1e-5):
    m = jnp.mean(x, axis=axis, keepdims=True)
    v = jnp.var(x, axis=axis, keepdims=True)
    return (x - m) / jnp.sqrt(v + eps)
def _scatter_add(tgt, idx, src, axis=0):
    return tgt.at[idx].add(src)
def _segment_sum(src, seg, n):
    return jax.ops.segment_sum(src, seg, n)
class _Rng:
    def __init__(self, key):
        self._k = key
    def _next(self):
        self._k, sub = jax.random.split(self._k)
        return sub
    def normal(self, shape):
        return jax.random.normal(self._next(), shape, dtype=jnp.bfloat16)
    def randint(self, lo, hi, shape):
        return jax.random.randint(self._next(), shape, lo, hi, dtype=jnp.int32)
    def uniform(self, shape, lo=0.0, hi=1.0):
        return jax.random.uniform(self._next(), shape, jnp.bfloat16, lo, hi)
    def permutation(self, n):
        return jax.random.permutation(self._next(), n)


kernel_name = 'interleave_layers__sliding_local_dilated__softmax_full_mha__prompt'

def setup_inputs():
    _rng = _Rng(jax.random.key(int.from_bytes(__import__("os").urandom(4), "little")))
    _w = (lambda a: (lambda t: t.astype(jnp.bfloat16) if jnp.issubdtype(t.dtype, jnp.floating) else t)(jnp.asarray(a)))
    def _A_setup():
        B, S, D = 1, 2048, 1024
        return {
            "x": _w((lambda *s: _rng.normal(s) * 0.05)(B, S, D)),
            "wqkv": _w((lambda *s: _rng.normal(s) * 0.05)(D, 3 * D)),
            "wo": _w((lambda *s: _rng.normal(s) * 0.05)(D, D)),
        }
    _A_in = _A_setup()

    def _B_setup():
        B, S, D = 1, 2048, 1024
        return {
            "x": _w((lambda *s: _rng.normal(s) * 0.05)(B, S, D)),
            "wqkv": _w((lambda *s: _rng.normal(s) * 0.05)(D, 3 * D)),
            "wo": _w((lambda *s: _rng.normal(s) * 0.05)(D, D)),
        }
    _B_in = _B_setup()

    return {
        "A_x": _A_in["x"],
        "A_wqkv": _A_in["wqkv"],
        "A_wo": _A_in["wo"],
        "B_x": _B_in["x"],
        "B_wqkv": _B_in["wqkv"],
        "B_wo": _B_in["wo"],
    }

def reference(A_x, A_wqkv, A_wo, B_x, B_wqkv, B_wo):
    def _A_ref(x, wqkv, wo):
        B, S, D = x.shape
        H = 32; Dh = D // H
        W, dil = 8, 2
        qkv = (lambda x, *d: x.transpose(*d))((x @ wqkv).reshape(B, S, 3, H, Dh), 2, 0, 3, 1, 4)
        q, k, v = qkv[0], qkv[1], qkv[2]
        scale = Dh ** -0.5
        pos = jnp.arange(S)
        off = jnp.arange(W) * dil
        idx = pos[:, None] - off[None, :]
        mask = idx >= 0
        idx_c = jnp.where(mask, idx, 0).reshape(-1)
        kg = k[:, :, idx_c, :].reshape(B, H, S, W, Dh)
        vg = v[:, :, idx_c, :].reshape(B, H, S, W, Dh)
        logits = jnp.einsum("bhsd,bhswd->bhsw", q, kg) * scale
        logits = jnp.where(mask[None, None, :, :], logits, -1e9)
        attn = _softmax(logits, axis=-1)
        o = jnp.einsum("bhsw,bhswd->bhsd", attn, vg)
        return (lambda x, *d: x.transpose(*d))(o, 0, 2, 1, 3).reshape(B, S, D) @ wo

    def _B_ref(x, wqkv, wo):
        B, S, D = x.shape
        H = 32; Dh = D // H
        qkv = (lambda x, *d: x.transpose(*d))((x @ wqkv).reshape(B, S, 3, H, Dh), 2, 0, 3, 1, 4)
        q, k, v = qkv[0], qkv[1], qkv[2]
        scale = Dh ** -0.5
        scores = jnp.einsum("bhqd,bhkd->bhqk", q, k) * scale
        p = _softmax(scores, axis=-1)
        o = jnp.einsum("bhqk,bhkd->bhqd", p, v)
        return (lambda x, *d: x.transpose(*d))(o, 0, 2, 1, 3).reshape(B, S, D) @ wo

    x = A_x
    x = x + _A_ref(_layernorm(x, axis=-1), A_wqkv, A_wo)
    x = x + _B_ref(_layernorm(x, axis=-1), B_wqkv, B_wo)
    x = x + _A_ref(_layernorm(x, axis=-1), A_wqkv, A_wo)
    x = x + _B_ref(_layernorm(x, axis=-1), B_wqkv, B_wo)
    return x
```

```python
import functools
import math

import jax
import jax.numpy as jnp
from jax import lax
import jax.experimental.pallas as pl
import jax.experimental.pallas.tpu as pltpu

S = 2048
D = 1024
H = 32
DH = 32
WIN = 8
DIL = 2
EPS = 1e-5
NT = D // 128
HALO = 16
QSCALE = (DH ** -0.5) * math.log2(math.e)

SB = 128
NSUB = 2
RB = SB * NSUB
RC = 32
TQ = 512
KC = 256
NC = S // KC
L_MAX = 2.0 ** 64

bf16 = jnp.bfloat16
f32 = jnp.float32
u32 = jnp.uint32

NN = (((1,), (0,)), ((), ()))
NTD = (((1,), (1,)), ((), ()))


def _pack(x):
    return pltpu.bitcast(x, u32)


def _unpack(x):
    return pltpu.bitcast(x, bf16)


def _layernorm(x):
    mu = jnp.mean(x, axis=-1, keepdims=True)
    xc = x - mu
    var = jnp.mean(xc * xc, axis=-1, keepdims=True)
    return (xc * lax.rsqrt(var + EPS)).astype(bf16)


def _kernel(x_ref, wa_ref, woa_ref, wqvt_ref, wk_ref, wob_ref, out_ref,
            xs, qa, ka, va, qt, kb, vt, ob, ot):
    xs[...] = x_ref[...].astype(f32)

    def local_attn(r0, s):
        outs = []
        for c in range(SB // RC):
            base = s * SB + c * RC
            q = [qa[t, base:base + RC, :] for t in range(NT)]
            logits = []
            for w in range(WIN):
                o0 = HALO + base - DIL * w
                acc = q[0] * ka[0, o0:o0 + RC, :]
                for t in range(1, NT):
                    acc = acc + q[t] * ka[t, o0:o0 + RC, :]
                acc = acc + pltpu.roll(acc, 64, 1)
                acc = acc + pltpu.roll(acc, 32, 1)
                if base == 0 and w > 0:
                    row = r0 + lax.broadcasted_iota(jnp.int32, (RC, 128), 0)
                    acc = jnp.where(row >= DIL * w, acc, -1e9)
                logits.append(acc)
            m = functools.reduce(jnp.maximum, logits)
            p = [jnp.exp2(lg - m) for lg in logits]
            inv = 1.0 / functools.reduce(lambda a, b: a + b, p)
            p = [pw * inv for pw in p]
            tiles = []
            for t in range(NT):
                acc = None
                for w in range(WIN):
                    o0 = HALO + base - DIL * w
                    term = p[w] * va[t, o0:o0 + RC, :]
                    acc = term if acc is None else acc + term
                tiles.append(acc.astype(bf16))
            outs.append(jnp.concatenate(tiles, axis=1))
        return jnp.concatenate(outs, axis=0)

    def row_body(r, carry):
        r0 = pl.multiple_of(r * RB, RB)
        rows = [pl.ds(r0 + s * SB, SB) for s in range(NSUB)]
        xn = [_layernorm(xs[rows[s], :]) for s in range(NSUB)]
        for s in range(NSUB):
            y = lax.dot_general(xn[s], wa_ref[...], NN, preferred_element_type=f32)
            for t in range(NT):
                qa[t, s * SB:(s + 1) * SB, :] = y[:, t * 128:(t + 1) * 128] * QSCALE
                ka[t, HALO + s * SB:HALO + (s + 1) * SB, :] = y[:, D + t * 128:D + (t + 1) * 128]
                va[t, HALO + s * SB:HALO + (s + 1) * SB, :] = y[:, 2 * D + t * 128:2 * D + (t + 1) * 128]
        xn2 = []
        for s in range(NSUB):
            o = local_attn(r0, s)
            x1 = xs[rows[s], :] + lax.dot_general(o, woa_ref[...], NN, preferred_element_type=f32)
            xs[rows[s], :] = x1
            xn2.append(_layernorm(x1))
        ka[:, 0:HALO, :] = ka[:, RB:RB + HALO, :]
        va[:, 0:HALO, :] = va[:, RB:RB + HALO, :]
        for s in range(NSUB):
            cols = pl.ds(r0 + s * SB, SB)
            yq = lax.dot_general(wqvt_ref[0:D, :], xn2[s], NTD, preferred_element_type=f32)
            qt[:, cols] = _pack((yq * QSCALE).astype(bf16))
            yv = lax.dot_general(wqvt_ref[D:2 * D, :], xn2[s], NTD, preferred_element_type=f32)
            vt[:, cols] = _pack(yv.astype(bf16))
            yk = lax.dot_general(xn2[s], wk_ref[...], NN, preferred_element_type=f32).astype(bf16)
            krows = pl.ds(pl.multiple_of((r0 + s * SB) // 2, SB // 2), SB // 2)
            for g in range(NT):
                kb[g, krows, :] = _pack(yk[:, g * 128:(g + 1) * 128])
        return carry

    def head_weights(g, hh, q0):
        w = qt[pl.ds(pl.multiple_of(g * 64 + hh * 16, 16), 16), pl.ds(q0, TQ)]
        parts = []
        if hh > 0:
            parts.append(jnp.zeros((16 * hh, TQ), u32))
        parts.append(w)
        if hh < 3:
            parts.append(jnp.zeros((16 * (3 - hh), TQ), u32))
        return _unpack(jnp.concatenate(parts, axis=0))

    def ref_max(g, q0):
        k0 = kb[g, 0:8, :]
        lane = lax.broadcasted_iota(jnp.int32, (8, 128), 1) // DH
        lhs = jnp.concatenate(
            [jnp.where(lane == hh, k0, jnp.zeros_like(k0)) for hh in range(4)], axis=0)
        w = _unpack(qt[pl.ds(pl.multiple_of(g * 64, 64), 64), pl.ds(q0, TQ)])
        s0 = jnp.dot(_unpack(lhs), w, preferred_element_type=f32)
        return jnp.concatenate(
            [jnp.broadcast_to(jnp.max(s0[16 * hh:16 * hh + 16], axis=0, keepdims=True), (8, TQ))
             for hh in range(4)], axis=0)

    def store_group(g, q0, o_t):
        ob[g, pl.ds(pl.multiple_of(q0 // 2, TQ // 2), TQ // 2), :] = _pack(o_t.T.astype(bf16))

    def attn_fast(q0):
        def group(g, carry):
            m_all, lmax = carry
            st = {}
            outs = []

            def qk(hh, c):
                if c == 0:
                    st[hh] = dict(w=head_weights(g, hh, q0), l=None, acc=None)
                kc = _unpack(kb[g, c * KC // 2:(c + 1) * KC // 2, :])
                return jnp.dot(kc, st[hh]["w"], preferred_element_type=f32)

            def pv(hh, c, s):
                d = st[hh]
                m = m_all[8 * hh:8 * hh + 8]
                p = jnp.exp2(s.reshape(KC // 8, 8, TQ) - m[None])
                lc = jnp.sum(p, axis=0)
                vc = _unpack(vt[pl.ds(pl.multiple_of(g * 64 + hh * 16, 16), 16), c * KC:(c + 1) * KC])
                o = jnp.dot(vc, p.reshape(KC, TQ).astype(bf16), preferred_element_type=f32)
                d["l"] = lc if c == 0 else d["l"] + lc
                d["acc"] = o if c == 0 else d["acc"] + o
                if c == NC - 1:
                    l = jnp.sum(d["l"], axis=0, keepdims=True)
                    d["lsum"] = l
                    outs.append(d["acc"] * (1.0 / l))

            m_next = None
            pend = None
            for hh in range(4):
                for c in range(NC):
                    if hh == 3 and c == 0:
                        m_next = ref_max(jnp.minimum(g + 1, NT - 1), q0)
                    s = qk(hh, c)
                    if pend is not None:
                        pv(*pend)
                    pend = (hh, c, s)
            pv(*pend)
            store_group(g, q0, jnp.concatenate(outs, axis=0))
            for hh in range(4):
                lmax = jnp.maximum(lmax, st[hh]["lsum"])
            return m_next, lmax

        _, lmax = lax.fori_loop(0, NT, group, (ref_max(0, q0), jnp.zeros((1, TQ), f32)))
        return lmax

    def attn_exact(q0):
        def group(g, carry):
            def head(hh, carry2):
                w = qt[pl.ds(pl.multiple_of(g * 64, 64), 64), pl.ds(q0, TQ)]
                row = lax.broadcasted_iota(jnp.int32, (64, TQ), 0) // 16
                w = _unpack(jnp.where(row == hh, w, jnp.zeros_like(w)))
                s = jnp.dot(_unpack(kb[g]), w, preferred_element_type=f32)
                p = jnp.exp2(s - jnp.max(s, axis=0, keepdims=True))
                l = jnp.sum(p, axis=0, keepdims=True)
                v = _unpack(vt[pl.ds(pl.multiple_of(g * 64 + hh * 16, 16), 16), :])
                o = jnp.dot(v, p.astype(bf16), preferred_element_type=f32)
                ot[pl.ds(pl.multiple_of(hh * DH, DH), DH), :] = o * (1.0 / l)
                return carry2
            lax.fori_loop(0, 4, head, 0)
            store_group(g, q0, ot[...])
            return carry
        lax.fori_loop(0, NT, group, 0)

    def q_body(qb, carry):
        q0 = pl.multiple_of(qb * TQ, TQ)
        lmax = attn_fast(q0)
        unsafe = jnp.max(jnp.where(lmax <= L_MAX, 0, 1))

        @pl.when(unsafe > 0)
        def _():
            attn_exact(q0)

        orows = pl.ds(pl.multiple_of(q0 // 2, TQ // 2), TQ // 2)
        o = jnp.concatenate([_unpack(ob[g, orows, :]) for g in range(NT)], axis=1)
        x2 = xs[pl.ds(q0, TQ), :] + lax.dot_general(o, wob_ref[...], NN, preferred_element_type=f32)
        xs[pl.ds(q0, TQ), :] = x2
        out_ref[pl.ds(q0, TQ), :] = x2.astype(bf16)
        return carry

    def layer_pair(l, carry):
        ka[:, 0:HALO, :] = jnp.zeros((NT, HALO, 128), f32)
        va[:, 0:HALO, :] = jnp.zeros((NT, HALO, 128), f32)
        lax.fori_loop(0, S // RB, row_body, 0)
        lax.fori_loop(0, S // TQ, q_body, 0)
        return carry

    lax.fori_loop(0, 2, layer_pair, 0)


@jax.jit
def pallas_interleave_layers__sliding_local_dilated__softmax_full_mha__prompt_kernel(
    A_x: jax.Array,
    A_wqkv: jax.Array,
    A_wo: jax.Array,
    B_x: jax.Array,
    B_wqkv: jax.Array,
    B_wo: jax.Array,
):
    del B_x
    x = A_x.reshape(S, D)
    wa = A_wqkv.reshape(D, 3, H, DH).transpose(0, 1, 3, 2).reshape(D, 3 * D)
    woa = A_wo.reshape(H, DH, D).transpose(1, 0, 2).reshape(D, D)
    wqvt = jnp.concatenate([B_wqkv[:, :D].T, B_wqkv[:, 2 * D:].T], axis=0)
    wk = B_wqkv[:, D:2 * D]
    out = pl.pallas_call(
        _kernel,
        out_shape=jax.ShapeDtypeStruct((S, D), bf16),
        scratch_shapes=[
            pltpu.VMEM((S, D), f32),
            pltpu.VMEM((NT, RB, 128), f32),
            pltpu.VMEM((NT, HALO + RB, 128), f32),
            pltpu.VMEM((NT, HALO + RB, 128), f32),
            pltpu.VMEM((D // 2, S), u32),
            pltpu.VMEM((NT, S // 2, 128), u32),
            pltpu.VMEM((D // 2, S), u32),
            pltpu.VMEM((NT, S // 2, 128), u32),
            pltpu.VMEM((128, TQ), f32),
        ],
        compiler_params=pltpu.CompilerParams(vmem_limit_bytes=110 * 1024 * 1024),
    )(x, wa, woa, wqvt, wk, B_wo)
    return out.reshape(1, S, D)
```

```python
import functools
import math

import jax
import jax.numpy as jnp
from jax import lax
import jax.experimental.pallas as pl
import jax.experimental.pallas.tpu as pltpu

S = 2048
D = 1024
H = 32
DH = 32
WIN = 8
DIL = 2
EPS = 1e-5
NT = D // 128
HALO = 16
QSCALE = (DH ** -0.5) * math.log2(math.e)

SB = 128
NSUB = 2
RB = SB * NSUB
RC = 32
TQ = 512
KC = 256
NC = S // KC
WCH = 512
NFLIGHT = 2
L_MAX = 2.0 ** 64

bf16 = jnp.bfloat16
f32 = jnp.float32
u32 = jnp.uint32

NN = (((1,), (0,)), ((), ()))
NTD = (((1,), (1,)), ((), ()))


def _pack(x):
    return pltpu.bitcast(x, u32)


def _unpack(x):
    return pltpu.bitcast(x, bf16)


def _layernorm(x):
    mu = jnp.mean(x, axis=-1, keepdims=True)
    xc = x - mu
    var = jnp.mean(xc * xc, axis=-1, keepdims=True)
    return (xc * lax.rsqrt(var + EPS)).astype(bf16)


def _kernel(x_hbm, wa_hbm, woa_hbm, wb_hbm, wob_hbm, out_hbm,
            xin, wa_raw, woa_raw, wb_raw, wob, outb,
            wat, woa, wqvt,
            xs, qa, ka, va, qt, kb, vt, ob, ot,
            sem_x, sem_wa, sem_w, sem_o):
    def x_copy(r):
        rows = pl.ds(r * RB, RB)
        return pltpu.make_async_copy(x_hbm.at[rows, :], xin.at[rows, :], sem_x.at[r])

    def wa_copy(i):
        cols = pl.ds(i * WCH, WCH)
        return pltpu.make_async_copy(wa_hbm.at[:, cols], wa_raw.at[:, cols], sem_wa.at[i])

    def wb_copy(i):
        cols = pl.ds(i * D, D)
        return pltpu.make_async_copy(wb_hbm.at[:, cols], wb_raw.at[:, cols], sem_w.at[i])

    woa_copy = pltpu.make_async_copy(woa_hbm, woa_raw, sem_w.at[3])
    wob_copy = pltpu.make_async_copy(wob_hbm, wob, sem_w.at[4])

    def out_copy(qb):
        rows = pl.ds(pl.multiple_of(qb * TQ, TQ), TQ)
        return pltpu.make_async_copy(outb.at[rows, :], out_hbm.at[rows, :], sem_o.at[qb])

    queue = ([wa_copy(i) for i in range(3 * D // WCH)]
             + [woa_copy, wb_copy(0), wb_copy(2), x_copy(0), wb_copy(1)]
             + [x_copy(r) for r in range(1, S // RB)] + [wob_copy])

    def start_next(n):
        for _ in range(min(n, len(queue))):
            queue.pop(0).start()

    start_next(NFLIGHT)

    ri = lax.broadcasted_iota(jnp.int32, (256, 256), 0)
    ci = lax.broadcasted_iota(jnp.int32, (256, 256), 1)
    sel = jnp.where(ci == (ri % 8) * DH + ri // 8, 1.0, 0.0).astype(bf16)
    eye = jnp.where(ri == ci, 1.0, 0.0).astype(bf16)[0:128, 0:128]

    def pair(a0, a1):
        both = jnp.concatenate([a0.reshape(DH, 8, D), a1.reshape(DH, 8, D)], axis=1)
        return _pack(both.reshape(DH * 16, D).astype(bf16)).reshape(DH, 8, D)

    for i in range(3 * D // WCH):
        wa_copy(i).wait()
        start_next(1)
        halves = [lax.dot_general(sel, wa_raw[:, i * WCH + j * 256:i * WCH + (j + 1) * 256], NTD,
                                  preferred_element_type=f32) for j in range(2)]
        wat[i // 2, :, i % 2, :, :] = pair(*halves)
    woa_copy.wait()
    start_next(1)
    for a in range(2):
        halves = [lax.dot_general(sel, woa_raw[a * 512 + j * 256:a * 512 + (j + 1) * 256, :], NN,
                                  preferred_element_type=f32) for j in range(2)]
        woa[:, a, :, :] = pair(*halves)
    for part, src in ((0, 0), (1, 2)):
        wb_copy(src).wait()
        start_next(1)
        for j in range(NT):
            wt = lax.dot_general(eye, wb_raw[:, src * D + j * 128:src * D + (j + 1) * 128], NTD,
                                 preferred_element_type=f32)
            wqvt[part * (D // 2) + j * 64:part * (D // 2) + (j + 1) * 64, :] = _pack(wt.astype(bf16))
    wb_copy(1).wait()
    start_next(len(queue))

    def local_attn(r0, s):
        outs = []
        for c in range(SB // RC):
            base = s * SB + c * RC
            q = [qa[t, base:base + RC, :] for t in range(NT)]
            logits = []
            for w in range(WIN):
                o0 = HALO + base - DIL * w
                acc = q[0] * ka[0, o0:o0 + RC, :]
                for t in range(1, NT):
                    acc = acc + q[t] * ka[t, o0:o0 + RC, :]
                acc = acc + pltpu.roll(acc, 64, 1)
                acc = acc + pltpu.roll(acc, 32, 1)
                if base == 0 and w > 0:
                    row = r0 + lax.broadcasted_iota(jnp.int32, (RC, 128), 0)
                    acc = jnp.where(row >= DIL * w, acc, -1e9)
                logits.append(acc)
            m = functools.reduce(jnp.maximum, logits)
            p = [jnp.exp2(lg - m) for lg in logits]
            inv = 1.0 / functools.reduce(lambda a, b: a + b, p)
            p = [pw * inv for pw in p]
            tiles = []
            for t in range(NT):
                acc = None
                for w in range(WIN):
                    o0 = HALO + base - DIL * w
                    term = p[w] * va[t, o0:o0 + RC, :]
                    acc = term if acc is None else acc + term
                tiles.append(acc.astype(bf16))
            outs.append(jnp.concatenate(tiles, axis=1))
        return jnp.concatenate(outs, axis=0)

    def row_body(r, l):
        r0 = pl.multiple_of(r * RB, RB)

        @pl.when(l == 0)
        def _():
            x_copy(r).wait()
            xs[pl.ds(r0, RB), :] = xin[pl.ds(r0, RB), :].astype(f32)

        rows = [pl.ds(r0 + s * SB, SB) for s in range(NSUB)]
        xn = [_layernorm(xs[rows[s], :]) for s in range(NSUB)]
        for s in range(NSUB):
            y = lax.dot_general(xn[s], _unpack(wat[...].reshape(3 * D // 2, D)), NTD,
                                preferred_element_type=f32)
            for t in range(NT):
                qa[t, s * SB:(s + 1) * SB, :] = y[:, t * 128:(t + 1) * 128] * QSCALE
                ka[t, HALO + s * SB:HALO + (s + 1) * SB, :] = y[:, D + t * 128:D + (t + 1) * 128]
                va[t, HALO + s * SB:HALO + (s + 1) * SB, :] = y[:, 2 * D + t * 128:2 * D + (t + 1) * 128]
        xn2 = []
        for s in range(NSUB):
            o = local_attn(r0, s)
            x1 = xs[rows[s], :] + lax.dot_general(o, _unpack(woa[...].reshape(D // 2, D)), NN,
                                                  preferred_element_type=f32)
            xs[rows[s], :] = x1
            xn2.append(_layernorm(x1))
        ka[:, 0:HALO, :] = ka[:, RB:RB + HALO, :]
        va[:, 0:HALO, :] = va[:, RB:RB + HALO, :]
        for s in range(NSUB):
            cols = pl.ds(r0 + s * SB, SB)
            yq = lax.dot_general(_unpack(wqvt[0:D // 2, :]), xn2[s], NTD, preferred_element_type=f32)
            qt[:, cols] = _pack((yq * QSCALE).astype(bf16))
            yv = lax.dot_general(_unpack(wqvt[D // 2:D, :]), xn2[s], NTD, preferred_element_type=f32)
            vt[:, cols] = _pack(yv.astype(bf16))
            yk = lax.dot_general(xn2[s], wb_raw[:, D:2 * D], NN, preferred_element_type=f32).astype(bf16)
            krows = pl.ds(pl.multiple_of((r0 + s * SB) // 2, SB // 2), SB // 2)
            for g in range(NT):
                kb[g, krows, :] = _pack(yk[:, g * 128:(g + 1) * 128])
        return l

    def head_weights(g, hh, q0):
        w = qt[pl.ds(pl.multiple_of(g * 64 + hh * 16, 16), 16), pl.ds(q0, TQ)]
        parts = []
        if hh > 0:
            parts.append(jnp.zeros((16 * hh, TQ), u32))
        parts.append(w)
        if hh < 3:
            parts.append(jnp.zeros((16 * (3 - hh), TQ), u32))
        return _unpack(jnp.concatenate(parts, axis=0))

    def ref_max(g, q0):
        k0 = kb[g, 0:8, :]
        lane = lax.broadcasted_iota(jnp.int32, (8, 128), 1) // DH
        lhs = jnp.concatenate(
            [jnp.where(lane == hh, k0, jnp.zeros_like(k0)) for hh in range(4)], axis=0)
        w = _unpack(qt[pl.ds(pl.multiple_of(g * 64, 64), 64), pl.ds(q0, TQ)])
        s0 = jnp.dot(_unpack(lhs), w, preferred_element_type=f32)
        return jnp.concatenate(
            [jnp.broadcast_to(jnp.max(s0[16 * hh:16 * hh + 16], axis=0, keepdims=True), (8, TQ))
             for hh in range(4)], axis=0)

    def store_group(g, q0, o_t):
        ob[g, pl.ds(pl.multiple_of(q0 // 2, TQ // 2), TQ // 2), :] = _pack(o_t.T.astype(bf16))

    def attn_fast(q0):
        def group(g, carry):
            m_all, lmax = carry
            st = {}
            outs = []

            def qk(hh, c):
                if c == 0:
                    st[hh] = dict(w=head_weights(g, hh, q0), l=None, acc=None)
                kc = _unpack(kb[g, c * KC // 2:(c + 1) * KC // 2, :])
                return jnp.dot(kc, st[hh]["w"], preferred_element_type=f32)

            def pv(hh, c, s):
                d = st[hh]
                m = m_all[8 * hh:8 * hh + 8]
                p = jnp.exp2(s.reshape(KC // 8, 8, TQ) - m[None])
                lc = jnp.sum(p, axis=0)
                vc = _unpack(vt[pl.ds(pl.multiple_of(g * 64 + hh * 16, 16), 16), c * KC:(c + 1) * KC])
                o = jnp.dot(vc, p.reshape(KC, TQ).astype(bf16), preferred_element_type=f32)
                d["l"] = lc if c == 0 else d["l"] + lc
                d["acc"] = o if c == 0 else d["acc"] + o
                if c == NC - 1:
                    l = jnp.sum(d["l"], axis=0, keepdims=True)
                    d["lsum"] = l
                    outs.append(d["acc"] * (1.0 / l))

            m_next = None
            pend = None
            for hh in range(4):
                for c in range(NC):
                    if hh == 3 and c == 0:
                        m_next = ref_max(jnp.minimum(g + 1, NT - 1), q0)
                    s = qk(hh, c)
                    if pend is not None:
                        pv(*pend)
                    pend = (hh, c, s)
            pv(*pend)
            store_group(g, q0, jnp.concatenate(outs, axis=0))
            for hh in range(4):
                lmax = jnp.maximum(lmax, st[hh]["lsum"])
            return m_next, lmax

        _, lmax = lax.fori_loop(0, NT, group, (ref_max(0, q0), jnp.zeros((1, TQ), f32)))
        return lmax

    def attn_exact(q0):
        def group(g, carry):
            def head(hh, carry2):
                w = qt[pl.ds(pl.multiple_of(g * 64, 64), 64), pl.ds(q0, TQ)]
                row = lax.broadcasted_iota(jnp.int32, (64, TQ), 0) // 16
                w = _unpack(jnp.where(row == hh, w, jnp.zeros_like(w)))
                s = jnp.dot(_unpack(kb[g]), w, preferred_element_type=f32)
                p = jnp.exp2(s - jnp.max(s, axis=0, keepdims=True))
                l = jnp.sum(p, axis=0, keepdims=True)
                v = _unpack(vt[pl.ds(pl.multiple_of(g * 64 + hh * 16, 16), 16), :])
                o = jnp.dot(v, p.astype(bf16), preferred_element_type=f32)
                ot[pl.ds(pl.multiple_of(hh * DH, DH), DH), :] = o * (1.0 / l)
                return carry2
            lax.fori_loop(0, 4, head, 0)
            store_group(g, q0, ot[...])
            return carry
        lax.fori_loop(0, NT, group, 0)

    def q_body(qb, l):
        q0 = pl.multiple_of(qb * TQ, TQ)
        lmax = attn_fast(q0)
        unsafe = jnp.max(jnp.where(lmax <= L_MAX, 0, 1))

        @pl.when(unsafe > 0)
        def _():
            attn_exact(q0)

        orows = pl.ds(pl.multiple_of(q0 // 2, TQ // 2), TQ // 2)
        o = jnp.concatenate([_unpack(ob[g, orows, :]) for g in range(NT)], axis=1)
        x2 = xs[pl.ds(q0, TQ), :] + lax.dot_general(o, wob[...], NN, preferred_element_type=f32)
        xs[pl.ds(q0, TQ), :] = x2
        outb[pl.ds(q0, TQ), :] = x2.astype(bf16)

        @pl.when(l == 1)
        def _():
            out_copy(qb).start()

        return l

    def layer_pair(l, carry):
        ka[:, 0:HALO, :] = jnp.zeros((NT, HALO, 128), f32)
        va[:, 0:HALO, :] = jnp.zeros((NT, HALO, 128), f32)
        lax.fori_loop(0, S // RB, row_body, l)

        @pl.when(l == 0)
        def _():
            wob_copy.wait()

        lax.fori_loop(0, S // TQ, q_body, l)
        return carry

    lax.fori_loop(0, 2, layer_pair, 0)
    for qb in range(S // TQ):
        out_copy(qb).wait()


@jax.jit
def pallas_interleave_layers__sliding_local_dilated__softmax_full_mha__prompt_kernel(
    A_x: jax.Array,
    A_wqkv: jax.Array,
    A_wo: jax.Array,
    B_x: jax.Array,
    B_wqkv: jax.Array,
    B_wo: jax.Array,
):
    del B_x
    x = A_x.reshape(S, D)
    hbm = pl.BlockSpec(memory_space=pl.ANY)
    out = pl.pallas_call(
        _kernel,
        out_shape=jax.ShapeDtypeStruct((S, D), bf16),
        in_specs=[hbm] * 5,
        out_specs=hbm,
        scratch_shapes=[
            pltpu.VMEM((S, D), bf16),
            pltpu.VMEM((D, 3 * D), bf16),
            pltpu.VMEM((D, D), bf16),
            pltpu.VMEM((D, 3 * D), bf16),
            pltpu.VMEM((D, D), bf16),
            pltpu.VMEM((S, D), bf16),
            pltpu.VMEM((3, DH, 2, 8, D), u32),
            pltpu.VMEM((DH, 2, 8, D), u32),
            pltpu.VMEM((D, D), u32),
            pltpu.VMEM((S, D), f32),
            pltpu.VMEM((NT, RB, 128), f32),
            pltpu.VMEM((NT, HALO + RB, 128), f32),
            pltpu.VMEM((NT, HALO + RB, 128), f32),
            pltpu.VMEM((D // 2, S), u32),
            pltpu.VMEM((NT, S // 2, 128), u32),
            pltpu.VMEM((D // 2, S), u32),
            pltpu.VMEM((NT, S // 2, 128), u32),
            pltpu.VMEM((128, TQ), f32),
            pltpu.SemaphoreType.DMA((S // RB,)),
            pltpu.SemaphoreType.DMA((3 * D // WCH,)),
            pltpu.SemaphoreType.DMA((5,)),
            pltpu.SemaphoreType.DMA((S // TQ,)),
        ],
        compiler_params=pltpu.CompilerParams(vmem_limit_bytes=110 * 1024 * 1024),
    )(x, A_wqkv, A_wo, B_wqkv, B_wo)
    return out.reshape(1, S, D)
```

```python
import functools
import math

import jax
import jax.numpy as jnp
from jax import lax
import jax.experimental.pallas as pl
import jax.experimental.pallas.tpu as pltpu

S = 2048
D = 1024
H = 32
DH = 32
WIN = 8
DIL = 2
EPS = 1e-5
NT = D // 128
HALO = 16
QSCALE = (DH ** -0.5) * math.log2(math.e)

SB = 128
NSUB = 2
RB = SB * NSUB
RC = 8
LOOK = 3
DEP_END = True
GATE_COL = 2 * D
TQ = 512
KC = 256
NC = S // KC
WCH = 512
NFLIGHT = 2
L_MAX = 2.0 ** 64

bf16 = jnp.bfloat16
f32 = jnp.float32
u32 = jnp.uint32

NN = (((1,), (0,)), ((), ()))
NTD = (((1,), (1,)), ((), ()))


def _pack(x):
    return pltpu.bitcast(x, u32)


def _unpack(x):
    return pltpu.bitcast(x, bf16)


def _layernorm(x):
    mu = jnp.mean(x, axis=-1, keepdims=True)
    xc = x - mu
    var = jnp.mean(xc * xc, axis=-1, keepdims=True)
    return (xc * lax.rsqrt(var + EPS)).astype(bf16)


def _kernel(x_hbm, wa_hbm, woa_hbm, wb_hbm, wob_hbm, out_hbm,
            xin, wa_raw, woa_raw, wb_raw, wob, outb,
            wat, woa, wqvt,
            xs, qa, ka, va, qt, kb, vt, ob, ot,
            sem_x, sem_wa, sem_w, sem_o):
    def x_copy(r):
        rows = pl.ds(r * RB, RB)
        return pltpu.make_async_copy(x_hbm.at[rows, :], xin.at[rows, :], sem_x.at[r])

    def wa_copy(i):
        cols = pl.ds(i * WCH, WCH)
        return pltpu.make_async_copy(wa_hbm.at[:, cols], wa_raw.at[:, cols], sem_wa.at[i])

    def wb_copy(i):
        cols = pl.ds(i * D, D)
        return pltpu.make_async_copy(wb_hbm.at[:, cols], wb_raw.at[:, cols], sem_w.at[i])

    woa_copy = pltpu.make_async_copy(woa_hbm, woa_raw, sem_w.at[3])
    wob_copy = pltpu.make_async_copy(wob_hbm, wob, sem_w.at[4])

    def out_copy(qb):
        rows = pl.ds(pl.multiple_of(qb * TQ, TQ), TQ)
        return pltpu.make_async_copy(outb.at[rows, :], out_hbm.at[rows, :], sem_o.at[qb])

    queue = ([wa_copy(i) for i in range(3 * D // WCH)]
             + [woa_copy, wb_copy(0), wb_copy(2), x_copy(0), wb_copy(1)]
             + [x_copy(r) for r in range(1, S // RB)] + [wob_copy])

    def start_next(n):
        for _ in range(min(n, len(queue))):
            queue.pop(0).start()

    start_next(NFLIGHT)

    ri = lax.broadcasted_iota(jnp.int32, (256, 256), 0)
    ci = lax.broadcasted_iota(jnp.int32, (256, 256), 1)
    sel = jnp.where(ci == (ri % 8) * DH + ri // 8, 1.0, 0.0).astype(bf16)
    eye = jnp.where(ri == ci, 1.0, 0.0).astype(bf16)[0:128, 0:128]

    def pair(a0, a1):
        both = jnp.concatenate([a0.reshape(DH, 8, D), a1.reshape(DH, 8, D)], axis=1)
        return _pack(both.reshape(DH * 16, D).astype(bf16)).reshape(DH, 8, D)

    for i in range(3 * D // WCH):
        wa_copy(i).wait()
        start_next(1)
        halves = [lax.dot_general(sel, wa_raw[:, i * WCH + j * 256:i * WCH + (j + 1) * 256], NTD,
                                  preferred_element_type=f32) for j in range(2)]
        wat[i // 2, :, i % 2, :, :] = pair(*halves)
    woa_copy.wait()
    start_next(1)
    for a in range(2):
        halves = [lax.dot_general(sel, woa_raw[a * 512 + j * 256:a * 512 + (j + 1) * 256, :], NN,
                                  preferred_element_type=f32) for j in range(2)]
        woa[:, a, :, :] = pair(*halves)
    for part, src in ((0, 0), (1, 2)):
        wb_copy(src).wait()
        start_next(1)
        for j in range(NT):
            wt = lax.dot_general(eye, wb_raw[:, src * D + j * 128:src * D + (j + 1) * 128], NTD,
                                 preferred_element_type=f32)
            wqvt[part * (D // 2) + j * 64:part * (D // 2) + (j + 1) * 64, :] = _pack(wt.astype(bf16))
    wb_copy(1).wait()
    start_next(len(queue))

    def local_attn(r0, s, first_dep):
        outs = []
        deps = []
        for c in range(SB // RC):
            base = s * SB + c * RC
            dep = deps[c - LOOK] if c >= LOOK else first_dep
            scale = jnp.maximum(QSCALE, jnp.minimum(dep, -3e38)) if dep is not None else QSCALE
            q = [qa[t, base:base + RC, :] * scale for t in range(NT)]
            logits = []
            for w in range(WIN):
                o0 = HALO + base - DIL * w
                acc = q[0] * ka[0, o0:o0 + RC, :]
                for t in range(1, NT):
                    acc = acc + q[t] * ka[t, o0:o0 + RC, :]
                acc = acc + pltpu.roll(acc, 64, 1)
                acc = acc + pltpu.roll(acc, 32, 1)
                if base < DIL * w:
                    row = r0 + base + lax.broadcasted_iota(jnp.int32, (RC, 128), 0)
                    acc = jnp.where(row >= DIL * w, acc, -1e9)
                logits.append(acc)
            m = functools.reduce(jnp.maximum, logits)
            p = [jnp.exp2(lg - m) for lg in logits]
            inv = 1.0 / functools.reduce(lambda a, b: a + b, p)
            p = [pw * inv for pw in p]
            tiles = []
            for t in range(NT):
                acc = None
                for w in range(WIN):
                    o0 = HALO + base - DIL * w
                    term = p[w] * va[t, o0:o0 + RC, :]
                    acc = term if acc is None else acc + term
                tiles.append(acc.astype(bf16))
            deps.append(acc if DEP_END else m)
            outs.append(jnp.concatenate(tiles, axis=1))
        return jnp.concatenate(outs, axis=0)

    def row_body(r, l):
        r0 = pl.multiple_of(r * RB, RB)

        @pl.when(l == 0)
        def _():
            x_copy(r).wait()
            xs[pl.ds(r0, RB), :] = xin[pl.ds(r0, RB), :].astype(f32)

        rows = [pl.ds(r0 + s * SB, SB) for s in range(NSUB)]
        xn = [_layernorm(xs[rows[s], :]) for s in range(NSUB)]
        firsts = []
        for s in range(NSUB):
            y = lax.dot_general(xn[s], _unpack(wat[...].reshape(3 * D // 2, D)), NTD,
                                preferred_element_type=f32)
            for t in range(NT):
                qa[t, s * SB:(s + 1) * SB, :] = y[:, t * 128:(t + 1) * 128]
                ka[t, HALO + s * SB:HALO + (s + 1) * SB, :] = y[:, D + t * 128:D + (t + 1) * 128]
                va[t, HALO + s * SB:HALO + (s + 1) * SB, :] = y[:, 2 * D + t * 128:2 * D + (t + 1) * 128]
            firsts.append(y[SB - RC:SB, GATE_COL - 128:GATE_COL] if GATE_COL else None)
        xn2 = []
        for s in range(NSUB):
            o = local_attn(r0, s, firsts[s])
            x1 = xs[rows[s], :] + lax.dot_general(o, _unpack(woa[...].reshape(D // 2, D)), NN,
                                                  preferred_element_type=f32)
            xs[rows[s], :] = x1
            xn2.append(_layernorm(x1))
        ka[:, 0:HALO, :] = ka[:, RB:RB + HALO, :]
        va[:, 0:HALO, :] = va[:, RB:RB + HALO, :]
        for s in range(NSUB):
            cols = pl.ds(r0 + s * SB, SB)
            yq = lax.dot_general(_unpack(wqvt[0:D // 2, :]), xn2[s], NTD, preferred_element_type=f32)
            qt[:, cols] = _pack((yq * QSCALE).astype(bf16))
            yv = lax.dot_general(_unpack(wqvt[D // 2:D, :]), xn2[s], NTD, preferred_element_type=f32)
            vt[:, cols] = _pack(yv.astype(bf16))
            yk = lax.dot_general(xn2[s], wb_raw[:, D:2 * D], NN, preferred_element_type=f32).astype(bf16)
            krows = pl.ds(pl.multiple_of((r0 + s * SB) // 2, SB // 2), SB // 2)
            for g in range(NT):
                kb[g, krows, :] = _pack(yk[:, g * 128:(g + 1) * 128])
        return l

    def head_weights(g, hh, q0):
        w = qt[pl.ds(pl.multiple_of(g * 64 + hh * 16, 16), 16), pl.ds(q0, TQ)]
        parts = []
        if hh > 0:
            parts.append(jnp.zeros((16 * hh, TQ), u32))
        parts.append(w)
        if hh < 3:
            parts.append(jnp.zeros((16 * (3 - hh), TQ), u32))
        return _unpack(jnp.concatenate(parts, axis=0))

    def ref_max(g, q0):
        k0 = kb[g, 0:8, :]
        lane = lax.broadcasted_iota(jnp.int32, (8, 128), 1) // DH
        lhs = jnp.concatenate(
            [jnp.where(lane == hh, k0, jnp.zeros_like(k0)) for hh in range(4)], axis=0)
        w = _unpack(qt[pl.ds(pl.multiple_of(g * 64, 64), 64), pl.ds(q0, TQ)])
        s0 = jnp.dot(_unpack(lhs), w, preferred_element_type=f32)
        return jnp.concatenate(
            [jnp.broadcast_to(jnp.max(s0[16 * hh:16 * hh + 16], axis=0, keepdims=True), (8, TQ))
             for hh in range(4)], axis=0)

    def store_group(g, q0, o_t):
        ob[g, pl.ds(pl.multiple_of(q0 // 2, TQ // 2), TQ // 2), :] = _pack(o_t.T.astype(bf16))

    def attn_fast(q0):
        def group(g, carry):
            m_all, lmax = carry
            st = {}
            outs = []

            def qk(hh, c):
                if c == 0:
                    st[hh] = dict(w=head_weights(g, hh, q0), l=None, acc=None)
                kc = _unpack(kb[g, c * KC // 2:(c + 1) * KC // 2, :])
                return jnp.dot(kc, st[hh]["w"], preferred_element_type=f32)

            def pv(hh, c, s):
                d = st[hh]
                m = m_all[8 * hh:8 * hh + 8]
                p = jnp.exp2(s.reshape(KC // 8, 8, TQ) - m[None])
                lc = jnp.sum(p, axis=0)
                vc = _unpack(vt[pl.ds(pl.multiple_of(g * 64 + hh * 16, 16), 16), c * KC:(c + 1) * KC])
                o = jnp.dot(vc, p.reshape(KC, TQ).astype(bf16), preferred_element_type=f32)
                d["l"] = lc if c == 0 else d["l"] + lc
                d["acc"] = o if c == 0 else d["acc"] + o
                if c == NC - 1:
                    l = jnp.sum(d["l"], axis=0, keepdims=True)
                    d["lsum"] = l
                    outs.append(d["acc"] * (1.0 / l))

            m_next = None
            pend = None
            for hh in range(4):
                for c in range(NC):
                    if hh == 3 and c == 0:
                        m_next = ref_max(jnp.minimum(g + 1, NT - 1), q0)
                    s = qk(hh, c)
                    if pend is not None:
                        pv(*pend)
                    pend = (hh, c, s)
            pv(*pend)
            store_group(g, q0, jnp.concatenate(outs, axis=0))
            for hh in range(4):
                lmax = jnp.maximum(lmax, st[hh]["lsum"])
            return m_next, lmax

        _, lmax = lax.fori_loop(0, NT, group, (ref_max(0, q0), jnp.zeros((1, TQ), f32)))
        return lmax

    def attn_exact(q0):
        def group(g, carry):
            def head(hh, carry2):
                w = qt[pl.ds(pl.multiple_of(g * 64, 64), 64), pl.ds(q0, TQ)]
                row = lax.broadcasted_iota(jnp.int32, (64, TQ), 0) // 16
                w = _unpack(jnp.where(row == hh, w, jnp.zeros_like(w)))
                s = jnp.dot(_unpack(kb[g]), w, preferred_element_type=f32)
                p = jnp.exp2(s - jnp.max(s, axis=0, keepdims=True))
                l = jnp.sum(p, axis=0, keepdims=True)
                v = _unpack(vt[pl.ds(pl.multiple_of(g * 64 + hh * 16, 16), 16), :])
                o = jnp.dot(v, p.astype(bf16), preferred_element_type=f32)
                ot[pl.ds(pl.multiple_of(hh * DH, DH), DH), :] = o * (1.0 / l)
                return carry2
            lax.fori_loop(0, 4, head, 0)
            store_group(g, q0, ot[...])
            return carry
        lax.fori_loop(0, NT, group, 0)

    def q_body(qb, l):
        q0 = pl.multiple_of(qb * TQ, TQ)
        lmax = attn_fast(q0)
        unsafe = jnp.max(jnp.where(lmax <= L_MAX, 0, 1))

        @pl.when(unsafe > 0)
        def _():
            attn_exact(q0)

        orows = pl.ds(pl.multiple_of(q0 // 2, TQ // 2), TQ // 2)
        o = jnp.concatenate([_unpack(ob[g, orows, :]) for g in range(NT)], axis=1)
        x2 = xs[pl.ds(q0, TQ), :] + lax.dot_general(o, wob[...], NN, preferred_element_type=f32)
        xs[pl.ds(q0, TQ), :] = x2
        outb[pl.ds(q0, TQ), :] = x2.astype(bf16)

        @pl.when(l == 1)
        def _():
            out_copy(qb).start()

        return l

    def layer_pair(l, carry):
        ka[:, 0:HALO, :] = jnp.zeros((NT, HALO, 128), f32)
        va[:, 0:HALO, :] = jnp.zeros((NT, HALO, 128), f32)
        lax.fori_loop(0, S // RB, row_body, l)

        @pl.when(l == 0)
        def _():
            wob_copy.wait()

        lax.fori_loop(0, S // TQ, q_body, l)
        return carry

    lax.fori_loop(0, 2, layer_pair, 0)
    for qb in range(S // TQ):
        out_copy(qb).wait()


@jax.jit
def pallas_interleave_layers__sliding_local_dilated__softmax_full_mha__prompt_kernel(
    A_x: jax.Array,
    A_wqkv: jax.Array,
    A_wo: jax.Array,
    B_x: jax.Array,
    B_wqkv: jax.Array,
    B_wo: jax.Array,
):
    del B_x
    x = A_x.reshape(S, D)
    hbm = pl.BlockSpec(memory_space=pl.ANY)
    out = pl.pallas_call(
        _kernel,
        out_shape=jax.ShapeDtypeStruct((S, D), bf16),
        in_specs=[hbm] * 5,
        out_specs=hbm,
        scratch_shapes=[
            pltpu.VMEM((S, D), bf16),
            pltpu.VMEM((D, 3 * D), bf16),
            pltpu.VMEM((D, D), bf16),
            pltpu.VMEM((D, 3 * D), bf16),
            pltpu.VMEM((D, D), bf16),
            pltpu.VMEM((S, D), bf16),
            pltpu.VMEM((3, DH, 2, 8, D), u32),
            pltpu.VMEM((DH, 2, 8, D), u32),
            pltpu.VMEM((D, D), u32),
            pltpu.VMEM((S, D), f32),
            pltpu.VMEM((NT, RB, 128), f32),
            pltpu.VMEM((NT, HALO + RB, 128), f32),
            pltpu.VMEM((NT, HALO + RB, 128), f32),
            pltpu.VMEM((D // 2, S), u32),
            pltpu.VMEM((NT, S // 2, 128), u32),
            pltpu.VMEM((D // 2, S), u32),
            pltpu.VMEM((NT, S // 2, 128), u32),
            pltpu.VMEM((128, TQ), f32),
            pltpu.SemaphoreType.DMA((S // RB,)),
            pltpu.SemaphoreType.DMA((3 * D // WCH,)),
            pltpu.SemaphoreType.DMA((5,)),
            pltpu.SemaphoreType.DMA((S // TQ,)),
        ],
        compiler_params=pltpu.CompilerParams(vmem_limit_bytes=110 * 1024 * 1024),
    )(x, A_wqkv, A_wo, B_wqkv, B_wo)
    return out.reshape(1, S, D)
```

```python
import functools
import math

import jax
import jax.numpy as jnp
from jax import lax
import jax.experimental.pallas as pl
import jax.experimental.pallas.tpu as pltpu

S = 2048
D = 1024
H = 32
DH = 32
WIN = 8
DIL = 2
EPS = 1e-5
NT = D // 128
HALO = 16
QSCALE = (DH ** -0.5) * math.log2(math.e)

SB = 128
NSUB = 2
RB = SB * NSUB
RC = 8
ROW_ORDER = [("a", 0), ("a", 1), ("o", 0), ("o", 1), ("b", 0), ("n", 0), ("b", 1)]
LOOK = 2
DEP_END = False
GATE_COL = 2 * D
TQ = 512
KC = 256
NC = S // KC
WCH = 512
WA_STARTS = (1, 1, 2, 1, 1, 2)
NFLIGHT = 3
L_MAX = 2.0 ** 64

bf16 = jnp.bfloat16
f32 = jnp.float32
u32 = jnp.uint32

NN = (((1,), (0,)), ((), ()))
NTD = (((1,), (1,)), ((), ()))


def _pack(x):
    return pltpu.bitcast(x, u32)


def _unpack(x):
    return pltpu.bitcast(x, bf16)


def _after(value, dep):
    if dep is None:
        return value
    return jnp.maximum(value, jnp.minimum(dep, -3e38))


def _tree(op, xs):
    xs = list(xs)
    while len(xs) > 1:
        xs = [op(xs[i], xs[i + 1]) if i + 1 < len(xs) else xs[i] for i in range(0, len(xs), 2)]
    return xs[0]


def _recip(x):
    r = pl.reciprocal(x, approx=True)
    return r * (2.0 - x * r)


def _layernorm(x):
    mu = jnp.mean(x, axis=-1, keepdims=True)
    xc = x - mu
    var = jnp.mean(xc * xc, axis=-1, keepdims=True)
    return (xc * lax.rsqrt(var + EPS)).astype(bf16)


def _kernel(x_hbm, wa_hbm, woa_hbm, wb_hbm, wob_hbm, out_hbm,
            xin, wa_raw, woa_raw, wb_raw, wob, outb,
            wat, wan, woa, wqvt, xnb,
            xs, qa, ka, va, qt, kb, vt, ob, ot,
            sem_x, sem_wa, sem_w, sem_o):
    def x_copy(r):
        rows = pl.ds(pl.multiple_of(r * RB, RB), RB)
        return pltpu.make_async_copy(x_hbm.at[rows, :], xin.at[rows, :], sem_x.at[r])

    def wa_copy(i):
        cols = pl.ds(pl.multiple_of(i * WCH, WCH), WCH)
        return pltpu.make_async_copy(wa_hbm.at[:, cols], wa_raw.at[:, cols], sem_wa.at[i])

    def wb_copy(i):
        cols = pl.ds(pl.multiple_of(i * D, D), D)
        return pltpu.make_async_copy(wb_hbm.at[:, cols], wb_raw.at[:, cols], sem_w.at[i])

    woa_copy = pltpu.make_async_copy(woa_hbm, woa_raw, sem_w.at[3])
    wob_copy = pltpu.make_async_copy(wob_hbm, wob, sem_w.at[4])

    def out_copy(qb):
        rows = pl.ds(pl.multiple_of(qb * TQ, TQ), TQ)
        return pltpu.make_async_copy(outb.at[rows, :], out_hbm.at[rows, :], sem_o.at[qb])

    n_wa = 3 * D // WCH
    queue = ([wa_copy(i) for i in range(n_wa)]
             + [woa_copy, wb_copy(0), wb_copy(2), x_copy(0), wb_copy(1)]
             + [x_copy(r) for r in range(1, S // RB)] + [wob_copy])
    for cp in queue[:NFLIGHT]:
        cp.start()
    queue = queue[NFLIGHT:]

    def start_in_loop(i, counts):
        for k, n in enumerate(counts):
            batch = [queue.pop(0) for _ in range(n)]

            @pl.when(i == k)
            def _():
                for cp in batch:
                    cp.start()

    def selection():
        ri = lax.broadcasted_iota(jnp.int32, (256, 256), 0)
        ci = lax.broadcasted_iota(jnp.int32, (256, 256), 1)
        return jnp.where(ci == (ri % 8) * DH + ri // 8, 1.0, 0.0).astype(bf16)

    def transpose(w):
        ri = lax.broadcasted_iota(jnp.int32, (128, 128), 0)
        ci = lax.broadcasted_iota(jnp.int32, (128, 128), 1)
        eye = jnp.where(ri == ci, 1.0, 0.0).astype(bf16)
        return lax.dot_general(eye, w, NTD, preferred_element_type=f32).astype(bf16)

    def pair(a0, a1):
        both = jnp.concatenate([a0.reshape(DH, 8, D), a1.reshape(DH, 8, D)], axis=1)
        return _pack(both.reshape(DH * 16, D).astype(bf16)).reshape(DH, 8, D)

    def prep_wa(i, carry):
        wa_copy(i).wait()
        start_in_loop(i, WA_STARTS)
        sel = selection()
        halves = [lax.dot_general(
            sel, wa_raw[:, pl.ds(pl.multiple_of(i * WCH + j * 256, 256), 256)], NTD,
            preferred_element_type=f32) for j in range(2)]
        wat[:, i % 2, :, :] = pair(*halves)

        @pl.when(i % 2 == 1)
        def _():
            wt = _unpack(wat[...].reshape(D // 2, D))
            cols = pl.ds(pl.multiple_of((i // 2) * D, D), D)
            for j in range(NT):
                wan[j * 64:(j + 1) * 64, cols] = _pack(transpose(wt[:, j * 128:(j + 1) * 128]))

        return carry

    def prep_woa(a, carry):
        sel = selection()
        halves = [lax.dot_general(
            sel, woa_raw[pl.ds(pl.multiple_of(a * 512 + j * 256, 256), 256), :], NN,
            preferred_element_type=f32) for j in range(2)]
        woa[:, a, :, :] = pair(*halves)
        return carry

    def prep_wb(part, carry):
        wb_copy(2 * part).wait()
        for j in range(NT):
            cols = pl.ds(pl.multiple_of(2 * part * D + j * 128, 128), 128)
            rows = pl.ds(pl.multiple_of(part * (D // 2) + j * 64, 64), 64)
            wqvt[rows, :] = _pack(transpose(wb_raw[:, cols]))
        return carry

    lax.fori_loop(0, n_wa, prep_wa, 0)
    woa_copy.wait()
    lax.fori_loop(0, 2, prep_woa, 0)
    lax.fori_loop(0, 2, prep_wb, 0)
    wb_copy(1).wait()
    for cp in queue:
        cp.start()

    def local_attn(r0, s, first_dep):
        outs = []
        deps = []
        for c in range(SB // RC):
            base = s * SB + c * RC
            scale = _after(QSCALE, deps[c - LOOK] if c >= LOOK else first_dep)
            logits = [None] * WIN
            for t in range(NT):
                q = qa[t, base:base + RC, :] * scale
                for w in range(WIN):
                    o0 = HALO + base - DIL * w
                    term = q * ka[t, o0:o0 + RC, :]
                    logits[w] = term if t == 0 else logits[w] + term
            for w in range(WIN):
                acc = logits[w]
                acc = acc + pltpu.roll(acc, 64, 1)
                acc = acc + pltpu.roll(acc, 32, 1)
                if base < DIL * w:
                    row = r0 + base + lax.broadcasted_iota(jnp.int32, (RC, 128), 0)
                    acc = jnp.where(row >= DIL * w, acc, -1e9)
                logits[w] = acc
            m = _tree(jnp.maximum, logits)
            p = [jnp.exp2(lg - m) for lg in logits]
            inv = _recip(_tree(jnp.add, p))
            tiles = []
            for t in range(NT):
                terms = [p[w] * va[t, HALO + base - DIL * w:HALO + base - DIL * w + RC, :]
                         for w in range(WIN)]
                acc = _tree(jnp.add, terms) * inv
                tiles.append(acc.astype(bf16))
            deps.append(acc if DEP_END else m)
            outs.append(jnp.concatenate(tiles, axis=1))
        return jnp.concatenate(outs, axis=0)

    def load_x(r, l):
        rows = pl.ds(pl.multiple_of(r * RB, RB), RB)
        x = jnp.where(l == 0, xin[rows, :].astype(f32), xs[rows, :])
        xs[rows, :] = x
        xnb[...] = _pack(_layernorm(x))

    def row_body(r, l):
        r0 = pl.multiple_of(r * RB, RB)
        rn = jnp.minimum(r + 1, S // RB - 1)

        @pl.when(jnp.logical_and(l == 0, r + 1 < S // RB))
        def _():
            x_copy(rn).wait()

        rows = [pl.ds(r0 + s * SB, SB) for s in range(NSUB)]
        gate = {}
        xn2 = {}

        def qkv_a(s):
            xn = _unpack(xnb[s * SB // 2:(s + 1) * SB // 2, :])
            y = lax.dot_general(xn, _unpack(wan[...]), NN, preferred_element_type=f32)
            for t in range(NT):
                qa[t, s * SB:(s + 1) * SB, :] = y[:, t * 128:(t + 1) * 128]
                ka[t, HALO + s * SB:HALO + (s + 1) * SB, :] = y[:, D + t * 128:D + (t + 1) * 128]
                va[t, HALO + s * SB:HALO + (s + 1) * SB, :] = y[:, 2 * D + t * 128:2 * D + (t + 1) * 128]
            gate[s] = y[SB - RC:SB, GATE_COL - 128:GATE_COL]

        def out_a(s):
            o = local_attn(r0, s, gate[s])
            x1 = xs[rows[s], :] + lax.dot_general(o, _unpack(woa[...].reshape(D // 2, D)), NN,
                                                  preferred_element_type=f32)
            xs[rows[s], :] = x1
            xn2[s] = _layernorm(x1)

        def qkv_b(s):
            cols = pl.ds(r0 + s * SB, SB)
            yq = lax.dot_general(_unpack(wqvt[0:D // 2, :]), xn2[s], NTD, preferred_element_type=f32)
            qt[:, cols] = _pack((yq * QSCALE).astype(bf16))
            yv = lax.dot_general(_unpack(wqvt[D // 2:D, :]), xn2[s], NTD, preferred_element_type=f32)
            vt[:, cols] = _pack(yv.astype(bf16))
            yk = lax.dot_general(xn2[s], wb_raw[:, D:2 * D], NN, preferred_element_type=f32).astype(bf16)
            krows = pl.ds(pl.multiple_of((r0 + s * SB) // 2, SB // 2), SB // 2)
            for g in range(NT):
                kb[g, krows, :] = _pack(yk[:, g * 128:(g + 1) * 128])

        steps = {"a": qkv_a, "o": out_a, "b": qkv_b}
        for name, s in ROW_ORDER:
            if name == "n":
                ka[:, 0:HALO, :] = ka[:, RB:RB + HALO, :]
                va[:, 0:HALO, :] = va[:, RB:RB + HALO, :]
                load_x(rn, jnp.where(r + 1 < S // RB, l, 1))
            else:
                steps[name](s)
        return l

    def head_weights(g, hh, q0):
        w = qt[pl.ds(pl.multiple_of(g * 64 + hh * 16, 16), 16), pl.ds(q0, TQ)]
        parts = []
        if hh > 0:
            parts.append(jnp.zeros((16 * hh, TQ), u32))
        parts.append(w)
        if hh < 3:
            parts.append(jnp.zeros((16 * (3 - hh), TQ), u32))
        return _unpack(jnp.concatenate(parts, axis=0))

    def ref_max(g, q0):
        k0 = kb[g, 0:8, :]
        lane = lax.broadcasted_iota(jnp.int32, (8, 128), 1) // DH
        lhs = jnp.concatenate(
            [jnp.where(lane == hh, k0, jnp.zeros_like(k0)) for hh in range(4)], axis=0)
        w = _unpack(qt[pl.ds(pl.multiple_of(g * 64, 64), 64), pl.ds(q0, TQ)])
        s0 = jnp.dot(_unpack(lhs), w, preferred_element_type=f32)
        return jnp.concatenate(
            [jnp.broadcast_to(jnp.max(s0[16 * hh:16 * hh + 16], axis=0, keepdims=True), (8, TQ))
             for hh in range(4)], axis=0)

    def store_group(g, q0, o_t):
        ob[g, pl.ds(pl.multiple_of(q0 // 2, TQ // 2), TQ // 2), :] = _pack(o_t.T.astype(bf16))

    def attn_fast(q0):
        def group(g, carry):
            m_all, lmax = carry
            st = {}
            outs = []

            def qk(hh, c):
                if c == 0:
                    st[hh] = dict(w=head_weights(g, hh, q0), l=None, acc=None)
                kc = _unpack(kb[g, c * KC // 2:(c + 1) * KC // 2, :])
                return jnp.dot(kc, st[hh]["w"], preferred_element_type=f32)

            def pv(hh, c, s):
                d = st[hh]
                m = m_all[8 * hh:8 * hh + 8]
                p = jnp.exp2(s.reshape(KC // 8, 8, TQ) - m[None])
                lc = jnp.sum(p, axis=0)
                vc = _unpack(vt[pl.ds(pl.multiple_of(g * 64 + hh * 16, 16), 16), c * KC:(c + 1) * KC])
                o = jnp.dot(vc, p.reshape(KC, TQ).astype(bf16), preferred_element_type=f32)
                d["l"] = lc if c == 0 else d["l"] + lc
                d["acc"] = o if c == 0 else d["acc"] + o
                if c == NC - 1:
                    l = jnp.sum(d["l"], axis=0, keepdims=True)
                    d["lsum"] = l
                    outs.append(d["acc"] * (1.0 / l))

            m_next = None
            pend = None
            for hh in range(4):
                for c in range(NC):
                    if hh == 3 and c == 0:
                        m_next = ref_max(jnp.minimum(g + 1, NT - 1), q0)
                    s = qk(hh, c)
                    if pend is not None:
                        pv(*pend)
                    pend = (hh, c, s)
            pv(*pend)
            store_group(g, q0, jnp.concatenate(outs, axis=0))
            for hh in range(4):
                lmax = jnp.maximum(lmax, st[hh]["lsum"])
            return m_next, lmax

        _, lmax = lax.fori_loop(0, NT, group, (ref_max(0, q0), jnp.zeros((1, TQ), f32)))
        return lmax

    def attn_exact(q0):
        def group(g, carry):
            def head(hh, carry2):
                w = qt[pl.ds(pl.multiple_of(g * 64, 64), 64), pl.ds(q0, TQ)]
                row = lax.broadcasted_iota(jnp.int32, (64, TQ), 0) // 16
                w = _unpack(jnp.where(row == hh, w, jnp.zeros_like(w)))
                s = jnp.dot(_unpack(kb[g]), w, preferred_element_type=f32)
                p = jnp.exp2(s - jnp.max(s, axis=0, keepdims=True))
                l = jnp.sum(p, axis=0, keepdims=True)
                v = _unpack(vt[pl.ds(pl.multiple_of(g * 64 + hh * 16, 16), 16), :])
                o = jnp.dot(v, p.astype(bf16), preferred_element_type=f32)
                ot[pl.ds(pl.multiple_of(hh * DH, DH), DH), :] = o * (1.0 / l)
                return carry2
            lax.fori_loop(0, 4, head, 0)
            store_group(g, q0, ot[...])
            return carry
        lax.fori_loop(0, NT, group, 0)

    def q_body(qb, l):
        q0 = pl.multiple_of(qb * TQ, TQ)
        lmax = attn_fast(q0)
        unsafe = jnp.max(jnp.where(lmax <= L_MAX, 0, 1))

        @pl.when(unsafe > 0)
        def _():
            attn_exact(q0)

        orows = pl.ds(pl.multiple_of(q0 // 2, TQ // 2), TQ // 2)
        o = jnp.concatenate([_unpack(ob[g, orows, :]) for g in range(NT)], axis=1)
        x2 = xs[pl.ds(q0, TQ), :] + lax.dot_general(o, wob[...], NN, preferred_element_type=f32)
        xs[pl.ds(q0, TQ), :] = x2
        outb[pl.ds(q0, TQ), :] = x2.astype(bf16)

        @pl.when(l == 1)
        def _():
            out_copy(qb).start()

        return l

    def layer_pair(l, carry):
        ka[:, 0:HALO, :] = jnp.zeros((NT, HALO, 128), f32)
        va[:, 0:HALO, :] = jnp.zeros((NT, HALO, 128), f32)

        @pl.when(l == 0)
        def _():
            x_copy(0).wait()

        load_x(0, l)
        lax.fori_loop(0, S // RB, row_body, l)

        @pl.when(l == 0)
        def _():
            wob_copy.wait()

        lax.fori_loop(0, S // TQ, q_body, l)
        return carry

    lax.fori_loop(0, 2, layer_pair, 0)
    for qb in range(S // TQ):
        out_copy(qb).wait()


@jax.jit
def pallas_interleave_layers__sliding_local_dilated__softmax_full_mha__prompt_kernel(
    A_x: jax.Array,
    A_wqkv: jax.Array,
    A_wo: jax.Array,
    B_x: jax.Array,
    B_wqkv: jax.Array,
    B_wo: jax.Array,
):
    del B_x
    x = A_x.reshape(S, D)
    hbm = pl.BlockSpec(memory_space=pl.ANY)
    out = pl.pallas_call(
        _kernel,
        out_shape=jax.ShapeDtypeStruct((S, D), bf16),
        in_specs=[hbm] * 5,
        out_specs=hbm,
        scratch_shapes=[
            pltpu.VMEM((S, D), bf16),
            pltpu.VMEM((D, 3 * D), bf16),
            pltpu.VMEM((D, D), bf16),
            pltpu.VMEM((D, 3 * D), bf16),
            pltpu.VMEM((D, D), bf16),
            pltpu.VMEM((S, D), bf16),
            pltpu.VMEM((DH, 2, 8, D), u32),
            pltpu.VMEM((D // 2, 3 * D), u32),
            pltpu.VMEM((DH, 2, 8, D), u32),
            pltpu.VMEM((D, D), u32),
            pltpu.VMEM((RB // 2, D), u32),
            pltpu.VMEM((S, D), f32),
            pltpu.VMEM((NT, RB, 128), f32),
            pltpu.VMEM((NT, HALO + RB, 128), f32),
            pltpu.VMEM((NT, HALO + RB, 128), f32),
            pltpu.VMEM((D // 2, S), u32),
            pltpu.VMEM((NT, S // 2, 128), u32),
            pltpu.VMEM((D // 2, S), u32),
            pltpu.VMEM((NT, S // 2, 128), u32),
            pltpu.VMEM((128, TQ), f32),
            pltpu.SemaphoreType.DMA((S // RB,)),
            pltpu.SemaphoreType.DMA((3 * D // WCH,)),
            pltpu.SemaphoreType.DMA((5,)),
            pltpu.SemaphoreType.DMA((S // TQ,)),
        ],
        compiler_params=pltpu.CompilerParams(vmem_limit_bytes=110 * 1024 * 1024),
    )(x, A_wqkv, A_wo, B_wqkv, B_wo)
    return out.reshape(1, S, D)
```

```python
import functools
import math

import jax
import jax.numpy as jnp
from jax import lax
import jax.experimental.pallas as pl
import jax.experimental.pallas.tpu as pltpu

S = 2048
D = 1024
H = 32
DH = 32
WIN = 8
DIL = 2
EPS = 1e-5
NT = D // 128
HALO = 16
QSCALE = (DH ** -0.5) * math.log2(math.e)

SB = 128
NSUB = 2
RB = SB * NSUB
RC = 8
ROW_ORDER = [("a", 0), ("a", 1), ("o", 0), ("o", 1), ("b", 0), ("n", 0), ("b", 1)]
LOOK = 2
DEP_END = False
GATE_COL = 2 * D
TQ = 512
KC = 256
NC = S // KC
HPB = 4
WCH = 512
WA_STARTS = (1, 1, 2, 1, 1, 2)
NFLIGHT = 3
L_MAX = 2.0 ** 64

bf16 = jnp.bfloat16
f32 = jnp.float32
u32 = jnp.uint32

NN = (((1,), (0,)), ((), ()))
NTD = (((1,), (1,)), ((), ()))


def _pack(x):
    return pltpu.bitcast(x, u32)


def _unpack(x):
    return pltpu.bitcast(x, bf16)


def _after(value, dep):
    if dep is None:
        return value
    return jnp.maximum(value, jnp.minimum(dep, -3e38))


def _tree(op, xs):
    xs = list(xs)
    while len(xs) > 1:
        xs = [op(xs[i], xs[i + 1]) if i + 1 < len(xs) else xs[i] for i in range(0, len(xs), 2)]
    return xs[0]


def _recip(x):
    r = pl.reciprocal(x, approx=True)
    return r * (2.0 - x * r)


def _layernorm(x):
    mu = jnp.mean(x, axis=-1, keepdims=True)
    xc = x - mu
    var = jnp.mean(xc * xc, axis=-1, keepdims=True)
    return (xc * lax.rsqrt(var + EPS)).astype(bf16)


def _kernel(x_hbm, wa_hbm, woa_hbm, wb_hbm, wob_hbm, out_hbm,
            xin, wa_raw, woa_raw, wb_raw, wob, outb,
            wat, wan, woa, wqvt, xnb,
            xs, qa, ka, va, qt, kb, vt, ob, ot, pp, invs,
            sem_x, sem_wa, sem_w, sem_o):
    def x_copy(r):
        rows = pl.ds(pl.multiple_of(r * RB, RB), RB)
        return pltpu.make_async_copy(x_hbm.at[rows, :], xin.at[rows, :], sem_x.at[r])

    def wa_copy(i):
        cols = pl.ds(pl.multiple_of(i * WCH, WCH), WCH)
        return pltpu.make_async_copy(wa_hbm.at[:, cols], wa_raw.at[:, cols], sem_wa.at[i])

    def wb_copy(i):
        cols = pl.ds(pl.multiple_of(i * D, D), D)
        return pltpu.make_async_copy(wb_hbm.at[:, cols], wb_raw.at[:, cols], sem_w.at[i])

    woa_copy = pltpu.make_async_copy(woa_hbm, woa_raw, sem_w.at[3])
    wob_copy = pltpu.make_async_copy(wob_hbm, wob, sem_w.at[4])

    def out_copy(qb):
        rows = pl.ds(pl.multiple_of(qb * TQ, TQ), TQ)
        return pltpu.make_async_copy(outb.at[rows, :], out_hbm.at[rows, :], sem_o.at[qb])

    n_wa = 3 * D // WCH
    queue = ([wa_copy(i) for i in range(n_wa)]
             + [woa_copy, wb_copy(0), wb_copy(2), x_copy(0), wb_copy(1)]
             + [x_copy(r) for r in range(1, S // RB)] + [wob_copy])
    for cp in queue[:NFLIGHT]:
        cp.start()
    queue = queue[NFLIGHT:]

    def start_in_loop(i, counts):
        for k, n in enumerate(counts):
            batch = [queue.pop(0) for _ in range(n)]

            @pl.when(i == k)
            def _():
                for cp in batch:
                    cp.start()

    def selection():
        ri = lax.broadcasted_iota(jnp.int32, (256, 256), 0)
        ci = lax.broadcasted_iota(jnp.int32, (256, 256), 1)
        return jnp.where(ci == (ri % 8) * DH + ri // 8, 1.0, 0.0).astype(bf16)

    def transpose(w):
        ri = lax.broadcasted_iota(jnp.int32, (128, 128), 0)
        ci = lax.broadcasted_iota(jnp.int32, (128, 128), 1)
        eye = jnp.where(ri == ci, 1.0, 0.0).astype(bf16)
        return lax.dot_general(eye, w, NTD, preferred_element_type=f32).astype(bf16)

    def pair(a0, a1):
        both = jnp.concatenate([a0.reshape(DH, 8, D), a1.reshape(DH, 8, D)], axis=1)
        return _pack(both.reshape(DH * 16, D).astype(bf16)).reshape(DH, 8, D)

    def prep_wa(i, carry):
        wa_copy(i).wait()
        start_in_loop(i, WA_STARTS)
        sel = selection()
        halves = [lax.dot_general(
            sel, wa_raw[:, pl.ds(pl.multiple_of(i * WCH + j * 256, 256), 256)], NTD,
            preferred_element_type=f32) for j in range(2)]
        wat[:, i % 2, :, :] = pair(*halves)

        @pl.when(i % 2 == 1)
        def _():
            wt = _unpack(wat[...].reshape(D // 2, D))
            cols = pl.ds(pl.multiple_of((i // 2) * D, D), D)
            for j in range(NT):
                wan[j * 64:(j + 1) * 64, cols] = _pack(transpose(wt[:, j * 128:(j + 1) * 128]))

        return carry

    def prep_woa(a, carry):
        sel = selection()
        halves = [lax.dot_general(
            sel, woa_raw[pl.ds(pl.multiple_of(a * 512 + j * 256, 256), 256), :], NN,
            preferred_element_type=f32) for j in range(2)]
        woa[:, a, :, :] = pair(*halves)
        return carry

    def prep_wb(part, carry):
        wb_copy(2 * part).wait()
        for j in range(NT):
            cols = pl.ds(pl.multiple_of(2 * part * D + j * 128, 128), 128)
            rows = pl.ds(pl.multiple_of(part * (D // 2) + j * 64, 64), 64)
            wqvt[rows, :] = _pack(transpose(wb_raw[:, cols]))
        return carry

    lax.fori_loop(0, n_wa, prep_wa, 0)
    woa_copy.wait()
    lax.fori_loop(0, 2, prep_woa, 0)
    lax.fori_loop(0, 2, prep_wb, 0)
    wb_copy(1).wait()
    for cp in queue:
        cp.start()

    def local_attn(r0, s, first_dep):
        outs = []
        deps = []
        for c in range(SB // RC):
            base = s * SB + c * RC
            scale = _after(QSCALE, deps[c - LOOK] if c >= LOOK else first_dep)
            logits = [None] * WIN
            for t in range(NT):
                q = qa[t, base:base + RC, :] * scale
                for w in range(WIN):
                    o0 = HALO + base - DIL * w
                    term = q * ka[t, o0:o0 + RC, :]
                    logits[w] = term if t == 0 else logits[w] + term
            for w in range(WIN):
                acc = logits[w]
                acc = acc + pltpu.roll(acc, 64, 1)
                acc = acc + pltpu.roll(acc, 32, 1)
                if base < DIL * w:
                    row = r0 + base + lax.broadcasted_iota(jnp.int32, (RC, 128), 0)
                    acc = jnp.where(row >= DIL * w, acc, -1e9)
                logits[w] = acc
            m = _tree(jnp.maximum, logits)
            p = [jnp.exp2(lg - m) for lg in logits]
            inv = _recip(_tree(jnp.add, p))
            tiles = []
            for t in range(NT):
                terms = [p[w] * va[t, HALO + base - DIL * w:HALO + base - DIL * w + RC, :]
                         for w in range(WIN)]
                acc = _tree(jnp.add, terms) * inv
                tiles.append(acc.astype(bf16))
            deps.append(acc if DEP_END else m)
            outs.append(jnp.concatenate(tiles, axis=1))
        return jnp.concatenate(outs, axis=0)

    def load_x(r, l):
        rows = pl.ds(pl.multiple_of(r * RB, RB), RB)
        x = jnp.where(l == 0, xin[rows, :].astype(f32), xs[rows, :])
        xs[rows, :] = x
        xnb[...] = _pack(_layernorm(x))

    def row_body(r, l):
        r0 = pl.multiple_of(r * RB, RB)
        rn = jnp.minimum(r + 1, S // RB - 1)

        @pl.when(jnp.logical_and(l == 0, r + 1 < S // RB))
        def _():
            x_copy(rn).wait()

        rows = [pl.ds(r0 + s * SB, SB) for s in range(NSUB)]
        gate = {}
        xn2 = {}

        def qkv_a(s):
            xn = _unpack(xnb[s * SB // 2:(s + 1) * SB // 2, :])
            y = lax.dot_general(xn, _unpack(wan[...]), NN, preferred_element_type=f32)
            for t in range(NT):
                qa[t, s * SB:(s + 1) * SB, :] = y[:, t * 128:(t + 1) * 128]
                ka[t, HALO + s * SB:HALO + (s + 1) * SB, :] = y[:, D + t * 128:D + (t + 1) * 128]
                va[t, HALO + s * SB:HALO + (s + 1) * SB, :] = y[:, 2 * D + t * 128:2 * D + (t + 1) * 128]
            gate[s] = y[SB - RC:SB, GATE_COL - 128:GATE_COL]

        def out_a(s):
            o = local_attn(r0, s, gate[s])
            x1 = xs[rows[s], :] + lax.dot_general(o, _unpack(woa[...].reshape(D // 2, D)), NN,
                                                  preferred_element_type=f32)
            xs[rows[s], :] = x1
            xn2[s] = _layernorm(x1)

        def qkv_b(s):
            cols = pl.ds(r0 + s * SB, SB)
            yq = lax.dot_general(_unpack(wqvt[0:D // 2, :]), xn2[s], NTD, preferred_element_type=f32)
            qt[:, cols] = _pack((yq * QSCALE).astype(bf16))
            yv = lax.dot_general(_unpack(wqvt[D // 2:D, :]), xn2[s], NTD, preferred_element_type=f32)
            vt[:, cols] = _pack(yv.astype(bf16))
            yk = lax.dot_general(xn2[s], wb_raw[:, D:2 * D], NN, preferred_element_type=f32).astype(bf16)
            krows = pl.ds(pl.multiple_of((r0 + s * SB) // 2, SB // 2), SB // 2)
            for g in range(NT):
                kb[g, krows, :] = _pack(yk[:, g * 128:(g + 1) * 128])

        steps = {"a": qkv_a, "o": out_a, "b": qkv_b}
        for name, s in ROW_ORDER:
            if name == "n":
                ka[:, 0:HALO, :] = ka[:, RB:RB + HALO, :]
                va[:, 0:HALO, :] = va[:, RB:RB + HALO, :]
                load_x(rn, jnp.where(r + 1 < S // RB, l, 1))
            else:
                steps[name](s)
        return l

    def head_weights(g, hh, q0):
        w = qt[pl.ds(pl.multiple_of(g * 64 + hh * 16, 16), 16), pl.ds(q0, TQ)]
        parts = []
        if hh > 0:
            parts.append(jnp.zeros((16 * hh, TQ), u32))
        parts.append(w)
        if hh < 3:
            parts.append(jnp.zeros((16 * (3 - hh), TQ), u32))
        return _unpack(jnp.concatenate(parts, axis=0))

    def ref_max(g, q0):
        k0 = kb[g, 0:8, :]
        lane = lax.broadcasted_iota(jnp.int32, (8, 128), 1) // DH
        lhs = jnp.concatenate(
            [jnp.where(lane == hh, k0, jnp.zeros_like(k0)) for hh in range(4)], axis=0)
        w = _unpack(qt[pl.ds(pl.multiple_of(g * 64, 64), 64), pl.ds(q0, TQ)])
        s0 = jnp.dot(_unpack(lhs), w, preferred_element_type=f32)
        return jnp.concatenate(
            [jnp.broadcast_to(jnp.max(s0[16 * hh:16 * hh + 16], axis=0, keepdims=True), (8, TQ))
             for hh in range(4)], axis=0)

    def v_rows(g, hh, c):
        rows = pl.ds(pl.multiple_of(g * 64 + hh * 16, 16), 16)
        return _unpack(vt[rows, c * KC:(c + 1) * KC])

    def finish_group(g):
        o = jnp.dot(v_rows(g, HPB - 1, NC - 1), _unpack(pp[...]), preferred_element_type=f32)
        last = (ot[3 * DH:4 * DH, :] + o) * invs[0:1, :]
        return jnp.concatenate([ot[0:3 * DH, :], last], axis=0).T.astype(bf16)

    def o_rows(q0):
        return pl.ds(pl.multiple_of(q0 // 2, TQ // 2), TQ // 2)

    def attn_fast(q0, m_first):
        def group(g, carry):
            m_all, lmax = carry
            st = {}

            def qk(hh, c):
                if c == 0:
                    st[hh] = dict(w=head_weights(g, hh, q0))
                kc = _unpack(kb[g, c * KC // 2:(c + 1) * KC // 2, :])
                return jnp.dot(kc, st[hh]["w"], preferred_element_type=f32)

            def pv(hh, c, s):
                d = st[hh]
                m = m_all[8 * hh:8 * hh + 8]
                p = jnp.exp2(s.reshape(KC // 8, 8, TQ) - m[None])
                lc = jnp.sum(p, axis=0)
                d["l"] = lc if c == 0 else d["l"] + lc
                p = p.reshape(KC, TQ).astype(bf16)
                if c == NC - 1:
                    d["lsum"] = jnp.sum(d["l"], axis=0, keepdims=True)
                if hh == HPB - 1 and c == NC - 1:
                    pp[...] = _pack(p)
                    ot[hh * DH:(hh + 1) * DH, :] = d["acc"]
                    invs[...] = jnp.broadcast_to(_recip(d["lsum"]), (8, TQ))
                    return
                o = jnp.dot(v_rows(g, hh, c), p, preferred_element_type=f32)
                d["acc"] = o if c == 0 else d["acc"] + o
                if c == NC - 1:
                    ot[hh * DH:(hh + 1) * DH, :] = d["acc"] * _recip(d["lsum"])

            m_next = None
            pend = None
            for hh in range(HPB):
                for c in range(NC):
                    if hh == HPB - 1 and c == 0:
                        m_next = ref_max(jnp.minimum(g + 1, NT - 1), q0)
                    s = qk(hh, c)
                    if pend is None:
                        ob[jnp.where(g == 0, NT, g - 1), o_rows(q0), :] = _pack(
                            finish_group(jnp.maximum(g - 1, 0)))
                    else:
                        pv(*pend)
                    pend = (hh, c, s)
            pv(*pend)
            for hh in range(HPB):
                lmax = jnp.maximum(lmax, st[hh]["lsum"])
            return m_next, lmax

        _, lmax = lax.fori_loop(0, NT, group, (m_first, jnp.zeros((1, TQ), f32)))
        return lmax

    def attn_exact(q0):
        def group(g, carry):
            def head(hh, carry2):
                w = qt[pl.ds(pl.multiple_of(g * 64, 64), 64), pl.ds(q0, TQ)]
                row = lax.broadcasted_iota(jnp.int32, (64, TQ), 0) // 16
                w = _unpack(jnp.where(row == hh, w, jnp.zeros_like(w)))
                s = jnp.dot(_unpack(kb[g]), w, preferred_element_type=f32)
                p = jnp.exp2(s - jnp.max(s, axis=0, keepdims=True))
                l = jnp.sum(p, axis=0, keepdims=True)
                v = _unpack(vt[pl.ds(pl.multiple_of(g * 64 + hh * 16, 16), 16), :])
                o = jnp.dot(v, p.astype(bf16), preferred_element_type=f32)
                ot[pl.ds(pl.multiple_of(hh * DH, DH), DH), :] = o * (1.0 / l)
                return carry2
            lax.fori_loop(0, 4, head, 0)
            ob[g, o_rows(q0), :] = _pack(ot[...].T.astype(bf16))
            return carry
        lax.fori_loop(0, NT, group, 0)
        pp[...] = jnp.zeros(pp.shape, u32)
        invs[...] = jnp.ones(invs.shape, f32)

    def q_body(qb, carry):
        l, m_first = carry
        q0 = pl.multiple_of(qb * TQ, TQ)
        lmax = attn_fast(q0, m_first)
        unsafe = jnp.max(jnp.where(lmax <= L_MAX, 0, 1))

        @pl.when(unsafe > 0)
        def _():
            attn_exact(q0)

        kd = (NT - 1) * 128
        half = TQ // 2
        o = jnp.concatenate([_unpack(ob[g, o_rows(q0), :]) for g in range(NT - 1)], axis=1)
        y0 = lax.dot_general(o[:half], wob[0:kd, :], NN, preferred_element_type=f32)
        o_last = finish_group(NT - 1)
        m_next = ref_max(0, pl.multiple_of(jnp.minimum(qb + 1, S // TQ - 1) * TQ, TQ))
        y1 = lax.dot_general(o[half:], wob[0:kd, :], NN, preferred_element_type=f32)
        y = jnp.concatenate([y0, y1], axis=0) + lax.dot_general(
            o_last, wob[kd:D, :], NN, preferred_element_type=f32)
        x2 = xs[pl.ds(q0, TQ), :] + y
        xs[pl.ds(q0, TQ), :] = x2
        outb[pl.ds(q0, TQ), :] = x2.astype(bf16)

        @pl.when(l == 1)
        def _():
            out_copy(qb).start()

        return l, m_next

    def layer_pair(l, carry):
        ka[:, 0:HALO, :] = jnp.zeros((NT, HALO, 128), f32)
        va[:, 0:HALO, :] = jnp.zeros((NT, HALO, 128), f32)

        @pl.when(l == 0)
        def _():
            x_copy(0).wait()

        load_x(0, l)
        lax.fori_loop(0, S // RB, row_body, l)

        @pl.when(l == 0)
        def _():
            wob_copy.wait()

        lax.fori_loop(0, S // TQ, q_body, (l, ref_max(0, 0)))
        return carry

    ot[...] = jnp.zeros(ot.shape, f32)
    pp[...] = jnp.zeros(pp.shape, u32)
    invs[...] = jnp.ones(invs.shape, f32)
    lax.fori_loop(0, 2, layer_pair, 0)
    for qb in range(S // TQ):
        out_copy(qb).wait()


@jax.jit
def pallas_interleave_layers__sliding_local_dilated__softmax_full_mha__prompt_kernel(
    A_x: jax.Array,
    A_wqkv: jax.Array,
    A_wo: jax.Array,
    B_x: jax.Array,
    B_wqkv: jax.Array,
    B_wo: jax.Array,
):
    del B_x
    x = A_x.reshape(S, D)
    hbm = pl.BlockSpec(memory_space=pl.ANY)
    out = pl.pallas_call(
        _kernel,
        out_shape=jax.ShapeDtypeStruct((S, D), bf16),
        in_specs=[hbm] * 5,
        out_specs=hbm,
        scratch_shapes=[
            pltpu.VMEM((S, D), bf16),
            pltpu.VMEM((D, 3 * D), bf16),
            pltpu.VMEM((D, D), bf16),
            pltpu.VMEM((D, 3 * D), bf16),
            pltpu.VMEM((D, D), bf16),
            pltpu.VMEM((S, D), bf16),
            pltpu.VMEM((DH, 2, 8, D), u32),
            pltpu.VMEM((D // 2, 3 * D), u32),
            pltpu.VMEM((DH, 2, 8, D), u32),
            pltpu.VMEM((D, D), u32),
            pltpu.VMEM((RB // 2, D), u32),
            pltpu.VMEM((S, D), f32),
            pltpu.VMEM((NT, RB, 128), f32),
            pltpu.VMEM((NT, HALO + RB, 128), f32),
            pltpu.VMEM((NT, HALO + RB, 128), f32),
            pltpu.VMEM((D // 2, S), u32),
            pltpu.VMEM((NT, S // 2, 128), u32),
            pltpu.VMEM((D // 2, S), u32),
            pltpu.VMEM((NT + 1, S // 2, 128), u32),
            pltpu.VMEM((128, TQ), f32),
            pltpu.VMEM((KC // 2, TQ), u32),
            pltpu.VMEM((8, TQ), f32),
            pltpu.SemaphoreType.DMA((S // RB,)),
            pltpu.SemaphoreType.DMA((3 * D // WCH,)),
            pltpu.SemaphoreType.DMA((5,)),
            pltpu.SemaphoreType.DMA((S // TQ,)),
        ],
        compiler_params=pltpu.CompilerParams(vmem_limit_bytes=110 * 1024 * 1024),
    )(x, A_wqkv, A_wo, B_wqkv, B_wo)
    return out.reshape(1, S, D)
```

```python
import functools
import math

import jax
import jax.numpy as jnp
from jax import lax
import jax.experimental.pallas as pl
import jax.experimental.pallas.tpu as pltpu

S = 2048
D = 1024
H = 32
DH = 32
WIN = 8
DIL = 2
EPS = 1e-5
NT = D // 128
HALO = 16
QSCALE = (DH ** -0.5) * math.log2(math.e)

SB = 128
NSUB = 2
RB = SB * NSUB
RC = 8
ROW_ORDER = [("a", 0), ("a", 1), ("o", 0), ("o", 1), ("b", 0), ("n", 0), ("b", 1)]
LC = 16
LN_LOOK = 2
LX_LOOK = 2
LN_RELOAD = False
LOOK = 2
DEP_END = False
GATE_COL = 2 * D
TQ = 512
KC = 256
NC = S // KC
HPB = 4
WCH = 512
WA_STARTS = (1, 1, 2, 1, 1, 2)
NFLIGHT = 3
L_MAX = 2.0 ** 64

bf16 = jnp.bfloat16
f32 = jnp.float32
u32 = jnp.uint32

NN = (((1,), (0,)), ((), ()))
NTD = (((1,), (1,)), ((), ()))


def _pack(x):
    return pltpu.bitcast(x, u32)


def _unpack(x):
    return pltpu.bitcast(x, bf16)


def _after(value, dep):
    if dep is None:
        return value
    return jnp.maximum(value, jnp.minimum(dep, -3e38))


def _tree(op, xs):
    xs = list(xs)
    while len(xs) > 1:
        xs = [op(xs[i], xs[i + 1]) if i + 1 < len(xs) else xs[i] for i in range(0, len(xs), 2)]
    return xs[0]


def _recip(x):
    r = pl.reciprocal(x, approx=True)
    return r * (2.0 - x * r)


def _layernorm(load, nrows, look, first_dep=None):
    outs = []
    deps = []
    for c in range(nrows // LC):
        dep = deps[c - look] if c >= look else first_dep
        x = load(c * LC, dep)
        inv_d = 1.0 / D if dep is None else _after(1.0 / D, dep[:, 0:1])
        mu = jnp.sum(x, axis=-1, keepdims=True) * inv_d
        xc = x - mu
        var = jnp.sum(xc * xc, axis=-1, keepdims=True) * (1.0 / D)
        y = xc * lax.rsqrt(var + EPS)
        deps.append(y[:, D - 128:])
        outs.append(y.astype(bf16))
    return jnp.concatenate(outs, axis=0)


def _kernel(x_hbm, wa_hbm, woa_hbm, wb_hbm, wob_hbm, out_hbm,
            xin, wa_raw, woa_raw, wb_raw, wob, outb,
            wat, wan, woa, wqvt, xnb,
            xs, qa, ka, va, qt, kb, vt, ob, ot, pp, invs,
            sem_x, sem_wa, sem_w, sem_o):
    def x_copy(r):
        rows = pl.ds(pl.multiple_of(r * RB, RB), RB)
        return pltpu.make_async_copy(x_hbm.at[rows, :], xin.at[rows, :], sem_x.at[r])

    def wa_copy(i):
        cols = pl.ds(pl.multiple_of(i * WCH, WCH), WCH)
        return pltpu.make_async_copy(wa_hbm.at[:, cols], wa_raw.at[:, cols], sem_wa.at[i])

    def wb_copy(i):
        cols = pl.ds(pl.multiple_of(i * D, D), D)
        return pltpu.make_async_copy(wb_hbm.at[:, cols], wb_raw.at[:, cols], sem_w.at[i])

    woa_copy = pltpu.make_async_copy(woa_hbm, woa_raw, sem_w.at[3])
    wob_copy = pltpu.make_async_copy(wob_hbm, wob, sem_w.at[4])

    def out_copy(qb):
        rows = pl.ds(pl.multiple_of(qb * TQ, TQ), TQ)
        return pltpu.make_async_copy(outb.at[rows, :], out_hbm.at[rows, :], sem_o.at[qb])

    n_wa = 3 * D // WCH
    queue = ([wa_copy(i) for i in range(n_wa)]
             + [woa_copy, wb_copy(0), wb_copy(2), x_copy(0), wb_copy(1)]
             + [x_copy(r) for r in range(1, S // RB)] + [wob_copy])
    for cp in queue[:NFLIGHT]:
        cp.start()
    queue = queue[NFLIGHT:]

    def start_in_loop(i, counts):
        for k, n in enumerate(counts):
            batch = [queue.pop(0) for _ in range(n)]

            @pl.when(i == k)
            def _():
                for cp in batch:
                    cp.start()

    def selection():
        ri = lax.broadcasted_iota(jnp.int32, (256, 256), 0)
        ci = lax.broadcasted_iota(jnp.int32, (256, 256), 1)
        return jnp.where(ci == (ri % 8) * DH + ri // 8, 1.0, 0.0).astype(bf16)

    def transpose(w):
        ri = lax.broadcasted_iota(jnp.int32, (128, 128), 0)
        ci = lax.broadcasted_iota(jnp.int32, (128, 128), 1)
        eye = jnp.where(ri == ci, 1.0, 0.0).astype(bf16)
        return lax.dot_general(eye, w, NTD, preferred_element_type=f32).astype(bf16)

    def pair(a0, a1):
        both = jnp.concatenate([a0.reshape(DH, 8, D), a1.reshape(DH, 8, D)], axis=1)
        return _pack(both.reshape(DH * 16, D).astype(bf16)).reshape(DH, 8, D)

    def prep_wa(i, carry):
        wa_copy(i).wait()
        start_in_loop(i, WA_STARTS)
        sel = selection()
        halves = [lax.dot_general(
            sel, wa_raw[:, pl.ds(pl.multiple_of(i * WCH + j * 256, 256), 256)], NTD,
            preferred_element_type=f32) for j in range(2)]
        wat[:, i % 2, :, :] = pair(*halves)

        @pl.when(i % 2 == 1)
        def _():
            wt = _unpack(wat[...].reshape(D // 2, D))
            cols = pl.ds(pl.multiple_of((i // 2) * D, D), D)
            for j in range(NT):
                wan[j * 64:(j + 1) * 64, cols] = _pack(transpose(wt[:, j * 128:(j + 1) * 128]))

        return carry

    def prep_woa(a, carry):
        sel = selection()
        halves = [lax.dot_general(
            sel, woa_raw[pl.ds(pl.multiple_of(a * 512 + j * 256, 256), 256), :], NN,
            preferred_element_type=f32) for j in range(2)]
        woa[:, a, :, :] = pair(*halves)
        return carry

    def prep_wb(part, carry):
        wb_copy(2 * part).wait()
        for j in range(NT):
            cols = pl.ds(pl.multiple_of(2 * part * D + j * 128, 128), 128)
            rows = pl.ds(pl.multiple_of(part * (D // 2) + j * 64, 64), 64)
            wqvt[rows, :] = _pack(transpose(wb_raw[:, cols]))
        return carry

    lax.fori_loop(0, n_wa, prep_wa, 0)
    woa_copy.wait()
    lax.fori_loop(0, 2, prep_woa, 0)
    lax.fori_loop(0, 2, prep_wb, 0)
    wb_copy(1).wait()
    for cp in queue:
        cp.start()

    def local_attn(r0, s, first_dep):
        outs = []
        deps = []
        for c in range(SB // RC):
            base = s * SB + c * RC
            scale = _after(QSCALE, deps[c - LOOK] if c >= LOOK else first_dep)
            logits = [None] * WIN
            for t in range(NT):
                q = qa[t, base:base + RC, :] * scale
                for w in range(WIN):
                    o0 = HALO + base - DIL * w
                    term = q * ka[t, o0:o0 + RC, :]
                    logits[w] = term if t == 0 else logits[w] + term
            for w in range(WIN):
                acc = logits[w]
                acc = acc + pltpu.roll(acc, 64, 1)
                acc = acc + pltpu.roll(acc, 32, 1)
                if base < DIL * w:
                    row = r0 + base + lax.broadcasted_iota(jnp.int32, (RC, 128), 0)
                    acc = jnp.where(row >= DIL * w, acc, -1e9)
                logits[w] = acc
            m = _tree(jnp.maximum, logits)
            p = [jnp.exp2(lg - m) for lg in logits]
            inv = _recip(_tree(jnp.add, p))
            tiles = []
            for t in range(NT):
                terms = [p[w] * va[t, HALO + base - DIL * w:HALO + base - DIL * w + RC, :]
                         for w in range(WIN)]
                acc = _tree(jnp.add, terms) * inv
                tiles.append(acc.astype(bf16))
            deps.append(acc if DEP_END else m)
            outs.append(jnp.concatenate(tiles, axis=1))
        return jnp.concatenate(outs, axis=0)

    def load_x(r, l, look):
        r0 = pl.multiple_of(r * RB, RB)

        def load(start, dep):
            rows = pl.ds(r0 + start, LC)
            lvec = _after(jnp.full((LC, 128), l, f32), dep)
            first = jnp.concatenate([lvec == 0.0] * NT, axis=1)
            x = jnp.where(first, xin[rows, :].astype(f32), xs[rows, :])
            xs[rows, :] = x
            return x

        xnb[...] = _pack(_layernorm(load, RB, look))

    def row_body(r, l):
        r0 = pl.multiple_of(r * RB, RB)
        rn = jnp.minimum(r + 1, S // RB - 1)

        @pl.when(jnp.logical_and(l == 0, r + 1 < S // RB))
        def _():
            x_copy(rn).wait()

        rows = [pl.ds(r0 + s * SB, SB) for s in range(NSUB)]
        gate = {}
        xn2 = {}

        def qkv_a(s):
            xn = _unpack(xnb[s * SB // 2:(s + 1) * SB // 2, :])
            y = lax.dot_general(xn, _unpack(wan[...]), NN, preferred_element_type=f32)
            for t in range(NT):
                qa[t, s * SB:(s + 1) * SB, :] = y[:, t * 128:(t + 1) * 128]
                ka[t, HALO + s * SB:HALO + (s + 1) * SB, :] = y[:, D + t * 128:D + (t + 1) * 128]
                va[t, HALO + s * SB:HALO + (s + 1) * SB, :] = y[:, 2 * D + t * 128:2 * D + (t + 1) * 128]
            gate[s] = y[SB - RC:SB, GATE_COL - 128:GATE_COL]

        def out_a(s):
            o = local_attn(r0, s, gate[s])
            x1 = xs[rows[s], :] + lax.dot_general(o, _unpack(woa[...].reshape(D // 2, D)), NN,
                                                  preferred_element_type=f32)
            xs[rows[s], :] = x1
            if LN_RELOAD:
                xn2[s] = _layernorm(lambda st, dep: xs[pl.ds(r0 + s * SB + st, LC), :], SB, LN_LOOK)
            else:
                xn2[s] = _layernorm(lambda st, dep: x1[st:st + LC], SB, LN_LOOK)

        def qkv_b(s):
            cols = pl.ds(r0 + s * SB, SB)
            yq = lax.dot_general(_unpack(wqvt[0:D // 2, :]), xn2[s], NTD, preferred_element_type=f32)
            qt[:, cols] = _pack((yq * QSCALE).astype(bf16))
            yv = lax.dot_general(_unpack(wqvt[D // 2:D, :]), xn2[s], NTD, preferred_element_type=f32)
            vt[:, cols] = _pack(yv.astype(bf16))
            yk = lax.dot_general(xn2[s], wb_raw[:, D:2 * D], NN, preferred_element_type=f32).astype(bf16)
            krows = pl.ds(pl.multiple_of((r0 + s * SB) // 2, SB // 2), SB // 2)
            for g in range(NT):
                kb[g, krows, :] = _pack(yk[:, g * 128:(g + 1) * 128])

        steps = {"a": qkv_a, "o": out_a, "b": qkv_b}
        for name, s in ROW_ORDER:
            if name == "n":
                ka[:, 0:HALO, :] = ka[:, RB:RB + HALO, :]
                va[:, 0:HALO, :] = va[:, RB:RB + HALO, :]
                load_x(rn, jnp.where(r + 1 < S // RB, l, 1), LX_LOOK)
            else:
                steps[name](s)
        return l

    def head_weights(g, hh, q0):
        w = qt[pl.ds(pl.multiple_of(g * 64 + hh * 16, 16), 16), pl.ds(q0, TQ)]
        parts = []
        if hh > 0:
            parts.append(jnp.zeros((16 * hh, TQ), u32))
        parts.append(w)
        if hh < 3:
            parts.append(jnp.zeros((16 * (3 - hh), TQ), u32))
        return _unpack(jnp.concatenate(parts, axis=0))

    def ref_max(g, q0):
        k0 = kb[g, 0:8, :]
        lane = lax.broadcasted_iota(jnp.int32, (8, 128), 1) // DH
        lhs = jnp.concatenate(
            [jnp.where(lane == hh, k0, jnp.zeros_like(k0)) for hh in range(4)], axis=0)
        w = _unpack(qt[pl.ds(pl.multiple_of(g * 64, 64), 64), pl.ds(q0, TQ)])
        s0 = jnp.dot(_unpack(lhs), w, preferred_element_type=f32)
        return jnp.concatenate(
            [jnp.broadcast_to(jnp.max(s0[16 * hh:16 * hh + 16], axis=0, keepdims=True), (8, TQ))
             for hh in range(4)], axis=0)

    def v_rows(g, hh, c):
        rows = pl.ds(pl.multiple_of(g * 64 + hh * 16, 16), 16)
        return _unpack(vt[rows, c * KC:(c + 1) * KC])

    def finish_group(g):
        o = jnp.dot(v_rows(g, HPB - 1, NC - 1), _unpack(pp[...]), preferred_element_type=f32)
        last = (ot[3 * DH:4 * DH, :] + o) * invs[0:1, :]
        return jnp.concatenate([ot[0:3 * DH, :], last], axis=0).T.astype(bf16)

    def o_rows(q0):
        return pl.ds(pl.multiple_of(q0 // 2, TQ // 2), TQ // 2)

    def attn_fast(q0, m_first):
        def group(g, carry):
            m_all, lmax = carry
            st = {}

            def qk(hh, c):
                if c == 0:
                    st[hh] = dict(w=head_weights(g, hh, q0))
                kc = _unpack(kb[g, c * KC // 2:(c + 1) * KC // 2, :])
                return jnp.dot(kc, st[hh]["w"], preferred_element_type=f32)

            def pv(hh, c, s):
                d = st[hh]
                m = m_all[8 * hh:8 * hh + 8]
                p = jnp.exp2(s.reshape(KC // 8, 8, TQ) - m[None])
                lc = jnp.sum(p, axis=0)
                d["l"] = lc if c == 0 else d["l"] + lc
                p = p.reshape(KC, TQ).astype(bf16)
                if c == NC - 1:
                    d["lsum"] = jnp.sum(d["l"], axis=0, keepdims=True)
                if hh == HPB - 1 and c == NC - 1:
                    pp[...] = _pack(p)
                    ot[hh * DH:(hh + 1) * DH, :] = d["acc"]
                    invs[...] = jnp.broadcast_to(_recip(d["lsum"]), (8, TQ))
                    return
                o = jnp.dot(v_rows(g, hh, c), p, preferred_element_type=f32)
                d["acc"] = o if c == 0 else d["acc"] + o
                if c == NC - 1:
                    ot[hh * DH:(hh + 1) * DH, :] = d["acc"] * _recip(d["lsum"])

            m_next = None
            pend = None
            for hh in range(HPB):
                for c in range(NC):
                    if hh == HPB - 1 and c == 0:
                        m_next = ref_max(jnp.minimum(g + 1, NT - 1), q0)
                    s = qk(hh, c)
                    if pend is None:
                        ob[jnp.where(g == 0, NT, g - 1), o_rows(q0), :] = _pack(
                            finish_group(jnp.maximum(g - 1, 0)))
                    else:
                        pv(*pend)
                    pend = (hh, c, s)
            pv(*pend)
            for hh in range(HPB):
                lmax = jnp.maximum(lmax, st[hh]["lsum"])
            return m_next, lmax

        _, lmax = lax.fori_loop(0, NT, group, (m_first, jnp.zeros((1, TQ), f32)))
        return lmax

    def attn_exact(q0):
        def group(g, carry):
            def head(hh, carry2):
                w = qt[pl.ds(pl.multiple_of(g * 64, 64), 64), pl.ds(q0, TQ)]
                row = lax.broadcasted_iota(jnp.int32, (64, TQ), 0) // 16
                w = _unpack(jnp.where(row == hh, w, jnp.zeros_like(w)))
                s = jnp.dot(_unpack(kb[g]), w, preferred_element_type=f32)
                p = jnp.exp2(s - jnp.max(s, axis=0, keepdims=True))
                l = jnp.sum(p, axis=0, keepdims=True)
                v = _unpack(vt[pl.ds(pl.multiple_of(g * 64 + hh * 16, 16), 16), :])
                o = jnp.dot(v, p.astype(bf16), preferred_element_type=f32)
                ot[pl.ds(pl.multiple_of(hh * DH, DH), DH), :] = o * (1.0 / l)
                return carry2
            lax.fori_loop(0, 4, head, 0)
            ob[g, o_rows(q0), :] = _pack(ot[...].T.astype(bf16))
            return carry
        lax.fori_loop(0, NT, group, 0)
        pp[...] = jnp.zeros(pp.shape, u32)
        invs[...] = jnp.ones(invs.shape, f32)

    def q_body(qb, carry):
        l, m_first = carry
        q0 = pl.multiple_of(qb * TQ, TQ)
        lmax = attn_fast(q0, m_first)
        unsafe = jnp.max(jnp.where(lmax <= L_MAX, 0, 1))

        @pl.when(unsafe > 0)
        def _():
            attn_exact(q0)

        kd = (NT - 1) * 128
        half = TQ // 2
        o = jnp.concatenate([_unpack(ob[g, o_rows(q0), :]) for g in range(NT - 1)], axis=1)
        y0 = lax.dot_general(o[:half], wob[0:kd, :], NN, preferred_element_type=f32)
        o_last = finish_group(NT - 1)
        m_next = ref_max(0, pl.multiple_of(jnp.minimum(qb + 1, S // TQ - 1) * TQ, TQ))
        y1 = lax.dot_general(o[half:], wob[0:kd, :], NN, preferred_element_type=f32)
        y = jnp.concatenate([y0, y1], axis=0) + lax.dot_general(
            o_last, wob[kd:D, :], NN, preferred_element_type=f32)
        x2 = xs[pl.ds(q0, TQ), :] + y
        xs[pl.ds(q0, TQ), :] = x2
        outb[pl.ds(q0, TQ), :] = x2.astype(bf16)

        @pl.when(l == 1)
        def _():
            out_copy(qb).start()

        return l, m_next

    def layer_pair(l, carry):
        ka[:, 0:HALO, :] = jnp.zeros((NT, HALO, 128), f32)
        va[:, 0:HALO, :] = jnp.zeros((NT, HALO, 128), f32)

        @pl.when(l == 0)
        def _():
            x_copy(0).wait()

        load_x(0, l, 8)
        lax.fori_loop(0, S // RB, row_body, l)

        @pl.when(l == 0)
        def _():
            wob_copy.wait()

        lax.fori_loop(0, S // TQ, q_body, (l, ref_max(0, 0)))
        return carry

    ot[...] = jnp.zeros(ot.shape, f32)
    pp[...] = jnp.zeros(pp.shape, u32)
    invs[...] = jnp.ones(invs.shape, f32)
    lax.fori_loop(0, 2, layer_pair, 0)
    for qb in range(S // TQ):
        out_copy(qb).wait()


@jax.jit
def pallas_interleave_layers__sliding_local_dilated__softmax_full_mha__prompt_kernel(
    A_x: jax.Array,
    A_wqkv: jax.Array,
    A_wo: jax.Array,
    B_x: jax.Array,
    B_wqkv: jax.Array,
    B_wo: jax.Array,
):
    del B_x
    x = A_x.reshape(S, D)
    hbm = pl.BlockSpec(memory_space=pl.ANY)
    out = pl.pallas_call(
        _kernel,
        out_shape=jax.ShapeDtypeStruct((S, D), bf16),
        in_specs=[hbm] * 5,
        out_specs=hbm,
        scratch_shapes=[
            pltpu.VMEM((S, D), bf16),
            pltpu.VMEM((D, 3 * D), bf16),
            pltpu.VMEM((D, D), bf16),
            pltpu.VMEM((D, 3 * D), bf16),
            pltpu.VMEM((D, D), bf16),
            pltpu.VMEM((S, D), bf16),
            pltpu.VMEM((DH, 2, 8, D), u32),
            pltpu.VMEM((D // 2, 3 * D), u32),
            pltpu.VMEM((DH, 2, 8, D), u32),
            pltpu.VMEM((D, D), u32),
            pltpu.VMEM((RB // 2, D), u32),
            pltpu.VMEM((S, D), f32),
            pltpu.VMEM((NT, RB, 128), f32),
            pltpu.VMEM((NT, HALO + RB, 128), f32),
            pltpu.VMEM((NT, HALO + RB, 128), f32),
            pltpu.VMEM((D // 2, S), u32),
            pltpu.VMEM((NT, S // 2, 128), u32),
            pltpu.VMEM((D // 2, S), u32),
            pltpu.VMEM((NT + 1, S // 2, 128), u32),
            pltpu.VMEM((128, TQ), f32),
            pltpu.VMEM((KC // 2, TQ), u32),
            pltpu.VMEM((8, TQ), f32),
            pltpu.SemaphoreType.DMA((S // RB,)),
            pltpu.SemaphoreType.DMA((3 * D // WCH,)),
            pltpu.SemaphoreType.DMA((5,)),
            pltpu.SemaphoreType.DMA((S // TQ,)),
        ],
        compiler_params=pltpu.CompilerParams(vmem_limit_bytes=110 * 1024 * 1024),
    )(x, A_wqkv, A_wo, B_wqkv, B_wo)
    return out.reshape(1, S, D)
```

```python
import functools
import math

import jax
import jax.numpy as jnp
from jax import lax
import jax.experimental.pallas as pl
import jax.experimental.pallas.tpu as pltpu

S = 2048
D = 1024
H = 32
DH = 32
WIN = 8
DIL = 2
EPS = 1e-5
NT = D // 128
HALO = 16
QSCALE = (DH ** -0.5) * math.log2(math.e)

SB = 128
NSUB = 2
RB = SB * NSUB
RC = 8
ROW_ORDER = [("a", 0), ("a", 1), ("o", 0), ("o", 1), ("b", 0), ("n", 0), ("b", 1)]
LC = 8
LN_LOOK = 2
LX_LOOK = 2
LN_RELOAD = False
LOOK = 2
DEP_END = False
GATE_COL = 2 * D
TQ = 512
KC = 256
NC = S // KC
HPB = 4
WCH = 512
WA_STARTS = (1, 1, 2, 1, 1, 2)
NFLIGHT = 3
L_MAX = 2.0 ** 64

bf16 = jnp.bfloat16
f32 = jnp.float32
u32 = jnp.uint32

NN = (((1,), (0,)), ((), ()))
NTD = (((1,), (1,)), ((), ()))


def _pack(x):
    return pltpu.bitcast(x, u32)


def _unpack(x):
    return pltpu.bitcast(x, bf16)


def _after(value, dep):
    if dep is None:
        return value
    return jnp.maximum(value, jnp.minimum(dep, -3e38))


def _tree(op, xs):
    xs = list(xs)
    while len(xs) > 1:
        xs = [op(xs[i], xs[i + 1]) if i + 1 < len(xs) else xs[i] for i in range(0, len(xs), 2)]
    return xs[0]


def _recip(x):
    r = pl.reciprocal(x, approx=True)
    return r * (2.0 - x * r)


def _layernorm(load, nrows, look, first_dep=None):
    outs = []
    deps = []
    for c in range(nrows // LC):
        dep = deps[c - look] if c >= look else first_dep
        x = load(c * LC, dep)
        mu = jnp.broadcast_to(jnp.sum(x, axis=-1, keepdims=True), (LC, 128)) * _after(1.0 / D, dep)
        xc = x - jnp.concatenate([mu] * NT, axis=1)
        var = jnp.sum(xc * xc, axis=-1, keepdims=True) * (1.0 / D)
        y = xc * lax.rsqrt(var + EPS)
        deps.append(y[:, D - 128:])
        outs.append(y)
    return jnp.concatenate(outs, axis=0).astype(bf16)


def _kernel(x_hbm, wa_hbm, woa_hbm, wb_hbm, wob_hbm, out_hbm,
            xin, wa_raw, woa_raw, wb_raw, wob, outb,
            wat, wan, woa, wqvt, xnb,
            xs, qa, ka, va, qt, kb, vt, ob, ot, pp, invs,
            sem_x, sem_wa, sem_w, sem_o):
    def x_copy(r):
        rows = pl.ds(pl.multiple_of(r * RB, RB), RB)
        return pltpu.make_async_copy(x_hbm.at[rows, :], xin.at[rows, :], sem_x.at[r])

    def wa_copy(i):
        cols = pl.ds(pl.multiple_of(i * WCH, WCH), WCH)
        return pltpu.make_async_copy(wa_hbm.at[:, cols], wa_raw.at[:, cols], sem_wa.at[i])

    def wb_copy(i):
        cols = pl.ds(pl.multiple_of(i * D, D), D)
        return pltpu.make_async_copy(wb_hbm.at[:, cols], wb_raw.at[:, cols], sem_w.at[i])

    woa_copy = pltpu.make_async_copy(woa_hbm, woa_raw, sem_w.at[3])
    wob_copy = pltpu.make_async_copy(wob_hbm, wob, sem_w.at[4])

    def out_copy(qb):
        rows = pl.ds(pl.multiple_of(qb * TQ, TQ), TQ)
        return pltpu.make_async_copy(outb.at[rows, :], out_hbm.at[rows, :], sem_o.at[qb])

    n_wa = 3 * D // WCH
    queue = ([wa_copy(i) for i in range(n_wa)]
             + [woa_copy, wb_copy(0), wb_copy(2), x_copy(0), wb_copy(1)]
             + [x_copy(r) for r in range(1, S // RB)] + [wob_copy])
    for cp in queue[:NFLIGHT]:
        cp.start()
    queue = queue[NFLIGHT:]

    def start_in_loop(i, counts):
        for k, n in enumerate(counts):
            batch = [queue.pop(0) for _ in range(n)]

            @pl.when(i == k)
            def _():
                for cp in batch:
                    cp.start()

    def selection():
        ri = lax.broadcasted_iota(jnp.int32, (256, 256), 0)
        ci = lax.broadcasted_iota(jnp.int32, (256, 256), 1)
        return jnp.where(ci == (ri % 8) * DH + ri // 8, 1.0, 0.0).astype(bf16)

    def transpose(w):
        ri = lax.broadcasted_iota(jnp.int32, (128, 128), 0)
        ci = lax.broadcasted_iota(jnp.int32, (128, 128), 1)
        eye = jnp.where(ri == ci, 1.0, 0.0).astype(bf16)
        return lax.dot_general(eye, w, NTD, preferred_element_type=f32).astype(bf16)

    def pair(a0, a1):
        both = jnp.concatenate([a0.reshape(DH, 8, D), a1.reshape(DH, 8, D)], axis=1)
        return _pack(both.reshape(DH * 16, D).astype(bf16)).reshape(DH, 8, D)

    def prep_wa(i, carry):
        wa_copy(i).wait()
        start_in_loop(i, WA_STARTS)
        sel = selection()
        halves = [lax.dot_general(
            sel, wa_raw[:, pl.ds(pl.multiple_of(i * WCH + j * 256, 256), 256)], NTD,
            preferred_element_type=f32) for j in range(2)]
        wat[:, i % 2, :, :] = pair(*halves)

        @pl.when(i % 2 == 1)
        def _():
            wt = _unpack(wat[...].reshape(D // 2, D))
            cols = pl.ds(pl.multiple_of((i // 2) * D, D), D)
            for j in range(NT):
                wan[j * 64:(j + 1) * 64, cols] = _pack(transpose(wt[:, j * 128:(j + 1) * 128]))

        return carry

    def prep_woa(a, carry):
        sel = selection()
        halves = [lax.dot_general(
            sel, woa_raw[pl.ds(pl.multiple_of(a * 512 + j * 256, 256), 256), :], NN,
            preferred_element_type=f32) for j in range(2)]
        woa[:, a, :, :] = pair(*halves)
        return carry

    def prep_wb(part, carry):
        wb_copy(2 * part).wait()
        for j in range(NT):
            cols = pl.ds(pl.multiple_of(2 * part * D + j * 128, 128), 128)
            rows = pl.ds(pl.multiple_of(part * (D // 2) + j * 64, 64), 64)
            wqvt[rows, :] = _pack(transpose(wb_raw[:, cols]))
        return carry

    lax.fori_loop(0, n_wa, prep_wa, 0)
    woa_copy.wait()
    lax.fori_loop(0, 2, prep_woa, 0)
    lax.fori_loop(0, 2, prep_wb, 0)
    wb_copy(1).wait()
    for cp in queue:
        cp.start()

    def local_attn(r0, s, first_dep):
        outs = []
        deps = []
        for c in range(SB // RC):
            base = s * SB + c * RC
            scale = _after(QSCALE, deps[c - LOOK] if c >= LOOK else first_dep)
            logits = [None] * WIN
            for t in range(NT):
                q = qa[t, base:base + RC, :] * scale
                for w in range(WIN):
                    o0 = HALO + base - DIL * w
                    term = q * ka[t, o0:o0 + RC, :]
                    logits[w] = term if t == 0 else logits[w] + term
            for w in range(WIN):
                acc = logits[w]
                acc = acc + pltpu.roll(acc, 64, 1)
                acc = acc + pltpu.roll(acc, 32, 1)
                if base < DIL * w:
                    row = r0 + base + lax.broadcasted_iota(jnp.int32, (RC, 128), 0)
                    acc = jnp.where(row >= DIL * w, acc, -1e9)
                logits[w] = acc
            m = _tree(jnp.maximum, logits)
            p = [jnp.exp2(lg - m) for lg in logits]
            inv = _recip(_tree(jnp.add, p))
            tiles = []
            for t in range(NT):
                terms = [p[w] * va[t, HALO + base - DIL * w:HALO + base - DIL * w + RC, :]
                         for w in range(WIN)]
                acc = _tree(jnp.add, terms) * inv
                tiles.append(acc.astype(bf16))
            deps.append(acc if DEP_END else m)
            outs.append(jnp.concatenate(tiles, axis=1))
        return jnp.concatenate(outs, axis=0)

    def load_x(r, l, look):
        r0 = pl.multiple_of(r * RB, RB)

        def load(start, dep):
            rows = pl.ds(r0 + start, LC)
            lvec = _after(jnp.full((LC, 128), l, f32), dep)
            first = jnp.concatenate([lvec == 0.0] * NT, axis=1)
            xi = xin[pl.ds(r0 + start // 16 * 16, 16), :].astype(f32)[start % 16:start % 16 + LC]
            x = jnp.where(first, xi, xs[rows, :])
            xs[rows, :] = x
            return x

        xnb[...] = _pack(_layernorm(load, RB, look))

    def row_body(r, l):
        r0 = pl.multiple_of(r * RB, RB)
        rn = jnp.minimum(r + 1, S // RB - 1)

        @pl.when(jnp.logical_and(l == 0, r + 1 < S // RB))
        def _():
            x_copy(rn).wait()

        rows = [pl.ds(r0 + s * SB, SB) for s in range(NSUB)]
        gate = {}
        xn2 = {}

        def qkv_a(s):
            xn = _unpack(xnb[s * SB // 2:(s + 1) * SB // 2, :])
            y = lax.dot_general(xn, _unpack(wan[...]), NN, preferred_element_type=f32)
            for t in range(NT):
                qa[t, s * SB:(s + 1) * SB, :] = y[:, t * 128:(t + 1) * 128]
                ka[t, HALO + s * SB:HALO + (s + 1) * SB, :] = y[:, D + t * 128:D + (t + 1) * 128]
                va[t, HALO + s * SB:HALO + (s + 1) * SB, :] = y[:, 2 * D + t * 128:2 * D + (t + 1) * 128]
            gate[s] = y[SB - RC:SB, GATE_COL - 128:GATE_COL]

        def out_a(s):
            o = local_attn(r0, s, gate[s])
            x1 = xs[rows[s], :] + lax.dot_general(o, _unpack(woa[...].reshape(D // 2, D)), NN,
                                                  preferred_element_type=f32)
            xs[rows[s], :] = x1
            if LN_RELOAD:
                xn2[s] = _layernorm(lambda st, dep: xs[pl.ds(r0 + s * SB + st, LC), :], SB, LN_LOOK)
            else:
                xn2[s] = _layernorm(lambda st, dep: x1[st:st + LC], SB, LN_LOOK)

        def qkv_b(s):
            cols = pl.ds(r0 + s * SB, SB)
            yq = lax.dot_general(_unpack(wqvt[0:D // 2, :]), xn2[s], NTD, preferred_element_type=f32)
            qt[:, cols] = _pack((yq * QSCALE).astype(bf16))
            yv = lax.dot_general(_unpack(wqvt[D // 2:D, :]), xn2[s], NTD, preferred_element_type=f32)
            vt[:, cols] = _pack(yv.astype(bf16))
            yk = lax.dot_general(xn2[s], wb_raw[:, D:2 * D], NN, preferred_element_type=f32).astype(bf16)
            krows = pl.ds(pl.multiple_of((r0 + s * SB) // 2, SB // 2), SB // 2)
            for g in range(NT):
                kb[g, krows, :] = _pack(yk[:, g * 128:(g + 1) * 128])

        steps = {"a": qkv_a, "o": out_a, "b": qkv_b}
        for name, s in ROW_ORDER:
            if name == "n":
                ka[:, 0:HALO, :] = ka[:, RB:RB + HALO, :]
                va[:, 0:HALO, :] = va[:, RB:RB + HALO, :]
                load_x(rn, jnp.where(r + 1 < S // RB, l, 1), LX_LOOK)
            else:
                steps[name](s)
        return l

    def head_weights(g, hh, q0):
        w = qt[pl.ds(pl.multiple_of(g * 64 + hh * 16, 16), 16), pl.ds(q0, TQ)]
        parts = []
        if hh > 0:
            parts.append(jnp.zeros((16 * hh, TQ), u32))
        parts.append(w)
        if hh < 3:
            parts.append(jnp.zeros((16 * (3 - hh), TQ), u32))
        return _unpack(jnp.concatenate(parts, axis=0))

    def v_rows(g, hh, c):
        rows = pl.ds(pl.multiple_of(g * 64 + hh * 16, 16), 16)
        return _unpack(vt[rows, c * KC:(c + 1) * KC])

    def finish_group(g):
        o = jnp.dot(v_rows(g, HPB - 1, NC - 1), _unpack(pp[...]), preferred_element_type=f32)
        last = (ot[3 * DH:4 * DH, :] + o) * invs[0:1, :]
        return jnp.concatenate([ot[0:3 * DH, :], last], axis=0).T.astype(bf16)

    def o_rows(q0):
        return pl.ds(pl.multiple_of(q0 // 2, TQ // 2), TQ // 2)

    def attn_fast(q0):
        def group(g, lmax):
            st = {}

            def qk(hh, c):
                if c == 0:
                    st[hh] = dict(w=head_weights(g, hh, q0))
                kc = _unpack(kb[g, c * KC // 2:(c + 1) * KC // 2, :])
                return jnp.dot(kc, st[hh]["w"], preferred_element_type=f32)

            def pv(hh, c, s):
                d = st[hh]
                if c == 0:
                    d["m"] = jnp.broadcast_to(jnp.max(s[0:8], axis=0, keepdims=True), (8, TQ))
                p = jnp.exp2(s.reshape(KC // 8, 8, TQ) - d["m"][None])
                lc = jnp.sum(p, axis=0)
                d["l"] = lc if c == 0 else d["l"] + lc
                p = p.reshape(KC, TQ).astype(bf16)
                if c == NC - 1:
                    d["lsum"] = jnp.sum(d["l"], axis=0, keepdims=True)
                if hh == HPB - 1 and c == NC - 1:
                    pp[...] = _pack(p)
                    ot[hh * DH:(hh + 1) * DH, :] = d["acc"]
                    invs[...] = jnp.broadcast_to(_recip(d["lsum"]), (8, TQ))
                    return
                o = jnp.dot(v_rows(g, hh, c), p, preferred_element_type=f32)
                d["acc"] = o if c == 0 else d["acc"] + o
                if c == NC - 1:
                    ot[hh * DH:(hh + 1) * DH, :] = d["acc"] * _recip(d["lsum"])

            pend = None
            for hh in range(HPB):
                for c in range(NC):
                    s = qk(hh, c)
                    if pend is None:
                        ob[jnp.where(g == 0, NT, g - 1), o_rows(q0), :] = _pack(
                            finish_group(jnp.maximum(g - 1, 0)))
                    else:
                        pv(*pend)
                    pend = (hh, c, s)
            pv(*pend)
            for hh in range(HPB):
                lmax = jnp.maximum(lmax, st[hh]["lsum"])
            return lmax

        return lax.fori_loop(0, NT, group, jnp.zeros((1, TQ), f32))

    def attn_exact(q0):
        def group(g, carry):
            def head(hh, carry2):
                w = qt[pl.ds(pl.multiple_of(g * 64, 64), 64), pl.ds(q0, TQ)]
                row = lax.broadcasted_iota(jnp.int32, (64, TQ), 0) // 16
                w = _unpack(jnp.where(row == hh, w, jnp.zeros_like(w)))
                s = jnp.dot(_unpack(kb[g]), w, preferred_element_type=f32)
                p = jnp.exp2(s - jnp.max(s, axis=0, keepdims=True))
                l = jnp.sum(p, axis=0, keepdims=True)
                v = _unpack(vt[pl.ds(pl.multiple_of(g * 64 + hh * 16, 16), 16), :])
                o = jnp.dot(v, p.astype(bf16), preferred_element_type=f32)
                ot[pl.ds(pl.multiple_of(hh * DH, DH), DH), :] = o * (1.0 / l)
                return carry2
            lax.fori_loop(0, 4, head, 0)
            ob[g, o_rows(q0), :] = _pack(ot[...].T.astype(bf16))
            return carry
        lax.fori_loop(0, NT, group, 0)
        pp[...] = jnp.zeros(pp.shape, u32)
        invs[...] = jnp.ones(invs.shape, f32)

    def q_body(qb, l):
        q0 = pl.multiple_of(qb * TQ, TQ)
        lmax = attn_fast(q0)
        unsafe = jnp.max(jnp.where(lmax <= L_MAX, 0, 1))

        @pl.when(unsafe > 0)
        def _():
            attn_exact(q0)

        kd = (NT - 1) * 128
        half = TQ // 2
        o = jnp.concatenate([_unpack(ob[g, o_rows(q0), :]) for g in range(NT - 1)], axis=1)
        y0 = lax.dot_general(o[:half], wob[0:kd, :], NN, preferred_element_type=f32)
        o_last = finish_group(NT - 1)
        y1 = lax.dot_general(o[half:], wob[0:kd, :], NN, preferred_element_type=f32)
        y = jnp.concatenate([y0, y1], axis=0) + lax.dot_general(
            o_last, wob[kd:D, :], NN, preferred_element_type=f32)
        x2 = xs[pl.ds(q0, TQ), :] + y
        xs[pl.ds(q0, TQ), :] = x2
        outb[pl.ds(q0, TQ), :] = x2.astype(bf16)

        @pl.when(l == 1)
        def _():
            out_copy(qb).start()

        return l

    def layer_pair(l, carry):
        ka[:, 0:HALO, :] = jnp.zeros((NT, HALO, 128), f32)
        va[:, 0:HALO, :] = jnp.zeros((NT, HALO, 128), f32)

        @pl.when(l == 0)
        def _():
            x_copy(0).wait()

        load_x(0, l, 8)
        lax.fori_loop(0, S // RB, row_body, l)

        @pl.when(l == 0)
        def _():
            wob_copy.wait()

        lax.fori_loop(0, S // TQ, q_body, l)
        return carry

    ot[...] = jnp.zeros(ot.shape, f32)
    pp[...] = jnp.zeros(pp.shape, u32)
    invs[...] = jnp.ones(invs.shape, f32)
    lax.fori_loop(0, 2, layer_pair, 0)
    for qb in range(S // TQ):
        out_copy(qb).wait()


@jax.jit
def pallas_interleave_layers__sliding_local_dilated__softmax_full_mha__prompt_kernel(
    A_x: jax.Array,
    A_wqkv: jax.Array,
    A_wo: jax.Array,
    B_x: jax.Array,
    B_wqkv: jax.Array,
    B_wo: jax.Array,
):
    del B_x
    x = A_x.reshape(S, D)
    hbm = pl.BlockSpec(memory_space=pl.ANY)
    out = pl.pallas_call(
        _kernel,
        out_shape=jax.ShapeDtypeStruct((S, D), bf16),
        in_specs=[hbm] * 5,
        out_specs=hbm,
        scratch_shapes=[
            pltpu.VMEM((S, D), bf16),
            pltpu.VMEM((D, 3 * D), bf16),
            pltpu.VMEM((D, D), bf16),
            pltpu.VMEM((D, 3 * D), bf16),
            pltpu.VMEM((D, D), bf16),
            pltpu.VMEM((S, D), bf16),
            pltpu.VMEM((DH, 2, 8, D), u32),
            pltpu.VMEM((D // 2, 3 * D), u32),
            pltpu.VMEM((DH, 2, 8, D), u32),
            pltpu.VMEM((D, D), u32),
            pltpu.VMEM((RB // 2, D), u32),
            pltpu.VMEM((S, D), f32),
            pltpu.VMEM((NT, RB, 128), f32),
            pltpu.VMEM((NT, HALO + RB, 128), f32),
            pltpu.VMEM((NT, HALO + RB, 128), f32),
            pltpu.VMEM((D // 2, S), u32),
            pltpu.VMEM((NT, S // 2, 128), u32),
            pltpu.VMEM((D // 2, S), u32),
            pltpu.VMEM((NT + 1, S // 2, 128), u32),
            pltpu.VMEM((128, TQ), f32),
            pltpu.VMEM((KC // 2, TQ), u32),
            pltpu.VMEM((8, TQ), f32),
            pltpu.SemaphoreType.DMA((S // RB,)),
            pltpu.SemaphoreType.DMA((3 * D // WCH,)),
            pltpu.SemaphoreType.DMA((5,)),
            pltpu.SemaphoreType.DMA((S // TQ,)),
        ],
        compiler_params=pltpu.CompilerParams(vmem_limit_bytes=110 * 1024 * 1024),
    )(x, A_wqkv, A_wo, B_wqkv, B_wo)
    return out.reshape(1, S, D)
```

```python
import functools
import math

import jax
import jax.numpy as jnp
from jax import lax
import jax.experimental.pallas as pl
import jax.experimental.pallas.tpu as pltpu

S = 2048
D = 1024
H = 32
DH = 32
WIN = 8
DIL = 2
EPS = 1e-5
NT = D // 128
HALO = 16
QSCALE = (DH ** -0.5) * math.log2(math.e)

SB = 128
NSUB = 2
RB = SB * NSUB
RC = 8
ROW_ORDER = [("a", 0), ("a", 1), ("o", 0), ("o", 1), ("b", 0), ("n", 0), ("b", 1)]
LC = 8
LN_LOOK = 2
LX_LOOK = 2
LN_RELOAD = False
LOOK = 2
DEP_END = False
GATE_COL = 2 * D
TQ = 512
KC = 256
NC = S // KC
OC = 128
HPB = 4
WCH = 512
WA_STARTS = (1, 1, 2, 1, 1, 2)
NFLIGHT = 3
L_MAX = 2.0 ** 64

bf16 = jnp.bfloat16
f32 = jnp.float32
u32 = jnp.uint32

NN = (((1,), (0,)), ((), ()))
NTD = (((1,), (1,)), ((), ()))


def _pack(x):
    return pltpu.bitcast(x, u32)


def _unpack(x):
    return pltpu.bitcast(x, bf16)


def _after(value, dep):
    if dep is None:
        return value
    return jnp.maximum(value, jnp.minimum(dep, -3e38))


def _tree(op, xs):
    xs = list(xs)
    while len(xs) > 1:
        xs = [op(xs[i], xs[i + 1]) if i + 1 < len(xs) else xs[i] for i in range(0, len(xs), 2)]
    return xs[0]


def _recip(x):
    r = pl.reciprocal(x, approx=True)
    return r * (2.0 - x * r)


def _layernorm(load, nrows, look, first_dep=None):
    outs = []
    deps = []
    for c in range(nrows // LC):
        dep = deps[c - look] if c >= look else first_dep
        x = load(c * LC, dep)
        mu = jnp.broadcast_to(jnp.sum(x, axis=-1, keepdims=True), (LC, 128)) * _after(1.0 / D, dep)
        xc = x - jnp.concatenate([mu] * NT, axis=1)
        var = jnp.sum(xc * xc, axis=-1, keepdims=True) * (1.0 / D)
        y = xc * lax.rsqrt(var + EPS)
        deps.append(y[:, D - 128:])
        outs.append(y)
    return jnp.concatenate(outs, axis=0).astype(bf16)


def _kernel(x_hbm, wa_hbm, woa_hbm, wb_hbm, wob_hbm, out_hbm,
            xin, wa_raw, woa_raw, wb_raw, wob, outb,
            wat, wan, woa, wqvt, xnb,
            xs, xs2, qa, ka, va, qt, kb, vt, ob, ot, pp, invs, lmx,
            sem_x, sem_wa, sem_w, sem_o):
    def x_copy(r):
        rows = pl.ds(pl.multiple_of(r * RB, RB), RB)
        return pltpu.make_async_copy(x_hbm.at[rows, :], xin.at[rows, :], sem_x.at[r])

    def wa_copy(i):
        cols = pl.ds(pl.multiple_of(i * WCH, WCH), WCH)
        return pltpu.make_async_copy(wa_hbm.at[:, cols], wa_raw.at[:, cols], sem_wa.at[i])

    def wb_copy(i):
        cols = pl.ds(pl.multiple_of(i * D, D), D)
        return pltpu.make_async_copy(wb_hbm.at[:, cols], wb_raw.at[:, cols], sem_w.at[i])

    woa_copy = pltpu.make_async_copy(woa_hbm, woa_raw, sem_w.at[3])
    wob_copy = pltpu.make_async_copy(wob_hbm, wob, sem_w.at[4])

    def out_copy(qb, j):
        rows = pl.ds(pl.multiple_of(qb * TQ + j * OC, OC), OC)
        return pltpu.make_async_copy(outb.at[rows, :], out_hbm.at[rows, :],
                                     sem_o.at[qb * (TQ // OC) + j])

    n_wa = 3 * D // WCH
    queue = ([wa_copy(i) for i in range(n_wa)]
             + [woa_copy, wb_copy(0), wb_copy(2), x_copy(0), wb_copy(1)]
             + [x_copy(r) for r in range(1, S // RB)] + [wob_copy])
    for cp in queue[:NFLIGHT]:
        cp.start()
    queue = queue[NFLIGHT:]

    def start_in_loop(i, counts):
        for k, n in enumerate(counts):
            batch = [queue.pop(0) for _ in range(n)]

            @pl.when(i == k)
            def _():
                for cp in batch:
                    cp.start()

    def selection():
        ri = lax.broadcasted_iota(jnp.int32, (256, 256), 0)
        ci = lax.broadcasted_iota(jnp.int32, (256, 256), 1)
        return jnp.where(ci == (ri % 8) * DH + ri // 8, 1.0, 0.0).astype(bf16)

    def transpose(w):
        ri = lax.broadcasted_iota(jnp.int32, (128, 128), 0)
        ci = lax.broadcasted_iota(jnp.int32, (128, 128), 1)
        eye = jnp.where(ri == ci, 1.0, 0.0).astype(bf16)
        return lax.dot_general(eye, w, NTD, preferred_element_type=f32).astype(bf16)

    def pair(a0, a1):
        both = jnp.concatenate([a0.reshape(DH, 8, D), a1.reshape(DH, 8, D)], axis=1)
        return _pack(both.reshape(DH * 16, D).astype(bf16)).reshape(DH, 8, D)

    def prep_wa(i, carry):
        wa_copy(i).wait()
        start_in_loop(i, WA_STARTS)
        sel = selection()
        halves = [lax.dot_general(
            sel, wa_raw[:, pl.ds(pl.multiple_of(i * WCH + j * 256, 256), 256)], NTD,
            preferred_element_type=f32) for j in range(2)]
        wat[:, i % 2, :, :] = pair(*halves)

        @pl.when(i % 2 == 1)
        def _():
            wt = _unpack(wat[...].reshape(D // 2, D))
            cols = pl.ds(pl.multiple_of((i // 2) * D, D), D)
            for j in range(NT):
                wan[j * 64:(j + 1) * 64, cols] = _pack(transpose(wt[:, j * 128:(j + 1) * 128]))

        return carry

    def prep_woa(a, carry):
        sel = selection()
        halves = [lax.dot_general(
            sel, woa_raw[pl.ds(pl.multiple_of(a * 512 + j * 256, 256), 256), :], NN,
            preferred_element_type=f32) for j in range(2)]
        woa[:, a, :, :] = pair(*halves)
        return carry

    def prep_wb(part, carry):
        wb_copy(2 * part).wait()
        for j in range(NT):
            cols = pl.ds(pl.multiple_of(2 * part * D + j * 128, 128), 128)
            rows = pl.ds(pl.multiple_of(part * (D // 2) + j * 64, 64), 64)
            wqvt[rows, :] = _pack(transpose(wb_raw[:, cols]))
        return carry

    lax.fori_loop(0, n_wa, prep_wa, 0)
    woa_copy.wait()
    lax.fori_loop(0, 2, prep_woa, 0)
    lax.fori_loop(0, 2, prep_wb, 0)
    wb_copy(1).wait()
    for cp in queue:
        cp.start()

    def local_attn(r0, s, first_dep):
        outs = []
        deps = []
        for c in range(SB // RC):
            base = s * SB + c * RC
            scale = _after(QSCALE, deps[c - LOOK] if c >= LOOK else first_dep)
            logits = [None] * WIN
            for t in range(NT):
                q = qa[t, base:base + RC, :] * scale
                for w in range(WIN):
                    o0 = HALO + base - DIL * w
                    term = q * ka[t, o0:o0 + RC, :]
                    logits[w] = term if t == 0 else logits[w] + term
            for w in range(WIN):
                acc = logits[w]
                acc = acc + pltpu.roll(acc, 64, 1)
                acc = acc + pltpu.roll(acc, 32, 1)
                if base < DIL * w:
                    row = r0 + base + lax.broadcasted_iota(jnp.int32, (RC, 128), 0)
                    acc = jnp.where(row >= DIL * w, acc, -1e9)
                logits[w] = acc
            m = _tree(jnp.maximum, logits)
            p = [jnp.exp2(lg - m) for lg in logits]
            inv = _recip(_tree(jnp.add, p))
            tiles = []
            for t in range(NT):
                terms = [p[w] * va[t, HALO + base - DIL * w:HALO + base - DIL * w + RC, :]
                         for w in range(WIN)]
                acc = _tree(jnp.add, terms) * inv
                tiles.append(acc.astype(bf16))
            deps.append(acc if DEP_END else m)
            outs.append(jnp.concatenate(tiles, axis=1))
        return jnp.concatenate(outs, axis=0)

    def load_x(r, l, look):
        r0 = pl.multiple_of(jnp.minimum(r, S // RB - 1) * RB, RB)
        w0 = pl.multiple_of(r * RB, RB)

        def load(start, dep):
            rows = pl.ds(r0 + start, LC)
            lvec = _after(jnp.full((LC, 128), l, f32), dep)
            first = jnp.concatenate([lvec == 0.0] * NT, axis=1)
            xi = xin[pl.ds(r0 + start // 16 * 16, 16), :].astype(f32)[start % 16:start % 16 + LC]
            x = jnp.where(first, xi, xs2[rows, :])
            xs[pl.ds(w0 + start, LC), :] = x
            return x

        xnb[...] = _pack(_layernorm(load, RB, look))

    def row_body(r, l):
        r0 = pl.multiple_of(r * RB, RB)
        rn = jnp.minimum(r + 1, S // RB - 1)

        @pl.when(jnp.logical_and(l == 0, r + 1 < S // RB))
        def _():
            x_copy(rn).wait()

        rows = [pl.ds(r0 + s * SB, SB) for s in range(NSUB)]
        gate = {}
        xn2 = {}

        def qkv_a(s):
            xn = _unpack(xnb[s * SB // 2:(s + 1) * SB // 2, :])
            y = lax.dot_general(xn, _unpack(wan[...]), NN, preferred_element_type=f32)
            for t in range(NT):
                qa[t, s * SB:(s + 1) * SB, :] = y[:, t * 128:(t + 1) * 128]
                ka[t, HALO + s * SB:HALO + (s + 1) * SB, :] = y[:, D + t * 128:D + (t + 1) * 128]
                va[t, HALO + s * SB:HALO + (s + 1) * SB, :] = y[:, 2 * D + t * 128:2 * D + (t + 1) * 128]
            gate[s] = y[SB - RC:SB, GATE_COL - 128:GATE_COL]

        def out_a(s):
            o = local_attn(r0, s, gate[s])
            x1 = xs[rows[s], :] + lax.dot_general(o, _unpack(woa[...].reshape(D // 2, D)), NN,
                                                  preferred_element_type=f32)
            xs[rows[s], :] = x1
            if LN_RELOAD:
                xn2[s] = _layernorm(lambda st, dep: xs[pl.ds(r0 + s * SB + st, LC), :], SB, LN_LOOK)
            else:
                xn2[s] = _layernorm(lambda st, dep: x1[st:st + LC], SB, LN_LOOK)

        def qkv_b(s):
            cols = pl.ds(r0 + s * SB, SB)
            yq = lax.dot_general(_unpack(wqvt[0:D // 2, :]), xn2[s], NTD, preferred_element_type=f32)
            qt[:, cols] = _pack((yq * QSCALE).astype(bf16))
            yv = lax.dot_general(_unpack(wqvt[D // 2:D, :]), xn2[s], NTD, preferred_element_type=f32)
            vt[:, cols] = _pack(yv.astype(bf16))
            yk = lax.dot_general(xn2[s], wb_raw[:, D:2 * D], NN, preferred_element_type=f32).astype(bf16)
            krows = pl.ds(pl.multiple_of((r0 + s * SB) // 2, SB // 2), SB // 2)
            for g in range(NT):
                kb[g, krows, :] = _pack(yk[:, g * 128:(g + 1) * 128])

        steps = {"a": qkv_a, "o": out_a, "b": qkv_b}
        for name, s in ROW_ORDER:
            if name == "n":
                ka[:, 0:HALO, :] = ka[:, RB:RB + HALO, :]
                va[:, 0:HALO, :] = va[:, RB:RB + HALO, :]
                load_x(r + 1, l, LX_LOOK)
            else:
                steps[name](s)
        return l

    def head_weights(g, hh, q0):
        w = qt[pl.ds(pl.multiple_of(g * 64 + hh * 16, 16), 16), pl.ds(q0, TQ)]
        parts = []
        if hh > 0:
            parts.append(jnp.zeros((16 * hh, TQ), u32))
        parts.append(w)
        if hh < 3:
            parts.append(jnp.zeros((16 * (3 - hh), TQ), u32))
        return _unpack(jnp.concatenate(parts, axis=0))

    def v_rows(g, hh, c):
        rows = pl.ds(pl.multiple_of(g * 64 + hh * 16, 16), 16)
        return _unpack(vt[rows, c * KC:(c + 1) * KC])

    def finish_group(g):
        o = jnp.dot(v_rows(g, HPB - 1, NC - 1), _unpack(pp[...]), preferred_element_type=f32)
        last = (ot[3 * DH:4 * DH, :] + o) * invs[0:1, :]
        return jnp.concatenate([ot[0:3 * DH, :], last], axis=0).T.astype(bf16)

    def o_rows(q0):
        return pl.ds(pl.multiple_of(q0 // 2, TQ // 2), TQ // 2)

    def attn_fast(q0):
        def group(g, lmax):
            st = {}

            def qk(hh, c):
                if c == 0:
                    st[hh] = dict(w=head_weights(g, hh, q0))
                kc = _unpack(kb[g, c * KC // 2:(c + 1) * KC // 2, :])
                return jnp.dot(kc, st[hh]["w"], preferred_element_type=f32)

            def pv(hh, c, s):
                d = st[hh]
                if c == 0:
                    d["m"] = jnp.broadcast_to(jnp.max(s[0:8], axis=0, keepdims=True), (8, TQ))
                p = jnp.exp2(s.reshape(KC // 8, 8, TQ) - d["m"][None])
                lc = jnp.sum(p, axis=0)
                d["l"] = lc if c == 0 else d["l"] + lc
                p = p.reshape(KC, TQ).astype(bf16)
                if c == NC - 1:
                    d["lsum"] = jnp.sum(d["l"], axis=0, keepdims=True)
                if hh == HPB - 1 and c == NC - 1:
                    pp[...] = _pack(p)
                    ot[hh * DH:(hh + 1) * DH, :] = d["acc"]
                    invs[...] = jnp.broadcast_to(_recip(d["lsum"]), (8, TQ))
                    return
                o = jnp.dot(v_rows(g, hh, c), p, preferred_element_type=f32)
                d["acc"] = o if c == 0 else d["acc"] + o
                if c == NC - 1:
                    ot[hh * DH:(hh + 1) * DH, :] = d["acc"] * _recip(d["lsum"])

            pend = None
            for hh in range(HPB):
                for c in range(NC):
                    s = qk(hh, c)
                    if pend is None:
                        ob[jnp.where(g == 0, NT, g - 1), o_rows(q0), :] = _pack(
                            finish_group(jnp.maximum(g - 1, 0)))
                    else:
                        pv(*pend)
                    pend = (hh, c, s)
            pv(*pend)
            for hh in range(HPB):
                lmax = jnp.maximum(lmax, st[hh]["lsum"])
            return lmax

        return lax.fori_loop(0, NT, group, jnp.zeros((1, TQ), f32))

    def attn_exact(q0):
        def group(g, carry):
            def head(hh, carry2):
                w = qt[pl.ds(pl.multiple_of(g * 64, 64), 64), pl.ds(q0, TQ)]
                row = lax.broadcasted_iota(jnp.int32, (64, TQ), 0) // 16
                w = _unpack(jnp.where(row == hh, w, jnp.zeros_like(w)))
                s = jnp.dot(_unpack(kb[g]), w, preferred_element_type=f32)
                p = jnp.exp2(s - jnp.max(s, axis=0, keepdims=True))
                l = jnp.sum(p, axis=0, keepdims=True)
                v = _unpack(vt[pl.ds(pl.multiple_of(g * 64 + hh * 16, 16), 16), :])
                o = jnp.dot(v, p.astype(bf16), preferred_element_type=f32)
                ot[pl.ds(pl.multiple_of(hh * DH, DH), DH), :] = o * (1.0 / l)
                return carry2
            lax.fori_loop(0, 4, head, 0)
            ob[g, o_rows(q0), :] = _pack(ot[...].T.astype(bf16))
            return carry
        lax.fori_loop(0, NT, group, 0)
        pp[...] = jnp.zeros(pp.shape, u32)
        invs[...] = jnp.ones(invs.shape, f32)

    def q_body(qb, l):
        q0 = pl.multiple_of(qb * TQ, TQ)

        def attempt(state):
            a, _ = state

            @pl.when(a == 0)
            def _():
                lmx[...] = jnp.broadcast_to(attn_fast(q0), (8, TQ))

            @pl.when(a == 1)
            def _():
                attn_exact(q0)

            @pl.when(jnp.logical_or(l == 1, a == 1))
            def _():
                for j in range(TQ // OC):
                    out_copy(qb, j).wait()

            kd = (NT - 1) * 128
            o = jnp.concatenate([_unpack(ob[g, o_rows(q0), :]) for g in range(NT - 1)], axis=1)
            o_last = None
            for j in range(TQ // OC):
                y = lax.dot_general(o[j * OC:(j + 1) * OC], wob[0:kd, :], NN,
                                    preferred_element_type=f32)
                if j == 0:
                    o_last = finish_group(NT - 1)
                    y_first = y
                    continue
                if j == 2:
                    bad = _tree(jnp.maximum, [jnp.where(lmx[:, i * 128:(i + 1) * 128] <= L_MAX, 0.0, 1.0)
                                              for i in range(TQ // 128)])
                    unsafe = jnp.max(bad)
                for jj in ((0, 1) if j == 1 else (j,)):
                    yj = (y_first if jj == 0 else y) + lax.dot_general(
                        o_last[jj * OC:(jj + 1) * OC], wob[kd:D, :], NN, preferred_element_type=f32)
                    rows = pl.ds(q0 + jj * OC, OC)
                    x2 = xs[rows, :] + yj
                    xs2[rows, :] = x2
                    outb[rows, :] = x2.astype(bf16)
                    out_copy(qb, jj).start()
            return a + 1, unsafe

        lax.while_loop(lambda st: jnp.logical_or(st[0] == 0, jnp.logical_and(st[0] == 1, st[1] > 0.5)),
                       attempt, (jnp.int32(0), jnp.float32(0)))
        return l

    def layer_pair(l, carry):
        ka[:, 0:HALO, :] = jnp.zeros((NT, HALO, 128), f32)
        va[:, 0:HALO, :] = jnp.zeros((NT, HALO, 128), f32)

        @pl.when(l == 0)
        def _():
            x_copy(0).wait()

        load_x(0, l, 8)
        lax.fori_loop(0, S // RB, row_body, l)

        @pl.when(l == 0)
        def _():
            wob_copy.wait()

        lax.fori_loop(0, S // TQ, q_body, l)
        return carry

    ot[...] = jnp.zeros(ot.shape, f32)
    pp[...] = jnp.zeros(pp.shape, u32)
    invs[...] = jnp.ones(invs.shape, f32)
    lax.fori_loop(0, 2, layer_pair, 0)
    for qb in range(S // TQ):
        for j in range(TQ // OC):
            out_copy(qb, j).wait()


@jax.jit
def pallas_interleave_layers__sliding_local_dilated__softmax_full_mha__prompt_kernel(
    A_x: jax.Array,
    A_wqkv: jax.Array,
    A_wo: jax.Array,
    B_x: jax.Array,
    B_wqkv: jax.Array,
    B_wo: jax.Array,
):
    del B_x
    x = A_x.reshape(S, D)
    hbm = pl.BlockSpec(memory_space=pl.ANY)
    out = pl.pallas_call(
        _kernel,
        out_shape=jax.ShapeDtypeStruct((S, D), bf16),
        in_specs=[hbm] * 5,
        out_specs=hbm,
        scratch_shapes=[
            pltpu.VMEM((S, D), bf16),
            pltpu.VMEM((D, 3 * D), bf16),
            pltpu.VMEM((D, D), bf16),
            pltpu.VMEM((D, 3 * D), bf16),
            pltpu.VMEM((D, D), bf16),
            pltpu.VMEM((S, D), bf16),
            pltpu.VMEM((DH, 2, 8, D), u32),
            pltpu.VMEM((D // 2, 3 * D), u32),
            pltpu.VMEM((DH, 2, 8, D), u32),
            pltpu.VMEM((D, D), u32),
            pltpu.VMEM((RB // 2, D), u32),
            pltpu.VMEM((S + RB, D), f32),
            pltpu.VMEM((S, D), f32),
            pltpu.VMEM((NT, RB, 128), f32),
            pltpu.VMEM((NT, HALO + RB, 128), f32),
            pltpu.VMEM((NT, HALO + RB, 128), f32),
            pltpu.VMEM((D // 2, S), u32),
            pltpu.VMEM((NT, S // 2, 128), u32),
            pltpu.VMEM((D // 2, S), u32),
            pltpu.VMEM((NT + 1, S // 2, 128), u32),
            pltpu.VMEM((128, TQ), f32),
            pltpu.VMEM((KC // 2, TQ), u32),
            pltpu.VMEM((8, TQ), f32),
            pltpu.VMEM((8, TQ), f32),
            pltpu.SemaphoreType.DMA((S // RB,)),
            pltpu.SemaphoreType.DMA((3 * D // WCH,)),
            pltpu.SemaphoreType.DMA((5,)),
            pltpu.SemaphoreType.DMA((S // OC,)),
        ],
        compiler_params=pltpu.CompilerParams(vmem_limit_bytes=110 * 1024 * 1024),
    )(x, A_wqkv, A_wo, B_wqkv, B_wo)
    return out.reshape(1, S, D)
```

```python
import functools
import math

import jax
import jax.numpy as jnp
from jax import lax
import jax.experimental.pallas as pl
import jax.experimental.pallas.tpu as pltpu

S = 2048
D = 1024
H = 32
DH = 32
WIN = 8
DIL = 2
EPS = 1e-5
NT = D // 128
HALO = 16
QSCALE = (DH ** -0.5) * math.log2(math.e)

SB = 128
NSUB = 2
RB = SB * NSUB
RC = 8
ROW_ORDER = [("a", 0), ("a", 1), ("o", 0), ("o", 1), ("b", 0), ("n", 0), ("b", 1)]
LC = 8
LN_LOOK = 2
LX_LOOK = 2
LN_RELOAD = False
LOOK = 2
DEP_END = False
GATE_COL = 2 * D
TQ = 512
KC = 256
NC = S // KC
OC = 128
HPB = 4
WCH = 512
WA_STARTS = (1, 1, 2, 1, 1, 2)
PITCH = 40
NFLIGHT = 3
L_MAX = 2.0 ** 64

bf16 = jnp.bfloat16
f32 = jnp.float32
u32 = jnp.uint32

NN = (((1,), (0,)), ((), ()))
NTD = (((1,), (1,)), ((), ()))


def _pack(x):
    return pltpu.bitcast(x, u32)


def _unpack(x):
    return pltpu.bitcast(x, bf16)


def _after(value, dep):
    if dep is None:
        return value
    return jnp.maximum(value, jnp.minimum(dep, -3e38))


def _tree(op, xs):
    xs = list(xs)
    while len(xs) > 1:
        xs = [op(xs[i], xs[i + 1]) if i + 1 < len(xs) else xs[i] for i in range(0, len(xs), 2)]
    return xs[0]


def _recip(x):
    r = pl.reciprocal(x, approx=True)
    return r * (2.0 - x * r)


def _layernorm(load, nrows, look, first_dep=None):
    outs = []
    deps = []
    for c in range(nrows // LC):
        dep = deps[c - look] if c >= look else first_dep
        x = load(c * LC, dep)
        mu = jnp.broadcast_to(jnp.sum(x, axis=-1, keepdims=True), (LC, 128)) * _after(1.0 / D, dep)
        xc = x - jnp.concatenate([mu] * NT, axis=1)
        var = jnp.sum(xc * xc, axis=-1, keepdims=True) * (1.0 / D)
        y = xc * lax.rsqrt(var + EPS)
        deps.append(y[:, D - 128:])
        outs.append(y)
    return jnp.concatenate(outs, axis=0).astype(bf16)


def _kernel(x_hbm, wa_hbm, woa_hbm, wb_hbm, wob_hbm, out_hbm,
            xin, wa_raw, woa_raw, wb_raw, wob, outb,
            stg, wan, woa, wqvt, xnb,
            xs, xs2, qa, ka, va, qt, kb, vt, ob, ot, pp, invs, lmx,
            sem_x, sem_wa, sem_w, sem_o):
    def x_copy(r):
        rows = pl.ds(pl.multiple_of(r * RB, RB), RB)
        return pltpu.make_async_copy(x_hbm.at[rows, :], xin.at[rows, :], sem_x.at[r])

    def wa_copy(i):
        cols = pl.ds(pl.multiple_of(i * WCH, WCH), WCH)
        return pltpu.make_async_copy(wa_hbm.at[:, cols], wa_raw.at[:, cols], sem_wa.at[i])

    def wb_copy(i):
        cols = pl.ds(pl.multiple_of(i * D, D), D)
        return pltpu.make_async_copy(wb_hbm.at[:, cols], wb_raw.at[:, cols], sem_w.at[i])

    woa_copy = pltpu.make_async_copy(woa_hbm, woa_raw, sem_w.at[3])
    wob_copy = pltpu.make_async_copy(wob_hbm, wob, sem_w.at[4])

    def out_copy(qb, j):
        rows = pl.ds(pl.multiple_of(qb * TQ + j * OC, OC), OC)
        return pltpu.make_async_copy(outb.at[rows, :], out_hbm.at[rows, :],
                                     sem_o.at[qb * (TQ // OC) + j])

    n_wa = 3 * D // WCH
    queue = ([wa_copy(i) for i in range(n_wa)]
             + [woa_copy, wb_copy(0), wb_copy(2), x_copy(0), wb_copy(1)]
             + [x_copy(r) for r in range(1, S // RB)] + [wob_copy])
    for cp in queue[:NFLIGHT]:
        cp.start()
    queue = queue[NFLIGHT:]

    batches = [[queue.pop(0) for _ in range(n)] for n in WA_STARTS]

    def start_in_loop(i, my_batches):
        for k, batch in enumerate(my_batches):
            @pl.when(i == k)
            def _():
                for cp in batch:
                    cp.start()

    def transpose(w):
        ri = lax.broadcasted_iota(jnp.int32, (128, 128), 0)
        ci = lax.broadcasted_iota(jnp.int32, (128, 128), 1)
        eye = jnp.where(ri == ci, 1.0, 0.0).astype(bf16)
        return lax.dot_general(eye, w, NTD, preferred_element_type=f32)

    def stage(j, rows):
        for hh in range(HPB):
            for t in range(NT):
                r = (j * HPB + hh) * PITCH
                stg[t, r:r + DH, :] = rows[hh * DH:(hh + 1) * DH, t * 128:(t + 1) * 128]

    def gather(t):
        return jnp.concatenate([stg[t, pl.ds(d, H, stride=PITCH), :].astype(bf16)
                                for d in range(DH)], axis=0)

    def prep_wa(part, carry):
        for half in range(2):
            i = 2 * part + half
            wa_copy(i).wait()
            start_in_loop(part, batches[half::2])
            for j in range(half * NT // 2, (half + 1) * NT // 2):
                cols = pl.ds(pl.multiple_of(part * D + j * 128, 128), 128)
                stage(j, transpose(wa_raw[:, cols]))
        cols = pl.ds(pl.multiple_of(part * D, D), D)
        for t in range(NT):
            wan[t * 64:(t + 1) * 64, cols] = _pack(transpose(gather(t)).astype(bf16))
        return carry

    def prep_woa():
        for j in range(NT):
            stage(j, woa_raw[j * 128:(j + 1) * 128, :].astype(f32))
        for t in range(NT):
            woa[:, t * 128:(t + 1) * 128] = _pack(gather(t))

    def prep_wb(part, carry):
        wb_copy(2 * part).wait()
        for j in range(NT):
            cols = pl.ds(pl.multiple_of(2 * part * D + j * 128, 128), 128)
            rows = pl.ds(pl.multiple_of(part * (D // 2) + j * 64, 64), 64)
            wqvt[rows, :] = _pack(transpose(wb_raw[:, cols]).astype(bf16))
        return carry

    lax.fori_loop(0, 3, prep_wa, 0)
    woa_copy.wait()
    prep_woa()
    lax.fori_loop(0, 2, prep_wb, 0)
    wb_copy(1).wait()
    for cp in queue:
        cp.start()

    def local_attn(r0, s, first_dep):
        outs = []
        deps = []
        for c in range(SB // RC):
            base = s * SB + c * RC
            scale = _after(QSCALE, deps[c - LOOK] if c >= LOOK else first_dep)
            logits = [None] * WIN
            for t in range(NT):
                q = qa[t, base:base + RC, :] * scale
                for w in range(WIN):
                    o0 = HALO + base - DIL * w
                    term = q * ka[t, o0:o0 + RC, :]
                    logits[w] = term if t == 0 else logits[w] + term
            for w in range(WIN):
                acc = logits[w]
                acc = acc + pltpu.roll(acc, 64, 1)
                acc = acc + pltpu.roll(acc, 32, 1)
                if base < DIL * w:
                    row = r0 + base + lax.broadcasted_iota(jnp.int32, (RC, 128), 0)
                    acc = jnp.where(row >= DIL * w, acc, -1e9)
                logits[w] = acc
            m = _tree(jnp.maximum, logits)
            p = [jnp.exp2(lg - m) for lg in logits]
            inv = _recip(_tree(jnp.add, p))
            tiles = []
            for t in range(NT):
                terms = [p[w] * va[t, HALO + base - DIL * w:HALO + base - DIL * w + RC, :]
                         for w in range(WIN)]
                acc = _tree(jnp.add, terms) * inv
                tiles.append(acc.astype(bf16))
            deps.append(acc if DEP_END else m)
            outs.append(jnp.concatenate(tiles, axis=1))
        return jnp.concatenate(outs, axis=0)

    def load_x(r, l, look):
        r0 = pl.multiple_of(jnp.minimum(r, S // RB - 1) * RB, RB)
        w0 = pl.multiple_of(r * RB, RB)

        def load(start, dep):
            rows = pl.ds(r0 + start, LC)
            lvec = _after(jnp.full((LC, 128), l, f32), dep)
            first = jnp.concatenate([lvec == 0.0] * NT, axis=1)
            xi = xin[pl.ds(r0 + start // 16 * 16, 16), :].astype(f32)[start % 16:start % 16 + LC]
            x = jnp.where(first, xi, xs2[rows, :])
            xs[pl.ds(w0 + start, LC), :] = x
            return x

        xnb[...] = _pack(_layernorm(load, RB, look))

    def row_body(r, l):
        r0 = pl.multiple_of(r * RB, RB)
        rn = jnp.minimum(r + 1, S // RB - 1)

        @pl.when(jnp.logical_and(l == 0, r + 1 < S // RB))
        def _():
            x_copy(rn).wait()

        rows = [pl.ds(r0 + s * SB, SB) for s in range(NSUB)]
        gate = {}
        xn2 = {}

        def qkv_a(s):
            xn = _unpack(xnb[s * SB // 2:(s + 1) * SB // 2, :])
            y = lax.dot_general(xn, _unpack(wan[...]), NN, preferred_element_type=f32)
            for t in range(NT):
                qa[t, s * SB:(s + 1) * SB, :] = y[:, t * 128:(t + 1) * 128]
                ka[t, HALO + s * SB:HALO + (s + 1) * SB, :] = y[:, D + t * 128:D + (t + 1) * 128]
                va[t, HALO + s * SB:HALO + (s + 1) * SB, :] = y[:, 2 * D + t * 128:2 * D + (t + 1) * 128]
            gate[s] = y[SB - RC:SB, GATE_COL - 128:GATE_COL]

        def out_a(s):
            o = local_attn(r0, s, gate[s])
            x1 = xs[rows[s], :] + lax.dot_general(o, _unpack(woa[...]), NN,
                                                  preferred_element_type=f32)
            xs[rows[s], :] = x1
            if LN_RELOAD:
                xn2[s] = _layernorm(lambda st, dep: xs[pl.ds(r0 + s * SB + st, LC), :], SB, LN_LOOK)
            else:
                xn2[s] = _layernorm(lambda st, dep: x1[st:st + LC], SB, LN_LOOK)

        def qkv_b(s):
            cols = pl.ds(r0 + s * SB, SB)
            yq = lax.dot_general(_unpack(wqvt[0:D // 2, :]), xn2[s], NTD, preferred_element_type=f32)
            qt[:, cols] = _pack((yq * QSCALE).astype(bf16))
            yv = lax.dot_general(_unpack(wqvt[D // 2:D, :]), xn2[s], NTD, preferred_element_type=f32)
            vt[:, cols] = _pack(yv.astype(bf16))
            yk = lax.dot_general(xn2[s], wb_raw[:, D:2 * D], NN, preferred_element_type=f32).astype(bf16)
            krows = pl.ds(pl.multiple_of((r0 + s * SB) // 2, SB // 2), SB // 2)
            for g in range(NT):
                kb[g, krows, :] = _pack(yk[:, g * 128:(g + 1) * 128])

        steps = {"a": qkv_a, "o": out_a, "b": qkv_b}
        for name, s in ROW_ORDER:
            if name == "n":
                ka[:, 0:HALO, :] = ka[:, RB:RB + HALO, :]
                va[:, 0:HALO, :] = va[:, RB:RB + HALO, :]
                load_x(r + 1, l, LX_LOOK)
            else:
                steps[name](s)
        return l

    def head_weights(g, hh, q0):
        w = qt[pl.ds(pl.multiple_of(g * 64 + hh * 16, 16), 16), pl.ds(q0, TQ)]
        parts = []
        if hh > 0:
            parts.append(jnp.zeros((16 * hh, TQ), u32))
        parts.append(w)
        if hh < 3:
            parts.append(jnp.zeros((16 * (3 - hh), TQ), u32))
        return _unpack(jnp.concatenate(parts, axis=0))

    def v_rows(g, hh, c):
        rows = pl.ds(pl.multiple_of(g * 64 + hh * 16, 16), 16)
        return _unpack(vt[rows, c * KC:(c + 1) * KC])

    def finish_group(g):
        o = jnp.dot(v_rows(g, HPB - 1, NC - 1), _unpack(pp[...]), preferred_element_type=f32)
        last = (ot[3 * DH:4 * DH, :] + o) * invs[0:1, :]
        return jnp.concatenate([ot[0:3 * DH, :], last], axis=0).T.astype(bf16)

    def o_rows(q0):
        return pl.ds(pl.multiple_of(q0 // 2, TQ // 2), TQ // 2)

    def attn_fast(q0):
        def group(g, lmax):
            st = {}

            def qk(hh, c):
                if c == 0:
                    st[hh] = dict(w=head_weights(g, hh, q0))
                kc = _unpack(kb[g, c * KC // 2:(c + 1) * KC // 2, :])
                return jnp.dot(kc, st[hh]["w"], preferred_element_type=f32)

            def pv(hh, c, s):
                d = st[hh]
                if c == 0:
                    d["m"] = jnp.broadcast_to(jnp.max(s[0:8], axis=0, keepdims=True), (8, TQ))
                p = jnp.exp2(s.reshape(KC // 8, 8, TQ) - d["m"][None])
                lc = jnp.sum(p, axis=0)
                d["l"] = lc if c == 0 else d["l"] + lc
                p = p.reshape(KC, TQ).astype(bf16)
                if c == NC - 1:
                    d["lsum"] = jnp.sum(d["l"], axis=0, keepdims=True)
                if hh == HPB - 1 and c == NC - 1:
                    pp[...] = _pack(p)
                    ot[hh * DH:(hh + 1) * DH, :] = d["acc"]
                    invs[...] = jnp.broadcast_to(_recip(d["lsum"]), (8, TQ))
                    return
                o = jnp.dot(v_rows(g, hh, c), p, preferred_element_type=f32)
                d["acc"] = o if c == 0 else d["acc"] + o
                if c == NC - 1:
                    ot[hh * DH:(hh + 1) * DH, :] = d["acc"] * _recip(d["lsum"])

            pend = None
            for hh in range(HPB):
                for c in range(NC):
                    s = qk(hh, c)
                    if pend is None:
                        ob[jnp.where(g == 0, NT, g - 1), o_rows(q0), :] = _pack(
                            finish_group(jnp.maximum(g - 1, 0)))
                    else:
                        pv(*pend)
                    pend = (hh, c, s)
            pv(*pend)
            for hh in range(HPB):
                lmax = jnp.maximum(lmax, st[hh]["lsum"])
            return lmax

        return lax.fori_loop(0, NT, group, jnp.zeros((1, TQ), f32))

    def attn_exact(q0):
        def group(g, carry):
            def head(hh, carry2):
                w = qt[pl.ds(pl.multiple_of(g * 64, 64), 64), pl.ds(q0, TQ)]
                row = lax.broadcasted_iota(jnp.int32, (64, TQ), 0) // 16
                w = _unpack(jnp.where(row == hh, w, jnp.zeros_like(w)))
                s = jnp.dot(_unpack(kb[g]), w, preferred_element_type=f32)
                p = jnp.exp2(s - jnp.max(s, axis=0, keepdims=True))
                l = jnp.sum(p, axis=0, keepdims=True)
                v = _unpack(vt[pl.ds(pl.multiple_of(g * 64 + hh * 16, 16), 16), :])
                o = jnp.dot(v, p.astype(bf16), preferred_element_type=f32)
                ot[pl.ds(pl.multiple_of(hh * DH, DH), DH), :] = o * (1.0 / l)
                return carry2
            lax.fori_loop(0, 4, head, 0)
            ob[g, o_rows(q0), :] = _pack(ot[...].T.astype(bf16))
            return carry
        lax.fori_loop(0, NT, group, 0)
        pp[...] = jnp.zeros(pp.shape, u32)
        invs[...] = jnp.ones(invs.shape, f32)

    def q_body(qb, l):
        q0 = pl.multiple_of(qb * TQ, TQ)

        def attempt(state):
            a, _ = state

            @pl.when(a == 0)
            def _():
                lmx[...] = jnp.broadcast_to(attn_fast(q0), (8, TQ))

            @pl.when(a == 1)
            def _():
                attn_exact(q0)

            @pl.when(jnp.logical_or(l == 1, a == 1))
            def _():
                for j in range(TQ // OC):
                    out_copy(qb, j).wait()

            kd = (NT - 1) * 128
            o = jnp.concatenate([_unpack(ob[g, o_rows(q0), :]) for g in range(NT - 1)], axis=1)
            o_last = None
            for j in range(TQ // OC):
                y = lax.dot_general(o[j * OC:(j + 1) * OC], wob[0:kd, :], NN,
                                    preferred_element_type=f32)
                if j == 0:
                    o_last = finish_group(NT - 1)
                    y_first = y
                    continue
                if j == 2:
                    bad = _tree(jnp.maximum, [jnp.where(lmx[:, i * 128:(i + 1) * 128] <= L_MAX, 0.0, 1.0)
                                              for i in range(TQ // 128)])
                    unsafe = jnp.max(bad)
                for jj in ((0, 1) if j == 1 else (j,)):
                    yj = (y_first if jj == 0 else y) + lax.dot_general(
                        o_last[jj * OC:(jj + 1) * OC], wob[kd:D, :], NN, preferred_element_type=f32)
                    rows = pl.ds(q0 + jj * OC, OC)
                    x2 = xs[rows, :] + yj
                    xs2[rows, :] = x2
                    outb[rows, :] = x2.astype(bf16)
                    out_copy(qb, jj).start()
            return a + 1, unsafe

        lax.while_loop(lambda st: jnp.logical_or(st[0] == 0, jnp.logical_and(st[0] == 1, st[1] > 0.5)),
                       attempt, (jnp.int32(0), jnp.float32(0)))
        return l

    def layer_pair(l, carry):
        ka[:, 0:HALO, :] = jnp.zeros((NT, HALO, 128), f32)
        va[:, 0:HALO, :] = jnp.zeros((NT, HALO, 128), f32)

        @pl.when(l == 0)
        def _():
            x_copy(0).wait()

        load_x(0, l, 8)
        lax.fori_loop(0, S // RB, row_body, l)

        @pl.when(l == 0)
        def _():
            wob_copy.wait()

        lax.fori_loop(0, S // TQ, q_body, l)
        return carry

    ot[...] = jnp.zeros(ot.shape, f32)
    pp[...] = jnp.zeros(pp.shape, u32)
    invs[...] = jnp.ones(invs.shape, f32)
    lax.fori_loop(0, 2, layer_pair, 0)
    for qb in range(S // TQ):
        for j in range(TQ // OC):
            out_copy(qb, j).wait()


@jax.jit
def pallas_interleave_layers__sliding_local_dilated__softmax_full_mha__prompt_kernel(
    A_x: jax.Array,
    A_wqkv: jax.Array,
    A_wo: jax.Array,
    B_x: jax.Array,
    B_wqkv: jax.Array,
    B_wo: jax.Array,
):
    del B_x
    x = A_x.reshape(S, D)
    hbm = pl.BlockSpec(memory_space=pl.ANY)
    out = pl.pallas_call(
        _kernel,
        out_shape=jax.ShapeDtypeStruct((S, D), bf16),
        in_specs=[hbm] * 5,
        out_specs=hbm,
        scratch_shapes=[
            pltpu.VMEM((S, D), bf16),
            pltpu.VMEM((D, 3 * D), bf16),
            pltpu.VMEM((D, D), bf16),
            pltpu.VMEM((D, 3 * D), bf16),
            pltpu.VMEM((D, D), bf16),
            pltpu.VMEM((S, D), bf16),
            pltpu.VMEM((NT, H * PITCH, 128), f32),
            pltpu.VMEM((D // 2, 3 * D), u32),
            pltpu.VMEM((D // 2, D), u32),
            pltpu.VMEM((D, D), u32),
            pltpu.VMEM((RB // 2, D), u32),
            pltpu.VMEM((S + RB, D), f32),
            pltpu.VMEM((S, D), f32),
            pltpu.VMEM((NT, RB, 128), f32),
            pltpu.VMEM((NT, HALO + RB, 128), f32),
            pltpu.VMEM((NT, HALO + RB, 128), f32),
            pltpu.VMEM((D // 2, S), u32),
            pltpu.VMEM((NT, S // 2, 128), u32),
            pltpu.VMEM((D // 2, S), u32),
            pltpu.VMEM((NT + 1, S // 2, 128), u32),
            pltpu.VMEM((128, TQ), f32),
            pltpu.VMEM((KC // 2, TQ), u32),
            pltpu.VMEM((8, TQ), f32),
            pltpu.VMEM((8, TQ), f32),
            pltpu.SemaphoreType.DMA((S // RB,)),
            pltpu.SemaphoreType.DMA((3 * D // WCH,)),
            pltpu.SemaphoreType.DMA((5,)),
            pltpu.SemaphoreType.DMA((S // OC,)),
        ],
        compiler_params=pltpu.CompilerParams(vmem_limit_bytes=110 * 1024 * 1024),
    )(x, A_wqkv, A_wo, B_wqkv, B_wo)
    return out.reshape(1, S, D)
```

```python
import functools
import math

import jax
import jax.numpy as jnp
from jax import lax
import jax.experimental.pallas as pl
import jax.experimental.pallas.tpu as pltpu

S = 2048
D = 1024
H = 32
DH = 32
WIN = 8
DIL = 2
EPS = 1e-5
NT = D // 128
HALO = 16
QSCALE = (DH ** -0.5) * math.log2(math.e)

SB = 128
NSUB = 2
RB = SB * NSUB
RC = 8
ROW_ORDER = [("a", 0), ("a", 1), ("o", 0), ("o", 1), ("b", 0), ("n", 0), ("b", 1)]
LC = 8
LN_LOOK = 2
LX_LOOK = 2
LN_RELOAD = False
LOOK = 2
DEP_END = False
GATE_COL = 2 * D
TQ = 512
KC = 256
NC = S // KC
OC = 128
HPB = 4
WCH = 512
WA_STARTS = (1, 1, 2, 1, 1, 2)
PITCH = 40
NFLIGHT = 3
L_MAX = 2.0 ** 64

bf16 = jnp.bfloat16
f32 = jnp.float32
u32 = jnp.uint32

NN = (((1,), (0,)), ((), ()))
NTD = (((1,), (1,)), ((), ()))


def _pack(x):
    return pltpu.bitcast(x, u32)


def _unpack(x):
    return pltpu.bitcast(x, bf16)


def _after(value, dep):
    if dep is None:
        return value
    return jnp.maximum(value, jnp.minimum(dep, -3e38))


def _tree(op, xs):
    xs = list(xs)
    while len(xs) > 1:
        xs = [op(xs[i], xs[i + 1]) if i + 1 < len(xs) else xs[i] for i in range(0, len(xs), 2)]
    return xs[0]


def _recip(x):
    r = pl.reciprocal(x, approx=True)
    return r * (2.0 - x * r)


def _layernorm(load, nrows, look, first_dep=None):
    outs = []
    deps = []
    for c in range(nrows // LC):
        dep = deps[c - look] if c >= look else first_dep
        x = load(c * LC, dep)
        mu = jnp.broadcast_to(jnp.sum(x, axis=-1, keepdims=True), (LC, 128)) * _after(1.0 / D, dep)
        xc = x - jnp.concatenate([mu] * NT, axis=1)
        var = jnp.sum(xc * xc, axis=-1, keepdims=True) * (1.0 / D)
        y = xc * lax.rsqrt(var + EPS)
        deps.append(y[:, D - 128:])
        outs.append(y)
    return jnp.concatenate(outs, axis=0).astype(bf16)


def _kernel(x_hbm, wa_hbm, woa_hbm, wb_hbm, wob_hbm, out_hbm,
            xin, wa_raw, woa_raw, wb_raw, wob, outb,
            stg, wan, woa, wqvt, xnb,
            xs, xs2, qa, ka, va, qt, kb, vt, ob, ot, pp, invs, lmx,
            sem_x, sem_wa, sem_w, sem_o):
    def x_copy(r):
        rows = pl.ds(pl.multiple_of(r * RB, RB), RB)
        return pltpu.make_async_copy(x_hbm.at[rows, :], xin.at[rows, :], sem_x.at[r])

    def wa_copy(i):
        cols = pl.ds(pl.multiple_of(i * WCH, WCH), WCH)
        return pltpu.make_async_copy(wa_hbm.at[:, cols], wa_raw.at[:, cols], sem_wa.at[i])

    def wb_copy(i):
        cols = pl.ds(pl.multiple_of(i * D, D), D)
        return pltpu.make_async_copy(wb_hbm.at[:, cols], wb_raw.at[:, cols], sem_w.at[i])

    woa_copy = pltpu.make_async_copy(woa_hbm, woa_raw, sem_w.at[3])
    wob_copy = pltpu.make_async_copy(wob_hbm, wob, sem_w.at[4])

    def out_copy(qb, j):
        rows = pl.ds(pl.multiple_of(qb * TQ + j * OC, OC), OC)
        return pltpu.make_async_copy(outb.at[rows, :], out_hbm.at[rows, :],
                                     sem_o.at[qb * (TQ // OC) + j])

    n_wa = 3 * D // WCH
    queue = ([wa_copy(i) for i in range(n_wa)]
             + [woa_copy, wb_copy(0), wb_copy(2), x_copy(0), wb_copy(1)]
             + [x_copy(r) for r in range(1, S // RB)] + [wob_copy])
    for cp in queue[:NFLIGHT]:
        cp.start()
    queue = queue[NFLIGHT:]

    batches = [[queue.pop(0) for _ in range(n)] for n in WA_STARTS]

    def start_in_loop(i, my_batches):
        for k, batch in enumerate(my_batches):
            @pl.when(i == k)
            def _():
                for cp in batch:
                    cp.start()

    def transpose(w):
        ri = lax.broadcasted_iota(jnp.int32, (128, 128), 0)
        ci = lax.broadcasted_iota(jnp.int32, (128, 128), 1)
        eye = jnp.where(ri == ci, 1.0, 0.0).astype(bf16)
        return lax.dot_general(eye, w, NTD, preferred_element_type=f32)

    def stage(j, rows):
        for hh in range(HPB):
            for t in range(NT):
                r = (j * HPB + hh) * PITCH
                stg[t, r:r + DH, :] = rows[hh * DH:(hh + 1) * DH, t * 128:(t + 1) * 128]

    def gather(t):
        return jnp.concatenate([stg[t, pl.ds(d, H, stride=PITCH), :].astype(bf16)
                                for d in range(DH)], axis=0)

    def prep_wa(part, carry):
        for half in range(2):
            i = 2 * part + half
            wa_copy(i).wait()
            start_in_loop(part, batches[half::2])
            for j in range(half * NT // 2, (half + 1) * NT // 2):
                cols = pl.ds(pl.multiple_of(part * D + j * 128, 128), 128)
                stage(j, transpose(wa_raw[:, cols]))
        cols = pl.ds(pl.multiple_of(part * D, D), D)
        for t in range(NT):
            wan[t * 64:(t + 1) * 64, cols] = _pack(transpose(gather(t)).astype(bf16))
        return carry

    def prep_woa():
        for j in range(NT):
            stage(j, woa_raw[j * 128:(j + 1) * 128, :].astype(f32))
        for t in range(NT):
            woa[:, t * 128:(t + 1) * 128] = _pack(gather(t))

    def prep_wb(part, carry):
        wb_copy(2 * part).wait()
        for j in range(NT):
            cols = pl.ds(pl.multiple_of(2 * part * D + j * 128, 128), 128)
            rows = pl.ds(pl.multiple_of(part * (D // 2) + j * 64, 64), 64)
            wqvt[rows, :] = _pack(transpose(wb_raw[:, cols]).astype(bf16))
        return carry

    lax.fori_loop(0, 3, prep_wa, 0)
    woa_copy.wait()
    prep_woa()
    lax.fori_loop(0, 2, prep_wb, 0)

    def local_attn(r0, s, first_dep):
        outs = []
        deps = []
        for c in range(SB // RC):
            base = s * SB + c * RC
            scale = _after(QSCALE, deps[c - LOOK] if c >= LOOK else first_dep)
            logits = [None] * WIN
            for t in range(NT):
                q = qa[t, base:base + RC, :] * scale
                for w in range(WIN):
                    o0 = HALO + base - DIL * w
                    term = q * ka[t, o0:o0 + RC, :]
                    logits[w] = term if t == 0 else logits[w] + term
            for w in range(WIN):
                acc = logits[w]
                acc = acc + pltpu.roll(acc, 64, 1)
                acc = acc + pltpu.roll(acc, 32, 1)
                if base < DIL * w:
                    row = r0 + base + lax.broadcasted_iota(jnp.int32, (RC, 128), 0)
                    acc = jnp.where(row >= DIL * w, acc, -1e9)
                logits[w] = acc
            m = _tree(jnp.maximum, logits)
            p = [jnp.exp2(lg - m) for lg in logits]
            inv = _recip(_tree(jnp.add, p))
            tiles = []
            for t in range(NT):
                terms = [p[w] * va[t, HALO + base - DIL * w:HALO + base - DIL * w + RC, :]
                         for w in range(WIN)]
                acc = _tree(jnp.add, terms) * inv
                tiles.append(acc.astype(bf16))
            deps.append(acc if DEP_END else m)
            outs.append(jnp.concatenate(tiles, axis=1))
        return jnp.concatenate(outs, axis=0)

    def load_x(r, l, look):
        r0 = pl.multiple_of(jnp.minimum(r, S // RB - 1) * RB, RB)
        w0 = pl.multiple_of(r * RB, RB)

        def load(start, dep):
            rows = pl.ds(r0 + start, LC)
            lvec = _after(jnp.full((LC, 128), l, f32), dep)
            first = jnp.concatenate([lvec == 0.0] * NT, axis=1)
            xi = xin[pl.ds(r0 + start // 16 * 16, 16), :].astype(f32)[start % 16:start % 16 + LC]
            x = jnp.where(first, xi, xs2[rows, :])
            xs[pl.ds(w0 + start, LC), :] = x
            return x

        xnb[...] = _pack(_layernorm(load, RB, look))

    def row_body(r, l):
        r0 = pl.multiple_of(r * RB, RB)
        rn = jnp.minimum(r + 1, S // RB - 1)

        @pl.when(jnp.logical_and(l == 0, r + 1 < S // RB))
        def _():
            x_copy(rn).wait()

        rows = [pl.ds(r0 + s * SB, SB) for s in range(NSUB)]
        gate = {}
        xn2 = {}

        def qkv_a(s):
            xn = _unpack(xnb[s * SB // 2:(s + 1) * SB // 2, :])
            y = lax.dot_general(xn, _unpack(wan[...]), NN, preferred_element_type=f32)
            for t in range(NT):
                qa[t, s * SB:(s + 1) * SB, :] = y[:, t * 128:(t + 1) * 128]
                ka[t, HALO + s * SB:HALO + (s + 1) * SB, :] = y[:, D + t * 128:D + (t + 1) * 128]
                va[t, HALO + s * SB:HALO + (s + 1) * SB, :] = y[:, 2 * D + t * 128:2 * D + (t + 1) * 128]
            gate[s] = y[SB - RC:SB, GATE_COL - 128:GATE_COL]

        def out_a(s):
            o = local_attn(r0, s, gate[s])
            x1 = xs[rows[s], :] + lax.dot_general(o, _unpack(woa[...]), NN,
                                                  preferred_element_type=f32)
            xs[rows[s], :] = x1
            if LN_RELOAD:
                xn2[s] = _layernorm(lambda st, dep: xs[pl.ds(r0 + s * SB + st, LC), :], SB, LN_LOOK)
            else:
                xn2[s] = _layernorm(lambda st, dep: x1[st:st + LC], SB, LN_LOOK)

        def qkv_b(s):
            cols = pl.ds(r0 + s * SB, SB)
            yq = lax.dot_general(_unpack(wqvt[0:D // 2, :]), xn2[s], NTD, preferred_element_type=f32)
            qt[:, cols] = _pack((yq * QSCALE).astype(bf16))
            yv = lax.dot_general(_unpack(wqvt[D // 2:D, :]), xn2[s], NTD, preferred_element_type=f32)
            vt[:, cols] = _pack(yv.astype(bf16))
            yk = lax.dot_general(xn2[s], wb_raw[:, D:2 * D], NN, preferred_element_type=f32).astype(bf16)
            krows = pl.ds(pl.multiple_of((r0 + s * SB) // 2, SB // 2), SB // 2)
            for g in range(NT):
                kb[g, krows, :] = _pack(yk[:, g * 128:(g + 1) * 128])

        steps = {"a": qkv_a, "o": out_a, "b": qkv_b}
        for name, s in ROW_ORDER:
            if name == "n":
                ka[:, 0:HALO, :] = ka[:, RB:RB + HALO, :]
                va[:, 0:HALO, :] = va[:, RB:RB + HALO, :]
                load_x(r + 1, l, LX_LOOK)
            else:
                steps[name](s)
        return l

    def head_weights(g, hh, q0):
        w = qt[pl.ds(pl.multiple_of(g * 64 + hh * 16, 16), 16), pl.ds(q0, TQ)]
        parts = []
        if hh > 0:
            parts.append(jnp.zeros((16 * hh, TQ), u32))
        parts.append(w)
        if hh < 3:
            parts.append(jnp.zeros((16 * (3 - hh), TQ), u32))
        return _unpack(jnp.concatenate(parts, axis=0))

    def v_rows(g, hh, c):
        rows = pl.ds(pl.multiple_of(g * 64 + hh * 16, 16), 16)
        return _unpack(vt[rows, c * KC:(c + 1) * KC])

    def finish_group(g):
        o = jnp.dot(v_rows(g, HPB - 1, NC - 1), _unpack(pp[...]), preferred_element_type=f32)
        last = (ot[3 * DH:4 * DH, :] + o) * invs[0:1, :]
        return jnp.concatenate([ot[0:3 * DH, :], last], axis=0).T.astype(bf16)

    def o_rows(q0):
        return pl.ds(pl.multiple_of(q0 // 2, TQ // 2), TQ // 2)

    def attn_fast(q0):
        def group(g, lmax):
            st = {}

            def qk(hh, c):
                if c == 0:
                    st[hh] = dict(w=head_weights(g, hh, q0))
                kc = _unpack(kb[g, c * KC // 2:(c + 1) * KC // 2, :])
                return jnp.dot(kc, st[hh]["w"], preferred_element_type=f32)

            def pv(hh, c, s):
                d = st[hh]
                if c == 0:
                    d["m"] = jnp.broadcast_to(jnp.max(s[0:8], axis=0, keepdims=True), (8, TQ))
                p = jnp.exp2(s.reshape(KC // 8, 8, TQ) - d["m"][None])
                lc = jnp.sum(p, axis=0)
                d["l"] = lc if c == 0 else d["l"] + lc
                p = p.reshape(KC, TQ).astype(bf16)
                if c == NC - 1:
                    d["lsum"] = jnp.sum(d["l"], axis=0, keepdims=True)
                if hh == HPB - 1 and c == NC - 1:
                    pp[...] = _pack(p)
                    ot[hh * DH:(hh + 1) * DH, :] = d["acc"]
                    invs[...] = jnp.broadcast_to(_recip(d["lsum"]), (8, TQ))
                    return
                o = jnp.dot(v_rows(g, hh, c), p, preferred_element_type=f32)
                d["acc"] = o if c == 0 else d["acc"] + o
                if c == NC - 1:
                    ot[hh * DH:(hh + 1) * DH, :] = d["acc"] * _recip(d["lsum"])

            pend = None
            for hh in range(HPB):
                for c in range(NC):
                    s = qk(hh, c)
                    if pend is None:
                        ob[jnp.where(g == 0, NT, g - 1), o_rows(q0), :] = _pack(
                            finish_group(jnp.maximum(g - 1, 0)))
                    else:
                        pv(*pend)
                    pend = (hh, c, s)
            pv(*pend)
            for hh in range(HPB):
                lmax = jnp.maximum(lmax, st[hh]["lsum"])
            return lmax

        return lax.fori_loop(0, NT, group, jnp.zeros((1, TQ), f32))

    def attn_exact(q0):
        def group(g, carry):
            def head(hh, carry2):
                w = qt[pl.ds(pl.multiple_of(g * 64, 64), 64), pl.ds(q0, TQ)]
                row = lax.broadcasted_iota(jnp.int32, (64, TQ), 0) // 16
                w = _unpack(jnp.where(row == hh, w, jnp.zeros_like(w)))
                s = jnp.dot(_unpack(kb[g]), w, preferred_element_type=f32)
                p = jnp.exp2(s - jnp.max(s, axis=0, keepdims=True))
                l = jnp.sum(p, axis=0, keepdims=True)
                v = _unpack(vt[pl.ds(pl.multiple_of(g * 64 + hh * 16, 16), 16), :])
                o = jnp.dot(v, p.astype(bf16), preferred_element_type=f32)
                ot[pl.ds(pl.multiple_of(hh * DH, DH), DH), :] = o * (1.0 / l)
                return carry2
            lax.fori_loop(0, 4, head, 0)
            ob[g, o_rows(q0), :] = _pack(ot[...].T.astype(bf16))
            return carry
        lax.fori_loop(0, NT, group, 0)
        pp[...] = jnp.zeros(pp.shape, u32)
        invs[...] = jnp.ones(invs.shape, f32)

    def q_body(qb, l):
        q0 = pl.multiple_of(qb * TQ, TQ)

        def attempt(state):
            a, _ = state

            @pl.when(a == 0)
            def _():
                lmx[...] = jnp.broadcast_to(attn_fast(q0), (8, TQ))

            @pl.when(a == 1)
            def _():
                attn_exact(q0)

            @pl.when(jnp.logical_or(l == 1, a == 1))
            def _():
                for j in range(TQ // OC):
                    out_copy(qb, j).wait()

            kd = (NT - 1) * 128
            o = jnp.concatenate([_unpack(ob[g, o_rows(q0), :]) for g in range(NT - 1)], axis=1)
            o_last = None
            for j in range(TQ // OC):
                y = lax.dot_general(o[j * OC:(j + 1) * OC], wob[0:kd, :], NN,
                                    preferred_element_type=f32)
                if j == 0:
                    o_last = finish_group(NT - 1)
                    y_first = y
                    continue
                if j == 2:
                    bad = _tree(jnp.maximum, [jnp.where(lmx[:, i * 128:(i + 1) * 128] <= L_MAX, 0.0, 1.0)
                                              for i in range(TQ // 128)])
                    unsafe = jnp.max(bad)
                for jj in ((0, 1) if j == 1 else (j,)):
                    yj = (y_first if jj == 0 else y) + lax.dot_general(
                        o_last[jj * OC:(jj + 1) * OC], wob[kd:D, :], NN, preferred_element_type=f32)
                    rows = pl.ds(q0 + jj * OC, OC)
                    x2 = xs[rows, :] + yj
                    xs2[rows, :] = x2
                    outb[rows, :] = x2.astype(bf16)
                    out_copy(qb, jj).start()
            return a + 1, unsafe

        lax.while_loop(lambda st: jnp.logical_or(st[0] == 0, jnp.logical_and(st[0] == 1, st[1] > 0.5)),
                       attempt, (jnp.int32(0), jnp.float32(0)))
        return l

    def layer_pair(l, carry):
        ka[:, 0:HALO, :] = jnp.zeros((NT, HALO, 128), f32)
        va[:, 0:HALO, :] = jnp.zeros((NT, HALO, 128), f32)

        @pl.when(l == 1)
        def _():
            load_x(0, l, 16)

        lax.fori_loop(0, S // RB, row_body, l)

        @pl.when(l == 0)
        def _():
            wob_copy.wait()

        lax.fori_loop(0, S // TQ, q_body, l)
        return carry

    x_copy(0).wait()
    load_x(0, 0, 16)
    wb_copy(1).wait()
    for cp in queue:
        cp.start()
    ot[...] = jnp.zeros(ot.shape, f32)
    pp[...] = jnp.zeros(pp.shape, u32)
    invs[...] = jnp.ones(invs.shape, f32)
    lax.fori_loop(0, 2, layer_pair, 0)
    for qb in range(S // TQ):
        for j in range(TQ // OC):
            out_copy(qb, j).wait()


@jax.jit
def pallas_interleave_layers__sliding_local_dilated__softmax_full_mha__prompt_kernel(
    A_x: jax.Array,
    A_wqkv: jax.Array,
    A_wo: jax.Array,
    B_x: jax.Array,
    B_wqkv: jax.Array,
    B_wo: jax.Array,
):
    del B_x
    x = A_x.reshape(S, D)
    hbm = pl.BlockSpec(memory_space=pl.ANY)
    out = pl.pallas_call(
        _kernel,
        out_shape=jax.ShapeDtypeStruct((S, D), bf16),
        in_specs=[hbm] * 5,
        out_specs=hbm,
        scratch_shapes=[
            pltpu.VMEM((S, D), bf16),
            pltpu.VMEM((D, 3 * D), bf16),
            pltpu.VMEM((D, D), bf16),
            pltpu.VMEM((D, 3 * D), bf16),
            pltpu.VMEM((D, D), bf16),
            pltpu.VMEM((S, D), bf16),
            pltpu.VMEM((NT, H * PITCH, 128), f32),
            pltpu.VMEM((D // 2, 3 * D), u32),
            pltpu.VMEM((D // 2, D), u32),
            pltpu.VMEM((D, D), u32),
            pltpu.VMEM((RB // 2, D), u32),
            pltpu.VMEM((S + RB, D), f32),
            pltpu.VMEM((S, D), f32),
            pltpu.VMEM((NT, RB, 128), f32),
            pltpu.VMEM((NT, HALO + RB, 128), f32),
            pltpu.VMEM((NT, HALO + RB, 128), f32),
            pltpu.VMEM((D // 2, S), u32),
            pltpu.VMEM((NT, S // 2, 128), u32),
            pltpu.VMEM((D // 2, S), u32),
            pltpu.VMEM((NT + 1, S // 2, 128), u32),
            pltpu.VMEM((128, TQ), f32),
            pltpu.VMEM((KC // 2, TQ), u32),
            pltpu.VMEM((8, TQ), f32),
            pltpu.VMEM((8, TQ), f32),
            pltpu.SemaphoreType.DMA((S // RB,)),
            pltpu.SemaphoreType.DMA((3 * D // WCH,)),
            pltpu.SemaphoreType.DMA((5,)),
            pltpu.SemaphoreType.DMA((S // OC,)),
        ],
        compiler_params=pltpu.CompilerParams(vmem_limit_bytes=110 * 1024 * 1024),
    )(x, A_wqkv, A_wo, B_wqkv, B_wo)
    return out.reshape(1, S, D)
```

```python
import functools
import math

import jax
import jax.numpy as jnp
from jax import lax
import jax.experimental.pallas as pl
import jax.experimental.pallas.tpu as pltpu

S = 2048
D = 1024
H = 32
DH = 32
WIN = 8
DIL = 2
EPS = 1e-5
NT = D // 128
HALO = 16
QSCALE = (DH ** -0.5) * math.log2(math.e)

SB = 128
NSUB = 2
RB = SB * NSUB
RC = 8
ROW_ORDER = [("a", 0), ("a", 1), ("o", 0), ("o", 1), ("b", 0), ("n", 0), ("b", 1)]
LC = 8
LN_LOOK = 2
LX_LOOK = 2
LN_RELOAD = False
LOOK = 2
DEP_END = False
GATE_COL = 2 * D
TQ = 512
KC = 256
NC = S // KC
OC = 128
GPB = 2
HPB = 4
WCH = 512
WA_STARTS = (1, 1, 2, 1, 1, 2)
PITCH = 40
NFLIGHT = 3
L_MAX = 2.0 ** 64

bf16 = jnp.bfloat16
f32 = jnp.float32
u32 = jnp.uint32

NN = (((1,), (0,)), ((), ()))
NTD = (((1,), (1,)), ((), ()))


def _pack(x):
    return pltpu.bitcast(x, u32)


def _unpack(x):
    return pltpu.bitcast(x, bf16)


def _after(value, dep):
    if dep is None:
        return value
    return jnp.maximum(value, jnp.minimum(dep, -3e38))


def _tree(op, xs):
    xs = list(xs)
    while len(xs) > 1:
        xs = [op(xs[i], xs[i + 1]) if i + 1 < len(xs) else xs[i] for i in range(0, len(xs), 2)]
    return xs[0]


def _recip(x):
    r = pl.reciprocal(x, approx=True)
    return r * (2.0 - x * r)


def _layernorm(load, nrows, look, first_dep=None):
    outs = []
    deps = []
    for c in range(nrows // LC):
        dep = deps[c - look] if c >= look else first_dep
        x = load(c * LC, dep)
        mu = jnp.broadcast_to(jnp.sum(x, axis=-1, keepdims=True), (LC, 128)) * _after(1.0 / D, dep)
        xc = x - jnp.concatenate([mu] * NT, axis=1)
        var = jnp.sum(xc * xc, axis=-1, keepdims=True) * (1.0 / D)
        y = xc * lax.rsqrt(var + EPS)
        deps.append(y[:, D - 128:])
        outs.append(y)
    return jnp.concatenate(outs, axis=0).astype(bf16)


def _kernel(x_hbm, wa_hbm, woa_hbm, wb_hbm, wob_hbm, out_hbm,
            xin, wa_raw, woa_raw, wb_raw, wob, outb,
            stg, wan, woa, wqvt, xnb,
            xs, xs2, qa, ka, va, qt, kb, vt, ob, ot, pp, invs, lmx,
            sem_x, sem_wa, sem_w, sem_o):
    def x_copy(r):
        rows = pl.ds(pl.multiple_of(r * RB, RB), RB)
        return pltpu.make_async_copy(x_hbm.at[rows, :], xin.at[rows, :], sem_x.at[r])

    def wa_copy(i):
        cols = pl.ds(pl.multiple_of(i * WCH, WCH), WCH)
        return pltpu.make_async_copy(wa_hbm.at[:, cols], wa_raw.at[:, cols], sem_wa.at[i])

    def wb_copy(i):
        cols = pl.ds(pl.multiple_of(i * D, D), D)
        return pltpu.make_async_copy(wb_hbm.at[:, cols], wb_raw.at[:, cols], sem_w.at[i])

    woa_copy = pltpu.make_async_copy(woa_hbm, woa_raw, sem_w.at[3])
    wob_copy = pltpu.make_async_copy(wob_hbm, wob, sem_w.at[4])

    def out_copy(qb, j):
        rows = pl.ds(pl.multiple_of(qb * TQ + j * OC, OC), OC)
        return pltpu.make_async_copy(outb.at[rows, :], out_hbm.at[rows, :],
                                     sem_o.at[qb * (TQ // OC) + j])

    n_wa = 3 * D // WCH
    queue = ([wa_copy(i) for i in range(n_wa)]
             + [woa_copy, wb_copy(0), wb_copy(2), x_copy(0), wb_copy(1)]
             + [x_copy(r) for r in range(1, S // RB)] + [wob_copy])
    for cp in queue[:NFLIGHT]:
        cp.start()
    queue = queue[NFLIGHT:]

    batches = [[queue.pop(0) for _ in range(n)] for n in WA_STARTS]

    def start_in_loop(i, my_batches):
        for k, batch in enumerate(my_batches):
            @pl.when(i == k)
            def _():
                for cp in batch:
                    cp.start()

    def transpose(w):
        ri = lax.broadcasted_iota(jnp.int32, (128, 128), 0)
        ci = lax.broadcasted_iota(jnp.int32, (128, 128), 1)
        eye = jnp.where(ri == ci, 1.0, 0.0).astype(bf16)
        return lax.dot_general(eye, w, NTD, preferred_element_type=f32)

    def stage(j, rows):
        for hh in range(HPB):
            r = pl.ds(pl.multiple_of((j * HPB + hh) * PITCH, 8), DH)
            for t in range(NT):
                stg[t, r, :] = rows[hh * DH:(hh + 1) * DH, t * 128:(t + 1) * 128]

    def gather(t):
        return jnp.concatenate([stg[t, pl.ds(d, H, stride=PITCH), :].astype(bf16)
                                for d in range(DH)], axis=0)

    def prep_wa(part, carry):
        for half in range(2):
            i = 2 * part + half
            wa_copy(i).wait()
            start_in_loop(part, batches[half::2])
            for j in range(half * NT // 2, (half + 1) * NT // 2):
                cols = pl.ds(pl.multiple_of(part * D + j * 128, 128), 128)
                stage(j, transpose(wa_raw[:, cols]))
        cols = pl.ds(pl.multiple_of(part * D, D), D)
        for t in range(NT):
            wan[t * 64:(t + 1) * 64, cols] = _pack(transpose(gather(t)).astype(bf16))
        return carry

    def prep_woa():
        def put(j, carry):
            stage(j, woa_raw[pl.ds(pl.multiple_of(j * 128, 128), 128), :].astype(f32))
            return carry

        def get(t, carry):
            woa[:, pl.ds(pl.multiple_of(t * 128, 128), 128)] = _pack(gather(t))
            return carry

        lax.fori_loop(0, NT, put, 0)
        lax.fori_loop(0, NT, get, 0)

    def prep_wb(part, carry):
        wb_copy(2 * part).wait()
        for j in range(NT):
            cols = pl.ds(pl.multiple_of(2 * part * D + j * 128, 128), 128)
            rows = pl.ds(pl.multiple_of(part * (D // 2) + j * 64, 64), 64)
            wqvt[rows, :] = _pack(transpose(wb_raw[:, cols]).astype(bf16))
        return carry

    lax.fori_loop(0, 3, prep_wa, 0)
    woa_copy.wait()
    prep_woa()
    lax.fori_loop(0, 2, prep_wb, 0)

    def local_attn(r0, s, first_dep):
        outs = []
        deps = []
        for c in range(SB // RC):
            base = s * SB + c * RC
            scale = _after(QSCALE, deps[c - LOOK] if c >= LOOK else first_dep)
            logits = [None] * WIN
            for t in range(NT):
                q = qa[t, base:base + RC, :] * scale
                for w in range(WIN):
                    o0 = HALO + base - DIL * w
                    term = q * ka[t, o0:o0 + RC, :]
                    logits[w] = term if t == 0 else logits[w] + term
            for w in range(WIN):
                acc = logits[w]
                acc = acc + pltpu.roll(acc, 64, 1)
                acc = acc + pltpu.roll(acc, 32, 1)
                if base < DIL * w:
                    row = r0 + base + lax.broadcasted_iota(jnp.int32, (RC, 128), 0)
                    acc = jnp.where(row >= DIL * w, acc, -1e9)
                logits[w] = acc
            m = _tree(jnp.maximum, logits)
            p = [jnp.exp2(lg - m) for lg in logits]
            inv = _recip(_tree(jnp.add, p))
            tiles = []
            for t in range(NT):
                terms = [p[w] * va[t, HALO + base - DIL * w:HALO + base - DIL * w + RC, :]
                         for w in range(WIN)]
                acc = _tree(jnp.add, terms) * inv
                tiles.append(acc.astype(bf16))
            deps.append(acc if DEP_END else m)
            outs.append(jnp.concatenate(tiles, axis=1))
        return jnp.concatenate(outs, axis=0)

    def load_x(r, l, look):
        r0 = pl.multiple_of(jnp.minimum(r, S // RB - 1) * RB, RB)
        w0 = pl.multiple_of(r * RB, RB)

        def load(start, dep):
            rows = pl.ds(r0 + start, LC)
            lvec = _after(jnp.full((LC, 128), l, f32), dep)
            first = jnp.concatenate([lvec == 0.0] * NT, axis=1)
            xi = xin[pl.ds(r0 + start // 16 * 16, 16), :].astype(f32)[start % 16:start % 16 + LC]
            x = jnp.where(first, xi, xs2[rows, :])
            xs[pl.ds(w0 + start, LC), :] = x
            return x

        xnb[...] = _pack(_layernorm(load, RB, look))

    def row_body(r, l):
        r0 = pl.multiple_of(r * RB, RB)
        rn = jnp.minimum(r + 1, S // RB - 1)

        @pl.when(jnp.logical_and(l == 0, r + 1 < S // RB))
        def _():
            x_copy(rn).wait()

        rows = [pl.ds(r0 + s * SB, SB) for s in range(NSUB)]
        gate = {}
        xn2 = {}

        def qkv_a(s):
            xn = _unpack(xnb[s * SB // 2:(s + 1) * SB // 2, :])
            y = lax.dot_general(xn, _unpack(wan[...]), NN, preferred_element_type=f32)
            for t in range(NT):
                qa[t, s * SB:(s + 1) * SB, :] = y[:, t * 128:(t + 1) * 128]
                ka[t, HALO + s * SB:HALO + (s + 1) * SB, :] = y[:, D + t * 128:D + (t + 1) * 128]
                va[t, HALO + s * SB:HALO + (s + 1) * SB, :] = y[:, 2 * D + t * 128:2 * D + (t + 1) * 128]
            gate[s] = y[SB - RC:SB, GATE_COL - 128:GATE_COL]

        def out_a(s):
            o = local_attn(r0, s, gate[s])
            x1 = xs[rows[s], :] + lax.dot_general(o, _unpack(woa[...]), NN,
                                                  preferred_element_type=f32)
            xs[rows[s], :] = x1
            if LN_RELOAD:
                xn2[s] = _layernorm(lambda st, dep: xs[pl.ds(r0 + s * SB + st, LC), :], SB, LN_LOOK)
            else:
                xn2[s] = _layernorm(lambda st, dep: x1[st:st + LC], SB, LN_LOOK)

        def qkv_b(s):
            cols = pl.ds(r0 + s * SB, SB)
            yq = lax.dot_general(_unpack(wqvt[0:D // 2, :]), xn2[s], NTD, preferred_element_type=f32)
            qt[:, cols] = _pack((yq * QSCALE).astype(bf16))
            yv = lax.dot_general(_unpack(wqvt[D // 2:D, :]), xn2[s], NTD, preferred_element_type=f32)
            vt[:, cols] = _pack(yv.astype(bf16))
            yk = lax.dot_general(xn2[s], wb_raw[:, D:2 * D], NN, preferred_element_type=f32).astype(bf16)
            krows = pl.ds(pl.multiple_of((r0 + s * SB) // 2, SB // 2), SB // 2)
            for g in range(NT):
                kb[g, krows, :] = _pack(yk[:, g * 128:(g + 1) * 128])

        steps = {"a": qkv_a, "o": out_a, "b": qkv_b}
        for name, s in ROW_ORDER:
            if name == "n":
                ka[:, 0:HALO, :] = ka[:, RB:RB + HALO, :]
                va[:, 0:HALO, :] = va[:, RB:RB + HALO, :]
                load_x(r + 1, l, LX_LOOK)
            else:
                steps[name](s)
        return l

    def head_weights(g, hh, q0):
        w = qt[pl.ds(pl.multiple_of(g * 64 + hh * 16, 16), 16), pl.ds(q0, TQ)]
        parts = []
        if hh > 0:
            parts.append(jnp.zeros((16 * hh, TQ), u32))
        parts.append(w)
        if hh < 3:
            parts.append(jnp.zeros((16 * (3 - hh), TQ), u32))
        return _unpack(jnp.concatenate(parts, axis=0))

    def v_rows(g, hh, c):
        rows = pl.ds(pl.multiple_of(g * 64 + hh * 16, 16), 16)
        return _unpack(vt[rows, c * KC:(c + 1) * KC])

    def finish_group(g):
        o = jnp.dot(v_rows(g, HPB - 1, NC - 1), _unpack(pp[...]), preferred_element_type=f32)
        last = (ot[3 * DH:4 * DH, :] + o) * invs[0:1, :]
        return jnp.concatenate([ot[0:3 * DH, :], last], axis=0).T.astype(bf16)

    def o_rows(q0):
        return pl.ds(pl.multiple_of(q0 // 2, TQ // 2), TQ // 2)

    def attn_fast(q0):
        def body(i, lmax):
            st = {}

            def qk(gg, hh, c):
                g = i * GPB + gg
                if c == 0:
                    st[gg, hh] = dict(w=head_weights(g, hh, q0))
                kc = _unpack(kb[g, c * KC // 2:(c + 1) * KC // 2, :])
                return jnp.dot(kc, st[gg, hh]["w"], preferred_element_type=f32)

            def pv(gg, hh, c, s):
                g = i * GPB + gg
                d = st[gg, hh]
                if c == 0:
                    d["m"] = jnp.broadcast_to(jnp.max(s[0:8], axis=0, keepdims=True), (8, TQ))
                p = jnp.exp2(s.reshape(KC // 8, 8, TQ) - d["m"][None])
                lc = jnp.sum(p, axis=0)
                d["l"] = lc if c == 0 else d["l"] + lc
                p = p.reshape(KC, TQ).astype(bf16)
                if c == NC - 1:
                    d["lsum"] = jnp.sum(d["l"], axis=0, keepdims=True)
                if gg == GPB - 1 and hh == HPB - 1 and c == NC - 1:
                    pp[...] = _pack(p)
                    ot[hh * DH:(hh + 1) * DH, :] = d["acc"]
                    invs[...] = jnp.broadcast_to(_recip(d["lsum"]), (8, TQ))
                    return
                o = jnp.dot(v_rows(g, hh, c), p, preferred_element_type=f32)
                d["acc"] = o if c == 0 else d["acc"] + o
                if c == NC - 1:
                    d["out"] = d["acc"] * _recip(d["lsum"])
                    if gg == GPB - 1:
                        ot[hh * DH:(hh + 1) * DH, :] = d["out"]
                    elif hh == HPB - 1:
                        o_t = jnp.concatenate([st[gg, k]["out"] for k in range(HPB)], axis=0)
                        ob[g, o_rows(q0), :] = _pack(o_t.T.astype(bf16))

            pend = None
            for gg in range(GPB):
                for hh in range(HPB):
                    for c in range(NC):
                        s = qk(gg, hh, c)
                        if pend is None:
                            ob[jnp.where(i == 0, NT, i * GPB - 1), o_rows(q0), :] = _pack(
                                finish_group(jnp.maximum(i * GPB - 1, 0)))
                        else:
                            pv(*pend)
                        pend = (gg, hh, c, s)
            pv(*pend)
            for d in st.values():
                lmax = jnp.maximum(lmax, d["lsum"])
            return lmax

        return lax.fori_loop(0, NT // GPB, body, jnp.zeros((1, TQ), f32))

    def attn_exact(q0):
        def group(g, carry):
            def head(hh, carry2):
                w = qt[pl.ds(pl.multiple_of(g * 64, 64), 64), pl.ds(q0, TQ)]
                row = lax.broadcasted_iota(jnp.int32, (64, TQ), 0) // 16
                w = _unpack(jnp.where(row == hh, w, jnp.zeros_like(w)))

                def scores(c):
                    kc = kb[g, pl.ds(pl.multiple_of(c * (KC // 2), KC // 2), KC // 2), :]
                    return jnp.dot(_unpack(kc), w, preferred_element_type=f32)

                def row_max(c, m):
                    return jnp.maximum(m, jnp.max(scores(c), axis=0, keepdims=True))

                m = lax.fori_loop(0, NC, row_max, jnp.full((1, TQ), -jnp.inf, f32))

                def accumulate(c, state):
                    l, acc = state
                    p = jnp.exp2(scores(c) - m)
                    v = vt[pl.ds(pl.multiple_of(g * 64 + hh * 16, 16), 16),
                           pl.ds(pl.multiple_of(c * KC, KC), KC)]
                    o = jnp.dot(_unpack(v), p.astype(bf16), preferred_element_type=f32)
                    return l + jnp.sum(p, axis=0, keepdims=True), acc + o

                l, acc = lax.fori_loop(0, NC, accumulate,
                                       (jnp.zeros((1, TQ), f32), jnp.zeros((DH, TQ), f32)))
                ot[pl.ds(pl.multiple_of(hh * DH, DH), DH), :] = acc * (1.0 / l)
                return carry2
            lax.fori_loop(0, HPB, head, 0)
            ob[g, o_rows(q0), :] = _pack(ot[...].T.astype(bf16))
            return carry
        lax.fori_loop(0, NT, group, 0)
        pp[...] = jnp.zeros(pp.shape, u32)
        invs[...] = jnp.ones(invs.shape, f32)

    def q_body(qb, l):
        q0 = pl.multiple_of(qb * TQ, TQ)

        def attempt(state):
            a, _ = state

            @pl.when(a == 0)
            def _():
                lmx[...] = jnp.broadcast_to(attn_fast(q0), (8, TQ))

            @pl.when(a == 1)
            def _():
                attn_exact(q0)

            @pl.when(jnp.logical_or(l == 1, a == 1))
            def _():
                for j in range(TQ // OC):
                    out_copy(qb, j).wait()

            kd = (NT - 1) * 128
            o = jnp.concatenate([_unpack(ob[g, o_rows(q0), :]) for g in range(NT - 1)], axis=1)
            o_last = None
            for j in range(TQ // OC):
                y = lax.dot_general(o[j * OC:(j + 1) * OC], wob[0:kd, :], NN,
                                    preferred_element_type=f32)
                if j == 0:
                    o_last = finish_group(NT - 1)
                    y_first = y
                    continue
                if j == 2:
                    bad = _tree(jnp.maximum, [jnp.where(lmx[:, i * 128:(i + 1) * 128] <= L_MAX, 0.0, 1.0)
                                              for i in range(TQ // 128)])
                    unsafe = jnp.max(bad)
                for jj in ((0, 1) if j == 1 else (j,)):
                    yj = (y_first if jj == 0 else y) + lax.dot_general(
                        o_last[jj * OC:(jj + 1) * OC], wob[kd:D, :], NN, preferred_element_type=f32)
                    rows = pl.ds(q0 + jj * OC, OC)
                    x2 = xs[rows, :] + yj
                    xs2[rows, :] = x2
                    outb[rows, :] = x2.astype(bf16)
                    out_copy(qb, jj).start()
            return a + 1, unsafe

        lax.while_loop(lambda st: jnp.logical_or(st[0] == 0, jnp.logical_and(st[0] == 1, st[1] > 0.5)),
                       attempt, (jnp.int32(0), jnp.float32(0)))
        return l

    def layer_pair(l, carry):
        ka[:, 0:HALO, :] = jnp.zeros((NT, HALO, 128), f32)
        va[:, 0:HALO, :] = jnp.zeros((NT, HALO, 128), f32)

        @pl.when(l == 1)
        def _():
            load_x(0, l, 16)

        lax.fori_loop(0, S // RB, row_body, l)

        @pl.when(l == 0)
        def _():
            wob_copy.wait()

        lax.fori_loop(0, S // TQ, q_body, l)
        return carry

    x_copy(0).wait()
    load_x(0, 0, 16)
    wb_copy(1).wait()
    for cp in queue:
        cp.start()
    ot[...] = jnp.zeros(ot.shape, f32)
    pp[...] = jnp.zeros(pp.shape, u32)
    invs[...] = jnp.ones(invs.shape, f32)
    lax.fori_loop(0, 2, layer_pair, 0)
    for qb in range(S // TQ):
        for j in range(TQ // OC):
            out_copy(qb, j).wait()


@jax.jit
def pallas_interleave_layers__sliding_local_dilated__softmax_full_mha__prompt_kernel(
    A_x: jax.Array,
    A_wqkv: jax.Array,
    A_wo: jax.Array,
    B_x: jax.Array,
    B_wqkv: jax.Array,
    B_wo: jax.Array,
):
    del B_x
    x = A_x.reshape(S, D)
    hbm = pl.BlockSpec(memory_space=pl.ANY)
    out = pl.pallas_call(
        _kernel,
        out_shape=jax.ShapeDtypeStruct((S, D), bf16),
        in_specs=[hbm] * 5,
        out_specs=hbm,
        scratch_shapes=[
            pltpu.VMEM((S, D), bf16),
            pltpu.VMEM((D, 3 * D), bf16),
            pltpu.VMEM((D, D), bf16),
            pltpu.VMEM((D, 3 * D), bf16),
            pltpu.VMEM((D, D), bf16),
            pltpu.VMEM((S, D), bf16),
            pltpu.VMEM((NT, H * PITCH, 128), f32),
            pltpu.VMEM((D // 2, 3 * D), u32),
            pltpu.VMEM((D // 2, D), u32),
            pltpu.VMEM((D, D), u32),
            pltpu.VMEM((RB // 2, D), u32),
            pltpu.VMEM((S + RB, D), f32),
            pltpu.VMEM((S, D), f32),
            pltpu.VMEM((NT, RB, 128), f32),
            pltpu.VMEM((NT, HALO + RB, 128), f32),
            pltpu.VMEM((NT, HALO + RB, 128), f32),
            pltpu.VMEM((D // 2, S), u32),
            pltpu.VMEM((NT, S // 2, 128), u32),
            pltpu.VMEM((D // 2, S), u32),
            pltpu.VMEM((NT + 1, S // 2, 128), u32),
            pltpu.VMEM((128, TQ), f32),
            pltpu.VMEM((KC // 2, TQ), u32),
            pltpu.VMEM((8, TQ), f32),
            pltpu.VMEM((8, TQ), f32),
            pltpu.SemaphoreType.DMA((S // RB,)),
            pltpu.SemaphoreType.DMA((3 * D // WCH,)),
            pltpu.SemaphoreType.DMA((5,)),
            pltpu.SemaphoreType.DMA((S // OC,)),
        ],
        compiler_params=pltpu.CompilerParams(vmem_limit_bytes=110 * 1024 * 1024),
    )(x, A_wqkv, A_wo, B_wqkv, B_wo)
    return out.reshape(1, S, D)
```

```python
import functools
import math

import jax
import jax.numpy as jnp
from jax import lax
import jax.experimental.pallas as pl
import jax.experimental.pallas.tpu as pltpu

S = 2048
D = 1024
H = 32
DH = 32
WIN = 8
DIL = 2
EPS = 1e-5
NT = D // 128
HALO = 16
QSCALE = (DH ** -0.5) * math.log2(math.e)

SB = 128
NSUB = 2
RB = SB * NSUB
RC = 8
ROW_ORDER = [("a", 0), ("a", 1), ("o", 0), ("o", 1), ("w", 0), ("l", 1), ("b", 0), ("n", 0), ("b", 1)]
LC = 8
LN_LOOK = 2
LX_LOOK = 2
LOOK = (2, 2)
DEP_END = (True, False)
GATE_COL = (2048, 2048)
TQ = 512
KC = 256
NC = S // KC
OC = 128
GPB = 2
HPB = 4
WCH = 512
WA_STARTS = (1, 1, 1, 2, 2, 2)
PITCH = 40
NFLIGHT = 3
L_MAX = 2.0 ** 64

bf16 = jnp.bfloat16
f32 = jnp.float32
u32 = jnp.uint32

NN = (((1,), (0,)), ((), ()))
NTD = (((1,), (1,)), ((), ()))


def _pack(x):
    return pltpu.bitcast(x, u32)


def _unpack(x):
    return pltpu.bitcast(x, bf16)


def _after(value, dep):
    if dep is None:
        return value
    return jnp.maximum(value, jnp.minimum(dep, -3e38))


def _tree(op, xs):
    xs = list(xs)
    while len(xs) > 1:
        xs = [op(xs[i], xs[i + 1]) if i + 1 < len(xs) else xs[i] for i in range(0, len(xs), 2)]
    return xs[0]


def _recip(x):
    r = pl.reciprocal(x, approx=True)
    return r * (2.0 - x * r)


def _layernorm(load, nrows, look, first_dep=None):
    outs = []
    deps = []
    for c in range(nrows // LC):
        dep = deps[c - look] if c >= look else first_dep
        x = load(c * LC, dep)
        mu = jnp.broadcast_to(jnp.sum(x, axis=-1, keepdims=True), (LC, 128)) * _after(1.0 / D, dep)
        xc = x - jnp.concatenate([mu] * NT, axis=1)
        var = jnp.sum(xc * xc, axis=-1, keepdims=True) * (1.0 / D)
        y = xc * lax.rsqrt(var + EPS)
        deps.append(y[:, D - 128:])
        outs.append(y)
    return jnp.concatenate(outs, axis=0).astype(bf16)


def _kernel(x_hbm, wa_hbm, woa_hbm, wb_hbm, wob_hbm, out_hbm,
            xin, wa_raw, woa_raw, wb_raw, wob, outb,
            stg, wan, woa, wqvt, xnb,
            xs, xs2, qa, ka, va, qt, kb, vt, ob, ot, pp, invs, lmx,
            sem_x, sem_wa, sem_w, sem_o):
    def x_copy(r):
        rows = pl.ds(pl.multiple_of(r * RB, RB), RB)
        return pltpu.make_async_copy(x_hbm.at[rows, :], xin.at[rows, :], sem_x.at[r])

    def wa_copy(i):
        cols = pl.ds(pl.multiple_of(i * WCH, WCH), WCH)
        return pltpu.make_async_copy(wa_hbm.at[:, cols], wa_raw.at[:, cols], sem_wa.at[i])

    def wb_copy(i):
        cols = pl.ds(pl.multiple_of(i * D, D), D)
        return pltpu.make_async_copy(wb_hbm.at[:, cols], wb_raw.at[:, cols], sem_w.at[i])

    woa_copy = pltpu.make_async_copy(woa_hbm, woa_raw, sem_w.at[3])
    wob_copy = pltpu.make_async_copy(wob_hbm, wob, sem_w.at[4])

    def out_copy(qb, j):
        rows = pl.ds(pl.multiple_of(qb * TQ + j * OC, OC), OC)
        return pltpu.make_async_copy(outb.at[rows, :], out_hbm.at[rows, :],
                                     sem_o.at[qb * (TQ // OC) + j])

    n_wa = 3 * D // WCH
    queue = ([wa_copy(i) for i in range(n_wa)]
             + [woa_copy, x_copy(0), x_copy(1), wb_copy(0), wb_copy(2), wb_copy(1)]
             + [x_copy(r) for r in range(2, S // RB)] + [wob_copy])
    for cp in queue[:NFLIGHT]:
        cp.start()
    queue = queue[NFLIGHT:]

    batches = [[queue.pop(0) for _ in range(n)] for n in WA_STARTS]

    def start_in_loop(i, my_batches):
        for k, batch in enumerate(my_batches):
            @pl.when(i == k)
            def _():
                for cp in batch:
                    cp.start()

    def transpose(w):
        ri = lax.broadcasted_iota(jnp.int32, (128, 128), 0)
        ci = lax.broadcasted_iota(jnp.int32, (128, 128), 1)
        eye = jnp.where(ri == ci, 1.0, 0.0).astype(bf16)
        return lax.dot_general(eye, w, NTD, preferred_element_type=f32)

    def stage(j, rows):
        for hh in range(HPB):
            r = pl.ds(pl.multiple_of((j * HPB + hh) * PITCH, 8), DH)
            for t in range(NT):
                stg[t, r, :] = rows[hh * DH:(hh + 1) * DH, t * 128:(t + 1) * 128]

    def gather(t):
        return jnp.concatenate([stg[t, pl.ds(d, H, stride=PITCH), :].astype(bf16)
                                for d in range(DH)], axis=0)

    def prep_wa(part, carry):
        for half in range(2):
            i = 2 * part + half
            wa_copy(i).wait()
            start_in_loop(part, batches[half::2])
            for j in range(half * NT // 2, (half + 1) * NT // 2):
                cols = pl.ds(pl.multiple_of(part * D + j * 128, 128), 128)
                stage(j, transpose(wa_raw[:, cols]))
        cols = pl.ds(pl.multiple_of(part * D, D), D)
        for t in range(NT):
            wan[t * 64:(t + 1) * 64, cols] = _pack(transpose(gather(t)).astype(bf16))
        return carry

    def prep_woa():
        def put(j, carry):
            stage(j, woa_raw[pl.ds(pl.multiple_of(j * 128, 128), 128), :].astype(f32))
            return carry

        def get(t, carry):
            woa[:, pl.ds(pl.multiple_of(t * 128, 128), 128)] = _pack(gather(t))
            return carry

        lax.fori_loop(0, NT, put, 0)
        lax.fori_loop(0, NT, get, 0)

    def prep_wb(part, carry):
        wb_copy(2 * part).wait()
        for j in range(NT):
            cols = pl.ds(pl.multiple_of(2 * part * D + j * 128, 128), 128)
            rows = pl.ds(pl.multiple_of(part * (D // 2) + j * 64, 64), 64)
            wqvt[rows, :] = _pack(transpose(wb_raw[:, cols]).astype(bf16))
        return carry

    lax.fori_loop(0, 3, prep_wa, 0)
    woa_copy.wait()
    prep_woa()

    def local_attn(r0, s, first_dep):
        outs = []
        deps = []
        for c in range(SB // RC):
            base = s * SB + c * RC
            scale = _after(QSCALE, deps[c - LOOK[s]] if c >= LOOK[s] else first_dep)
            logits = [None] * WIN
            for t in range(NT):
                q = qa[t, base:base + RC, :] * scale
                for w in range(WIN):
                    o0 = HALO + base - DIL * w
                    term = q * ka[t, o0:o0 + RC, :]
                    logits[w] = term if t == 0 else logits[w] + term
            for w in range(WIN):
                acc = logits[w]
                acc = acc + pltpu.roll(acc, 64, 1)
                acc = acc + pltpu.roll(acc, 32, 1)
                if base < DIL * w:
                    row = r0 + base + lax.broadcasted_iota(jnp.int32, (RC, 128), 0)
                    acc = jnp.where(row >= DIL * w, acc, -1e9)
                logits[w] = acc
            m = _tree(jnp.maximum, logits)
            p = [jnp.exp2(lg - m) for lg in logits]
            inv = _recip(_tree(jnp.add, p))
            tiles = []
            for t in range(NT):
                terms = [p[w] * va[t, HALO + base - DIL * w:HALO + base - DIL * w + RC, :]
                         for w in range(WIN)]
                acc = _tree(jnp.add, terms) * inv
                tiles.append(acc.astype(bf16))
            deps.append(acc if DEP_END[s] else m)
            outs.append(jnp.concatenate(tiles, axis=1))
        return jnp.concatenate(outs, axis=0)

    def load_x(r, l, look):
        r0 = pl.multiple_of(jnp.minimum(r, S // RB - 1) * RB, RB)
        w0 = pl.multiple_of(r * RB, RB)

        def load(start, dep):
            rows = pl.ds(r0 + start, LC)
            lvec = _after(jnp.full((LC, 128), l, f32), dep)
            first = jnp.concatenate([lvec == 0.0] * NT, axis=1)
            xi = xin[pl.ds(r0 + start // 16 * 16, 16), :].astype(f32)[start % 16:start % 16 + LC]
            x = jnp.where(first, xi, xs2[rows, :])
            xs[pl.ds(w0 + start, LC), :] = x
            return x

        xnb[...] = _pack(_layernorm(load, RB, look))

    def row_body(r, l):
        r0 = pl.multiple_of(r * RB, RB)
        rn = jnp.minimum(r + 1, S // RB - 1)

        @pl.when(jnp.logical_and(l == 0, r + 1 < S // RB))
        def _():
            x_copy(rn).wait()

        rows = [pl.ds(r0 + s * SB, SB) for s in range(NSUB)]
        gate = {}
        xn2 = {}

        def qkv_a(s):
            xn = _unpack(xnb[s * SB // 2:(s + 1) * SB // 2, :])
            y = lax.dot_general(xn, _unpack(wan[...]), NN, preferred_element_type=f32)
            for t in range(NT):
                qa[t, s * SB:(s + 1) * SB, :] = y[:, t * 128:(t + 1) * 128]
                ka[t, HALO + s * SB:HALO + (s + 1) * SB, :] = y[:, D + t * 128:D + (t + 1) * 128]
                va[t, HALO + s * SB:HALO + (s + 1) * SB, :] = y[:, 2 * D + t * 128:2 * D + (t + 1) * 128]
            gate[s] = y[SB - RC:SB, GATE_COL[s] - 128:GATE_COL[s]]

        def out_a(s):
            o = local_attn(r0, s, gate[s])
            x1 = xs[rows[s], :] + lax.dot_general(o, _unpack(woa[...]), NN,
                                                  preferred_element_type=f32)
            xs[rows[s], :] = x1
            if s < NSUB - 1:
                xn2[s] = _layernorm(lambda st, dep: x1[st:st + LC], SB, LN_LOOK)

        def norm_b(s):
            xn2[s] = _layernorm(lambda st, dep: xs[pl.ds(r0 + s * SB + st, LC), :], SB, LN_LOOK)

        def weights_b(_):
            @pl.when(jnp.logical_and(l == 0, r == 0))
            def _():
                lax.fori_loop(0, 2, prep_wb, 0)
                wb_copy(1).wait()
                for cp in queue:
                    cp.start()

        def qkv_b(s):
            cols = pl.ds(r0 + s * SB, SB)
            yq = lax.dot_general(_unpack(wqvt[0:D // 2, :]), xn2[s], NTD, preferred_element_type=f32)
            qt[:, cols] = _pack((yq * QSCALE).astype(bf16))
            yv = lax.dot_general(_unpack(wqvt[D // 2:D, :]), xn2[s], NTD, preferred_element_type=f32)
            vt[:, cols] = _pack(yv.astype(bf16))
            yk = lax.dot_general(xn2[s], wb_raw[:, D:2 * D], NN, preferred_element_type=f32).astype(bf16)
            krows = pl.ds(pl.multiple_of((r0 + s * SB) // 2, SB // 2), SB // 2)
            for g in range(NT):
                kb[g, krows, :] = _pack(yk[:, g * 128:(g + 1) * 128])

        steps = {"a": qkv_a, "o": out_a, "b": qkv_b, "w": weights_b, "l": norm_b}
        for name, s in ROW_ORDER:
            if name == "n":
                ka[:, 0:HALO, :] = ka[:, RB:RB + HALO, :]
                va[:, 0:HALO, :] = va[:, RB:RB + HALO, :]
                load_x(r + 1, l, LX_LOOK)
            else:
                steps[name](s)
        return l

    def head_weights(g, hh, q0):
        w = qt[pl.ds(pl.multiple_of(g * 64 + hh * 16, 16), 16), pl.ds(q0, TQ)]
        parts = []
        if hh > 0:
            parts.append(jnp.zeros((16 * hh, TQ), u32))
        parts.append(w)
        if hh < 3:
            parts.append(jnp.zeros((16 * (3 - hh), TQ), u32))
        return _unpack(jnp.concatenate(parts, axis=0))

    def v_rows(g, hh, c):
        rows = pl.ds(pl.multiple_of(g * 64 + hh * 16, 16), 16)
        return _unpack(vt[rows, c * KC:(c + 1) * KC])

    def finish_group(g):
        o = jnp.dot(v_rows(g, HPB - 1, NC - 1), _unpack(pp[...]), preferred_element_type=f32)
        last = (ot[3 * DH:4 * DH, :] + o) * invs[0:1, :]
        return jnp.concatenate([ot[0:3 * DH, :], last], axis=0).T.astype(bf16)

    def o_rows(q0):
        return pl.ds(pl.multiple_of(q0 // 2, TQ // 2), TQ // 2)

    def attn_fast(q0):
        def body(i, lmax):
            st = {}

            def qk(gg, hh, c):
                g = i * GPB + gg
                if c == 0:
                    st[gg, hh] = dict(w=head_weights(g, hh, q0))
                kc = _unpack(kb[g, c * KC // 2:(c + 1) * KC // 2, :])
                return jnp.dot(kc, st[gg, hh]["w"], preferred_element_type=f32)

            def pv(gg, hh, c, s):
                g = i * GPB + gg
                d = st[gg, hh]
                if c == 0:
                    d["m"] = jnp.broadcast_to(jnp.max(s[0:8], axis=0, keepdims=True), (8, TQ))
                p = jnp.exp2(s.reshape(KC // 8, 8, TQ) - d["m"][None])
                lc = jnp.sum(p, axis=0)
                d["l"] = lc if c == 0 else d["l"] + lc
                p = p.reshape(KC, TQ).astype(bf16)
                if c == NC - 1:
                    d["lsum"] = jnp.sum(d["l"], axis=0, keepdims=True)
                if gg == GPB - 1 and hh == HPB - 1 and c == NC - 1:
                    pp[...] = _pack(p)
                    ot[hh * DH:(hh + 1) * DH, :] = d["acc"]
                    invs[...] = jnp.broadcast_to(_recip(d["lsum"]), (8, TQ))
                    return
                o = jnp.dot(v_rows(g, hh, c), p, preferred_element_type=f32)
                d["acc"] = o if c == 0 else d["acc"] + o
                if c == NC - 1:
                    d["out"] = d["acc"] * _recip(d["lsum"])
                    if gg == GPB - 1:
                        ot[hh * DH:(hh + 1) * DH, :] = d["out"]
                    elif hh == HPB - 1:
                        o_t = jnp.concatenate([st[gg, k]["out"] for k in range(HPB)], axis=0)
                        ob[g, o_rows(q0), :] = _pack(o_t.T.astype(bf16))

            pend = None
            for gg in range(GPB):
                for hh in range(HPB):
                    for c in range(NC):
                        s = qk(gg, hh, c)
                        if pend is None:
                            ob[jnp.where(i == 0, NT, i * GPB - 1), o_rows(q0), :] = _pack(
                                finish_group(jnp.maximum(i * GPB - 1, 0)))
                        else:
                            pv(*pend)
                        pend = (gg, hh, c, s)
            pv(*pend)
            for d in st.values():
                lmax = jnp.maximum(lmax, d["lsum"])
            return lmax

        return lax.fori_loop(0, NT // GPB, body, jnp.zeros((1, TQ), f32))

    def attn_exact(q0):
        def group(g, carry):
            def head(hh, carry2):
                w = qt[pl.ds(pl.multiple_of(g * 64, 64), 64), pl.ds(q0, TQ)]
                row = lax.broadcasted_iota(jnp.int32, (64, TQ), 0) // 16
                w = _unpack(jnp.where(row == hh, w, jnp.zeros_like(w)))

                def scores(c):
                    kc = kb[g, pl.ds(pl.multiple_of(c * (KC // 2), KC // 2), KC // 2), :]
                    return jnp.dot(_unpack(kc), w, preferred_element_type=f32)

                def row_max(c, m):
                    return jnp.maximum(m, jnp.max(scores(c), axis=0, keepdims=True))

                m = lax.fori_loop(0, NC, row_max, jnp.full((1, TQ), -jnp.inf, f32))

                def accumulate(c, state):
                    l, acc = state
                    p = jnp.exp2(scores(c) - m)
                    v = vt[pl.ds(pl.multiple_of(g * 64 + hh * 16, 16), 16),
                           pl.ds(pl.multiple_of(c * KC, KC), KC)]
                    o = jnp.dot(_unpack(v), p.astype(bf16), preferred_element_type=f32)
                    return l + jnp.sum(p, axis=0, keepdims=True), acc + o

                l, acc = lax.fori_loop(0, NC, accumulate,
                                       (jnp.zeros((1, TQ), f32), jnp.zeros((DH, TQ), f32)))
                ot[pl.ds(pl.multiple_of(hh * DH, DH), DH), :] = acc * (1.0 / l)
                return carry2
            lax.fori_loop(0, HPB, head, 0)
            ob[g, o_rows(q0), :] = _pack(ot[...].T.astype(bf16))
            return carry
        lax.fori_loop(0, NT, group, 0)
        pp[...] = jnp.zeros(pp.shape, u32)
        invs[...] = jnp.ones(invs.shape, f32)

    def q_body(qb, l):
        q0 = pl.multiple_of(qb * TQ, TQ)

        def attempt(state):
            a, _ = state

            @pl.when(a == 0)
            def _():
                lmx[...] = jnp.broadcast_to(attn_fast(q0), (8, TQ))

            @pl.when(a == 1)
            def _():
                attn_exact(q0)

            @pl.when(jnp.logical_or(l == 1, a == 1))
            def _():
                for j in range(TQ // OC):
                    out_copy(qb, j).wait()

            kd = (NT - 1) * 128
            o = jnp.concatenate([_unpack(ob[g, o_rows(q0), :]) for g in range(NT - 1)], axis=1)
            o_last = None
            for j in range(TQ // OC):
                y = lax.dot_general(o[j * OC:(j + 1) * OC], wob[0:kd, :], NN,
                                    preferred_element_type=f32)
                if j == 0:
                    o_last = finish_group(NT - 1)
                    y_first = y
                    continue
                if j == 2:
                    bad = _tree(jnp.maximum, [jnp.where(lmx[:, i * 128:(i + 1) * 128] <= L_MAX, 0.0, 1.0)
                                              for i in range(TQ // 128)])
                    unsafe = jnp.max(bad)
                for jj in ((0, 1) if j == 1 else (j,)):
                    yj = (y_first if jj == 0 else y) + lax.dot_general(
                        o_last[jj * OC:(jj + 1) * OC], wob[kd:D, :], NN, preferred_element_type=f32)
                    rows = pl.ds(q0 + jj * OC, OC)
                    x2 = xs[rows, :] + yj
                    xs2[rows, :] = x2
                    outb[rows, :] = x2.astype(bf16)
                    out_copy(qb, jj).start()
            return a + 1, unsafe

        lax.while_loop(lambda st: jnp.logical_or(st[0] == 0, jnp.logical_and(st[0] == 1, st[1] > 0.5)),
                       attempt, (jnp.int32(0), jnp.float32(0)))
        return l

    def layer_pair(l, carry):
        ka[:, 0:HALO, :] = jnp.zeros((NT, HALO, 128), f32)
        va[:, 0:HALO, :] = jnp.zeros((NT, HALO, 128), f32)

        @pl.when(l == 1)
        def _():
            load_x(0, l, 16)

        lax.fori_loop(0, S // RB, row_body, l)

        @pl.when(l == 0)
        def _():
            wob_copy.wait()

        lax.fori_loop(0, S // TQ, q_body, l)
        return carry

    x_copy(0).wait()
    load_x(0, 0, 16)
    ot[...] = jnp.zeros(ot.shape, f32)
    pp[...] = jnp.zeros(pp.shape, u32)
    invs[...] = jnp.ones(invs.shape, f32)
    lax.fori_loop(0, 2, layer_pair, 0)
    for qb in range(S // TQ):
        for j in range(TQ // OC):
            out_copy(qb, j).wait()


@jax.jit
def pallas_interleave_layers__sliding_local_dilated__softmax_full_mha__prompt_kernel(
    A_x: jax.Array,
    A_wqkv: jax.Array,
    A_wo: jax.Array,
    B_x: jax.Array,
    B_wqkv: jax.Array,
    B_wo: jax.Array,
):
    del B_x
    x = A_x.reshape(S, D)
    hbm = pl.BlockSpec(memory_space=pl.ANY)
    out = pl.pallas_call(
        _kernel,
        out_shape=jax.ShapeDtypeStruct((S, D), bf16),
        in_specs=[hbm] * 5,
        out_specs=hbm,
        scratch_shapes=[
            pltpu.VMEM((S, D), bf16),
            pltpu.VMEM((D, 3 * D), bf16),
            pltpu.VMEM((D, D), bf16),
            pltpu.VMEM((D, 3 * D), bf16),
            pltpu.VMEM((D, D), bf16),
            pltpu.VMEM((S, D), bf16),
            pltpu.VMEM((NT, H * PITCH, 128), f32),
            pltpu.VMEM((D // 2, 3 * D), u32),
            pltpu.VMEM((D // 2, D), u32),
            pltpu.VMEM((D, D), u32),
            pltpu.VMEM((RB // 2, D), u32),
            pltpu.VMEM((S + RB, D), f32),
            pltpu.VMEM((S, D), f32),
            pltpu.VMEM((NT, RB, 128), f32),
            pltpu.VMEM((NT, HALO + RB, 128), f32),
            pltpu.VMEM((NT, HALO + RB, 128), f32),
            pltpu.VMEM((D // 2, S), u32),
            pltpu.VMEM((NT, S // 2, 128), u32),
            pltpu.VMEM((D // 2, S), u32),
            pltpu.VMEM((NT + 1, S // 2, 128), u32),
            pltpu.VMEM((128, TQ), f32),
            pltpu.VMEM((KC // 2, TQ), u32),
            pltpu.VMEM((8, TQ), f32),
            pltpu.VMEM((8, TQ), f32),
            pltpu.SemaphoreType.DMA((S // RB,)),
            pltpu.SemaphoreType.DMA((3 * D // WCH,)),
            pltpu.SemaphoreType.DMA((5,)),
            pltpu.SemaphoreType.DMA((S // OC,)),
        ],
        compiler_params=pltpu.CompilerParams(vmem_limit_bytes=110 * 1024 * 1024),
    )(x, A_wqkv, A_wo, B_wqkv, B_wo)
    return out.reshape(1, S, D)
```

```python
import functools
import math

import jax
import jax.numpy as jnp
from jax import lax
import jax.experimental.pallas as pl
import jax.experimental.pallas.tpu as pltpu

S = 2048
D = 1024
H = 32
DH = 32
WIN = 8
DIL = 2
EPS = 1e-5
NT = D // 128
HALO = 16
QSCALE = (DH ** -0.5) * math.log2(math.e)

SB = 128
NSUB = 2
RB = SB * NSUB
RC = 8
ROW_ORDER = [("a", 0), ("a", 1), ("o", 0), ("o", 1), ("w", 0), ("l", 1), ("b", 0), ("n", 0), ("b", 1)]
LC = 8
LN_LOOK = 2
LX_LOOK = 2
LOOK = (2, 2)
DEP_END = (True, False)
GATE_COL = (2048, 2048)
TQ = 512
KC = 256
NC = S // KC
OC = 128
GPB = 2
HPB = 4
WCH = 512
WA_STARTS = (1, 1, 1, 2, 2, 2)
PITCH = 40
NFLIGHT = 3
L_MAX = 2.0 ** 64
V_EXP = 50

bf16 = jnp.bfloat16
f32 = jnp.float32
u32 = jnp.uint32

NN = (((1,), (0,)), ((), ()))
NTD = (((1,), (1,)), ((), ()))


def _pack(x):
    return pltpu.bitcast(x, u32)


def _unpack(x):
    return pltpu.bitcast(x, bf16)


def _after(value, dep):
    if dep is None:
        return value
    return jnp.maximum(value, jnp.minimum(dep, -3e38))


def _tree(op, xs):
    xs = list(xs)
    while len(xs) > 1:
        xs = [op(xs[i], xs[i + 1]) if i + 1 < len(xs) else xs[i] for i in range(0, len(xs), 2)]
    return xs[0]


def _recip(x):
    r = pl.reciprocal(x, approx=True)
    return r * (2.0 - x * r)


def _too_large(packed):
    bias = 0x8000 - ((127 + V_EXP) << 7)
    t = (packed & jnp.uint32(0x7F807F80)) + jnp.uint32(bias << 16 | bias)
    return _tree(jnp.bitwise_or, [t[i:i + 8] for i in range(0, t.shape[0], 8)])


def _layernorm(load, nrows, look, first_dep=None):
    outs = []
    deps = []
    for c in range(nrows // LC):
        dep = deps[c - look] if c >= look else first_dep
        x = load(c * LC, dep)
        mu = jnp.broadcast_to(jnp.sum(x, axis=-1, keepdims=True), (LC, 128)) * _after(1.0 / D, dep)
        xc = x - jnp.concatenate([mu] * NT, axis=1)
        var = jnp.sum(xc * xc, axis=-1, keepdims=True) * (1.0 / D)
        y = xc * lax.rsqrt(var + EPS)
        deps.append(y[:, D - 128:])
        outs.append(y)
    return jnp.concatenate(outs, axis=0).astype(bf16)


def _kernel(x_hbm, wa_hbm, woa_hbm, wb_hbm, wob_hbm, out_hbm,
            xin, wa_raw, woa_raw, wb_raw, wob, outb,
            stg, wan, woa, wqvt, xnb,
            xs, xs2, qa, ka, va, qt, kb, vt, ob, ot, pp, invs, lmx, vbig,
            sem_x, sem_wa, sem_w, sem_o):
    def x_copy(r):
        rows = pl.ds(pl.multiple_of(r * RB, RB), RB)
        return pltpu.make_async_copy(x_hbm.at[rows, :], xin.at[rows, :], sem_x.at[r])

    def wa_copy(i):
        cols = pl.ds(pl.multiple_of(i * WCH, WCH), WCH)
        return pltpu.make_async_copy(wa_hbm.at[:, cols], wa_raw.at[:, cols], sem_wa.at[i])

    def wb_copy(i):
        cols = pl.ds(pl.multiple_of(i * D, D), D)
        return pltpu.make_async_copy(wb_hbm.at[:, cols], wb_raw.at[:, cols], sem_w.at[i])

    woa_copy = pltpu.make_async_copy(woa_hbm, woa_raw, sem_w.at[3])
    wob_copy = pltpu.make_async_copy(wob_hbm, wob, sem_w.at[4])

    def out_copy(qb, j):
        rows = pl.ds(pl.multiple_of(qb * TQ + j * OC, OC), OC)
        return pltpu.make_async_copy(outb.at[rows, :], out_hbm.at[rows, :],
                                     sem_o.at[qb * (TQ // OC) + j])

    n_wa = 3 * D // WCH
    queue = ([wa_copy(i) for i in range(n_wa)]
             + [woa_copy, x_copy(0), x_copy(1), wb_copy(0), wb_copy(2), wb_copy(1)]
             + [x_copy(r) for r in range(2, S // RB)] + [wob_copy])
    for cp in queue[:NFLIGHT]:
        cp.start()
    queue = queue[NFLIGHT:]

    batches = [[queue.pop(0) for _ in range(n)] for n in WA_STARTS]

    def start_in_loop(i, my_batches):
        for k, batch in enumerate(my_batches):
            @pl.when(i == k)
            def _():
                for cp in batch:
                    cp.start()

    def transpose(w):
        ri = lax.broadcasted_iota(jnp.int32, (128, 128), 0)
        ci = lax.broadcasted_iota(jnp.int32, (128, 128), 1)
        eye = jnp.where(ri == ci, 1.0, 0.0).astype(bf16)
        return lax.dot_general(eye, w, NTD, preferred_element_type=f32)

    def stage(j, rows):
        for hh in range(HPB):
            r = pl.ds(pl.multiple_of((j * HPB + hh) * PITCH, 8), DH)
            for t in range(NT):
                stg[t, r, :] = rows[hh * DH:(hh + 1) * DH, t * 128:(t + 1) * 128]

    def gather(t):
        return jnp.concatenate([stg[t, pl.ds(d, H, stride=PITCH), :].astype(bf16)
                                for d in range(DH)], axis=0)

    def prep_wa(part, carry):
        for half in range(2):
            i = 2 * part + half
            wa_copy(i).wait()
            start_in_loop(part, batches[half::2])
            for j in range(half * NT // 2, (half + 1) * NT // 2):
                cols = pl.ds(pl.multiple_of(part * D + j * 128, 128), 128)
                stage(j, transpose(wa_raw[:, cols]))
        cols = pl.ds(pl.multiple_of(part * D, D), D)
        for t in range(NT):
            wan[t * 64:(t + 1) * 64, cols] = _pack(transpose(gather(t)).astype(bf16))
        return carry

    def prep_woa():
        def put(j, carry):
            stage(j, woa_raw[pl.ds(pl.multiple_of(j * 128, 128), 128), :].astype(f32))
            return carry

        def get(t, carry):
            woa[:, pl.ds(pl.multiple_of(t * 128, 128), 128)] = _pack(gather(t))
            return carry

        lax.fori_loop(0, NT, put, 0)
        lax.fori_loop(0, NT, get, 0)

    def prep_wb(part, carry):
        wb_copy(2 * part).wait()
        for j in range(NT):
            cols = pl.ds(pl.multiple_of(2 * part * D + j * 128, 128), 128)
            rows = pl.ds(pl.multiple_of(part * (D // 2) + j * 64, 64), 64)
            wqvt[rows, :] = _pack(transpose(wb_raw[:, cols]).astype(bf16))
        return carry

    lax.fori_loop(0, 3, prep_wa, 0)
    woa_copy.wait()
    prep_woa()

    def local_attn(r0, s, first_dep):
        outs = []
        deps = []
        for c in range(SB // RC):
            base = s * SB + c * RC
            scale = _after(QSCALE, deps[c - LOOK[s]] if c >= LOOK[s] else first_dep)
            logits = [None] * WIN
            for t in range(NT):
                q = qa[t, base:base + RC, :] * scale
                for w in range(WIN):
                    o0 = HALO + base - DIL * w
                    term = q * ka[t, o0:o0 + RC, :]
                    logits[w] = term if t == 0 else logits[w] + term
            for w in range(WIN):
                acc = logits[w]
                acc = acc + pltpu.roll(acc, 64, 1)
                acc = acc + pltpu.roll(acc, 32, 1)
                if base < DIL * w:
                    row = r0 + base + lax.broadcasted_iota(jnp.int32, (RC, 128), 0)
                    acc = jnp.where(row >= DIL * w, acc, -1e9)
                logits[w] = acc
            m = _tree(jnp.maximum, logits)
            p = [jnp.exp2(lg - m) for lg in logits]
            inv = _recip(_tree(jnp.add, p))
            tiles = []
            for t in range(NT):
                terms = [p[w] * va[t, HALO + base - DIL * w:HALO + base - DIL * w + RC, :]
                         for w in range(WIN)]
                acc = _tree(jnp.add, terms) * inv
                tiles.append(acc.astype(bf16))
            deps.append(acc if DEP_END[s] else m)
            outs.append(jnp.concatenate(tiles, axis=1))
        return jnp.concatenate(outs, axis=0)

    def load_x(r, l, look):
        r0 = pl.multiple_of(jnp.minimum(r, S // RB - 1) * RB, RB)
        w0 = pl.multiple_of(r * RB, RB)

        def load(start, dep):
            rows = pl.ds(r0 + start, LC)
            lvec = _after(jnp.full((LC, 128), l, f32), dep)
            first = jnp.concatenate([lvec == 0.0] * NT, axis=1)
            xi = xin[pl.ds(r0 + start // 16 * 16, 16), :].astype(f32)[start % 16:start % 16 + LC]
            x = jnp.where(first, xi, xs2[rows, :])
            xs[pl.ds(w0 + start, LC), :] = x
            return x

        xnb[...] = _pack(_layernorm(load, RB, look))

    def row_body(r, l):
        r0 = pl.multiple_of(r * RB, RB)
        rn = jnp.minimum(r + 1, S // RB - 1)

        @pl.when(jnp.logical_and(l == 0, r + 1 < S // RB))
        def _():
            x_copy(rn).wait()

        rows = [pl.ds(r0 + s * SB, SB) for s in range(NSUB)]
        gate = {}
        xn2 = {}

        def qkv_a(s):
            xn = _unpack(xnb[s * SB // 2:(s + 1) * SB // 2, :])
            y = lax.dot_general(xn, _unpack(wan[...]), NN, preferred_element_type=f32)
            for t in range(NT):
                qa[t, s * SB:(s + 1) * SB, :] = y[:, t * 128:(t + 1) * 128]
                ka[t, HALO + s * SB:HALO + (s + 1) * SB, :] = y[:, D + t * 128:D + (t + 1) * 128]
                va[t, HALO + s * SB:HALO + (s + 1) * SB, :] = y[:, 2 * D + t * 128:2 * D + (t + 1) * 128]
            gate[s] = y[SB - RC:SB, GATE_COL[s] - 128:GATE_COL[s]]

        def out_a(s):
            o = local_attn(r0, s, gate[s])
            x1 = xs[rows[s], :] + lax.dot_general(o, _unpack(woa[...]), NN,
                                                  preferred_element_type=f32)
            xs[rows[s], :] = x1
            if s < NSUB - 1:
                xn2[s] = _layernorm(lambda st, dep: x1[st:st + LC], SB, LN_LOOK)

        def norm_b(s):
            xn2[s] = _layernorm(lambda st, dep: xs[pl.ds(r0 + s * SB + st, LC), :], SB, LN_LOOK)

        def weights_b(_):
            @pl.when(jnp.logical_and(l == 0, r == 0))
            def _():
                lax.fori_loop(0, 2, prep_wb, 0)
                wb_copy(1).wait()
                for cp in queue:
                    cp.start()

        def qkv_b(s):
            cols = pl.ds(r0 + s * SB, SB)
            yq = lax.dot_general(_unpack(wqvt[0:D // 2, :]), xn2[s], NTD, preferred_element_type=f32)
            qt[:, cols] = _pack((yq * QSCALE).astype(bf16))
            yv = lax.dot_general(_unpack(wqvt[D // 2:D, :]), xn2[s], NTD, preferred_element_type=f32)
            v_t = _pack(yv.astype(bf16))
            vt[:, cols] = v_t
            vbig[...] = vbig[...] | _too_large(v_t)
            yk = lax.dot_general(xn2[s], wb_raw[:, D:2 * D], NN, preferred_element_type=f32).astype(bf16)
            krows = pl.ds(pl.multiple_of((r0 + s * SB) // 2, SB // 2), SB // 2)
            for g in range(NT):
                kb[g, krows, :] = _pack(yk[:, g * 128:(g + 1) * 128])

        steps = {"a": qkv_a, "o": out_a, "b": qkv_b, "w": weights_b, "l": norm_b}
        for name, s in ROW_ORDER:
            if name == "n":
                ka[:, 0:HALO, :] = ka[:, RB:RB + HALO, :]
                va[:, 0:HALO, :] = va[:, RB:RB + HALO, :]
                load_x(r + 1, l, LX_LOOK)
            else:
                steps[name](s)
        return l

    def head_weights(g, hh, q0):
        w = qt[pl.ds(pl.multiple_of(g * 64 + hh * 16, 16), 16), pl.ds(q0, TQ)]
        parts = []
        if hh > 0:
            parts.append(jnp.zeros((16 * hh, TQ), u32))
        parts.append(w)
        if hh < 3:
            parts.append(jnp.zeros((16 * (3 - hh), TQ), u32))
        return _unpack(jnp.concatenate(parts, axis=0))

    def v_rows(g, hh, c):
        rows = pl.ds(pl.multiple_of(g * 64 + hh * 16, 16), 16)
        return _unpack(vt[rows, c * KC:(c + 1) * KC])

    def finish_group(g):
        o = jnp.dot(v_rows(g, HPB - 1, NC - 1), _unpack(pp[...]), preferred_element_type=f32)
        last = (ot[3 * DH:4 * DH, :] + o) * invs[0:1, :]
        return jnp.concatenate([ot[0:3 * DH, :], last], axis=0).T.astype(bf16)

    def o_rows(q0):
        return pl.ds(pl.multiple_of(q0 // 2, TQ // 2), TQ // 2)

    def attn_fast(q0):
        def body(i, lmax):
            st = {}

            def qk(gg, hh, c):
                g = i * GPB + gg
                if c == 0:
                    st[gg, hh] = dict(w=head_weights(g, hh, q0))
                kc = _unpack(kb[g, c * KC // 2:(c + 1) * KC // 2, :])
                return jnp.dot(kc, st[gg, hh]["w"], preferred_element_type=f32)

            def pv(gg, hh, c, s):
                g = i * GPB + gg
                d = st[gg, hh]
                if c == 0:
                    d["m"] = jnp.broadcast_to(jnp.max(s[0:8], axis=0, keepdims=True), (8, TQ))
                p = jnp.exp2(s.reshape(KC // 8, 8, TQ) - d["m"][None])
                lc = jnp.sum(p, axis=0)
                d["l"] = lc if c == 0 else d["l"] + lc
                p = p.reshape(KC, TQ).astype(bf16)
                if c == NC - 1:
                    d["lsum"] = jnp.sum(d["l"], axis=0, keepdims=True)
                if gg == GPB - 1 and hh == HPB - 1 and c == NC - 1:
                    pp[...] = _pack(p)
                    ot[hh * DH:(hh + 1) * DH, :] = d["acc"]
                    invs[...] = jnp.broadcast_to(_recip(d["lsum"]), (8, TQ))
                    return
                o = jnp.dot(v_rows(g, hh, c), p, preferred_element_type=f32)
                d["acc"] = o if c == 0 else d["acc"] + o
                if c == NC - 1:
                    d["out"] = d["acc"] * _recip(d["lsum"])
                    if gg == GPB - 1:
                        ot[hh * DH:(hh + 1) * DH, :] = d["out"]
                    elif hh == HPB - 1:
                        o_t = jnp.concatenate([st[gg, k]["out"] for k in range(HPB)], axis=0)
                        ob[g, o_rows(q0), :] = _pack(o_t.T.astype(bf16))

            pend = None
            for gg in range(GPB):
                for hh in range(HPB):
                    for c in range(NC):
                        s = qk(gg, hh, c)
                        if pend is None:
                            ob[jnp.where(i == 0, NT, i * GPB - 1), o_rows(q0), :] = _pack(
                                finish_group(jnp.maximum(i * GPB - 1, 0)))
                        else:
                            pv(*pend)
                        pend = (gg, hh, c, s)
            pv(*pend)
            for d in st.values():
                lmax = jnp.maximum(lmax, d["lsum"])
            return lmax

        return lax.fori_loop(0, NT // GPB, body, jnp.zeros((1, TQ), f32))

    def attn_exact(q0):
        def group(g, carry):
            def head(hh, carry2):
                w = qt[pl.ds(pl.multiple_of(g * 64, 64), 64), pl.ds(q0, TQ)]
                row = lax.broadcasted_iota(jnp.int32, (64, TQ), 0) // 16
                w = _unpack(jnp.where(row == hh, w, jnp.zeros_like(w)))

                def scores(c):
                    kc = kb[g, pl.ds(pl.multiple_of(c * (KC // 2), KC // 2), KC // 2), :]
                    return jnp.dot(_unpack(kc), w, preferred_element_type=f32)

                def row_max(c, m):
                    return jnp.maximum(m, jnp.max(scores(c), axis=0, keepdims=True))

                m = lax.fori_loop(0, NC, row_max, jnp.full((1, TQ), -jnp.inf, f32))

                def accumulate(c, state):
                    l, acc = state
                    p = jnp.exp2(scores(c) - m)
                    v = vt[pl.ds(pl.multiple_of(g * 64 + hh * 16, 16), 16),
                           pl.ds(pl.multiple_of(c * KC, KC), KC)]
                    o = jnp.dot(_unpack(v), p.astype(bf16), preferred_element_type=f32)
                    return l + jnp.sum(p, axis=0, keepdims=True), acc + o

                l, acc = lax.fori_loop(0, NC, accumulate,
                                       (jnp.zeros((1, TQ), f32), jnp.zeros((DH, TQ), f32)))
                ot[pl.ds(pl.multiple_of(hh * DH, DH), DH), :] = acc * (1.0 / l)
                return carry2
            lax.fori_loop(0, HPB, head, 0)
            ob[g, o_rows(q0), :] = _pack(ot[...].T.astype(bf16))
            return carry
        lax.fori_loop(0, NT, group, 0)
        pp[...] = jnp.zeros(pp.shape, u32)
        invs[...] = jnp.ones(invs.shape, f32)

    def q_body(qb, l):
        q0 = pl.multiple_of(qb * TQ, TQ)

        def attempt(state):
            a, _ = state

            @pl.when(a == 0)
            def _():
                lmx[...] = jnp.broadcast_to(attn_fast(q0), (8, TQ))

            @pl.when(a == 1)
            def _():
                attn_exact(q0)

            @pl.when(jnp.logical_or(l == 1, a == 1))
            def _():
                for j in range(TQ // OC):
                    out_copy(qb, j).wait()

            kd = (NT - 1) * 128
            o = jnp.concatenate([_unpack(ob[g, o_rows(q0), :]) for g in range(NT - 1)], axis=1)
            o_last = None
            for j in range(TQ // OC):
                y = lax.dot_general(o[j * OC:(j + 1) * OC], wob[0:kd, :], NN,
                                    preferred_element_type=f32)
                if j == 0:
                    o_last = finish_group(NT - 1)
                    y_first = y
                    continue
                if j == 2:
                    bad = _tree(jnp.maximum, [jnp.where(lmx[:, i * 128:(i + 1) * 128] <= L_MAX, 0.0, 1.0)
                                              for i in range(TQ // 128)])
                    v_ok = (vbig[...] & jnp.uint32(0x80008000)) == 0
                    unsafe = jnp.max(jnp.where(v_ok, bad, 1.0))
                for jj in ((0, 1) if j == 1 else (j,)):
                    yj = (y_first if jj == 0 else y) + lax.dot_general(
                        o_last[jj * OC:(jj + 1) * OC], wob[kd:D, :], NN, preferred_element_type=f32)
                    rows = pl.ds(q0 + jj * OC, OC)
                    x2 = xs[rows, :] + yj
                    xs2[rows, :] = x2
                    outb[rows, :] = x2.astype(bf16)
                    out_copy(qb, jj).start()
            return a + 1, unsafe

        lax.while_loop(lambda st: jnp.logical_or(st[0] == 0, jnp.logical_and(st[0] == 1, st[1] > 0.5)),
                       attempt, (jnp.int32(0), jnp.float32(0)))
        return l

    def layer_pair(l, carry):
        ka[:, 0:HALO, :] = jnp.zeros((NT, HALO, 128), f32)
        va[:, 0:HALO, :] = jnp.zeros((NT, HALO, 128), f32)
        vbig[...] = jnp.zeros(vbig.shape, u32)

        @pl.when(l == 1)
        def _():
            load_x(0, l, 16)

        lax.fori_loop(0, S // RB, row_body, l)

        @pl.when(l == 0)
        def _():
            wob_copy.wait()

        lax.fori_loop(0, S // TQ, q_body, l)
        return carry

    x_copy(0).wait()
    load_x(0, 0, 16)
    ot[...] = jnp.zeros(ot.shape, f32)
    pp[...] = jnp.zeros(pp.shape, u32)
    invs[...] = jnp.ones(invs.shape, f32)
    lax.fori_loop(0, 2, layer_pair, 0)
    for qb in range(S // TQ):
        for j in range(TQ // OC):
            out_copy(qb, j).wait()


@jax.jit
def pallas_interleave_layers__sliding_local_dilated__softmax_full_mha__prompt_kernel(
    A_x: jax.Array,
    A_wqkv: jax.Array,
    A_wo: jax.Array,
    B_x: jax.Array,
    B_wqkv: jax.Array,
    B_wo: jax.Array,
):
    del B_x
    x = A_x.reshape(S, D)
    hbm = pl.BlockSpec(memory_space=pl.ANY)
    out = pl.pallas_call(
        _kernel,
        out_shape=jax.ShapeDtypeStruct((S, D), bf16),
        in_specs=[hbm] * 5,
        out_specs=hbm,
        scratch_shapes=[
            pltpu.VMEM((S, D), bf16),
            pltpu.VMEM((D, 3 * D), bf16),
            pltpu.VMEM((D, D), bf16),
            pltpu.VMEM((D, 3 * D), bf16),
            pltpu.VMEM((D, D), bf16),
            pltpu.VMEM((S, D), bf16),
            pltpu.VMEM((NT, H * PITCH, 128), f32),
            pltpu.VMEM((D // 2, 3 * D), u32),
            pltpu.VMEM((D // 2, D), u32),
            pltpu.VMEM((D, D), u32),
            pltpu.VMEM((RB // 2, D), u32),
            pltpu.VMEM((S + RB, D), f32),
            pltpu.VMEM((S, D), f32),
            pltpu.VMEM((NT, RB, 128), f32),
            pltpu.VMEM((NT, HALO + RB, 128), f32),
            pltpu.VMEM((NT, HALO + RB, 128), f32),
            pltpu.VMEM((D // 2, S), u32),
            pltpu.VMEM((NT, S // 2, 128), u32),
            pltpu.VMEM((D // 2, S), u32),
            pltpu.VMEM((NT + 1, S // 2, 128), u32),
            pltpu.VMEM((128, TQ), f32),
            pltpu.VMEM((KC // 2, TQ), u32),
            pltpu.VMEM((8, TQ), f32),
            pltpu.VMEM((8, TQ), f32),
            pltpu.VMEM((8, 128), u32),
            pltpu.SemaphoreType.DMA((S // RB,)),
            pltpu.SemaphoreType.DMA((3 * D // WCH,)),
            pltpu.SemaphoreType.DMA((5,)),
            pltpu.SemaphoreType.DMA((S // OC,)),
        ],
        compiler_params=pltpu.CompilerParams(vmem_limit_bytes=110 * 1024 * 1024),
    )(x, A_wqkv, A_wo, B_wqkv, B_wo)
    return out.reshape(1, S, D)
```

```python
import functools
import math

import jax
import jax.numpy as jnp
from jax import lax
import jax.experimental.pallas as pl
import jax.experimental.pallas.tpu as pltpu

S = 2048
D = 1024
H = 32
DH = 32
WIN = 8
DIL = 2
EPS = 1e-5
NT = D // 128
HALO = 16
QSCALE = (DH ** -0.5) * math.log2(math.e)

SB = 128
NSUB = 2
RB = SB * NSUB
RC = 8
ROW_ORDER = [("a", 0), ("a", 1), ("o", 0), ("o", 1), ("w", 0), ("l", 1), ("b", 0), ("n", 0), ("b", 1)]
LC = 8
LN_LOOK = 2
LX_LOOK = 1
NDUP = 1
TILE_GATE = 1
PV_GATE = 1
T_OUTER = True
PV_TREE = False
LOOK = (2, 2)
DEP_END = (True, False)
GATE_COL = (2048, 2048)
TQ = 512
KC = 256
NC = S // KC
OC = 128
GPB = 2
HPB = 4
WCH = 512
WA_STARTS = (1, 1, 1, 2, 2, 2)
PITCH = 40
NFLIGHT = 3
L_MAX = 2.0 ** 64
V_EXP = 50

bf16 = jnp.bfloat16
f32 = jnp.float32
u32 = jnp.uint32

NN = (((1,), (0,)), ((), ()))
NTD = (((1,), (1,)), ((), ()))


def _pack(x):
    return pltpu.bitcast(x, u32)


def _unpack(x):
    return pltpu.bitcast(x, bf16)


def _after(value, dep):
    if dep is None:
        return value
    return jnp.maximum(value, jnp.minimum(dep, -3e38))


def _tree(op, xs):
    xs = list(xs)
    while len(xs) > 1:
        xs = [op(xs[i], xs[i + 1]) if i + 1 < len(xs) else xs[i] for i in range(0, len(xs), 2)]
    return xs[0]


def _recip(x):
    r = pl.reciprocal(x, approx=True)
    return r * (2.0 - x * r)


def _too_large(packed):
    bias = 0x8000 - ((127 + V_EXP) << 7)
    t = (packed & jnp.uint32(0x7F807F80)) + jnp.uint32(bias << 16 | bias)
    return _tree(jnp.bitwise_or, [t[i:i + 8] for i in range(0, t.shape[0], 8)])


def _layernorm(load, nrows, look, first_dep=None):
    outs = []
    deps = []
    for c in range(nrows // LC):
        dep = deps[c - look] if c >= look else first_dep
        x = load(c * LC, dep)
        mu = jnp.broadcast_to(jnp.sum(x, axis=-1, keepdims=True), (LC, 128)) * _after(1.0 / D, dep)
        xc = x - jnp.concatenate([mu] * NT, axis=1)
        var = jnp.sum(xc * xc, axis=-1, keepdims=True) * (1.0 / D)
        y = xc * lax.rsqrt(var + EPS)
        deps.append(y[:, D - 128:])
        outs.append(y)
    return jnp.concatenate(outs, axis=0).astype(bf16)


def _kernel(x_hbm, wa_hbm, woa_hbm, wb_hbm, wob_hbm, out_hbm,
            xin, wa_raw, woa_raw, wb_raw, wob, outb,
            stg, wan, woa, wqvt, xnb,
            xs, xs2, qa, ka, va, qt, kb, vt, ob, ot, pp, invs, lmx, vbig,
            sem_x, sem_wa, sem_w, sem_o):
    def x_copy(r):
        rows = pl.ds(pl.multiple_of(r * RB, RB), RB)
        return pltpu.make_async_copy(x_hbm.at[rows, :], xin.at[rows, :], sem_x.at[r])

    def wa_copy(i):
        cols = pl.ds(pl.multiple_of(i * WCH, WCH), WCH)
        return pltpu.make_async_copy(wa_hbm.at[:, cols], wa_raw.at[:, cols], sem_wa.at[i])

    def wb_copy(i):
        cols = pl.ds(pl.multiple_of(i * D, D), D)
        return pltpu.make_async_copy(wb_hbm.at[:, cols], wb_raw.at[:, cols], sem_w.at[i])

    woa_copy = pltpu.make_async_copy(woa_hbm, woa_raw, sem_w.at[3])
    wob_copy = pltpu.make_async_copy(wob_hbm, wob, sem_w.at[4])

    def out_copy(qb, j):
        rows = pl.ds(pl.multiple_of(qb * TQ + j * OC, OC), OC)
        return pltpu.make_async_copy(outb.at[rows, :], out_hbm.at[rows, :],
                                     sem_o.at[qb * (TQ // OC) + j])

    n_wa = 3 * D // WCH
    queue = ([wa_copy(i) for i in range(n_wa)]
             + [woa_copy, x_copy(0), x_copy(1), wb_copy(0), wb_copy(2), wb_copy(1)]
             + [x_copy(r) for r in range(2, S // RB)] + [wob_copy])
    for cp in queue[:NFLIGHT]:
        cp.start()
    queue = queue[NFLIGHT:]

    batches = [[queue.pop(0) for _ in range(n)] for n in WA_STARTS]

    def start_in_loop(i, my_batches):
        for k, batch in enumerate(my_batches):
            @pl.when(i == k)
            def _():
                for cp in batch:
                    cp.start()

    def transpose(w):
        ri = lax.broadcasted_iota(jnp.int32, (128, 128), 0)
        ci = lax.broadcasted_iota(jnp.int32, (128, 128), 1)
        eye = jnp.where(ri == ci, 1.0, 0.0).astype(bf16)
        return lax.dot_general(eye, w, NTD, preferred_element_type=f32)

    def stage(j, rows):
        for hh in range(HPB):
            r = pl.ds(pl.multiple_of((j * HPB + hh) * PITCH, 8), DH)
            for t in range(NT):
                stg[t, r, :] = rows[hh * DH:(hh + 1) * DH, t * 128:(t + 1) * 128]

    def gather(t):
        return jnp.concatenate([stg[t, pl.ds(d, H, stride=PITCH), :].astype(bf16)
                                for d in range(DH)], axis=0)

    def prep_wa(part, carry):
        for half in range(2):
            i = 2 * part + half
            wa_copy(i).wait()
            start_in_loop(part, batches[half::2])
            for j in range(half * NT // 2, (half + 1) * NT // 2):
                cols = pl.ds(pl.multiple_of(part * D + j * 128, 128), 128)
                stage(j, transpose(wa_raw[:, cols]))
        cols = pl.ds(pl.multiple_of(part * D, D), D)
        for t in range(NT):
            wan[t * 64:(t + 1) * 64, cols] = _pack(transpose(gather(t)).astype(bf16))
        return carry

    def prep_woa():
        def put(j, carry):
            stage(j, woa_raw[pl.ds(pl.multiple_of(j * 128, 128), 128), :].astype(f32))
            return carry

        def get(t, carry):
            woa[:, pl.ds(pl.multiple_of(t * 128, 128), 128)] = _pack(gather(t))
            return carry

        lax.fori_loop(0, NT, put, 0)
        lax.fori_loop(0, NT, get, 0)

    def prep_wb(part, carry):
        wb_copy(2 * part).wait()
        for j in range(NT):
            cols = pl.ds(pl.multiple_of(2 * part * D + j * 128, 128), 128)
            rows = pl.ds(pl.multiple_of(part * (D // 2) + j * 64, 64), 64)
            wqvt[rows, :] = _pack(transpose(wb_raw[:, cols]).astype(bf16))
        return carry

    lax.fori_loop(0, 3, prep_wa, 0)
    woa_copy.wait()
    prep_woa()

    def local_attn(r0, s, first_dep):
        outs = []
        deps = []
        for c in range(SB // RC):
            base = s * SB + c * RC
            scale = _after(QSCALE, deps[c - LOOK[s]] if c >= LOOK[s] else first_dep)
            logits = [None] * WIN
            dup = NT * (c % NDUP)
            if T_OUTER:
                for t in range(NT):
                    if TILE_GATE and t > 0 and t % TILE_GATE == 0:
                        scale = _after(QSCALE, logits[WIN - 1])
                    q = qa[t, base:base + RC, :] * scale
                    for w in range(WIN):
                        o0 = HALO + base - DIL * w
                        term = q * ka[t + dup, o0:o0 + RC, :]
                        logits[w] = term if t == 0 else logits[w] + term
            else:
                q = [qa[t, base:base + RC, :] * scale for t in range(NT)]
                for w in range(WIN):
                    o0 = HALO + base - DIL * w
                    terms = [q[t] * ka[t + dup, o0:o0 + RC, :] for t in range(NT)]
                    logits[w] = functools.reduce(jnp.add, terms)
            for w in range(WIN):
                acc = logits[w]
                acc = acc + pltpu.roll(acc, 64, 1)
                acc = acc + pltpu.roll(acc, 32, 1)
                if base < DIL * w:
                    row = r0 + base + lax.broadcasted_iota(jnp.int32, (RC, 128), 0)
                    acc = jnp.where(row >= DIL * w, acc, -1e9)
                logits[w] = acc
            m = _tree(jnp.maximum, logits)
            p = [jnp.exp2(lg - m) for lg in logits]
            inv = _recip(_tree(jnp.add, p))
            tiles = []
            done = []
            for t in range(NT):
                if PV_GATE and t >= PV_GATE:
                    p[0] = _after(p[0], done[t - PV_GATE])
                terms = [p[w] * va[t + dup, HALO + base - DIL * w:HALO + base - DIL * w + RC, :]
                         for w in range(WIN)]
                acc = (_tree(jnp.add, terms) if PV_TREE else functools.reduce(jnp.add, terms)) * inv
                tiles.append(acc.astype(bf16))
                done.append(acc)
            deps.append(acc if DEP_END[s] else m)
            outs.append(jnp.concatenate(tiles, axis=1))
        return jnp.concatenate(outs, axis=0)

    def load_x(r, l, look):
        r0 = pl.multiple_of(jnp.minimum(r, S // RB - 1) * RB, RB)
        w0 = pl.multiple_of(r * RB, RB)

        def load(start, dep):
            rows = pl.ds(r0 + start, LC)
            lvec = _after(jnp.full((LC, 128), l, f32), dep)
            first = jnp.concatenate([lvec == 0.0] * NT, axis=1)
            xi = xin[pl.ds(r0 + start // 16 * 16, 16), :].astype(f32)[start % 16:start % 16 + LC]
            x = jnp.where(first, xi, xs2[rows, :])
            xs[pl.ds(w0 + start, LC), :] = x
            return x

        xnb[...] = _pack(_layernorm(load, RB, look))

    def row_body(r, l):
        r0 = pl.multiple_of(r * RB, RB)
        rn = jnp.minimum(r + 1, S // RB - 1)

        @pl.when(jnp.logical_and(l == 0, r + 1 < S // RB))
        def _():
            x_copy(rn).wait()

        rows = [pl.ds(r0 + s * SB, SB) for s in range(NSUB)]
        gate = {}
        xn2 = {}

        def qkv_a(s):
            xn = _unpack(xnb[s * SB // 2:(s + 1) * SB // 2, :])
            y = lax.dot_general(xn, _unpack(wan[...]), NN, preferred_element_type=f32)
            for t in range(NT):
                qa[t, s * SB:(s + 1) * SB, :] = y[:, t * 128:(t + 1) * 128]
                for dup in range(0, NDUP * NT, NT):
                    new = slice(HALO + s * SB, HALO + (s + 1) * SB)
                    ka[t + dup, new, :] = y[:, D + t * 128:D + (t + 1) * 128]
                    va[t + dup, new, :] = y[:, 2 * D + t * 128:2 * D + (t + 1) * 128]
            gate[s] = y[SB - RC:SB, GATE_COL[s] - 128:GATE_COL[s]]

        def out_a(s):
            o = local_attn(r0, s, gate[s])
            x1 = xs[rows[s], :] + lax.dot_general(o, _unpack(woa[...]), NN,
                                                  preferred_element_type=f32)
            xs[rows[s], :] = x1
            if s < NSUB - 1:
                xn2[s] = _layernorm(lambda st, dep: x1[st:st + LC], SB, LN_LOOK)

        def norm_b(s):
            xn2[s] = _layernorm(lambda st, dep: xs[pl.ds(r0 + s * SB + st, LC), :], SB, LN_LOOK)

        def weights_b(_):
            @pl.when(jnp.logical_and(l == 0, r == 0))
            def _():
                lax.fori_loop(0, 2, prep_wb, 0)
                wb_copy(1).wait()
                for cp in queue:
                    cp.start()

        def qkv_b(s):
            cols = pl.ds(r0 + s * SB, SB)
            yq = lax.dot_general(_unpack(wqvt[0:D // 2, :]), xn2[s], NTD, preferred_element_type=f32)
            qt[:, cols] = _pack((yq * QSCALE).astype(bf16))
            yv = lax.dot_general(_unpack(wqvt[D // 2:D, :]), xn2[s], NTD, preferred_element_type=f32)
            v_t = _pack(yv.astype(bf16))
            vt[:, cols] = v_t
            vbig[...] = vbig[...] | _too_large(v_t)
            yk = lax.dot_general(xn2[s], wb_raw[:, D:2 * D], NN, preferred_element_type=f32).astype(bf16)
            krows = pl.ds(pl.multiple_of((r0 + s * SB) // 2, SB // 2), SB // 2)
            for g in range(NT):
                kb[g, krows, :] = _pack(yk[:, g * 128:(g + 1) * 128])

        steps = {"a": qkv_a, "o": out_a, "b": qkv_b, "w": weights_b, "l": norm_b}
        for name, s in ROW_ORDER:
            if name == "n":
                ka[:, 0:HALO, :] = ka[:, RB:RB + HALO, :]
                va[:, 0:HALO, :] = va[:, RB:RB + HALO, :]
                load_x(r + 1, l, LX_LOOK)
            else:
                steps[name](s)
        return l

    def head_weights(g, hh, q0):
        w = qt[pl.ds(pl.multiple_of(g * 64 + hh * 16, 16), 16), pl.ds(q0, TQ)]
        parts = []
        if hh > 0:
            parts.append(jnp.zeros((16 * hh, TQ), u32))
        parts.append(w)
        if hh < 3:
            parts.append(jnp.zeros((16 * (3 - hh), TQ), u32))
        return _unpack(jnp.concatenate(parts, axis=0))

    def v_rows(g, hh, c):
        rows = pl.ds(pl.multiple_of(g * 64 + hh * 16, 16), 16)
        return _unpack(vt[rows, c * KC:(c + 1) * KC])

    def finish_group(g):
        o = jnp.dot(v_rows(g, HPB - 1, NC - 1), _unpack(pp[...]), preferred_element_type=f32)
        last = (ot[3 * DH:4 * DH, :] + o) * invs[0:1, :]
        return jnp.concatenate([ot[0:3 * DH, :], last], axis=0).T.astype(bf16)

    def o_rows(q0):
        return pl.ds(pl.multiple_of(q0 // 2, TQ // 2), TQ // 2)

    def attn_fast(q0):
        def body(i, lmax):
            st = {}

            def qk(gg, hh, c):
                g = i * GPB + gg
                if c == 0:
                    st[gg, hh] = dict(w=head_weights(g, hh, q0))
                kc = _unpack(kb[g, c * KC // 2:(c + 1) * KC // 2, :])
                return jnp.dot(kc, st[gg, hh]["w"], preferred_element_type=f32)

            def pv(gg, hh, c, s):
                g = i * GPB + gg
                d = st[gg, hh]
                if c == 0:
                    d["m"] = jnp.broadcast_to(jnp.max(s[0:8], axis=0, keepdims=True), (8, TQ))
                p = jnp.exp2(s.reshape(KC // 8, 8, TQ) - d["m"][None])
                lc = jnp.sum(p, axis=0)
                d["l"] = lc if c == 0 else d["l"] + lc
                p = p.reshape(KC, TQ).astype(bf16)
                if c == NC - 1:
                    d["lsum"] = jnp.sum(d["l"], axis=0, keepdims=True)
                if gg == GPB - 1 and hh == HPB - 1 and c == NC - 1:
                    pp[...] = _pack(p)
                    ot[hh * DH:(hh + 1) * DH, :] = d["acc"]
                    invs[...] = jnp.broadcast_to(_recip(d["lsum"]), (8, TQ))
                    return
                o = jnp.dot(v_rows(g, hh, c), p, preferred_element_type=f32)
                d["acc"] = o if c == 0 else d["acc"] + o
                if c == NC - 1:
                    d["out"] = d["acc"] * _recip(d["lsum"])
                    if gg == GPB - 1:
                        ot[hh * DH:(hh + 1) * DH, :] = d["out"]
                    elif hh == HPB - 1:
                        o_t = jnp.concatenate([st[gg, k]["out"] for k in range(HPB)], axis=0)
                        ob[g, o_rows(q0), :] = _pack(o_t.T.astype(bf16))

            pend = None
            for gg in range(GPB):
                for hh in range(HPB):
                    for c in range(NC):
                        s = qk(gg, hh, c)
                        if pend is None:
                            ob[jnp.where(i == 0, NT, i * GPB - 1), o_rows(q0), :] = _pack(
                                finish_group(jnp.maximum(i * GPB - 1, 0)))
                        else:
                            pv(*pend)
                        pend = (gg, hh, c, s)
            pv(*pend)
            for d in st.values():
                lmax = jnp.maximum(lmax, d["lsum"])
            return lmax

        return lax.fori_loop(0, NT // GPB, body, jnp.zeros((1, TQ), f32))

    def attn_exact(q0):
        def group(g, carry):
            def head(hh, carry2):
                w = qt[pl.ds(pl.multiple_of(g * 64, 64), 64), pl.ds(q0, TQ)]
                row = lax.broadcasted_iota(jnp.int32, (64, TQ), 0) // 16
                w = _unpack(jnp.where(row == hh, w, jnp.zeros_like(w)))

                def scores(c):
                    kc = kb[g, pl.ds(pl.multiple_of(c * (KC // 2), KC // 2), KC // 2), :]
                    return jnp.dot(_unpack(kc), w, preferred_element_type=f32)

                def row_max(c, m):
                    return jnp.maximum(m, jnp.max(scores(c), axis=0, keepdims=True))

                m = lax.fori_loop(0, NC, row_max, jnp.full((1, TQ), -jnp.inf, f32))

                def accumulate(c, state):
                    l, acc = state
                    p = jnp.exp2(scores(c) - m)
                    v = vt[pl.ds(pl.multiple_of(g * 64 + hh * 16, 16), 16),
                           pl.ds(pl.multiple_of(c * KC, KC), KC)]
                    o = jnp.dot(_unpack(v), p.astype(bf16), preferred_element_type=f32)
                    return l + jnp.sum(p, axis=0, keepdims=True), acc + o

                l, acc = lax.fori_loop(0, NC, accumulate,
                                       (jnp.zeros((1, TQ), f32), jnp.zeros((DH, TQ), f32)))
                ot[pl.ds(pl.multiple_of(hh * DH, DH), DH), :] = acc * (1.0 / l)
                return carry2
            lax.fori_loop(0, HPB, head, 0)
            ob[g, o_rows(q0), :] = _pack(ot[...].T.astype(bf16))
            return carry
        lax.fori_loop(0, NT, group, 0)
        pp[...] = jnp.zeros(pp.shape, u32)
        invs[...] = jnp.ones(invs.shape, f32)

    def q_body(qb, l):
        q0 = pl.multiple_of(qb * TQ, TQ)

        def attempt(state):
            a, _ = state

            @pl.when(a == 0)
            def _():
                lmx[...] = jnp.broadcast_to(attn_fast(q0), (8, TQ))

            @pl.when(a == 1)
            def _():
                attn_exact(q0)

            @pl.when(jnp.logical_or(l == 1, a == 1))
            def _():
                for j in range(TQ // OC):
                    out_copy(qb, j).wait()

            kd = (NT - 1) * 128
            o = jnp.concatenate([_unpack(ob[g, o_rows(q0), :]) for g in range(NT - 1)], axis=1)
            o_last = None
            for j in range(TQ // OC):
                y = lax.dot_general(o[j * OC:(j + 1) * OC], wob[0:kd, :], NN,
                                    preferred_element_type=f32)
                if j == 0:
                    o_last = finish_group(NT - 1)
                    y_first = y
                    continue
                if j == 2:
                    bad = _tree(jnp.maximum, [jnp.where(lmx[:, i * 128:(i + 1) * 128] <= L_MAX, 0.0, 1.0)
                                              for i in range(TQ // 128)])
                    v_ok = (vbig[...] & jnp.uint32(0x80008000)) == 0
                    unsafe = jnp.max(jnp.where(v_ok, bad, 1.0))
                for jj in ((0, 1) if j == 1 else (j,)):
                    yj = (y_first if jj == 0 else y) + lax.dot_general(
                        o_last[jj * OC:(jj + 1) * OC], wob[kd:D, :], NN, preferred_element_type=f32)
                    rows = pl.ds(q0 + jj * OC, OC)
                    x2 = xs[rows, :] + yj
                    xs2[rows, :] = x2
                    outb[rows, :] = x2.astype(bf16)
                    out_copy(qb, jj).start()
            return a + 1, unsafe

        lax.while_loop(lambda st: jnp.logical_or(st[0] == 0, jnp.logical_and(st[0] == 1, st[1] > 0.5)),
                       attempt, (jnp.int32(0), jnp.float32(0)))
        return l

    def layer_pair(l, carry):
        ka[:, 0:HALO, :] = jnp.zeros((NDUP * NT, HALO, 128), f32)
        va[:, 0:HALO, :] = jnp.zeros((NDUP * NT, HALO, 128), f32)
        vbig[...] = jnp.zeros(vbig.shape, u32)

        @pl.when(l == 1)
        def _():
            load_x(0, l, 16)

        lax.fori_loop(0, S // RB, row_body, l)

        @pl.when(l == 0)
        def _():
            wob_copy.wait()

        lax.fori_loop(0, S // TQ, q_body, l)
        return carry

    x_copy(0).wait()
    load_x(0, 0, 16)
    ot[...] = jnp.zeros(ot.shape, f32)
    pp[...] = jnp.zeros(pp.shape, u32)
    invs[...] = jnp.ones(invs.shape, f32)
    lax.fori_loop(0, 2, layer_pair, 0)
    for qb in range(S // TQ):
        for j in range(TQ // OC):
            out_copy(qb, j).wait()


@jax.jit
def pallas_interleave_layers__sliding_local_dilated__softmax_full_mha__prompt_kernel(
    A_x: jax.Array,
    A_wqkv: jax.Array,
    A_wo: jax.Array,
    B_x: jax.Array,
    B_wqkv: jax.Array,
    B_wo: jax.Array,
):
    del B_x
    x = A_x.reshape(S, D)
    hbm = pl.BlockSpec(memory_space=pl.ANY)
    out = pl.pallas_call(
        _kernel,
        out_shape=jax.ShapeDtypeStruct((S, D), bf16),
        in_specs=[hbm] * 5,
        out_specs=hbm,
        scratch_shapes=[
            pltpu.VMEM((S, D), bf16),
            pltpu.VMEM((D, 3 * D), bf16),
            pltpu.VMEM((D, D), bf16),
            pltpu.VMEM((D, 3 * D), bf16),
            pltpu.VMEM((D, D), bf16),
            pltpu.VMEM((S, D), bf16),
            pltpu.VMEM((NT, H * PITCH, 128), f32),
            pltpu.VMEM((D // 2, 3 * D), u32),
            pltpu.VMEM((D // 2, D), u32),
            pltpu.VMEM((D, D), u32),
            pltpu.VMEM((RB // 2, D), u32),
            pltpu.VMEM((S + RB, D), f32),
            pltpu.VMEM((S, D), f32),
            pltpu.VMEM((NT, RB, 128), f32),
            pltpu.VMEM((NDUP * NT, HALO + RB, 128), f32),
            pltpu.VMEM((NDUP * NT, HALO + RB, 128), f32),
            pltpu.VMEM((D // 2, S), u32),
            pltpu.VMEM((NT, S // 2, 128), u32),
            pltpu.VMEM((D // 2, S), u32),
            pltpu.VMEM((NT + 1, S // 2, 128), u32),
            pltpu.VMEM((128, TQ), f32),
            pltpu.VMEM((KC // 2, TQ), u32),
            pltpu.VMEM((8, TQ), f32),
            pltpu.VMEM((8, TQ), f32),
            pltpu.VMEM((8, 128), u32),
            pltpu.SemaphoreType.DMA((S // RB,)),
            pltpu.SemaphoreType.DMA((3 * D // WCH,)),
            pltpu.SemaphoreType.DMA((5,)),
            pltpu.SemaphoreType.DMA((S // OC,)),
        ],
        compiler_params=pltpu.CompilerParams(vmem_limit_bytes=110 * 1024 * 1024),
    )(x, A_wqkv, A_wo, B_wqkv, B_wo)
    return out.reshape(1, S, D)
```

```python
import functools
import math

import jax
import jax.numpy as jnp
from jax import lax
import jax.experimental.pallas as pl
import jax.experimental.pallas.tpu as pltpu

S = 2048
D = 1024
H = 32
DH = 32
WIN = 8
DIL = 2
EPS = 1e-5
NT = D // 128
HALO = 16
QSCALE = (DH ** -0.5) * math.log2(math.e)

SB = 128
NSUB = 2
RB = SB * NSUB
RC = 8
ROW_ORDER = [("a", 0), ("a", 1), ("o", 0), ("o", 1), ("w", 0), ("l", 1), ("b", 0), ("n", 0), ("b", 1)]
LC = 8
LN_LOOK = 2
LX_LOOK = 1
NDUP = 1
TILE_GATE = 1
PV_GATE = 1
T_OUTER = True
PV_TREE = False
LOOK = (2, 2)
DEP_END = (True, False)
GATE_COL = (2048, 2048)
TQ = 512
KC = 256
NC = S // KC
OC = 128
GPB = 2
HPB = 4
WCH = 512
WA_STARTS = (1, 1, 1, 2, 2, 2)
PITCH = 40
NFLIGHT = 3
L_MAX = 2.0 ** 64
V_EXP = 50

bf16 = jnp.bfloat16
f32 = jnp.float32
u32 = jnp.uint32

NN = (((1,), (0,)), ((), ()))
NTD = (((1,), (1,)), ((), ()))


def _pack(x):
    return pltpu.bitcast(x, u32)


def _unpack(x):
    return pltpu.bitcast(x, bf16)


def _after(value, dep):
    if dep is None:
        return value
    return jnp.maximum(value, jnp.minimum(dep, -3e38))


def _tree(op, xs):
    xs = list(xs)
    while len(xs) > 1:
        xs = [op(xs[i], xs[i + 1]) if i + 1 < len(xs) else xs[i] for i in range(0, len(xs), 2)]
    return xs[0]


def _recip(x):
    r = pl.reciprocal(x, approx=True)
    return r * (2.0 - x * r)


def _too_large(packed):
    bias = 0x8000 - ((127 + V_EXP) << 7)
    t = (packed & jnp.uint32(0x7F807F80)) + jnp.uint32(bias << 16 | bias)
    return _tree(jnp.bitwise_or, [t[i:i + 8] for i in range(0, t.shape[0], 8)])


def _layernorm(load, nrows, look, first_dep=None):
    outs = []
    deps = []
    for c in range(nrows // LC):
        dep = deps[c - look] if c >= look else first_dep
        x = load(c * LC, dep)
        mu = jnp.broadcast_to(jnp.sum(x, axis=-1, keepdims=True), (LC, 128)) * _after(1.0 / D, dep)
        xc = x - jnp.concatenate([mu] * NT, axis=1)
        var = jnp.sum(xc * xc, axis=-1, keepdims=True) * (1.0 / D)
        y = xc * lax.rsqrt(var + EPS)
        deps.append(y[:, D - 128:])
        outs.append(y)
    return jnp.concatenate(outs, axis=0).astype(bf16)


def _kernel(x_hbm, wa_hbm, woa_hbm, wb_hbm, wob_hbm, out_hbm,
            xin, wa_raw, woa_raw, wb_raw, wob, outb,
            stg, wan, woa, xnb,
            xs, xs2, qa, ka, va, qt, kb, vt, ob, ot, pp, invs, lmx, vbig,
            sem_x, sem_wa, sem_w, sem_o):
    def x_copy(r):
        rows = pl.ds(pl.multiple_of(r * RB, RB), RB)
        return pltpu.make_async_copy(x_hbm.at[rows, :], xin.at[rows, :], sem_x.at[r])

    def wa_copy(i):
        cols = pl.ds(pl.multiple_of(i * WCH, WCH), WCH)
        return pltpu.make_async_copy(wa_hbm.at[:, cols], wa_raw.at[:, cols], sem_wa.at[i])

    def wb_copy(i):
        cols = pl.ds(pl.multiple_of(i * D, D), D)
        return pltpu.make_async_copy(wb_hbm.at[:, cols], wb_raw.at[:, cols], sem_w.at[i])

    woa_copy = pltpu.make_async_copy(woa_hbm, woa_raw, sem_w.at[3])
    wob_copy = pltpu.make_async_copy(wob_hbm, wob, sem_w.at[4])

    def out_copy(qb, j):
        rows = pl.ds(pl.multiple_of(qb * TQ + j * OC, OC), OC)
        return pltpu.make_async_copy(outb.at[rows, :], out_hbm.at[rows, :],
                                     sem_o.at[qb * (TQ // OC) + j])

    n_wa = 3 * D // WCH
    queue = ([wa_copy(i) for i in range(n_wa)]
             + [woa_copy, x_copy(0), x_copy(1), wb_copy(0), wb_copy(2), wb_copy(1)]
             + [x_copy(r) for r in range(2, S // RB)] + [wob_copy])
    for cp in queue[:NFLIGHT]:
        cp.start()
    queue = queue[NFLIGHT:]

    batches = [[queue.pop(0) for _ in range(n)] for n in WA_STARTS]

    def start_in_loop(i, my_batches):
        for k, batch in enumerate(my_batches):
            @pl.when(i == k)
            def _():
                for cp in batch:
                    cp.start()

    def transpose(w):
        ri = lax.broadcasted_iota(jnp.int32, (128, 128), 0)
        ci = lax.broadcasted_iota(jnp.int32, (128, 128), 1)
        eye = jnp.where(ri == ci, 1.0, 0.0).astype(bf16)
        return lax.dot_general(eye, w, NTD, preferred_element_type=f32)

    def stage(j, rows):
        for hh in range(HPB):
            r = pl.ds(pl.multiple_of((j * HPB + hh) * PITCH, 8), DH)
            for t in range(NT):
                stg[t, r, :] = rows[hh * DH:(hh + 1) * DH, t * 128:(t + 1) * 128]

    def gather(t):
        return jnp.concatenate([stg[t, pl.ds(d, H, stride=PITCH), :].astype(bf16)
                                for d in range(DH)], axis=0)

    def prep_wa(part, carry):
        for half in range(2):
            i = 2 * part + half
            wa_copy(i).wait()
            start_in_loop(part, batches[half::2])
            for j in range(half * NT // 2, (half + 1) * NT // 2):
                cols = pl.ds(pl.multiple_of(part * D + j * 128, 128), 128)
                stage(j, transpose(wa_raw[:, cols]))
        cols = pl.ds(pl.multiple_of(part * D, D), D)
        for t in range(NT):
            wan[t * 64:(t + 1) * 64, cols] = _pack(transpose(gather(t)).astype(bf16))
        return carry

    def prep_woa():
        def put(j, carry):
            stage(j, woa_raw[pl.ds(pl.multiple_of(j * 128, 128), 128), :].astype(f32))
            return carry

        def get(t, carry):
            woa[:, pl.ds(pl.multiple_of(t * 128, 128), 128)] = _pack(gather(t))
            return carry

        lax.fori_loop(0, NT, put, 0)
        lax.fori_loop(0, NT, get, 0)

    lax.fori_loop(0, 3, prep_wa, 0)
    woa_copy.wait()
    prep_woa()

    def local_attn(r0, s, first_dep):
        outs = []
        deps = []
        for c in range(SB // RC):
            base = s * SB + c * RC
            scale = _after(QSCALE, deps[c - LOOK[s]] if c >= LOOK[s] else first_dep)
            logits = [None] * WIN
            dup = NT * (c % NDUP)
            if T_OUTER:
                for t in range(NT):
                    if TILE_GATE and t > 0 and t % TILE_GATE == 0:
                        scale = _after(QSCALE, logits[WIN - 1])
                    q = qa[t, base:base + RC, :] * scale
                    for w in range(WIN):
                        o0 = HALO + base - DIL * w
                        term = q * ka[t + dup, o0:o0 + RC, :]
                        logits[w] = term if t == 0 else logits[w] + term
            else:
                q = [qa[t, base:base + RC, :] * scale for t in range(NT)]
                for w in range(WIN):
                    o0 = HALO + base - DIL * w
                    terms = [q[t] * ka[t + dup, o0:o0 + RC, :] for t in range(NT)]
                    logits[w] = functools.reduce(jnp.add, terms)
            for w in range(WIN):
                acc = logits[w]
                acc = acc + pltpu.roll(acc, 64, 1)
                acc = acc + pltpu.roll(acc, 32, 1)
                if base < DIL * w:
                    row = r0 + base + lax.broadcasted_iota(jnp.int32, (RC, 128), 0)
                    acc = jnp.where(row >= DIL * w, acc, -1e9)
                logits[w] = acc
            m = _tree(jnp.maximum, logits)
            p = [jnp.exp2(lg - m) for lg in logits]
            inv = _recip(_tree(jnp.add, p))
            tiles = []
            done = []
            for t in range(NT):
                if PV_GATE and t >= PV_GATE:
                    p[0] = _after(p[0], done[t - PV_GATE])
                terms = [p[w] * va[t + dup, HALO + base - DIL * w:HALO + base - DIL * w + RC, :]
                         for w in range(WIN)]
                acc = (_tree(jnp.add, terms) if PV_TREE else functools.reduce(jnp.add, terms)) * inv
                tiles.append(acc.astype(bf16))
                done.append(acc)
            deps.append(acc if DEP_END[s] else m)
            outs.append(jnp.concatenate(tiles, axis=1))
        return jnp.concatenate(outs, axis=0)

    def load_x(r, l, look):
        r0 = pl.multiple_of(jnp.minimum(r, S // RB - 1) * RB, RB)
        w0 = pl.multiple_of(r * RB, RB)

        def load(start, dep):
            rows = pl.ds(r0 + start, LC)
            lvec = _after(jnp.full((LC, 128), l, f32), dep)
            first = jnp.concatenate([lvec == 0.0] * NT, axis=1)
            xi = xin[pl.ds(r0 + start // 16 * 16, 16), :].astype(f32)[start % 16:start % 16 + LC]
            x = jnp.where(first, xi, xs2[rows, :])
            xs[pl.ds(w0 + start, LC), :] = x
            return x

        xnb[...] = _pack(_layernorm(load, RB, look))

    def row_body(r, l):
        r0 = pl.multiple_of(r * RB, RB)
        rn = jnp.minimum(r + 1, S // RB - 1)

        @pl.when(jnp.logical_and(l == 0, r + 1 < S // RB))
        def _():
            x_copy(rn).wait()

        rows = [pl.ds(r0 + s * SB, SB) for s in range(NSUB)]
        gate = {}
        xn2 = {}

        def qkv_a(s):
            xn = _unpack(xnb[s * SB // 2:(s + 1) * SB // 2, :])
            y = lax.dot_general(xn, _unpack(wan[...]), NN, preferred_element_type=f32)
            for t in range(NT):
                qa[t, s * SB:(s + 1) * SB, :] = y[:, t * 128:(t + 1) * 128]
                for dup in range(0, NDUP * NT, NT):
                    new = slice(HALO + s * SB, HALO + (s + 1) * SB)
                    ka[t + dup, new, :] = y[:, D + t * 128:D + (t + 1) * 128]
                    va[t + dup, new, :] = y[:, 2 * D + t * 128:2 * D + (t + 1) * 128]
            gate[s] = y[SB - RC:SB, GATE_COL[s] - 128:GATE_COL[s]]

        def out_a(s):
            o = local_attn(r0, s, gate[s])
            x1 = xs[rows[s], :] + lax.dot_general(o, _unpack(woa[...]), NN,
                                                  preferred_element_type=f32)
            xs[rows[s], :] = x1
            if s < NSUB - 1:
                xn2[s] = _layernorm(lambda st, dep: x1[st:st + LC], SB, LN_LOOK)

        def norm_b(s):
            xn2[s] = _layernorm(lambda st, dep: xs[pl.ds(r0 + s * SB + st, LC), :], SB, LN_LOOK)

        def weights_b(_):
            @pl.when(jnp.logical_and(l == 0, r == 0))
            def _():
                for i in range(3):
                    wb_copy(i).wait()
                for cp in queue:
                    cp.start()

        def qkv_b(s):
            cols = pl.ds(r0 + s * SB, SB)
            yq = lax.dot_general(xn2[s], wb_raw[:, 0:D], NN, preferred_element_type=f32)
            qt[:, cols] = _pack((yq * QSCALE).T.astype(bf16))
            yv = lax.dot_general(xn2[s], wb_raw[:, 2 * D:3 * D], NN, preferred_element_type=f32).T
            v_t = _pack(yv.astype(bf16))
            vt[:, cols] = v_t
            vbig[...] = vbig[...] | _too_large(v_t)
            yk = lax.dot_general(xn2[s], wb_raw[:, D:2 * D], NN, preferred_element_type=f32).astype(bf16)
            krows = pl.ds(pl.multiple_of((r0 + s * SB) // 2, SB // 2), SB // 2)
            for g in range(NT):
                kb[g, krows, :] = _pack(yk[:, g * 128:(g + 1) * 128])

        steps = {"a": qkv_a, "o": out_a, "b": qkv_b, "w": weights_b, "l": norm_b}
        for name, s in ROW_ORDER:
            if name == "n":
                ka[:, 0:HALO, :] = ka[:, RB:RB + HALO, :]
                va[:, 0:HALO, :] = va[:, RB:RB + HALO, :]
                load_x(r + 1, l, LX_LOOK)
            else:
                steps[name](s)
        return l

    def head_weights(g, hh, q0):
        w = qt[pl.ds(pl.multiple_of(g * 64 + hh * 16, 16), 16), pl.ds(q0, TQ)]
        parts = []
        if hh > 0:
            parts.append(jnp.zeros((16 * hh, TQ), u32))
        parts.append(w)
        if hh < 3:
            parts.append(jnp.zeros((16 * (3 - hh), TQ), u32))
        return _unpack(jnp.concatenate(parts, axis=0))

    def v_rows(g, hh, c):
        rows = pl.ds(pl.multiple_of(g * 64 + hh * 16, 16), 16)
        return _unpack(vt[rows, c * KC:(c + 1) * KC])

    def finish_group(g):
        o = jnp.dot(v_rows(g, HPB - 1, NC - 1), _unpack(pp[...]), preferred_element_type=f32)
        last = (ot[3 * DH:4 * DH, :] + o) * invs[0:1, :]
        return jnp.concatenate([ot[0:3 * DH, :], last], axis=0).T.astype(bf16)

    def o_rows(q0):
        return pl.ds(pl.multiple_of(q0 // 2, TQ // 2), TQ // 2)

    def attn_fast(q0):
        def body(i, lmax):
            st = {}

            def qk(gg, hh, c):
                g = i * GPB + gg
                if c == 0:
                    st[gg, hh] = dict(w=head_weights(g, hh, q0))
                kc = _unpack(kb[g, c * KC // 2:(c + 1) * KC // 2, :])
                return jnp.dot(kc, st[gg, hh]["w"], preferred_element_type=f32)

            def pv(gg, hh, c, s):
                g = i * GPB + gg
                d = st[gg, hh]
                if c == 0:
                    d["m"] = jnp.broadcast_to(jnp.max(s[0:8], axis=0, keepdims=True), (8, TQ))
                p = jnp.exp2(s.reshape(KC // 8, 8, TQ) - d["m"][None])
                lc = jnp.sum(p, axis=0)
                d["l"] = lc if c == 0 else d["l"] + lc
                p = p.reshape(KC, TQ).astype(bf16)
                if c == NC - 1:
                    d["lsum"] = jnp.sum(d["l"], axis=0, keepdims=True)
                if gg == GPB - 1 and hh == HPB - 1 and c == NC - 1:
                    pp[...] = _pack(p)
                    ot[hh * DH:(hh + 1) * DH, :] = d["acc"]
                    invs[...] = jnp.broadcast_to(_recip(d["lsum"]), (8, TQ))
                    return
                o = jnp.dot(v_rows(g, hh, c), p, preferred_element_type=f32)
                d["acc"] = o if c == 0 else d["acc"] + o
                if c == NC - 1:
                    d["out"] = d["acc"] * _recip(d["lsum"])
                    if gg == GPB - 1:
                        ot[hh * DH:(hh + 1) * DH, :] = d["out"]
                    elif hh == HPB - 1:
                        o_t = jnp.concatenate([st[gg, k]["out"] for k in range(HPB)], axis=0)
                        ob[g, o_rows(q0), :] = _pack(o_t.T.astype(bf16))

            pend = None
            for gg in range(GPB):
                for hh in range(HPB):
                    for c in range(NC):
                        s = qk(gg, hh, c)
                        if pend is None:
                            ob[jnp.where(i == 0, NT, i * GPB - 1), o_rows(q0), :] = _pack(
                                finish_group(jnp.maximum(i * GPB - 1, 0)))
                        else:
                            pv(*pend)
                        pend = (gg, hh, c, s)
            pv(*pend)
            for d in st.values():
                lmax = jnp.maximum(lmax, d["lsum"])
            return lmax

        return lax.fori_loop(0, NT // GPB, body, jnp.zeros((1, TQ), f32))

    def attn_exact(q0):
        def group(g, carry):
            def head(hh, carry2):
                w = qt[pl.ds(pl.multiple_of(g * 64, 64), 64), pl.ds(q0, TQ)]
                row = lax.broadcasted_iota(jnp.int32, (64, TQ), 0) // 16
                w = _unpack(jnp.where(row == hh, w, jnp.zeros_like(w)))

                def scores(c):
                    kc = kb[g, pl.ds(pl.multiple_of(c * (KC // 2), KC // 2), KC // 2), :]
                    return jnp.dot(_unpack(kc), w, preferred_element_type=f32)

                def row_max(c, m):
                    return jnp.maximum(m, jnp.max(scores(c), axis=0, keepdims=True))

                m = lax.fori_loop(0, NC, row_max, jnp.full((1, TQ), -jnp.inf, f32))

                def accumulate(c, state):
                    l, acc = state
                    p = jnp.exp2(scores(c) - m)
                    v = vt[pl.ds(pl.multiple_of(g * 64 + hh * 16, 16), 16),
                           pl.ds(pl.multiple_of(c * KC, KC), KC)]
                    o = jnp.dot(_unpack(v), p.astype(bf16), preferred_element_type=f32)
                    return l + jnp.sum(p, axis=0, keepdims=True), acc + o

                l, acc = lax.fori_loop(0, NC, accumulate,
                                       (jnp.zeros((1, TQ), f32), jnp.zeros((DH, TQ), f32)))
                ot[pl.ds(pl.multiple_of(hh * DH, DH), DH), :] = acc * (1.0 / l)
                return carry2
            lax.fori_loop(0, HPB, head, 0)
            ob[g, o_rows(q0), :] = _pack(ot[...].T.astype(bf16))
            return carry
        lax.fori_loop(0, NT, group, 0)
        pp[...] = jnp.zeros(pp.shape, u32)
        invs[...] = jnp.ones(invs.shape, f32)

    def q_body(qb, l):
        q0 = pl.multiple_of(qb * TQ, TQ)

        def attempt(state):
            a, _ = state

            @pl.when(a == 0)
            def _():
                lmx[...] = jnp.broadcast_to(attn_fast(q0), (8, TQ))

            @pl.when(a == 1)
            def _():
                attn_exact(q0)

            @pl.when(jnp.logical_or(l == 1, a == 1))
            def _():
                for j in range(TQ // OC):
                    out_copy(qb, j).wait()

            kd = (NT - 1) * 128
            o = jnp.concatenate([_unpack(ob[g, o_rows(q0), :]) for g in range(NT - 1)], axis=1)
            o_last = None
            for j in range(TQ // OC):
                y = lax.dot_general(o[j * OC:(j + 1) * OC], wob[0:kd, :], NN,
                                    preferred_element_type=f32)
                if j == 0:
                    o_last = finish_group(NT - 1)
                    y_first = y
                    continue
                if j == 2:
                    bad = _tree(jnp.maximum, [jnp.where(lmx[:, i * 128:(i + 1) * 128] <= L_MAX, 0.0, 1.0)
                                              for i in range(TQ // 128)])
                    v_ok = (vbig[...] & jnp.uint32(0x80008000)) == 0
                    unsafe = jnp.max(jnp.where(v_ok, bad, 1.0))
                for jj in ((0, 1) if j == 1 else (j,)):
                    yj = (y_first if jj == 0 else y) + lax.dot_general(
                        o_last[jj * OC:(jj + 1) * OC], wob[kd:D, :], NN, preferred_element_type=f32)
                    rows = pl.ds(q0 + jj * OC, OC)
                    x2 = xs[rows, :] + yj
                    xs2[rows, :] = x2
                    outb[rows, :] = x2.astype(bf16)
                    out_copy(qb, jj).start()
            return a + 1, unsafe

        lax.while_loop(lambda st: jnp.logical_or(st[0] == 0, jnp.logical_and(st[0] == 1, st[1] > 0.5)),
                       attempt, (jnp.int32(0), jnp.float32(0)))
        return l

    def layer_pair(l, carry):
        ka[:, 0:HALO, :] = jnp.zeros((NDUP * NT, HALO, 128), f32)
        va[:, 0:HALO, :] = jnp.zeros((NDUP * NT, HALO, 128), f32)
        vbig[...] = jnp.zeros(vbig.shape, u32)

        @pl.when(l == 1)
        def _():
            load_x(0, l, 16)

        lax.fori_loop(0, S // RB, row_body, l)

        @pl.when(l == 0)
        def _():
            wob_copy.wait()

        lax.fori_loop(0, S // TQ, q_body, l)
        return carry

    x_copy(0).wait()
    load_x(0, 0, 16)
    ot[...] = jnp.zeros(ot.shape, f32)
    pp[...] = jnp.zeros(pp.shape, u32)
    invs[...] = jnp.ones(invs.shape, f32)
    lax.fori_loop(0, 2, layer_pair, 0)
    for qb in range(S // TQ):
        for j in range(TQ // OC):
            out_copy(qb, j).wait()


@jax.jit
def pallas_interleave_layers__sliding_local_dilated__softmax_full_mha__prompt_kernel(
    A_x: jax.Array,
    A_wqkv: jax.Array,
    A_wo: jax.Array,
    B_x: jax.Array,
    B_wqkv: jax.Array,
    B_wo: jax.Array,
):
    del B_x
    x = A_x.reshape(S, D)
    hbm = pl.BlockSpec(memory_space=pl.ANY)
    out = pl.pallas_call(
        _kernel,
        out_shape=jax.ShapeDtypeStruct((S, D), bf16),
        in_specs=[hbm] * 5,
        out_specs=hbm,
        scratch_shapes=[
            pltpu.VMEM((S, D), bf16),
            pltpu.VMEM((D, 3 * D), bf16),
            pltpu.VMEM((D, D), bf16),
            pltpu.VMEM((D, 3 * D), bf16),
            pltpu.VMEM((D, D), bf16),
            pltpu.VMEM((S, D), bf16),
            pltpu.VMEM((NT, H * PITCH, 128), f32),
            pltpu.VMEM((D // 2, 3 * D), u32),
            pltpu.VMEM((D // 2, D), u32),
            pltpu.VMEM((RB // 2, D), u32),
            pltpu.VMEM((S + RB, D), f32),
            pltpu.VMEM((S, D), f32),
            pltpu.VMEM((NT, RB, 128), f32),
            pltpu.VMEM((NDUP * NT, HALO + RB, 128), f32),
            pltpu.VMEM((NDUP * NT, HALO + RB, 128), f32),
            pltpu.VMEM((D // 2, S), u32),
            pltpu.VMEM((NT, S // 2, 128), u32),
            pltpu.VMEM((D // 2, S), u32),
            pltpu.VMEM((NT + 1, S // 2, 128), u32),
            pltpu.VMEM((128, TQ), f32),
            pltpu.VMEM((KC // 2, TQ), u32),
            pltpu.VMEM((8, TQ), f32),
            pltpu.VMEM((8, TQ), f32),
            pltpu.VMEM((8, 128), u32),
            pltpu.SemaphoreType.DMA((S // RB,)),
            pltpu.SemaphoreType.DMA((3 * D // WCH,)),
            pltpu.SemaphoreType.DMA((5,)),
            pltpu.SemaphoreType.DMA((S // OC,)),
        ],
        compiler_params=pltpu.CompilerParams(vmem_limit_bytes=110 * 1024 * 1024),
    )(x, A_wqkv, A_wo, B_wqkv, B_wo)
    return out.reshape(1, S, D)
```

```python
import functools
import math

import jax
import jax.numpy as jnp
from jax import lax
import jax.experimental.pallas as pl
import jax.experimental.pallas.tpu as pltpu

S = 2048
D = 1024
H = 32
DH = 32
WIN = 8
DIL = 2
EPS = 1e-5
NT = D // 128
HALO = 16
QSCALE = (DH ** -0.5) * math.log2(math.e)

SB = 128
NSUB = 2
RB = SB * NSUB
RC = 8
ROW_ORDER = [("a", 0), ("a", 1), ("o", 0), ("o", 1), ("w", 0), ("l", 1), ("b", 0), ("n", 0), ("b", 1)]
LC = 8
LN_LOOK = 2
LX_LOOK = 1
NDUP = 1
TILE_GATE = 1
PV_GATE = 1
T_OUTER = True
PV_TREE = False
LOOK = (2, 2)
DEP_END = (True, False)
GATE_COL = (2048, 2048)
TQ = 512
KC = 256
NC = S // KC
OC = 128
GPB = 2
HPB = 4
WA_STARTS = (1, 1, 1, 1, 1, 2, 2, 3)
WPITCH = 20
PITCH = 40
NFLIGHT = 3
L_MAX = 2.0 ** 64
V_EXP = 50

bf16 = jnp.bfloat16
f32 = jnp.float32
u32 = jnp.uint32

NN = (((1,), (0,)), ((), ()))
NTD = (((1,), (1,)), ((), ()))


def _pack(x):
    return pltpu.bitcast(x, u32)


def _unpack(x):
    return pltpu.bitcast(x, bf16)


def _after(value, dep):
    if dep is None:
        return value
    return jnp.maximum(value, jnp.minimum(dep, -3e38))


def _tree(op, xs):
    xs = list(xs)
    while len(xs) > 1:
        xs = [op(xs[i], xs[i + 1]) if i + 1 < len(xs) else xs[i] for i in range(0, len(xs), 2)]
    return xs[0]


def _recip(x):
    r = pl.reciprocal(x, approx=True)
    return r * (2.0 - x * r)


def _too_large(packed):
    bias = 0x8000 - ((127 + V_EXP) << 7)
    t = (packed & jnp.uint32(0x7F807F80)) + jnp.uint32(bias << 16 | bias)
    return _tree(jnp.bitwise_or, [t[i:i + 8] for i in range(0, t.shape[0], 8)])


def _layernorm(load, nrows, look, first_dep=None):
    outs = []
    deps = []
    for c in range(nrows // LC):
        dep = deps[c - look] if c >= look else first_dep
        x = load(c * LC, dep)
        mu = jnp.broadcast_to(jnp.sum(x, axis=-1, keepdims=True), (LC, 128)) * _after(1.0 / D, dep)
        xc = x - jnp.concatenate([mu] * NT, axis=1)
        var = jnp.sum(xc * xc, axis=-1, keepdims=True) * (1.0 / D)
        y = xc * lax.rsqrt(var + EPS)
        deps.append(y[:, D - 128:])
        outs.append(y)
    return jnp.concatenate(outs, axis=0).astype(bf16)


def _kernel(x_hbm, wa_hbm, woa_hbm, wb_hbm, wob_hbm, out_hbm,
            xin, wa_raw, woa_raw, wb_raw, wob, outb,
            stg, stw, wan, woa, xnb,
            xs, xs2, qa, ka, va, qt, kb, vt, ob, ot, pp, invs, lmx, vbig,
            sem_x, sem_wa, sem_w, sem_o):
    def x_copy(r):
        rows = pl.ds(pl.multiple_of(r * RB, RB), RB)
        return pltpu.make_async_copy(x_hbm.at[rows, :], xin.at[rows, :], sem_x.at[r])

    def wa_copy(i):
        rows = pl.ds(pl.multiple_of(i * 128, 128), 128)
        return pltpu.make_async_copy(wa_hbm.at[rows, :], wa_raw.at[rows, :], sem_wa.at[i])

    def wb_copy(i):
        cols = pl.ds(pl.multiple_of(i * D, D), D)
        return pltpu.make_async_copy(wb_hbm.at[:, cols], wb_raw.at[:, cols], sem_w.at[i])

    def woa_copy(i):
        cols = pl.ds(pl.multiple_of(i * (D // 2), D // 2), D // 2)
        return pltpu.make_async_copy(woa_hbm.at[:, cols], woa_raw.at[:, cols], sem_w.at[3 + i])

    wob_copy = pltpu.make_async_copy(wob_hbm, wob, sem_w.at[5])

    def out_copy(qb, j):
        rows = pl.ds(pl.multiple_of(qb * TQ + j * OC, OC), OC)
        return pltpu.make_async_copy(outb.at[rows, :], out_hbm.at[rows, :],
                                     sem_o.at[qb * (TQ // OC) + j])

    queue = ([wa_copy(i) for i in range(NT)]
             + [x_copy(0), woa_copy(0), woa_copy(1), x_copy(1), wb_copy(0), wb_copy(2), wb_copy(1)]
             + [x_copy(r) for r in range(2, S // RB)] + [wob_copy])
    for cp in queue[:NFLIGHT]:
        cp.start()
    queue = queue[NFLIGHT:]

    batches = [[queue.pop(0) for _ in range(n)] for n in WA_STARTS]

    def start_in_loop(i, my_batches):
        for k, batch in enumerate(my_batches):
            @pl.when(i == k)
            def _():
                for cp in batch:
                    cp.start()

    def transpose(w):
        ri = lax.broadcasted_iota(jnp.int32, (128, 128), 0)
        ci = lax.broadcasted_iota(jnp.int32, (128, 128), 1)
        eye = jnp.where(ri == ci, 1.0, 0.0).astype(bf16)
        return lax.dot_general(eye, w, NTD, preferred_element_type=f32)

    def prep_wa(t, carry):
        wa_copy(t).wait()
        start_in_loop(t, batches)
        rows = pl.ds(pl.multiple_of(t * 128, 128), 128)

        def forward(part):
            for j in range(NT):
                wt = transpose(wa_raw[rows, part * D + j * 128:part * D + (j + 1) * 128])
                for hh in range(HPB):
                    r = (j * HPB + hh) * PITCH
                    stg[part, r:r + DH, :] = wt[hh * DH:(hh + 1) * DH]

        def back(part):
            regrouped = jnp.concatenate([stg[part, pl.ds(d, H, stride=PITCH), :].astype(bf16)
                                         for d in range(DH)], axis=0)
            wan[pl.ds(pl.multiple_of(t * 64, 64), 64), part * D:(part + 1) * D] = _pack(
                transpose(regrouped).astype(bf16))

        forward(0)
        forward(1)
        back(0)
        forward(2)
        back(1)
        back(2)
        return carry

    def prep_woa(t, carry):
        cols = pl.ds(pl.multiple_of(t * 128, 128), 128)
        w = _pack(woa_raw[:, cols])
        for h in range(H):
            stw[h * WPITCH:h * WPITCH + DH // 2, :] = w[h * (DH // 2):(h + 1) * (DH // 2)]
        lo = jnp.uint32(0xFFFF)
        for j in range(DH // 2):
            even = stw[pl.ds(j, H // 2, stride=2 * WPITCH), :]
            odd = stw[pl.ds(WPITCH + j, H // 2, stride=2 * WPITCH), :]
            woa[2 * j * 16:(2 * j + 1) * 16, cols] = (even & lo) | (odd << 16)
            woa[(2 * j + 1) * 16:(2 * j + 2) * 16, cols] = (even >> 16) | (odd & ~lo)
        return carry

    lax.fori_loop(0, NT, prep_wa, 0)

    def local_attn(r0, s, first_dep):
        outs = []
        deps = []
        for c in range(SB // RC):
            base = s * SB + c * RC
            scale = _after(QSCALE, deps[c - LOOK[s]] if c >= LOOK[s] else first_dep)
            logits = [None] * WIN
            dup = NT * (c % NDUP)
            if T_OUTER:
                for t in range(NT):
                    if TILE_GATE and t > 0 and t % TILE_GATE == 0:
                        scale = _after(QSCALE, logits[WIN - 1])
                    q = qa[t, base:base + RC, :] * scale
                    for w in range(WIN):
                        o0 = HALO + base - DIL * w
                        term = q * ka[t + dup, o0:o0 + RC, :]
                        logits[w] = term if t == 0 else logits[w] + term
            else:
                q = [qa[t, base:base + RC, :] * scale for t in range(NT)]
                for w in range(WIN):
                    o0 = HALO + base - DIL * w
                    terms = [q[t] * ka[t + dup, o0:o0 + RC, :] for t in range(NT)]
                    logits[w] = functools.reduce(jnp.add, terms)
            for w in range(WIN):
                acc = logits[w]
                acc = acc + pltpu.roll(acc, 64, 1)
                acc = acc + pltpu.roll(acc, 32, 1)
                if base < DIL * w:
                    row = r0 + base + lax.broadcasted_iota(jnp.int32, (RC, 128), 0)
                    acc = jnp.where(row >= DIL * w, acc, -1e9)
                logits[w] = acc
            m = _tree(jnp.maximum, logits)
            p = [jnp.exp2(lg - m) for lg in logits]
            inv = _recip(_tree(jnp.add, p))
            tiles = []
            done = []
            for t in range(NT):
                if PV_GATE and t >= PV_GATE:
                    p[0] = _after(p[0], done[t - PV_GATE])
                terms = [p[w] * va[t + dup, HALO + base - DIL * w:HALO + base - DIL * w + RC, :]
                         for w in range(WIN)]
                acc = (_tree(jnp.add, terms) if PV_TREE else functools.reduce(jnp.add, terms)) * inv
                tiles.append(acc.astype(bf16))
                done.append(acc)
            deps.append(acc if DEP_END[s] else m)
            outs.append(jnp.concatenate(tiles, axis=1))
        return jnp.concatenate(outs, axis=0)

    def load_x(r, l, look):
        r0 = pl.multiple_of(jnp.minimum(r, S // RB - 1) * RB, RB)
        w0 = pl.multiple_of(r * RB, RB)

        def load(start, dep):
            rows = pl.ds(r0 + start, LC)
            lvec = _after(jnp.full((LC, 128), l, f32), dep)
            first = jnp.concatenate([lvec == 0.0] * NT, axis=1)
            xi = xin[pl.ds(r0 + start // 16 * 16, 16), :].astype(f32)[start % 16:start % 16 + LC]
            x = jnp.where(first, xi, xs2[rows, :])
            xs[pl.ds(w0 + start, LC), :] = x
            return x

        xnb[...] = _pack(_layernorm(load, RB, look))

    def row_body(r, l):
        r0 = pl.multiple_of(r * RB, RB)
        rn = jnp.minimum(r + 1, S // RB - 1)

        @pl.when(jnp.logical_and(l == 0, r + 1 < S // RB))
        def _():
            x_copy(rn).wait()

        rows = [pl.ds(r0 + s * SB, SB) for s in range(NSUB)]
        gate = {}
        xn2 = {}

        def qkv_a(s):
            xn = _unpack(xnb[s * SB // 2:(s + 1) * SB // 2, :])
            y = lax.dot_general(xn, _unpack(wan[...]), NN, preferred_element_type=f32)
            for t in range(NT):
                qa[t, s * SB:(s + 1) * SB, :] = y[:, t * 128:(t + 1) * 128]
                for dup in range(0, NDUP * NT, NT):
                    new = slice(HALO + s * SB, HALO + (s + 1) * SB)
                    ka[t + dup, new, :] = y[:, D + t * 128:D + (t + 1) * 128]
                    va[t + dup, new, :] = y[:, 2 * D + t * 128:2 * D + (t + 1) * 128]
            gate[s] = y[SB - RC:SB, GATE_COL[s] - 128:GATE_COL[s]]

        def out_a(s):
            o = local_attn(r0, s, gate[s])
            x1 = xs[rows[s], :] + lax.dot_general(o, _unpack(woa[...]), NN,
                                                  preferred_element_type=f32)
            xs[rows[s], :] = x1
            if s < NSUB - 1:
                xn2[s] = _layernorm(lambda st, dep: x1[st:st + LC], SB, LN_LOOK)

        def norm_b(s):
            xn2[s] = _layernorm(lambda st, dep: xs[pl.ds(r0 + s * SB + st, LC), :], SB, LN_LOOK)

        def weights_b(_):
            @pl.when(jnp.logical_and(l == 0, r == 0))
            def _():
                for i in range(3):
                    wb_copy(i).wait()
                for cp in queue:
                    cp.start()

        def qkv_b(s):
            cols = pl.ds(r0 + s * SB, SB)
            yq = lax.dot_general(xn2[s], wb_raw[:, 0:D], NN, preferred_element_type=f32)
            qt[:, cols] = _pack((yq * QSCALE).T.astype(bf16))
            yv = lax.dot_general(xn2[s], wb_raw[:, 2 * D:3 * D], NN, preferred_element_type=f32).T
            v_t = _pack(yv.astype(bf16))
            vt[:, cols] = v_t
            vbig[...] = vbig[...] | _too_large(v_t)
            yk = lax.dot_general(xn2[s], wb_raw[:, D:2 * D], NN, preferred_element_type=f32).astype(bf16)
            krows = pl.ds(pl.multiple_of((r0 + s * SB) // 2, SB // 2), SB // 2)
            for g in range(NT):
                kb[g, krows, :] = _pack(yk[:, g * 128:(g + 1) * 128])

        steps = {"a": qkv_a, "o": out_a, "b": qkv_b, "w": weights_b, "l": norm_b}
        for name, s in ROW_ORDER:
            if name == "n":
                ka[:, 0:HALO, :] = ka[:, RB:RB + HALO, :]
                va[:, 0:HALO, :] = va[:, RB:RB + HALO, :]
                load_x(r + 1, l, LX_LOOK)
            else:
                steps[name](s)
        return l

    def head_weights(g, hh, q0):
        w = qt[pl.ds(pl.multiple_of(g * 64 + hh * 16, 16), 16), pl.ds(q0, TQ)]
        parts = []
        if hh > 0:
            parts.append(jnp.zeros((16 * hh, TQ), u32))
        parts.append(w)
        if hh < 3:
            parts.append(jnp.zeros((16 * (3 - hh), TQ), u32))
        return _unpack(jnp.concatenate(parts, axis=0))

    def v_rows(g, hh, c):
        rows = pl.ds(pl.multiple_of(g * 64 + hh * 16, 16), 16)
        return _unpack(vt[rows, c * KC:(c + 1) * KC])

    def finish_group(g):
        o = jnp.dot(v_rows(g, HPB - 1, NC - 1), _unpack(pp[...]), preferred_element_type=f32)
        last = (ot[3 * DH:4 * DH, :] + o) * invs[0:1, :]
        return jnp.concatenate([ot[0:3 * DH, :], last], axis=0).T.astype(bf16)

    def o_rows(q0):
        return pl.ds(pl.multiple_of(q0 // 2, TQ // 2), TQ // 2)

    def attn_fast(q0):
        def body(i, lmax):
            st = {}

            def qk(gg, hh, c):
                g = i * GPB + gg
                if c == 0:
                    st[gg, hh] = dict(w=head_weights(g, hh, q0))
                kc = _unpack(kb[g, c * KC // 2:(c + 1) * KC // 2, :])
                return jnp.dot(kc, st[gg, hh]["w"], preferred_element_type=f32)

            def pv(gg, hh, c, s):
                g = i * GPB + gg
                d = st[gg, hh]
                if c == 0:
                    d["m"] = jnp.broadcast_to(jnp.max(s[0:8], axis=0, keepdims=True), (8, TQ))
                p = jnp.exp2(s.reshape(KC // 8, 8, TQ) - d["m"][None])
                lc = jnp.sum(p, axis=0)
                d["l"] = lc if c == 0 else d["l"] + lc
                p = p.reshape(KC, TQ).astype(bf16)
                if c == NC - 1:
                    d["lsum"] = jnp.sum(d["l"], axis=0, keepdims=True)
                if gg == GPB - 1 and hh == HPB - 1 and c == NC - 1:
                    pp[...] = _pack(p)
                    ot[hh * DH:(hh + 1) * DH, :] = d["acc"]
                    invs[...] = jnp.broadcast_to(_recip(d["lsum"]), (8, TQ))
                    return
                o = jnp.dot(v_rows(g, hh, c), p, preferred_element_type=f32)
                d["acc"] = o if c == 0 else d["acc"] + o
                if c == NC - 1:
                    d["out"] = d["acc"] * _recip(d["lsum"])
                    if gg == GPB - 1:
                        ot[hh * DH:(hh + 1) * DH, :] = d["out"]
                    elif hh == HPB - 1:
                        o_t = jnp.concatenate([st[gg, k]["out"] for k in range(HPB)], axis=0)
                        ob[g, o_rows(q0), :] = _pack(o_t.T.astype(bf16))

            pend = None
            for gg in range(GPB):
                for hh in range(HPB):
                    for c in range(NC):
                        s = qk(gg, hh, c)
                        if pend is None:
                            ob[jnp.where(i == 0, NT, i * GPB - 1), o_rows(q0), :] = _pack(
                                finish_group(jnp.maximum(i * GPB - 1, 0)))
                        else:
                            pv(*pend)
                        pend = (gg, hh, c, s)
            pv(*pend)
            for d in st.values():
                lmax = jnp.maximum(lmax, d["lsum"])
            return lmax

        return lax.fori_loop(0, NT // GPB, body, jnp.zeros((1, TQ), f32))

    def attn_exact(q0):
        def group(g, carry):
            def head(hh, carry2):
                w = qt[pl.ds(pl.multiple_of(g * 64, 64), 64), pl.ds(q0, TQ)]
                row = lax.broadcasted_iota(jnp.int32, (64, TQ), 0) // 16
                w = _unpack(jnp.where(row == hh, w, jnp.zeros_like(w)))

                def scores(c):
                    kc = kb[g, pl.ds(pl.multiple_of(c * (KC // 2), KC // 2), KC // 2), :]
                    return jnp.dot(_unpack(kc), w, preferred_element_type=f32)

                def row_max(c, m):
                    return jnp.maximum(m, jnp.max(scores(c), axis=0, keepdims=True))

                m = lax.fori_loop(0, NC, row_max, jnp.full((1, TQ), -jnp.inf, f32))

                def accumulate(c, state):
                    l, acc = state
                    p = jnp.exp2(scores(c) - m)
                    v = vt[pl.ds(pl.multiple_of(g * 64 + hh * 16, 16), 16),
                           pl.ds(pl.multiple_of(c * KC, KC), KC)]
                    o = jnp.dot(_unpack(v), p.astype(bf16), preferred_element_type=f32)
                    return l + jnp.sum(p, axis=0, keepdims=True), acc + o

                l, acc = lax.fori_loop(0, NC, accumulate,
                                       (jnp.zeros((1, TQ), f32), jnp.zeros((DH, TQ), f32)))
                ot[pl.ds(pl.multiple_of(hh * DH, DH), DH), :] = acc * (1.0 / l)
                return carry2
            lax.fori_loop(0, HPB, head, 0)
            ob[g, o_rows(q0), :] = _pack(ot[...].T.astype(bf16))
            return carry
        lax.fori_loop(0, NT, group, 0)
        pp[...] = jnp.zeros(pp.shape, u32)
        invs[...] = jnp.ones(invs.shape, f32)

    def q_body(qb, l):
        q0 = pl.multiple_of(qb * TQ, TQ)

        def attempt(state):
            a, _ = state

            @pl.when(a == 0)
            def _():
                lmx[...] = jnp.broadcast_to(attn_fast(q0), (8, TQ))

            @pl.when(a == 1)
            def _():
                attn_exact(q0)

            @pl.when(jnp.logical_or(l == 1, a == 1))
            def _():
                for j in range(TQ // OC):
                    out_copy(qb, j).wait()

            kd = (NT - 1) * 128
            o = jnp.concatenate([_unpack(ob[g, o_rows(q0), :]) for g in range(NT - 1)], axis=1)
            o_last = None
            for j in range(TQ // OC):
                y = lax.dot_general(o[j * OC:(j + 1) * OC], wob[0:kd, :], NN,
                                    preferred_element_type=f32)
                if j == 0:
                    o_last = finish_group(NT - 1)
                    y_first = y
                    continue
                if j == 2:
                    bad = _tree(jnp.maximum, [jnp.where(lmx[:, i * 128:(i + 1) * 128] <= L_MAX, 0.0, 1.0)
                                              for i in range(TQ // 128)])
                    v_ok = (vbig[...] & jnp.uint32(0x80008000)) == 0
                    unsafe = jnp.max(jnp.where(v_ok, bad, 1.0))
                for jj in ((0, 1) if j == 1 else (j,)):
                    yj = (y_first if jj == 0 else y) + lax.dot_general(
                        o_last[jj * OC:(jj + 1) * OC], wob[kd:D, :], NN, preferred_element_type=f32)
                    rows = pl.ds(q0 + jj * OC, OC)
                    x2 = xs[rows, :] + yj
                    xs2[rows, :] = x2
                    outb[rows, :] = x2.astype(bf16)
                    out_copy(qb, jj).start()
            return a + 1, unsafe

        lax.while_loop(lambda st: jnp.logical_or(st[0] == 0, jnp.logical_and(st[0] == 1, st[1] > 0.5)),
                       attempt, (jnp.int32(0), jnp.float32(0)))
        return l

    def layer_pair(l, carry):
        ka[:, 0:HALO, :] = jnp.zeros((NDUP * NT, HALO, 128), f32)
        va[:, 0:HALO, :] = jnp.zeros((NDUP * NT, HALO, 128), f32)
        vbig[...] = jnp.zeros(vbig.shape, u32)

        @pl.when(l == 1)
        def _():
            load_x(0, l, 32)

        lax.fori_loop(0, S // RB, row_body, l)

        @pl.when(l == 0)
        def _():
            wob_copy.wait()

        lax.fori_loop(0, S // TQ, q_body, l)
        return carry

    x_copy(0).wait()
    load_x(0, 0, 32)
    for i in range(2):
        woa_copy(i).wait()
        lax.fori_loop(i * NT // 2, (i + 1) * NT // 2, prep_woa, 0)
    ot[...] = jnp.zeros(ot.shape, f32)
    pp[...] = jnp.zeros(pp.shape, u32)
    invs[...] = jnp.ones(invs.shape, f32)
    lax.fori_loop(0, 2, layer_pair, 0)
    for qb in range(S // TQ):
        for j in range(TQ // OC):
            out_copy(qb, j).wait()


@jax.jit
def pallas_interleave_layers__sliding_local_dilated__softmax_full_mha__prompt_kernel(
    A_x: jax.Array,
    A_wqkv: jax.Array,
    A_wo: jax.Array,
    B_x: jax.Array,
    B_wqkv: jax.Array,
    B_wo: jax.Array,
):
    del B_x
    x = A_x.reshape(S, D)
    hbm = pl.BlockSpec(memory_space=pl.ANY)
    out = pl.pallas_call(
        _kernel,
        out_shape=jax.ShapeDtypeStruct((S, D), bf16),
        in_specs=[hbm] * 5,
        out_specs=hbm,
        scratch_shapes=[
            pltpu.VMEM((S, D), bf16),
            pltpu.VMEM((D, 3 * D), bf16),
            pltpu.VMEM((D, D), bf16),
            pltpu.VMEM((D, 3 * D), bf16),
            pltpu.VMEM((D, D), bf16),
            pltpu.VMEM((S, D), bf16),
            pltpu.VMEM((3, H * PITCH, 128), f32),
            pltpu.VMEM((H * WPITCH, 128), u32),
            pltpu.VMEM((D // 2, 3 * D), u32),
            pltpu.VMEM((D // 2, D), u32),
            pltpu.VMEM((RB // 2, D), u32),
            pltpu.VMEM((S + RB, D), f32),
            pltpu.VMEM((S, D), f32),
            pltpu.VMEM((NT, RB, 128), f32),
            pltpu.VMEM((NDUP * NT, HALO + RB, 128), f32),
            pltpu.VMEM((NDUP * NT, HALO + RB, 128), f32),
            pltpu.VMEM((D // 2, S), u32),
            pltpu.VMEM((NT, S // 2, 128), u32),
            pltpu.VMEM((D // 2, S), u32),
            pltpu.VMEM((NT + 1, S // 2, 128), u32),
            pltpu.VMEM((128, TQ), f32),
            pltpu.VMEM((KC // 2, TQ), u32),
            pltpu.VMEM((8, TQ), f32),
            pltpu.VMEM((8, TQ), f32),
            pltpu.VMEM((8, 128), u32),
            pltpu.SemaphoreType.DMA((S // RB,)),
            pltpu.SemaphoreType.DMA((NT,)),
            pltpu.SemaphoreType.DMA((6,)),
            pltpu.SemaphoreType.DMA((S // OC,)),
        ],
        compiler_params=pltpu.CompilerParams(vmem_limit_bytes=110 * 1024 * 1024),
    )(x, A_wqkv, A_wo, B_wqkv, B_wo)
    return out.reshape(1, S, D)
```

```python
import functools
import math

import jax
import jax.numpy as jnp
from jax import lax
import jax.experimental.pallas as pl
import jax.experimental.pallas.tpu as pltpu

S = 2048
D = 1024
H = 32
DH = 32
WIN = 8
DIL = 2
EPS = 1e-5
NT = D // 128
HALO = 16
QSCALE = (DH ** -0.5) * math.log2(math.e)

SB = 128
NSUB = 2
RB = SB * NSUB
RC = 8
ROW_ORDER = [("a", 0), ("a", 1), ("o", 0), ("o", 1), ("w", 0), ("l", 1), ("b", 0), ("n", 0), ("b", 1)]
LC = 8
LN_LOOK = 2
LX_LOOK = 1
NDUP = 1
TILE_GATE = 1
PV_GATE = 1
T_OUTER = True
PV_TREE = False
LOOK = (2, 2)
DEP_END = (True, False)
GATE_COL = (2048, 2048)
TQ = 512
KC = 256
NC = S // KC
OC = 128
GPB = 2
HPB = 4
NWO = 4
WA_STARTS = (2, 1, 2, 1, 2, 1, 1, 0)
LATE_AT = 3
XLU_TILES = (8, 8, 0)
WPITCH = 20
PITCH = 40
NFLIGHT = 3
L_MAX = 2.0 ** 64
V_EXP = 50

bf16 = jnp.bfloat16
f32 = jnp.float32
u32 = jnp.uint32

NN = (((1,), (0,)), ((), ()))
NTD = (((1,), (1,)), ((), ()))


def _pack(x):
    return pltpu.bitcast(x, u32)


def _unpack(x):
    return pltpu.bitcast(x, bf16)


def _after(value, dep):
    if dep is None:
        return value
    return jnp.maximum(value, jnp.minimum(dep, -3e38))


def _tree(op, xs):
    xs = list(xs)
    while len(xs) > 1:
        xs = [op(xs[i], xs[i + 1]) if i + 1 < len(xs) else xs[i] for i in range(0, len(xs), 2)]
    return xs[0]


def _recip(x):
    r = pl.reciprocal(x, approx=True)
    return r * (2.0 - x * r)


def _too_large(packed):
    bias = 0x8000 - ((127 + V_EXP) << 7)
    t = (packed & jnp.uint32(0x7F807F80)) + jnp.uint32(bias << 16 | bias)
    return _tree(jnp.bitwise_or, [t[i:i + 8] for i in range(0, t.shape[0], 8)])


def _layernorm(load, nrows, look, first_dep=None):
    outs = []
    deps = []
    for c in range(nrows // LC):
        dep = deps[c - look] if c >= look else first_dep
        x = load(c * LC, dep)
        mu = jnp.broadcast_to(jnp.sum(x, axis=-1, keepdims=True), (LC, 128)) * _after(1.0 / D, dep)
        xc = x - jnp.concatenate([mu] * NT, axis=1)
        var = jnp.sum(xc * xc, axis=-1, keepdims=True) * (1.0 / D)
        y = xc * lax.rsqrt(var + EPS)
        deps.append(y[:, D - 128:])
        outs.append(y)
    return jnp.concatenate(outs, axis=0).astype(bf16)


def _kernel(x_hbm, wa_hbm, woa_hbm, wb_hbm, wob_hbm, out_hbm,
            xin, wa_raw, woa_raw, wb_raw, wob, outb,
            stg, stw, wan, woa, xnb,
            xs, xs2, qa, ka, va, qt, kb, vt, ob, ot, pp, invs, lmx, vbig,
            sem_x, sem_wa, sem_w, sem_o):
    def x_copy(r):
        rows = pl.ds(pl.multiple_of(r * RB, RB), RB)
        return pltpu.make_async_copy(x_hbm.at[rows, :], xin.at[rows, :], sem_x.at[r])

    def wa_copy(i):
        rows = pl.ds(pl.multiple_of(i * 128, 128), 128)
        return pltpu.make_async_copy(wa_hbm.at[rows, :], wa_raw.at[rows, :], sem_wa.at[i])

    def wb_copy(i):
        cols = pl.ds(pl.multiple_of(i * D, D), D)
        return pltpu.make_async_copy(wb_hbm.at[:, cols], wb_raw.at[:, cols], sem_w.at[i])

    def woa_copy(i):
        cols = pl.ds(pl.multiple_of(i * (D // NWO), D // NWO), D // NWO)
        return pltpu.make_async_copy(woa_hbm.at[:, cols], woa_raw.at[:, cols], sem_w.at[4 + i])

    wob_copy = pltpu.make_async_copy(wob_hbm, wob, sem_w.at[3])

    def out_copy(qb, j):
        rows = pl.ds(pl.multiple_of(qb * TQ + j * OC, OC), OC)
        return pltpu.make_async_copy(outb.at[rows, :], out_hbm.at[rows, :],
                                     sem_o.at[qb * (TQ // OC) + j])

    queue = ([wa_copy(i) for i in range(NT)]
             + [x_copy(0)] + [woa_copy(i) for i in range(NWO)]
             + [x_copy(1), wb_copy(0), wb_copy(2), wb_copy(1)]
             + [x_copy(r) for r in range(2, S // RB)] + [wob_copy])
    for cp in queue[:NFLIGHT]:
        cp.start()
    queue = queue[NFLIGHT:]

    batches = [[queue.pop(0) for _ in range(n)] for n in WA_STARTS]
    late = [queue.pop(0) for _ in range(NT + 5 + NWO - NFLIGHT - sum(WA_STARTS))]

    def start_in_loop(i, my_batches):
        for k, batch in enumerate(my_batches):
            @pl.when(i == k)
            def _():
                for cp in batch:
                    cp.start()

    def transpose(w):
        ri = lax.broadcasted_iota(jnp.int32, (128, 128), 0)
        ci = lax.broadcasted_iota(jnp.int32, (128, 128), 1)
        eye = jnp.where(ri == ci, 1.0, 0.0).astype(bf16)
        return lax.dot_general(eye, w, NTD, preferred_element_type=f32)

    def prep_wa(t, carry):
        wa_copy(t).wait()
        start_in_loop(t, batches)
        rows = pl.ds(pl.multiple_of(t * 128, 128), 128)

        def forward(part):
            for j in range(NT):
                wt = transpose(wa_raw[rows, part * D + j * 128:part * D + (j + 1) * 128])
                for hh in range(HPB):
                    r = (j * HPB + hh) * PITCH
                    stg[part, r:r + DH, :] = wt[hh * DH:(hh + 1) * DH]

        def back(part):
            regrouped = jnp.concatenate([stg[part, pl.ds(d, H, stride=PITCH), :]
                                         for d in range(DH)], axis=0)
            n = XLU_TILES[part] * 128
            pieces = []
            if n > 0:
                pieces.append(regrouped[:n].T)
            if n < D:
                pieces.append(transpose(regrouped[n:].astype(bf16)))
            wan[pl.ds(pl.multiple_of(t * 64, 64), 64), part * D:(part + 1) * D] = _pack(
                jnp.concatenate(pieces, axis=1).astype(bf16))

        forward(0)
        forward(1)
        back(0)
        forward(2)
        back(1)
        back(2)
        return carry

    def prep_woa(t, carry):
        cols = pl.ds(pl.multiple_of(t * 128, 128), 128)
        w = _pack(woa_raw[:, cols])
        for h in range(H):
            stw[h * WPITCH:h * WPITCH + DH // 2, :] = w[h * (DH // 2):(h + 1) * (DH // 2)]
        lo = jnp.uint32(0xFFFF)
        for j in range(DH // 2):
            even = stw[pl.ds(j, H // 2, stride=2 * WPITCH), :]
            odd = stw[pl.ds(WPITCH + j, H // 2, stride=2 * WPITCH), :]
            woa[2 * j * 16:(2 * j + 1) * 16, cols] = (even & lo) | (odd << 16)
            woa[(2 * j + 1) * 16:(2 * j + 2) * 16, cols] = (even >> 16) | (odd & ~lo)
        return carry

    ot[...] = jnp.zeros(ot.shape, f32)
    pp[...] = jnp.zeros(pp.shape, u32)
    invs[...] = jnp.ones(invs.shape, f32)
    lax.fori_loop(0, NT, prep_wa, 0)

    def local_attn(r0, s, first_dep):
        outs = []
        deps = []
        for c in range(SB // RC):
            base = s * SB + c * RC
            scale = _after(QSCALE, deps[c - LOOK[s]] if c >= LOOK[s] else first_dep)
            logits = [None] * WIN
            dup = NT * (c % NDUP)
            if T_OUTER:
                for t in range(NT):
                    if TILE_GATE and t > 0 and t % TILE_GATE == 0:
                        scale = _after(QSCALE, logits[WIN - 1])
                    q = qa[t, base:base + RC, :] * scale
                    for w in range(WIN):
                        o0 = HALO + base - DIL * w
                        term = q * ka[t + dup, o0:o0 + RC, :]
                        logits[w] = term if t == 0 else logits[w] + term
            else:
                q = [qa[t, base:base + RC, :] * scale for t in range(NT)]
                for w in range(WIN):
                    o0 = HALO + base - DIL * w
                    terms = [q[t] * ka[t + dup, o0:o0 + RC, :] for t in range(NT)]
                    logits[w] = functools.reduce(jnp.add, terms)
            for w in range(WIN):
                acc = logits[w]
                acc = acc + pltpu.roll(acc, 64, 1)
                acc = acc + pltpu.roll(acc, 32, 1)
                if base < DIL * w:
                    row = r0 + base + lax.broadcasted_iota(jnp.int32, (RC, 128), 0)
                    acc = jnp.where(row >= DIL * w, acc, -1e9)
                logits[w] = acc
            m = _tree(jnp.maximum, logits)
            p = [jnp.exp2(lg - m) for lg in logits]
            inv = _recip(_tree(jnp.add, p))
            tiles = []
            done = []
            for t in range(NT):
                if PV_GATE and t >= PV_GATE:
                    p[0] = _after(p[0], done[t - PV_GATE])
                terms = [p[w] * va[t + dup, HALO + base - DIL * w:HALO + base - DIL * w + RC, :]
                         for w in range(WIN)]
                acc = (_tree(jnp.add, terms) if PV_TREE else functools.reduce(jnp.add, terms)) * inv
                tiles.append(acc.astype(bf16))
                done.append(acc)
            deps.append(acc if DEP_END[s] else m)
            outs.append(jnp.concatenate(tiles, axis=1))
        return jnp.concatenate(outs, axis=0)

    def load_x(r, l, look):
        r0 = pl.multiple_of(jnp.minimum(r, S // RB - 1) * RB, RB)
        w0 = pl.multiple_of(r * RB, RB)

        def load(start, dep):
            rows = pl.ds(r0 + start, LC)
            lvec = _after(jnp.full((LC, 128), l, f32), dep)
            first = jnp.concatenate([lvec == 0.0] * NT, axis=1)
            xi = xin[pl.ds(r0 + start // 16 * 16, 16), :].astype(f32)[start % 16:start % 16 + LC]
            x = jnp.where(first, xi, xs2[rows, :])
            xs[pl.ds(w0 + start, LC), :] = x
            return x

        xnb[...] = _pack(_layernorm(load, RB, look))

    def row_body(r, l):
        r0 = pl.multiple_of(r * RB, RB)
        rn = jnp.minimum(r + 1, S // RB - 1)

        rows = [pl.ds(r0 + s * SB, SB) for s in range(NSUB)]
        gate = {}
        xn2 = {}

        def qkv_a(s):
            xn = _unpack(xnb[s * SB // 2:(s + 1) * SB // 2, :])
            y = lax.dot_general(xn, _unpack(wan[...]), NN, preferred_element_type=f32)
            for t in range(NT):
                qa[t, s * SB:(s + 1) * SB, :] = y[:, t * 128:(t + 1) * 128]
                for dup in range(0, NDUP * NT, NT):
                    new = slice(HALO + s * SB, HALO + (s + 1) * SB)
                    ka[t + dup, new, :] = y[:, D + t * 128:D + (t + 1) * 128]
                    va[t + dup, new, :] = y[:, 2 * D + t * 128:2 * D + (t + 1) * 128]
            gate[s] = y[SB - RC:SB, GATE_COL[s] - 128:GATE_COL[s]]

        def out_a(s):
            o = local_attn(r0, s, gate[s])
            x1 = xs[rows[s], :] + lax.dot_general(o, _unpack(woa[...]), NN,
                                                  preferred_element_type=f32)
            xs[rows[s], :] = x1
            if s < NSUB - 1:
                xn2[s] = _layernorm(lambda st, dep: x1[st:st + LC], SB, LN_LOOK)

        def norm_b(s):
            xn2[s] = _layernorm(lambda st, dep: xs[pl.ds(r0 + s * SB + st, LC), :], SB, LN_LOOK)

        def weights_b(_):
            @pl.when(jnp.logical_and(l == 0, r == 0))
            def _():
                for i in range(3):
                    wb_copy(i).wait()
                for cp in queue:
                    cp.start()

            @pl.when(jnp.logical_and(l == 0, r + 1 < S // RB))
            def _():
                x_copy(rn).wait()

        def qkv_b(s):
            cols = pl.ds(r0 + s * SB, SB)
            yq = lax.dot_general(xn2[s], wb_raw[:, 0:D], NN, preferred_element_type=f32)
            qt[:, cols] = _pack((yq * QSCALE).T.astype(bf16))
            yv = lax.dot_general(xn2[s], wb_raw[:, 2 * D:3 * D], NN, preferred_element_type=f32).T
            v_t = _pack(yv.astype(bf16))
            vt[:, cols] = v_t
            vbig[...] = vbig[...] | _too_large(v_t)
            yk = lax.dot_general(xn2[s], wb_raw[:, D:2 * D], NN, preferred_element_type=f32).astype(bf16)
            krows = pl.ds(pl.multiple_of((r0 + s * SB) // 2, SB // 2), SB // 2)
            for g in range(NT):
                kb[g, krows, :] = _pack(yk[:, g * 128:(g + 1) * 128])

        steps = {"a": qkv_a, "o": out_a, "b": qkv_b, "w": weights_b, "l": norm_b}
        for name, s in ROW_ORDER:
            if name == "n":
                ka[:, 0:HALO, :] = ka[:, RB:RB + HALO, :]
                va[:, 0:HALO, :] = va[:, RB:RB + HALO, :]
                load_x(r + 1, l, LX_LOOK)
            else:
                steps[name](s)
        return l

    def head_weights(g, hh, q0):
        w = qt[pl.ds(pl.multiple_of(g * 64 + hh * 16, 16), 16), pl.ds(q0, TQ)]
        parts = []
        if hh > 0:
            parts.append(jnp.zeros((16 * hh, TQ), u32))
        parts.append(w)
        if hh < 3:
            parts.append(jnp.zeros((16 * (3 - hh), TQ), u32))
        return _unpack(jnp.concatenate(parts, axis=0))

    def v_rows(g, hh, c):
        rows = pl.ds(pl.multiple_of(g * 64 + hh * 16, 16), 16)
        return _unpack(vt[rows, c * KC:(c + 1) * KC])

    def finish_group(g):
        o = jnp.dot(v_rows(g, HPB - 1, NC - 1), _unpack(pp[...]), preferred_element_type=f32)
        last = (ot[3 * DH:4 * DH, :] + o) * invs[0:1, :]
        return jnp.concatenate([ot[0:3 * DH, :], last], axis=0).T.astype(bf16)

    def o_rows(q0):
        return pl.ds(pl.multiple_of(q0 // 2, TQ // 2), TQ // 2)

    def attn_fast(q0):
        def body(i, lmax):
            st = {}

            def qk(gg, hh, c):
                g = i * GPB + gg
                if c == 0:
                    st[gg, hh] = dict(w=head_weights(g, hh, q0))
                kc = _unpack(kb[g, c * KC // 2:(c + 1) * KC // 2, :])
                return jnp.dot(kc, st[gg, hh]["w"], preferred_element_type=f32)

            def pv(gg, hh, c, s):
                g = i * GPB + gg
                d = st[gg, hh]
                if c == 0:
                    d["m"] = jnp.broadcast_to(jnp.max(s[0:8], axis=0, keepdims=True), (8, TQ))
                p = jnp.exp2(s.reshape(KC // 8, 8, TQ) - d["m"][None])
                lc = jnp.sum(p, axis=0)
                d["l"] = lc if c == 0 else d["l"] + lc
                p = p.reshape(KC, TQ).astype(bf16)
                if c == NC - 1:
                    d["lsum"] = jnp.sum(d["l"], axis=0, keepdims=True)
                if gg == GPB - 1 and hh == HPB - 1 and c == NC - 1:
                    pp[...] = _pack(p)
                    ot[hh * DH:(hh + 1) * DH, :] = d["acc"]
                    invs[...] = jnp.broadcast_to(_recip(d["lsum"]), (8, TQ))
                    return
                o = jnp.dot(v_rows(g, hh, c), p, preferred_element_type=f32)
                d["acc"] = o if c == 0 else d["acc"] + o
                if c == NC - 1:
                    d["out"] = d["acc"] * _recip(d["lsum"])
                    if gg == GPB - 1:
                        ot[hh * DH:(hh + 1) * DH, :] = d["out"]
                    elif hh == HPB - 1:
                        o_t = jnp.concatenate([st[gg, k]["out"] for k in range(HPB)], axis=0)
                        ob[g, o_rows(q0), :] = _pack(o_t.T.astype(bf16))

            pend = None
            for gg in range(GPB):
                for hh in range(HPB):
                    for c in range(NC):
                        s = qk(gg, hh, c)
                        if pend is None:
                            ob[jnp.where(i == 0, NT, i * GPB - 1), o_rows(q0), :] = _pack(
                                finish_group(jnp.maximum(i * GPB - 1, 0)))
                        else:
                            pv(*pend)
                        pend = (gg, hh, c, s)
            pv(*pend)
            for d in st.values():
                lmax = jnp.maximum(lmax, d["lsum"])
            return lmax

        return lax.fori_loop(0, NT // GPB, body, jnp.zeros((1, TQ), f32))

    def attn_exact(q0):
        def group(g, carry):
            def head(hh, carry2):
                w = qt[pl.ds(pl.multiple_of(g * 64, 64), 64), pl.ds(q0, TQ)]
                row = lax.broadcasted_iota(jnp.int32, (64, TQ), 0) // 16
                w = _unpack(jnp.where(row == hh, w, jnp.zeros_like(w)))

                def scores(c):
                    kc = kb[g, pl.ds(pl.multiple_of(c * (KC // 2), KC // 2), KC // 2), :]
                    return jnp.dot(_unpack(kc), w, preferred_element_type=f32)

                def row_max(c, m):
                    return jnp.maximum(m, jnp.max(scores(c), axis=0, keepdims=True))

                m = lax.fori_loop(0, NC, row_max, jnp.full((1, TQ), -jnp.inf, f32))

                def accumulate(c, state):
                    l, acc = state
                    p = jnp.exp2(scores(c) - m)
                    v = vt[pl.ds(pl.multiple_of(g * 64 + hh * 16, 16), 16),
                           pl.ds(pl.multiple_of(c * KC, KC), KC)]
                    o = jnp.dot(_unpack(v), p.astype(bf16), preferred_element_type=f32)
                    return l + jnp.sum(p, axis=0, keepdims=True), acc + o

                l, acc = lax.fori_loop(0, NC, accumulate,
                                       (jnp.zeros((1, TQ), f32), jnp.zeros((DH, TQ), f32)))
                ot[pl.ds(pl.multiple_of(hh * DH, DH), DH), :] = acc * (1.0 / l)
                return carry2
            lax.fori_loop(0, HPB, head, 0)
            ob[g, o_rows(q0), :] = _pack(ot[...].T.astype(bf16))
            return carry
        lax.fori_loop(0, NT, group, 0)
        pp[...] = jnp.zeros(pp.shape, u32)
        invs[...] = jnp.ones(invs.shape, f32)

    def q_body(qb, l):
        q0 = pl.multiple_of(qb * TQ, TQ)

        def attempt(state):
            a, _ = state

            @pl.when(a == 0)
            def _():
                lmx[...] = jnp.broadcast_to(attn_fast(q0), (8, TQ))

            @pl.when(a == 1)
            def _():
                attn_exact(q0)

            @pl.when(jnp.logical_or(l == 1, a == 1))
            def _():
                for j in range(TQ // OC):
                    out_copy(qb, j).wait()

            kd = (NT - 1) * 128
            o = jnp.concatenate([_unpack(ob[g, o_rows(q0), :]) for g in range(NT - 1)], axis=1)
            o_last = None
            for j in range(TQ // OC):
                y = lax.dot_general(o[j * OC:(j + 1) * OC], wob[0:kd, :], NN,
                                    preferred_element_type=f32)
                if j == 0:
                    o_last = finish_group(NT - 1)
                    y_first = y
                    continue
                if j == 2:
                    bad = _tree(jnp.maximum, [jnp.where(lmx[:, i * 128:(i + 1) * 128] <= L_MAX, 0.0, 1.0)
                                              for i in range(TQ // 128)])
                    v_ok = (vbig[...] & jnp.uint32(0x80008000)) == 0
                    unsafe = jnp.max(jnp.where(v_ok, bad, 1.0))
                for jj in ((0, 1) if j == 1 else (j,)):
                    yj = (y_first if jj == 0 else y) + lax.dot_general(
                        o_last[jj * OC:(jj + 1) * OC], wob[kd:D, :], NN, preferred_element_type=f32)
                    rows = pl.ds(q0 + jj * OC, OC)
                    x2 = xs[rows, :] + yj
                    xs2[rows, :] = x2
                    outb[rows, :] = x2.astype(bf16)
                    out_copy(qb, jj).start()
            return a + 1, unsafe

        lax.while_loop(lambda st: jnp.logical_or(st[0] == 0, jnp.logical_and(st[0] == 1, st[1] > 0.5)),
                       attempt, (jnp.int32(0), jnp.float32(0)))
        return l

    def layer_pair(l, carry):
        ka[:, 0:HALO, :] = jnp.zeros((NDUP * NT, HALO, 128), f32)
        va[:, 0:HALO, :] = jnp.zeros((NDUP * NT, HALO, 128), f32)
        vbig[...] = jnp.zeros(vbig.shape, u32)

        @pl.when(l == 1)
        def _():
            load_x(0, l, 32)

        lax.fori_loop(0, S // RB, row_body, l)

        @pl.when(l == 0)
        def _():
            wob_copy.wait()

        lax.fori_loop(0, S // TQ, q_body, l)
        return carry

    x_copy(0).wait()
    load_x(0, 0, 32)
    for i in range(NWO):
        woa_copy(i).wait()
        if i == LATE_AT:
            for cp in late:
                cp.start()
        lax.fori_loop(i * NT // NWO, (i + 1) * NT // NWO, prep_woa, 0)
    lax.fori_loop(0, 2, layer_pair, 0)
    for qb in range(S // TQ):
        for j in range(TQ // OC):
            out_copy(qb, j).wait()


@jax.jit
def pallas_interleave_layers__sliding_local_dilated__softmax_full_mha__prompt_kernel(
    A_x: jax.Array,
    A_wqkv: jax.Array,
    A_wo: jax.Array,
    B_x: jax.Array,
    B_wqkv: jax.Array,
    B_wo: jax.Array,
):
    del B_x
    x = A_x.reshape(S, D)
    hbm = pl.BlockSpec(memory_space=pl.ANY)
    out = pl.pallas_call(
        _kernel,
        out_shape=jax.ShapeDtypeStruct((S, D), bf16),
        in_specs=[hbm] * 5,
        out_specs=hbm,
        scratch_shapes=[
            pltpu.VMEM((S, D), bf16),
            pltpu.VMEM((D, 3 * D), bf16),
            pltpu.VMEM((D, D), bf16),
            pltpu.VMEM((D, 3 * D), bf16),
            pltpu.VMEM((D, D), bf16),
            pltpu.VMEM((S, D), bf16),
            pltpu.VMEM((3, H * PITCH, 128), f32),
            pltpu.VMEM((H * WPITCH, 128), u32),
            pltpu.VMEM((D // 2, 3 * D), u32),
            pltpu.VMEM((D // 2, D), u32),
            pltpu.VMEM((RB // 2, D), u32),
            pltpu.VMEM((S + RB, D), f32),
            pltpu.VMEM((S, D), f32),
            pltpu.VMEM((NT, RB, 128), f32),
            pltpu.VMEM((NDUP * NT, HALO + RB, 128), f32),
            pltpu.VMEM((NDUP * NT, HALO + RB, 128), f32),
            pltpu.VMEM((D // 2, S), u32),
            pltpu.VMEM((NT, S // 2, 128), u32),
            pltpu.VMEM((D // 2, S), u32),
            pltpu.VMEM((NT + 1, S // 2, 128), u32),
            pltpu.VMEM((128, TQ), f32),
            pltpu.VMEM((KC // 2, TQ), u32),
            pltpu.VMEM((8, TQ), f32),
            pltpu.VMEM((8, TQ), f32),
            pltpu.VMEM((8, 128), u32),
            pltpu.SemaphoreType.DMA((S // RB,)),
            pltpu.SemaphoreType.DMA((NT,)),
            pltpu.SemaphoreType.DMA((4 + NWO,)),
            pltpu.SemaphoreType.DMA((S // OC,)),
        ],
        compiler_params=pltpu.CompilerParams(vmem_limit_bytes=110 * 1024 * 1024),
    )(x, A_wqkv, A_wo, B_wqkv, B_wo)
    return out.reshape(1, S, D)
```

```python
import functools
import math

import jax
import jax.numpy as jnp
from jax import lax
import jax.experimental.pallas as pl
import jax.experimental.pallas.tpu as pltpu

S = 2048
D = 1024
H = 32
DH = 32
WIN = 8
DIL = 2
EPS = 1e-5
NT = D // 128
HALO = 16
QSCALE = (DH ** -0.5) * math.log2(math.e)

SB = 128
NSUB = 2
RB = SB * NSUB
RC = 8
ROW_HEAD = [("a", 0), ("a", 1), ("o", 0), ("o", 1), ("w", 0), ("l", 1)]
ROW_TAILS = [
    [("b", (0, 0, 1)), ("b", (2, 0, 1)), ("b", (1, 0, 1)), ("n", 0), ("b", (0, 1, 1)), ("b", (2, 1, 1)), ("b", (1, 1, 1))],
    [("b", (0, 0, 1)), ("n", 0), ("b", (2, 0, 2)), ("b", (0, 1, 1)), ("b", (1, 0, 2))],
    [("b", (0, 0, 1)), ("b", (2, 0, 2)), ("n", 0), ("b", (0, 1, 1)), ("b", (1, 0, 2))],
    [("b", (1, 0, 1)), ("n", 0), ("b", (2, 0, 2)), ("b", (0, 0, 2)), ("b", (1, 1, 1))],
    [("b", (0, 0, 1)), ("b", (2, 0, 1)), ("n", 0), ("b", (0, 1, 1)), ("b", (2, 1, 1)), ("b", (1, 0, 2))],
]
TAIL = 4
ROW_ORDER = ROW_HEAD + ROW_TAILS[TAIL]
LC = 8
LN_LOOK = 2
LX_LOOK = 1
NDUP = 1
TILE_GATE = 1
PV_GATE = 1
T_OUTER = True
PV_TREE = False
LOOK = (2, 2)
DEP_END = (True, False)
GATE_COL = (2048, 2048)
TQ = 512
KC = 256
NC = S // KC
OC = 128
GPB = 2
HPB = 4
NWO = 4
WA_STARTS = (2, 1, 2, 1, 2, 1, 1, 0)
LATE_AT = 3
XLU_TILES = (8, 8, 0)
WPITCH = 20
PITCH = 40
NFLIGHT = 3
L_MAX = 2.0 ** 64
V_EXP = 50

bf16 = jnp.bfloat16
f32 = jnp.float32
u32 = jnp.uint32

NN = (((1,), (0,)), ((), ()))
NTD = (((1,), (1,)), ((), ()))


def _pack(x):
    return pltpu.bitcast(x, u32)


def _unpack(x):
    return pltpu.bitcast(x, bf16)


def _after(value, dep):
    if dep is None:
        return value
    return jnp.maximum(value, jnp.minimum(dep, -3e38))


def _tree(op, xs):
    xs = list(xs)
    while len(xs) > 1:
        xs = [op(xs[i], xs[i + 1]) if i + 1 < len(xs) else xs[i] for i in range(0, len(xs), 2)]
    return xs[0]


def _recip(x):
    r = pl.reciprocal(x, approx=True)
    return r * (2.0 - x * r)


def _too_large(packed):
    bias = 0x8000 - ((127 + V_EXP) << 7)
    t = (packed & jnp.uint32(0x7F807F80)) + jnp.uint32(bias << 16 | bias)
    return _tree(jnp.bitwise_or, [t[i:i + 8] for i in range(0, t.shape[0], 8)])


def _layernorm(load, nrows, look, first_dep=None):
    outs = []
    deps = []
    for c in range(nrows // LC):
        dep = deps[c - look] if c >= look else first_dep
        x = load(c * LC, dep)
        mu = jnp.broadcast_to(jnp.sum(x, axis=-1, keepdims=True), (LC, 128)) * _after(1.0 / D, dep)
        xc = x - jnp.concatenate([mu] * NT, axis=1)
        var = jnp.sum(xc * xc, axis=-1, keepdims=True) * (1.0 / D)
        y = xc * lax.rsqrt(var + EPS)
        deps.append(y[:, D - 128:])
        outs.append(y)
    return jnp.concatenate(outs, axis=0).astype(bf16)


def _kernel(x_hbm, wa_hbm, woa_hbm, wb_hbm, wob_hbm, out_hbm,
            xin, wa_raw, woa_raw, wb_raw, wob, outb,
            stg, stw, wan, woa, xnb,
            xs, xs2, qa, ka, va, qt, kb, vt, ob, ot, pp, invs, lmx, vbig,
            sem_x, sem_wa, sem_w, sem_o):
    def x_copy(r):
        rows = pl.ds(pl.multiple_of(r * RB, RB), RB)
        return pltpu.make_async_copy(x_hbm.at[rows, :], xin.at[rows, :], sem_x.at[r])

    def wa_copy(i):
        rows = pl.ds(pl.multiple_of(i * 128, 128), 128)
        return pltpu.make_async_copy(wa_hbm.at[rows, :], wa_raw.at[rows, :], sem_wa.at[i])

    def wb_copy(i):
        cols = pl.ds(pl.multiple_of(i * D, D), D)
        return pltpu.make_async_copy(wb_hbm.at[:, cols], wb_raw.at[:, cols], sem_w.at[i])

    def woa_copy(i):
        cols = pl.ds(pl.multiple_of(i * (D // NWO), D // NWO), D // NWO)
        return pltpu.make_async_copy(woa_hbm.at[:, cols], woa_raw.at[:, cols], sem_w.at[4 + i])

    wob_copy = pltpu.make_async_copy(wob_hbm, wob, sem_w.at[3])

    def out_copy(qb, j):
        rows = pl.ds(pl.multiple_of(qb * TQ + j * OC, OC), OC)
        return pltpu.make_async_copy(outb.at[rows, :], out_hbm.at[rows, :],
                                     sem_o.at[qb * (TQ // OC) + j])

    queue = ([wa_copy(i) for i in range(NT)]
             + [x_copy(0)] + [woa_copy(i) for i in range(NWO)]
             + [x_copy(1), wb_copy(0), wb_copy(2), wb_copy(1)]
             + [x_copy(r) for r in range(2, S // RB)] + [wob_copy])
    for cp in queue[:NFLIGHT]:
        cp.start()
    queue = queue[NFLIGHT:]

    batches = [[queue.pop(0) for _ in range(n)] for n in WA_STARTS]
    late = [queue.pop(0) for _ in range(NT + 5 + NWO - NFLIGHT - sum(WA_STARTS))]

    def start_in_loop(i, my_batches):
        for k, batch in enumerate(my_batches):
            @pl.when(i == k)
            def _():
                for cp in batch:
                    cp.start()

    def transpose(w):
        ri = lax.broadcasted_iota(jnp.int32, (128, 128), 0)
        ci = lax.broadcasted_iota(jnp.int32, (128, 128), 1)
        eye = jnp.where(ri == ci, 1.0, 0.0).astype(bf16)
        return lax.dot_general(eye, w, NTD, preferred_element_type=f32)

    def prep_wa(t, carry):
        wa_copy(t).wait()
        start_in_loop(t, batches)
        rows = pl.ds(pl.multiple_of(t * 128, 128), 128)

        def forward(part):
            for j in range(NT):
                wt = transpose(wa_raw[rows, part * D + j * 128:part * D + (j + 1) * 128])
                for hh in range(HPB):
                    r = (j * HPB + hh) * PITCH
                    stg[part, r:r + DH, :] = wt[hh * DH:(hh + 1) * DH]

        def back(part):
            regrouped = jnp.concatenate([stg[part, pl.ds(d, H, stride=PITCH), :]
                                         for d in range(DH)], axis=0)
            n = XLU_TILES[part] * 128
            pieces = []
            if n > 0:
                pieces.append(regrouped[:n].T)
            if n < D:
                pieces.append(transpose(regrouped[n:].astype(bf16)))
            wan[pl.ds(pl.multiple_of(t * 64, 64), 64), part * D:(part + 1) * D] = _pack(
                jnp.concatenate(pieces, axis=1).astype(bf16))

        forward(0)
        forward(1)
        back(0)
        forward(2)
        back(1)
        back(2)
        return carry

    def prep_woa(t, carry):
        cols = pl.ds(pl.multiple_of(t * 128, 128), 128)
        w = _pack(woa_raw[:, cols])
        for h in range(H):
            stw[h * WPITCH:h * WPITCH + DH // 2, :] = w[h * (DH // 2):(h + 1) * (DH // 2)]
        lo = jnp.uint32(0xFFFF)
        for j in range(DH // 2):
            even = stw[pl.ds(j, H // 2, stride=2 * WPITCH), :]
            odd = stw[pl.ds(WPITCH + j, H // 2, stride=2 * WPITCH), :]
            woa[2 * j * 16:(2 * j + 1) * 16, cols] = (even & lo) | (odd << 16)
            woa[(2 * j + 1) * 16:(2 * j + 2) * 16, cols] = (even >> 16) | (odd & ~lo)
        return carry

    ot[...] = jnp.zeros(ot.shape, f32)
    pp[...] = jnp.zeros(pp.shape, u32)
    invs[...] = jnp.ones(invs.shape, f32)
    lax.fori_loop(0, NT, prep_wa, 0)

    def local_attn(r0, s, first_dep):
        outs = []
        deps = []
        for c in range(SB // RC):
            base = s * SB + c * RC
            scale = _after(QSCALE, deps[c - LOOK[s]] if c >= LOOK[s] else first_dep)
            logits = [None] * WIN
            dup = NT * (c % NDUP)
            if T_OUTER:
                for t in range(NT):
                    if TILE_GATE and t > 0 and t % TILE_GATE == 0:
                        scale = _after(QSCALE, logits[WIN - 1])
                    q = qa[t, base:base + RC, :] * scale
                    for w in range(WIN):
                        o0 = HALO + base - DIL * w
                        term = q * ka[t + dup, o0:o0 + RC, :]
                        logits[w] = term if t == 0 else logits[w] + term
            else:
                q = [qa[t, base:base + RC, :] * scale for t in range(NT)]
                for w in range(WIN):
                    o0 = HALO + base - DIL * w
                    terms = [q[t] * ka[t + dup, o0:o0 + RC, :] for t in range(NT)]
                    logits[w] = functools.reduce(jnp.add, terms)
            for w in range(WIN):
                acc = logits[w]
                acc = acc + pltpu.roll(acc, 64, 1)
                acc = acc + pltpu.roll(acc, 32, 1)
                if base < DIL * w:
                    row = r0 + base + lax.broadcasted_iota(jnp.int32, (RC, 128), 0)
                    acc = jnp.where(row >= DIL * w, acc, -1e9)
                logits[w] = acc
            m = _tree(jnp.maximum, logits)
            p = [jnp.exp2(lg - m) for lg in logits]
            inv = _recip(_tree(jnp.add, p))
            tiles = []
            done = []
            for t in range(NT):
                if PV_GATE and t >= PV_GATE:
                    p[0] = _after(p[0], done[t - PV_GATE])
                terms = [p[w] * va[t + dup, HALO + base - DIL * w:HALO + base - DIL * w + RC, :]
                         for w in range(WIN)]
                acc = (_tree(jnp.add, terms) if PV_TREE else functools.reduce(jnp.add, terms)) * inv
                tiles.append(acc.astype(bf16))
                done.append(acc)
            deps.append(acc if DEP_END[s] else m)
            outs.append(jnp.concatenate(tiles, axis=1))
        return jnp.concatenate(outs, axis=0)

    def load_x(r, l, look):
        r0 = pl.multiple_of(jnp.minimum(r, S // RB - 1) * RB, RB)
        w0 = pl.multiple_of(r * RB, RB)

        def load(start, dep):
            rows = pl.ds(r0 + start, LC)
            lvec = _after(jnp.full((LC, 128), l, f32), dep)
            first = jnp.concatenate([lvec == 0.0] * NT, axis=1)
            xi = xin[pl.ds(r0 + start // 16 * 16, 16), :].astype(f32)[start % 16:start % 16 + LC]
            x = jnp.where(first, xi, xs2[rows, :])
            xs[pl.ds(w0 + start, LC), :] = x
            return x

        xnb[...] = _pack(_layernorm(load, RB, look))

    def row_body(r, l):
        r0 = pl.multiple_of(r * RB, RB)
        rn = jnp.minimum(r + 1, S // RB - 1)

        rows = [pl.ds(r0 + s * SB, SB) for s in range(NSUB)]
        gate = {}
        xn2 = {}

        def qkv_a(s):
            xn = _unpack(xnb[s * SB // 2:(s + 1) * SB // 2, :])
            y = lax.dot_general(xn, _unpack(wan[...]), NN, preferred_element_type=f32)
            for t in range(NT):
                qa[t, s * SB:(s + 1) * SB, :] = y[:, t * 128:(t + 1) * 128]
                for dup in range(0, NDUP * NT, NT):
                    new = slice(HALO + s * SB, HALO + (s + 1) * SB)
                    ka[t + dup, new, :] = y[:, D + t * 128:D + (t + 1) * 128]
                    va[t + dup, new, :] = y[:, 2 * D + t * 128:2 * D + (t + 1) * 128]
            gate[s] = y[SB - RC:SB, GATE_COL[s] - 128:GATE_COL[s]]

        def out_a(s):
            o = local_attn(r0, s, gate[s])
            x1 = xs[rows[s], :] + lax.dot_general(o, _unpack(woa[...]), NN,
                                                  preferred_element_type=f32)
            xs[rows[s], :] = x1
            if s < NSUB - 1:
                xn2[s] = _layernorm(lambda st, dep: x1[st:st + LC], SB, LN_LOOK)

        def norm_b(s):
            xn2[s] = _layernorm(lambda st, dep: xs[pl.ds(r0 + s * SB + st, LC), :], SB, LN_LOOK)

        def weights_b(_):
            @pl.when(jnp.logical_and(l == 0, r == 0))
            def _():
                for i in range(3):
                    wb_copy(i).wait()
                for cp in queue:
                    cp.start()

            @pl.when(jnp.logical_and(l == 0, r + 1 < S // RB))
            def _():
                x_copy(rn).wait()

        def proj_b(arg):
            part, s, n = arg
            xn = jnp.concatenate([xn2[s + i] for i in range(n)], axis=0)
            y = lax.dot_general(xn, wb_raw[:, part * D:(part + 1) * D], NN, preferred_element_type=f32)
            cols = pl.ds(r0 + s * SB, n * SB)
            if part == 0:
                qt[:, cols] = _pack((y * QSCALE).T.astype(bf16))
            elif part == 2:
                v_t = _pack(y.T.astype(bf16))
                vt[:, cols] = v_t
                for i in range(n):
                    vbig[...] = vbig[...] | _too_large(v_t[:, i * SB:(i + 1) * SB])
            else:
                krows = pl.ds(pl.multiple_of((r0 + s * SB) // 2, SB // 2), n * SB // 2)
                y = y.astype(bf16)
                for g in range(NT):
                    kb[g, krows, :] = _pack(y[:, g * 128:(g + 1) * 128])

        steps = {"a": qkv_a, "o": out_a, "b": proj_b, "w": weights_b, "l": norm_b}
        for name, s in ROW_ORDER:
            if name == "n":
                ka[:, 0:HALO, :] = ka[:, RB:RB + HALO, :]
                va[:, 0:HALO, :] = va[:, RB:RB + HALO, :]
                load_x(r + 1, l, LX_LOOK)
            else:
                steps[name](s)
        return l

    def head_weights(g, hh, q0):
        w = qt[pl.ds(pl.multiple_of(g * 64 + hh * 16, 16), 16), pl.ds(q0, TQ)]
        parts = []
        if hh > 0:
            parts.append(jnp.zeros((16 * hh, TQ), u32))
        parts.append(w)
        if hh < 3:
            parts.append(jnp.zeros((16 * (3 - hh), TQ), u32))
        return _unpack(jnp.concatenate(parts, axis=0))

    def v_rows(g, hh, c):
        rows = pl.ds(pl.multiple_of(g * 64 + hh * 16, 16), 16)
        return _unpack(vt[rows, c * KC:(c + 1) * KC])

    def finish_group(g):
        o = jnp.dot(v_rows(g, HPB - 1, NC - 1), _unpack(pp[...]), preferred_element_type=f32)
        last = (ot[3 * DH:4 * DH, :] + o) * invs[0:1, :]
        return jnp.concatenate([ot[0:3 * DH, :], last], axis=0).T.astype(bf16)

    def o_rows(q0):
        return pl.ds(pl.multiple_of(q0 // 2, TQ // 2), TQ // 2)

    def attn_fast(q0):
        def body(i, lmax):
            st = {}

            def qk(gg, hh, c):
                g = i * GPB + gg
                if c == 0:
                    st[gg, hh] = dict(w=head_weights(g, hh, q0))
                kc = _unpack(kb[g, c * KC // 2:(c + 1) * KC // 2, :])
                return jnp.dot(kc, st[gg, hh]["w"], preferred_element_type=f32)

            def pv(gg, hh, c, s):
                g = i * GPB + gg
                d = st[gg, hh]
                if c == 0:
                    d["m"] = jnp.broadcast_to(jnp.max(s[0:8], axis=0, keepdims=True), (8, TQ))
                p = jnp.exp2(s.reshape(KC // 8, 8, TQ) - d["m"][None])
                lc = jnp.sum(p, axis=0)
                d["l"] = lc if c == 0 else d["l"] + lc
                p = p.reshape(KC, TQ).astype(bf16)
                if c == NC - 1:
                    d["lsum"] = jnp.sum(d["l"], axis=0, keepdims=True)
                if gg == GPB - 1 and hh == HPB - 1 and c == NC - 1:
                    pp[...] = _pack(p)
                    ot[hh * DH:(hh + 1) * DH, :] = d["acc"]
                    invs[...] = jnp.broadcast_to(_recip(d["lsum"]), (8, TQ))
                    return
                o = jnp.dot(v_rows(g, hh, c), p, preferred_element_type=f32)
                d["acc"] = o if c == 0 else d["acc"] + o
                if c == NC - 1:
                    d["out"] = d["acc"] * _recip(d["lsum"])
                    if gg == GPB - 1:
                        ot[hh * DH:(hh + 1) * DH, :] = d["out"]
                    elif hh == HPB - 1:
                        o_t = jnp.concatenate([st[gg, k]["out"] for k in range(HPB)], axis=0)
                        ob[g, o_rows(q0), :] = _pack(o_t.T.astype(bf16))

            pend = None
            for gg in range(GPB):
                for hh in range(HPB):
                    for c in range(NC):
                        s = qk(gg, hh, c)
                        if pend is None:
                            ob[jnp.where(i == 0, NT, i * GPB - 1), o_rows(q0), :] = _pack(
                                finish_group(jnp.maximum(i * GPB - 1, 0)))
                        else:
                            pv(*pend)
                        pend = (gg, hh, c, s)
            pv(*pend)
            for d in st.values():
                lmax = jnp.maximum(lmax, d["lsum"])
            return lmax

        return lax.fori_loop(0, NT // GPB, body, jnp.zeros((1, TQ), f32))

    def attn_exact(q0):
        def group(g, carry):
            def head(hh, carry2):
                w = qt[pl.ds(pl.multiple_of(g * 64, 64), 64), pl.ds(q0, TQ)]
                row = lax.broadcasted_iota(jnp.int32, (64, TQ), 0) // 16
                w = _unpack(jnp.where(row == hh, w, jnp.zeros_like(w)))

                def scores(c):
                    kc = kb[g, pl.ds(pl.multiple_of(c * (KC // 2), KC // 2), KC // 2), :]
                    return jnp.dot(_unpack(kc), w, preferred_element_type=f32)

                def row_max(c, m):
                    return jnp.maximum(m, jnp.max(scores(c), axis=0, keepdims=True))

                m = lax.fori_loop(0, NC, row_max, jnp.full((1, TQ), -jnp.inf, f32))

                def accumulate(c, state):
                    l, acc = state
                    p = jnp.exp2(scores(c) - m)
                    v = vt[pl.ds(pl.multiple_of(g * 64 + hh * 16, 16), 16),
                           pl.ds(pl.multiple_of(c * KC, KC), KC)]
                    o = jnp.dot(_unpack(v), p.astype(bf16), preferred_element_type=f32)
                    return l + jnp.sum(p, axis=0, keepdims=True), acc + o

                l, acc = lax.fori_loop(0, NC, accumulate,
                                       (jnp.zeros((1, TQ), f32), jnp.zeros((DH, TQ), f32)))
                ot[pl.ds(pl.multiple_of(hh * DH, DH), DH), :] = acc * (1.0 / l)
                return carry2
            lax.fori_loop(0, HPB, head, 0)
            ob[g, o_rows(q0), :] = _pack(ot[...].T.astype(bf16))
            return carry
        lax.fori_loop(0, NT, group, 0)
        pp[...] = jnp.zeros(pp.shape, u32)
        invs[...] = jnp.ones(invs.shape, f32)

    def q_body(qb, l):
        q0 = pl.multiple_of(qb * TQ, TQ)

        def attempt(state):
            a, _ = state

            @pl.when(a == 0)
            def _():
                lmx[...] = jnp.broadcast_to(attn_fast(q0), (8, TQ))

            @pl.when(a == 1)
            def _():
                attn_exact(q0)

            @pl.when(jnp.logical_or(l == 1, a == 1))
            def _():
                for j in range(TQ // OC):
                    out_copy(qb, j).wait()

            kd = (NT - 1) * 128
            o = jnp.concatenate([_unpack(ob[g, o_rows(q0), :]) for g in range(NT - 1)], axis=1)
            o_last = None
            for j in range(TQ // OC):
                y = lax.dot_general(o[j * OC:(j + 1) * OC], wob[0:kd, :], NN,
                                    preferred_element_type=f32)
                if j == 0:
                    o_last = finish_group(NT - 1)
                    y_first = y
                    continue
                if j == 2:
                    bad = _tree(jnp.maximum, [jnp.where(lmx[:, i * 128:(i + 1) * 128] <= L_MAX, 0.0, 1.0)
                                              for i in range(TQ // 128)])
                    v_ok = (vbig[...] & jnp.uint32(0x80008000)) == 0
                    unsafe = jnp.max(jnp.where(v_ok, bad, 1.0))
                for jj in ((0, 1) if j == 1 else (j,)):
                    yj = (y_first if jj == 0 else y) + lax.dot_general(
                        o_last[jj * OC:(jj + 1) * OC], wob[kd:D, :], NN, preferred_element_type=f32)
                    rows = pl.ds(q0 + jj * OC, OC)
                    x2 = xs[rows, :] + yj
                    xs2[rows, :] = x2
                    outb[rows, :] = x2.astype(bf16)
                    out_copy(qb, jj).start()
            return a + 1, unsafe

        lax.while_loop(lambda st: jnp.logical_or(st[0] == 0, jnp.logical_and(st[0] == 1, st[1] > 0.5)),
                       attempt, (jnp.int32(0), jnp.float32(0)))
        return l

    def layer_pair(l, carry):
        ka[:, 0:HALO, :] = jnp.zeros((NDUP * NT, HALO, 128), f32)
        va[:, 0:HALO, :] = jnp.zeros((NDUP * NT, HALO, 128), f32)
        vbig[...] = jnp.zeros(vbig.shape, u32)

        @pl.when(l == 1)
        def _():
            load_x(0, l, 32)

        lax.fori_loop(0, S // RB, row_body, l)

        @pl.when(l == 0)
        def _():
            wob_copy.wait()

        lax.fori_loop(0, S // TQ, q_body, l)
        return carry

    x_copy(0).wait()
    load_x(0, 0, 32)
    for i in range(NWO):
        woa_copy(i).wait()
        if i == LATE_AT:
            for cp in late:
                cp.start()
        lax.fori_loop(i * NT // NWO, (i + 1) * NT // NWO, prep_woa, 0)
    lax.fori_loop(0, 2, layer_pair, 0)
    for qb in range(S // TQ):
        for j in range(TQ // OC):
            out_copy(qb, j).wait()


@jax.jit
def pallas_interleave_layers__sliding_local_dilated__softmax_full_mha__prompt_kernel(
    A_x: jax.Array,
    A_wqkv: jax.Array,
    A_wo: jax.Array,
    B_x: jax.Array,
    B_wqkv: jax.Array,
    B_wo: jax.Array,
):
    del B_x
    x = A_x.reshape(S, D)
    hbm = pl.BlockSpec(memory_space=pl.ANY)
    out = pl.pallas_call(
        _kernel,
        out_shape=jax.ShapeDtypeStruct((S, D), bf16),
        in_specs=[hbm] * 5,
        out_specs=hbm,
        scratch_shapes=[
            pltpu.VMEM((S, D), bf16),
            pltpu.VMEM((D, 3 * D), bf16),
            pltpu.VMEM((D, D), bf16),
            pltpu.VMEM((D, 3 * D), bf16),
            pltpu.VMEM((D, D), bf16),
            pltpu.VMEM((S, D), bf16),
            pltpu.VMEM((3, H * PITCH, 128), f32),
            pltpu.VMEM((H * WPITCH, 128), u32),
            pltpu.VMEM((D // 2, 3 * D), u32),
            pltpu.VMEM((D // 2, D), u32),
            pltpu.VMEM((RB // 2, D), u32),
            pltpu.VMEM((S + RB, D), f32),
            pltpu.VMEM((S, D), f32),
            pltpu.VMEM((NT, RB, 128), f32),
            pltpu.VMEM((NDUP * NT, HALO + RB, 128), f32),
            pltpu.VMEM((NDUP * NT, HALO + RB, 128), f32),
            pltpu.VMEM((D // 2, S), u32),
            pltpu.VMEM((NT, S // 2, 128), u32),
            pltpu.VMEM((D // 2, S), u32),
            pltpu.VMEM((NT + 1, S // 2, 128), u32),
            pltpu.VMEM((128, TQ), f32),
            pltpu.VMEM((KC // 2, TQ), u32),
            pltpu.VMEM((8, TQ), f32),
            pltpu.VMEM((8, TQ), f32),
            pltpu.VMEM((8, 128), u32),
            pltpu.SemaphoreType.DMA((S // RB,)),
            pltpu.SemaphoreType.DMA((NT,)),
            pltpu.SemaphoreType.DMA((4 + NWO,)),
            pltpu.SemaphoreType.DMA((S // OC,)),
        ],
        compiler_params=pltpu.CompilerParams(vmem_limit_bytes=110 * 1024 * 1024),
    )(x, A_wqkv, A_wo, B_wqkv, B_wo)
    return out.reshape(1, S, D)
```

```python
import functools
import math

import jax
import jax.numpy as jnp
from jax import lax
import jax.experimental.pallas as pl
import jax.experimental.pallas.tpu as pltpu

S = 2048
D = 1024
H = 32
DH = 32
WIN = 8
DIL = 2
EPS = 1e-5
NT = D // 128
HALO = 16
QSCALE = (DH ** -0.5) * math.log2(math.e)

SB = 128
NSUB = 2
RB = SB * NSUB
RC = 8
ROW_HEAD = [("a", 0), ("a", 1), ("o", 0), ("o", 1), ("w", 0), ("l", 1)]
ROW_TAILS = [
    [("b", (0, 0, 1)), ("b", (2, 0, 1)), ("b", (1, 0, 1)), ("n", 0), ("b", (0, 1, 1)), ("b", (2, 1, 1)), ("b", (1, 1, 1))],
    [("b", (0, 0, 1)), ("n", 0), ("b", (2, 0, 2)), ("b", (0, 1, 1)), ("b", (1, 0, 2))],
    [("b", (0, 0, 1)), ("b", (2, 0, 2)), ("n", 0), ("b", (0, 1, 1)), ("b", (1, 0, 2))],
    [("b", (1, 0, 1)), ("n", 0), ("b", (2, 0, 2)), ("b", (0, 0, 2)), ("b", (1, 1, 1))],
    [("b", (0, 0, 1)), ("b", (2, 0, 1)), ("n", 0), ("b", (0, 1, 1)), ("b", (2, 1, 1)), ("b", (1, 0, 2))],
]
TAIL = 0
ROW_ORDER = ROW_HEAD + ROW_TAILS[TAIL]
LC = 8
LN_LOOK = (2, 1)
LX_LOOK = 1
NDUP = 1
TILE_GATE = (2, 2)
PV_GATE = (1, 1)
T_OUTER = True
PV_TREE = True
LOOK = (1, 2)
DEP_END = (False, False)
GATE_COL = (2048, 2048)
TQ = 512
KC = 256
NC = S // KC
OC = 128
GPB = 2
HPB = 4
NWO = 4
WA_STARTS = (2, 1, 2, 1, 2, 1, 1, 0)
LATE_AT = 3
XLU_TILES = (8, 8, 0)
WPITCH = 20
PITCH = 40
NFLIGHT = 3
L_MAX = 2.0 ** 64
V_EXP = 50

bf16 = jnp.bfloat16
f32 = jnp.float32
u32 = jnp.uint32

NN = (((1,), (0,)), ((), ()))
NTD = (((1,), (1,)), ((), ()))


def _pack(x):
    return pltpu.bitcast(x, u32)


def _unpack(x):
    return pltpu.bitcast(x, bf16)


def _after(value, dep):
    if dep is None:
        return value
    return jnp.maximum(value, jnp.minimum(dep, -3e38))


def _tree(op, xs):
    xs = list(xs)
    while len(xs) > 1:
        xs = [op(xs[i], xs[i + 1]) if i + 1 < len(xs) else xs[i] for i in range(0, len(xs), 2)]
    return xs[0]


def _recip(x):
    r = pl.reciprocal(x, approx=True)
    return r * (2.0 - x * r)


def _too_large(packed):
    bias = 0x8000 - ((127 + V_EXP) << 7)
    t = (packed & jnp.uint32(0x7F807F80)) + jnp.uint32(bias << 16 | bias)
    return _tree(jnp.bitwise_or, [t[i:i + 8] for i in range(0, t.shape[0], 8)])


def _layernorm(load, nrows, look, first_dep=None):
    outs = []
    deps = []
    for c in range(nrows // LC):
        dep = deps[c - look] if c >= look else first_dep
        x = load(c * LC, dep)
        mu = jnp.broadcast_to(jnp.sum(x, axis=-1, keepdims=True), (LC, 128)) * _after(1.0 / D, dep)
        xc = x - jnp.concatenate([mu] * NT, axis=1)
        var = jnp.sum(xc * xc, axis=-1, keepdims=True) * (1.0 / D)
        y = xc * lax.rsqrt(var + EPS)
        deps.append(y[:, D - 128:])
        outs.append(y)
    return jnp.concatenate(outs, axis=0).astype(bf16)


def _kernel(x_hbm, wa_hbm, woa_hbm, wb_hbm, wob_hbm, out_hbm,
            xin, wa_raw, woa_raw, wb_raw, wob, outb,
            stg, stw, wan, woa, xnb,
            xs, xs2, qa, ka, va, qt, kb, vt, ob, ot, pp, invs, lmx, vbig,
            sem_x, sem_wa, sem_w, sem_o):
    def x_copy(r):
        rows = pl.ds(pl.multiple_of(r * RB, RB), RB)
        return pltpu.make_async_copy(x_hbm.at[rows, :], xin.at[rows, :], sem_x.at[r])

    def wa_copy(i):
        rows = pl.ds(pl.multiple_of(i * 128, 128), 128)
        return pltpu.make_async_copy(wa_hbm.at[rows, :], wa_raw.at[rows, :], sem_wa.at[i])

    def wb_copy(i):
        cols = pl.ds(pl.multiple_of(i * D, D), D)
        return pltpu.make_async_copy(wb_hbm.at[:, cols], wb_raw.at[:, cols], sem_w.at[i])

    def woa_copy(i):
        cols = pl.ds(pl.multiple_of(i * (D // NWO), D // NWO), D // NWO)
        return pltpu.make_async_copy(woa_hbm.at[:, cols], woa_raw.at[:, cols], sem_w.at[4 + i])

    wob_copy = pltpu.make_async_copy(wob_hbm, wob, sem_w.at[3])

    def out_copy(qb, j):
        rows = pl.ds(pl.multiple_of(qb * TQ + j * OC, OC), OC)
        return pltpu.make_async_copy(outb.at[rows, :], out_hbm.at[rows, :],
                                     sem_o.at[qb * (TQ // OC) + j])

    queue = ([wa_copy(i) for i in range(NT)]
             + [x_copy(0)] + [woa_copy(i) for i in range(NWO)]
             + [x_copy(1), wb_copy(0), wb_copy(2), wb_copy(1)]
             + [x_copy(r) for r in range(2, S // RB)] + [wob_copy])
    for cp in queue[:NFLIGHT]:
        cp.start()
    queue = queue[NFLIGHT:]

    batches = [[queue.pop(0) for _ in range(n)] for n in WA_STARTS]
    late = [queue.pop(0) for _ in range(NT + 5 + NWO - NFLIGHT - sum(WA_STARTS))]

    def start_in_loop(i, my_batches):
        for k, batch in enumerate(my_batches):
            @pl.when(i == k)
            def _():
                for cp in batch:
                    cp.start()

    def transpose(w):
        ri = lax.broadcasted_iota(jnp.int32, (128, 128), 0)
        ci = lax.broadcasted_iota(jnp.int32, (128, 128), 1)
        eye = jnp.where(ri == ci, 1.0, 0.0).astype(bf16)
        return lax.dot_general(eye, w, NTD, preferred_element_type=f32)

    def prep_wa(t, carry):
        wa_copy(t).wait()
        start_in_loop(t, batches)
        rows = pl.ds(pl.multiple_of(t * 128, 128), 128)

        def forward(part):
            for j in range(NT):
                wt = transpose(wa_raw[rows, part * D + j * 128:part * D + (j + 1) * 128])
                for hh in range(HPB):
                    r = (j * HPB + hh) * PITCH
                    stg[part, r:r + DH, :] = wt[hh * DH:(hh + 1) * DH]

        def back(part):
            regrouped = jnp.concatenate([stg[part, pl.ds(d, H, stride=PITCH), :]
                                         for d in range(DH)], axis=0)
            n = XLU_TILES[part] * 128
            pieces = []
            if n > 0:
                pieces.append(regrouped[:n].T)
            if n < D:
                pieces.append(transpose(regrouped[n:].astype(bf16)))
            wan[pl.ds(pl.multiple_of(t * 64, 64), 64), part * D:(part + 1) * D] = _pack(
                jnp.concatenate(pieces, axis=1).astype(bf16))

        forward(0)
        forward(1)
        back(0)
        forward(2)
        back(1)
        back(2)
        return carry

    def prep_woa(t, carry):
        cols = pl.ds(pl.multiple_of(t * 128, 128), 128)
        w = _pack(woa_raw[:, cols])
        for h in range(H):
            stw[h * WPITCH:h * WPITCH + DH // 2, :] = w[h * (DH // 2):(h + 1) * (DH // 2)]
        lo = jnp.uint32(0xFFFF)
        for j in range(DH // 2):
            even = stw[pl.ds(j, H // 2, stride=2 * WPITCH), :]
            odd = stw[pl.ds(WPITCH + j, H // 2, stride=2 * WPITCH), :]
            woa[2 * j * 16:(2 * j + 1) * 16, cols] = (even & lo) | (odd << 16)
            woa[(2 * j + 1) * 16:(2 * j + 2) * 16, cols] = (even >> 16) | (odd & ~lo)
        return carry

    ot[...] = jnp.zeros(ot.shape, f32)
    pp[...] = jnp.zeros(pp.shape, u32)
    invs[...] = jnp.ones(invs.shape, f32)
    lax.fori_loop(0, NT, prep_wa, 0)

    def local_attn(r0, s, first_dep):
        outs = []
        deps = []
        for c in range(SB // RC):
            base = s * SB + c * RC
            scale = _after(QSCALE, deps[c - LOOK[s]] if c >= LOOK[s] else first_dep)
            logits = [None] * WIN
            dup = NT * (c % NDUP)
            if T_OUTER:
                for t in range(NT):
                    if TILE_GATE[s] and t > 0 and t % TILE_GATE[s] == 0:
                        scale = _after(QSCALE, logits[WIN - 1])
                    q = qa[t, base:base + RC, :] * scale
                    for w in range(WIN):
                        o0 = HALO + base - DIL * w
                        term = q * ka[t + dup, o0:o0 + RC, :]
                        logits[w] = term if t == 0 else logits[w] + term
            else:
                q = [qa[t, base:base + RC, :] * scale for t in range(NT)]
                for w in range(WIN):
                    o0 = HALO + base - DIL * w
                    terms = [q[t] * ka[t + dup, o0:o0 + RC, :] for t in range(NT)]
                    logits[w] = functools.reduce(jnp.add, terms)
            for w in range(WIN):
                acc = logits[w]
                acc = acc + pltpu.roll(acc, 64, 1)
                acc = acc + pltpu.roll(acc, 32, 1)
                if base < DIL * w:
                    row = r0 + base + lax.broadcasted_iota(jnp.int32, (RC, 128), 0)
                    acc = jnp.where(row >= DIL * w, acc, -1e9)
                logits[w] = acc
            m = _tree(jnp.maximum, logits)
            p = [jnp.exp2(lg - m) for lg in logits]
            inv = _recip(_tree(jnp.add, p))
            tiles = []
            done = []
            for t in range(NT):
                if PV_GATE[s] and t >= PV_GATE[s]:
                    p[0] = _after(p[0], done[t - PV_GATE[s]])
                terms = [p[w] * va[t + dup, HALO + base - DIL * w:HALO + base - DIL * w + RC, :]
                         for w in range(WIN)]
                acc = (_tree(jnp.add, terms) if PV_TREE else functools.reduce(jnp.add, terms)) * inv
                tiles.append(acc.astype(bf16))
                done.append(acc)
            deps.append(acc if DEP_END[s] else m)
            outs.append(jnp.concatenate(tiles, axis=1))
        return jnp.concatenate(outs, axis=0)

    def load_x(r, l, look):
        r0 = pl.multiple_of(jnp.minimum(r, S // RB - 1) * RB, RB)
        w0 = pl.multiple_of(r * RB, RB)

        def load(start, dep):
            rows = pl.ds(r0 + start, LC)
            lvec = _after(jnp.full((LC, 128), l, f32), dep)
            first = jnp.concatenate([lvec == 0.0] * NT, axis=1)
            xi = xin[pl.ds(r0 + start // 16 * 16, 16), :].astype(f32)[start % 16:start % 16 + LC]
            x = jnp.where(first, xi, xs2[rows, :])
            xs[pl.ds(w0 + start, LC), :] = x
            return x

        xnb[...] = _pack(_layernorm(load, RB, look))

    def row_body(r, l):
        r0 = pl.multiple_of(r * RB, RB)
        rn = jnp.minimum(r + 1, S // RB - 1)

        rows = [pl.ds(r0 + s * SB, SB) for s in range(NSUB)]
        gate = {}
        xn2 = {}

        def qkv_a(s):
            xn = _unpack(xnb[s * SB // 2:(s + 1) * SB // 2, :])
            y = lax.dot_general(xn, _unpack(wan[...]), NN, preferred_element_type=f32)
            for t in range(NT):
                qa[t, s * SB:(s + 1) * SB, :] = y[:, t * 128:(t + 1) * 128]
                for dup in range(0, NDUP * NT, NT):
                    new = slice(HALO + s * SB, HALO + (s + 1) * SB)
                    ka[t + dup, new, :] = y[:, D + t * 128:D + (t + 1) * 128]
                    va[t + dup, new, :] = y[:, 2 * D + t * 128:2 * D + (t + 1) * 128]
            gate[s] = y[SB - RC:SB, GATE_COL[s] - 128:GATE_COL[s]]

        def out_a(s):
            o = local_attn(r0, s, gate[s])
            x1 = xs[rows[s], :] + lax.dot_general(o, _unpack(woa[...]), NN,
                                                  preferred_element_type=f32)
            xs[rows[s], :] = x1
            if s < NSUB - 1:
                xn2[s] = _layernorm(lambda st, dep: x1[st:st + LC], SB, LN_LOOK[s])

        def norm_b(s):
            xn2[s] = _layernorm(lambda st, dep: xs[pl.ds(r0 + s * SB + st, LC), :], SB, LN_LOOK[s])

        def weights_b(_):
            @pl.when(jnp.logical_and(l == 0, r == 0))
            def _():
                for i in range(3):
                    wb_copy(i).wait()
                for cp in queue:
                    cp.start()

            @pl.when(jnp.logical_and(l == 0, r + 1 < S // RB))
            def _():
                x_copy(rn).wait()

        def proj_b(arg):
            part, s, n = arg
            xn = jnp.concatenate([xn2[s + i] for i in range(n)], axis=0)
            y = lax.dot_general(xn, wb_raw[:, part * D:(part + 1) * D], NN, preferred_element_type=f32)
            cols = pl.ds(r0 + s * SB, n * SB)
            if part == 0:
                qt[:, cols] = _pack((y * QSCALE).T.astype(bf16))
            elif part == 2:
                v_t = _pack(y.T.astype(bf16))
                vt[:, cols] = v_t
                for i in range(n):
                    vbig[...] = vbig[...] | _too_large(v_t[:, i * SB:(i + 1) * SB])
            else:
                krows = pl.ds(pl.multiple_of((r0 + s * SB) // 2, SB // 2), n * SB // 2)
                y = y.astype(bf16)
                for g in range(NT):
                    kb[g, krows, :] = _pack(y[:, g * 128:(g + 1) * 128])

        steps = {"a": qkv_a, "o": out_a, "b": proj_b, "w": weights_b, "l": norm_b}
        for name, s in ROW_ORDER:
            if name == "n":
                ka[:, 0:HALO, :] = ka[:, RB:RB + HALO, :]
                va[:, 0:HALO, :] = va[:, RB:RB + HALO, :]
                load_x(r + 1, l, LX_LOOK)
            else:
                steps[name](s)
        return l

    def head_weights(g, hh, q0):
        w = qt[pl.ds(pl.multiple_of(g * 64 + hh * 16, 16), 16), pl.ds(q0, TQ)]
        parts = []
        if hh > 0:
            parts.append(jnp.zeros((16 * hh, TQ), u32))
        parts.append(w)
        if hh < 3:
            parts.append(jnp.zeros((16 * (3 - hh), TQ), u32))
        return _unpack(jnp.concatenate(parts, axis=0))

    def v_rows(g, hh, c):
        rows = pl.ds(pl.multiple_of(g * 64 + hh * 16, 16), 16)
        return _unpack(vt[rows, c * KC:(c + 1) * KC])

    def finish_group(g):
        o = jnp.dot(v_rows(g, HPB - 1, NC - 1), _unpack(pp[...]), preferred_element_type=f32)
        last = (ot[3 * DH:4 * DH, :] + o) * invs[0:1, :]
        return jnp.concatenate([ot[0:3 * DH, :], last], axis=0).T.astype(bf16)

    def o_rows(q0):
        return pl.ds(pl.multiple_of(q0 // 2, TQ // 2), TQ // 2)

    def attn_fast(q0):
        def body(i, lmax):
            st = {}

            def qk(gg, hh, c):
                g = i * GPB + gg
                if c == 0:
                    st[gg, hh] = dict(w=head_weights(g, hh, q0))
                kc = _unpack(kb[g, c * KC // 2:(c + 1) * KC // 2, :])
                return jnp.dot(kc, st[gg, hh]["w"], preferred_element_type=f32)

            def pv(gg, hh, c, s):
                g = i * GPB + gg
                d = st[gg, hh]
                if c == 0:
                    d["m"] = jnp.broadcast_to(jnp.max(s[0:8], axis=0, keepdims=True), (8, TQ))
                p = jnp.exp2(s.reshape(KC // 8, 8, TQ) - d["m"][None])
                lc = jnp.sum(p, axis=0)
                d["l"] = lc if c == 0 else d["l"] + lc
                p = p.reshape(KC, TQ).astype(bf16)
                if c == NC - 1:
                    d["lsum"] = jnp.sum(d["l"], axis=0, keepdims=True)
                if gg == GPB - 1 and hh == HPB - 1 and c == NC - 1:
                    pp[...] = _pack(p)
                    ot[hh * DH:(hh + 1) * DH, :] = d["acc"]
                    invs[...] = jnp.broadcast_to(_recip(d["lsum"]), (8, TQ))
                    return
                o = jnp.dot(v_rows(g, hh, c), p, preferred_element_type=f32)
                d["acc"] = o if c == 0 else d["acc"] + o
                if c == NC - 1:
                    d["out"] = d["acc"] * _recip(d["lsum"])
                    if gg == GPB - 1:
                        ot[hh * DH:(hh + 1) * DH, :] = d["out"]
                    elif hh == HPB - 1:
                        o_t = jnp.concatenate([st[gg, k]["out"] for k in range(HPB)], axis=0)
                        ob[g, o_rows(q0), :] = _pack(o_t.T.astype(bf16))

            pend = None
            for gg in range(GPB):
                for hh in range(HPB):
                    for c in range(NC):
                        s = qk(gg, hh, c)
                        if pend is None:
                            ob[jnp.where(i == 0, NT, i * GPB - 1), o_rows(q0), :] = _pack(
                                finish_group(jnp.maximum(i * GPB - 1, 0)))
                        else:
                            pv(*pend)
                        pend = (gg, hh, c, s)
            pv(*pend)
            for d in st.values():
                lmax = jnp.maximum(lmax, d["lsum"])
            return lmax

        return lax.fori_loop(0, NT // GPB, body, jnp.zeros((1, TQ), f32))

    def attn_exact(q0):
        def group(g, carry):
            def head(hh, carry2):
                w = qt[pl.ds(pl.multiple_of(g * 64, 64), 64), pl.ds(q0, TQ)]
                row = lax.broadcasted_iota(jnp.int32, (64, TQ), 0) // 16
                w = _unpack(jnp.where(row == hh, w, jnp.zeros_like(w)))

                def scores(c):
                    kc = kb[g, pl.ds(pl.multiple_of(c * (KC // 2), KC // 2), KC // 2), :]
                    return jnp.dot(_unpack(kc), w, preferred_element_type=f32)

                def row_max(c, m):
                    return jnp.maximum(m, jnp.max(scores(c), axis=0, keepdims=True))

                m = lax.fori_loop(0, NC, row_max, jnp.full((1, TQ), -jnp.inf, f32))

                def accumulate(c, state):
                    l, acc = state
                    p = jnp.exp2(scores(c) - m)
                    v = vt[pl.ds(pl.multiple_of(g * 64 + hh * 16, 16), 16),
                           pl.ds(pl.multiple_of(c * KC, KC), KC)]
                    o = jnp.dot(_unpack(v), p.astype(bf16), preferred_element_type=f32)
                    return l + jnp.sum(p, axis=0, keepdims=True), acc + o

                l, acc = lax.fori_loop(0, NC, accumulate,
                                       (jnp.zeros((1, TQ), f32), jnp.zeros((DH, TQ), f32)))
                ot[pl.ds(pl.multiple_of(hh * DH, DH), DH), :] = acc * (1.0 / l)
                return carry2
            lax.fori_loop(0, HPB, head, 0)
            ob[g, o_rows(q0), :] = _pack(ot[...].T.astype(bf16))
            return carry
        lax.fori_loop(0, NT, group, 0)
        pp[...] = jnp.zeros(pp.shape, u32)
        invs[...] = jnp.ones(invs.shape, f32)

    def q_body(qb, l):
        q0 = pl.multiple_of(qb * TQ, TQ)

        def attempt(state):
            a, _ = state

            @pl.when(a == 0)
            def _():
                lmx[...] = jnp.broadcast_to(attn_fast(q0), (8, TQ))

            @pl.when(a == 1)
            def _():
                attn_exact(q0)

            @pl.when(jnp.logical_or(l == 1, a == 1))
            def _():
                for j in range(TQ // OC):
                    out_copy(qb, j).wait()

            kd = (NT - 1) * 128
            o = jnp.concatenate([_unpack(ob[g, o_rows(q0), :]) for g in range(NT - 1)], axis=1)
            o_last = None
            for j in range(TQ // OC):
                y = lax.dot_general(o[j * OC:(j + 1) * OC], wob[0:kd, :], NN,
                                    preferred_element_type=f32)
                if j == 0:
                    o_last = finish_group(NT - 1)
                    y_first = y
                    continue
                if j == 2:
                    bad = _tree(jnp.maximum, [jnp.where(lmx[:, i * 128:(i + 1) * 128] <= L_MAX, 0.0, 1.0)
                                              for i in range(TQ // 128)])
                    v_ok = (vbig[...] & jnp.uint32(0x80008000)) == 0
                    unsafe = jnp.max(jnp.where(v_ok, bad, 1.0))
                for jj in ((0, 1) if j == 1 else (j,)):
                    yj = (y_first if jj == 0 else y) + lax.dot_general(
                        o_last[jj * OC:(jj + 1) * OC], wob[kd:D, :], NN, preferred_element_type=f32)
                    rows = pl.ds(q0 + jj * OC, OC)
                    x2 = xs[rows, :] + yj
                    xs2[rows, :] = x2
                    outb[rows, :] = x2.astype(bf16)
                    out_copy(qb, jj).start()
            return a + 1, unsafe

        lax.while_loop(lambda st: jnp.logical_or(st[0] == 0, jnp.logical_and(st[0] == 1, st[1] > 0.5)),
                       attempt, (jnp.int32(0), jnp.float32(0)))
        return l

    def layer_pair(l, carry):
        ka[:, 0:HALO, :] = jnp.zeros((NDUP * NT, HALO, 128), f32)
        va[:, 0:HALO, :] = jnp.zeros((NDUP * NT, HALO, 128), f32)
        vbig[...] = jnp.zeros(vbig.shape, u32)

        @pl.when(l == 1)
        def _():
            load_x(0, l, 32)

        lax.fori_loop(0, S // RB, row_body, l)

        @pl.when(l == 0)
        def _():
            wob_copy.wait()

        lax.fori_loop(0, S // TQ, q_body, l)
        return carry

    x_copy(0).wait()
    load_x(0, 0, 32)
    for i in range(NWO):
        woa_copy(i).wait()
        if i == LATE_AT:
            for cp in late:
                cp.start()
        lax.fori_loop(i * NT // NWO, (i + 1) * NT // NWO, prep_woa, 0)
    lax.fori_loop(0, 2, layer_pair, 0)
    for qb in range(S // TQ):
        for j in range(TQ // OC):
            out_copy(qb, j).wait()


@jax.jit
def pallas_interleave_layers__sliding_local_dilated__softmax_full_mha__prompt_kernel(
    A_x: jax.Array,
    A_wqkv: jax.Array,
    A_wo: jax.Array,
    B_x: jax.Array,
    B_wqkv: jax.Array,
    B_wo: jax.Array,
):
    del B_x
    x = A_x.reshape(S, D)
    hbm = pl.BlockSpec(memory_space=pl.ANY)
    out = pl.pallas_call(
        _kernel,
        out_shape=jax.ShapeDtypeStruct((S, D), bf16),
        in_specs=[hbm] * 5,
        out_specs=hbm,
        scratch_shapes=[
            pltpu.VMEM((S, D), bf16),
            pltpu.VMEM((D, 3 * D), bf16),
            pltpu.VMEM((D, D), bf16),
            pltpu.VMEM((D, 3 * D), bf16),
            pltpu.VMEM((D, D), bf16),
            pltpu.VMEM((S, D), bf16),
            pltpu.VMEM((3, H * PITCH, 128), f32),
            pltpu.VMEM((H * WPITCH, 128), u32),
            pltpu.VMEM((D // 2, 3 * D), u32),
            pltpu.VMEM((D // 2, D), u32),
            pltpu.VMEM((RB // 2, D), u32),
            pltpu.VMEM((S + RB, D), f32),
            pltpu.VMEM((S, D), f32),
            pltpu.VMEM((NT, RB, 128), f32),
            pltpu.VMEM((NDUP * NT, HALO + RB, 128), f32),
            pltpu.VMEM((NDUP * NT, HALO + RB, 128), f32),
            pltpu.VMEM((D // 2, S), u32),
            pltpu.VMEM((NT, S // 2, 128), u32),
            pltpu.VMEM((D // 2, S), u32),
            pltpu.VMEM((NT + 1, S // 2, 128), u32),
            pltpu.VMEM((128, TQ), f32),
            pltpu.VMEM((KC // 2, TQ), u32),
            pltpu.VMEM((8, TQ), f32),
            pltpu.VMEM((8, TQ), f32),
            pltpu.VMEM((8, 128), u32),
            pltpu.SemaphoreType.DMA((S // RB,)),
            pltpu.SemaphoreType.DMA((NT,)),
            pltpu.SemaphoreType.DMA((4 + NWO,)),
            pltpu.SemaphoreType.DMA((S // OC,)),
        ],
        compiler_params=pltpu.CompilerParams(vmem_limit_bytes=110 * 1024 * 1024),
    )(x, A_wqkv, A_wo, B_wqkv, B_wo)
    return out.reshape(1, S, D)
```

```python
import functools
import math

import jax
import jax.numpy as jnp
from jax import lax
import jax.experimental.pallas as pl
import jax.experimental.pallas.tpu as pltpu

S = 2048
D = 1024
H = 32
DH = 32
WIN = 8
DIL = 2
EPS = 1e-5
NT = D // 128
HALO = 16
QSCALE = (DH ** -0.5) * math.log2(math.e)

SB = 128
NSUB = 2
RB = SB * NSUB
RC = 8
ROW_HEADS = [[("a", 0), ("a", 1), ("o", 0), ("h", 0), ("l", 0), ("o", 1), ("w", 0), ("l", 1)],
             [("a", 0), ("a", 1), ("o", 0), ("h", 0), ("l", 0), ("o", 1), ("r", 1), ("w", 0), ("m", 1)]]
HEAD = 1
ROW_HEAD = ROW_HEADS[HEAD]
ROW_TAILS = [
    [("b", (0, 0, 1)), ("b", (2, 0, 1)), ("b", (1, 0, 1)), ("n", 0), ("b", (0, 1, 1)), ("b", (2, 1, 1)), ("b", (1, 1, 1))],
    [("b", (0, 0, 1)), ("n", 0), ("b", (2, 0, 2)), ("b", (0, 1, 1)), ("b", (1, 0, 2))],
    [("b", (0, 0, 1)), ("b", (2, 0, 2)), ("n", 0), ("b", (0, 1, 1)), ("b", (1, 0, 2))],
    [("b", (1, 0, 1)), ("n", 0), ("b", (2, 0, 2)), ("b", (0, 0, 2)), ("b", (1, 1, 1))],
    [("b", (0, 0, 1)), ("b", (2, 0, 1)), ("n", 0), ("b", (0, 1, 1)), ("b", (2, 1, 1)), ("b", (1, 0, 2))],
]
TAIL = 0
ROW_ORDER = ROW_HEAD + ROW_TAILS[TAIL]
LC = 8
LN_LOOK = (2, 1)
LX_LOOK = 1
NDUP = 1
TILE_GATE = (2, 2)
PV_GATE = (1, 1)
T_OUTER = True
PV_TREE = True
LOOK = (1, 2)
DEP_END = (False, False)
GATE_COL = (2048, 2048)
TQ = 512
KC = 256
NC = S // KC
OC = 128
WOB_PACK = False
T1O = 4
T1_ORDERS = [
    [("m", 0), ("f", 0), ("m", 1), ("r", 0), ("r", 1), ("m", 2), ("c", 0), ("r", 2), ("m", 3), ("r", 3)],
    [("m", 0), ("f", 0), ("r", 0), ("w", 1), ("c", 0), ("w", 2), ("w", 3)],
    [("f", 0), ("m", 0), ("w", 1), ("r", 0), ("c", 0), ("w", 2), ("w", 3)],
    [("m", 0), ("f", 0), ("w", 1), ("c", 0), ("w", 2), ("r", 0), ("w", 3)],
    [("f", 0), ("w", 0), ("w", 1), ("c", 0), ("w", 2), ("w", 3)],
    [("m", 0), ("m", 1), ("f", 0), ("w", 2), ("r", 0), ("r", 1), ("c", 0), ("w", 3)],
]
GPB = 2
HPB = 4
NWO = 4
WA_STARTS = (2, 1, 2, 1, 2, 1, 1, 0)
LATE_AT = 3
XLU_TILES = (8, 8, 0)
WPITCH = 20
PITCH = 40
NFLIGHT = 3
L_MAX = 2.0 ** 64
V_EXP = 50

bf16 = jnp.bfloat16
f32 = jnp.float32
u32 = jnp.uint32

NN = (((1,), (0,)), ((), ()))
NTD = (((1,), (1,)), ((), ()))


def _pack(x):
    return pltpu.bitcast(x, u32)


def _unpack(x):
    return pltpu.bitcast(x, bf16)


def _after(value, dep):
    if dep is None:
        return value
    return jnp.maximum(value, jnp.minimum(dep, -3e38))


def _tree(op, xs):
    xs = list(xs)
    while len(xs) > 1:
        xs = [op(xs[i], xs[i + 1]) if i + 1 < len(xs) else xs[i] for i in range(0, len(xs), 2)]
    return xs[0]


def _recip(x):
    r = pl.reciprocal(x, approx=True)
    return r * (2.0 - x * r)


def _too_large(packed):
    bias = 0x8000 - ((127 + V_EXP) << 7)
    t = (packed & jnp.uint32(0x7F807F80)) + jnp.uint32(bias << 16 | bias)
    return _tree(jnp.bitwise_or, [t[i:i + 8] for i in range(0, t.shape[0], 8)])


def _layernorm(load, nrows, look, first_dep=None):
    outs = []
    deps = []
    for c in range(nrows // LC):
        dep = deps[c - look] if c >= look else first_dep
        x = load(c * LC, dep)
        mu = jnp.broadcast_to(jnp.sum(x, axis=-1, keepdims=True), (LC, 128)) * _after(1.0 / D, dep)
        xc = x - jnp.concatenate([mu] * NT, axis=1)
        var = jnp.sum(xc * xc, axis=-1, keepdims=True) * (1.0 / D)
        y = xc * lax.rsqrt(var + EPS)
        deps.append(y[:, D - 128:])
        outs.append(y)
    return jnp.concatenate(outs, axis=0).astype(bf16)


def _kernel(x_hbm, wa_hbm, woa_hbm, wb_hbm, wob_hbm, out_hbm,
            xin, wa_raw, woa_raw, wb_raw, wob, wobp, outb,
            stg, stw, wan, woa, xnb,
            xs, xs2, qa, ka, va, qt, kb, vt, ob, ot, pp, invs, lmx, vbig,
            sem_x, sem_wa, sem_w, sem_o):
    def x_copy(r):
        rows = pl.ds(pl.multiple_of(r * RB, RB), RB)
        return pltpu.make_async_copy(x_hbm.at[rows, :], xin.at[rows, :], sem_x.at[r])

    def wa_copy(i):
        rows = pl.ds(pl.multiple_of(i * 128, 128), 128)
        return pltpu.make_async_copy(wa_hbm.at[rows, :], wa_raw.at[rows, :], sem_wa.at[i])

    wb_copy = pltpu.make_async_copy(wb_hbm, wb_raw, sem_w.at[0])

    def woa_copy(i):
        cols = pl.ds(pl.multiple_of(i * (D // NWO), D // NWO), D // NWO)
        return pltpu.make_async_copy(woa_hbm.at[:, cols], woa_raw.at[:, cols], sem_w.at[2 + i])

    wob_copy = pltpu.make_async_copy(wob_hbm, wob, sem_w.at[1])

    def out_copy(qb, j):
        rows = pl.ds(pl.multiple_of(qb * TQ + j * OC, OC), OC)
        return pltpu.make_async_copy(outb.at[rows, :], out_hbm.at[rows, :],
                                     sem_o.at[qb * (TQ // OC) + j])

    queue = ([wa_copy(i) for i in range(NT)]
             + [x_copy(0)] + [woa_copy(i) for i in range(NWO)]
             + [x_copy(1), wb_copy]
             + [x_copy(r) for r in range(2, S // RB)] + [wob_copy])
    for cp in queue[:NFLIGHT]:
        cp.start()
    queue = queue[NFLIGHT:]

    batches = [[queue.pop(0) for _ in range(n)] for n in WA_STARTS]
    late = [queue.pop(0) for _ in range(NT + 3 + NWO - NFLIGHT - sum(WA_STARTS))]

    def start_in_loop(i, my_batches):
        for k, batch in enumerate(my_batches):
            @pl.when(i == k)
            def _():
                for cp in batch:
                    cp.start()

    def transpose(w):
        ri = lax.broadcasted_iota(jnp.int32, (128, 128), 0)
        ci = lax.broadcasted_iota(jnp.int32, (128, 128), 1)
        eye = jnp.where(ri == ci, 1.0, 0.0).astype(bf16)
        return lax.dot_general(eye, w, NTD, preferred_element_type=f32)

    def prep_wa(t, carry):
        wa_copy(t).wait()
        start_in_loop(t, batches)
        rows = pl.ds(pl.multiple_of(t * 128, 128), 128)

        def forward(part):
            for j in range(NT):
                wt = transpose(wa_raw[rows, part * D + j * 128:part * D + (j + 1) * 128])
                for hh in range(HPB):
                    r = (j * HPB + hh) * PITCH
                    stg[part, r:r + DH, :] = wt[hh * DH:(hh + 1) * DH]

        def back(part):
            regrouped = jnp.concatenate([stg[part, pl.ds(d, H, stride=PITCH), :]
                                         for d in range(DH)], axis=0)
            n = XLU_TILES[part] * 128
            pieces = []
            if n > 0:
                pieces.append(regrouped[:n].T)
            if n < D:
                pieces.append(transpose(regrouped[n:].astype(bf16)))
            wan[pl.ds(pl.multiple_of(t * 64, 64), 64), part * D:(part + 1) * D] = _pack(
                jnp.concatenate(pieces, axis=1).astype(bf16))

        forward(0)
        forward(1)
        back(0)
        forward(2)
        back(1)
        back(2)
        return carry

    def prep_woa(t, carry):
        cols = pl.ds(pl.multiple_of(t * 128, 128), 128)
        w = _pack(woa_raw[:, cols])
        for h in range(H):
            stw[h * WPITCH:h * WPITCH + DH // 2, :] = w[h * (DH // 2):(h + 1) * (DH // 2)]
        lo = jnp.uint32(0xFFFF)
        for j in range(DH // 2):
            even = stw[pl.ds(j, H // 2, stride=2 * WPITCH), :]
            odd = stw[pl.ds(WPITCH + j, H // 2, stride=2 * WPITCH), :]
            woa[2 * j * 16:(2 * j + 1) * 16, cols] = (even & lo) | (odd << 16)
            woa[(2 * j + 1) * 16:(2 * j + 2) * 16, cols] = (even >> 16) | (odd & ~lo)
        return carry

    ot[...] = jnp.zeros(ot.shape, f32)
    pp[...] = jnp.zeros(pp.shape, u32)
    invs[...] = jnp.ones(invs.shape, f32)
    lax.fori_loop(0, NT, prep_wa, 0)

    def local_attn(r0, s, first_dep):
        outs = []
        deps = []
        for c in range(SB // RC):
            base = s * SB + c * RC
            scale = _after(QSCALE, deps[c - LOOK[s]] if c >= LOOK[s] else first_dep)
            logits = [None] * WIN
            dup = NT * (c % NDUP)
            if T_OUTER:
                for t in range(NT):
                    if TILE_GATE[s] and t > 0 and t % TILE_GATE[s] == 0:
                        scale = _after(QSCALE, logits[WIN - 1])
                    q = qa[t, base:base + RC, :] * scale
                    for w in range(WIN):
                        o0 = HALO + base - DIL * w
                        term = q * ka[t + dup, o0:o0 + RC, :]
                        logits[w] = term if t == 0 else logits[w] + term
            else:
                q = [qa[t, base:base + RC, :] * scale for t in range(NT)]
                for w in range(WIN):
                    o0 = HALO + base - DIL * w
                    terms = [q[t] * ka[t + dup, o0:o0 + RC, :] for t in range(NT)]
                    logits[w] = functools.reduce(jnp.add, terms)
            for w in range(WIN):
                acc = logits[w]
                acc = acc + pltpu.roll(acc, 64, 1)
                acc = acc + pltpu.roll(acc, 32, 1)
                if base < DIL * w:
                    row = r0 + base + lax.broadcasted_iota(jnp.int32, (RC, 128), 0)
                    acc = jnp.where(row >= DIL * w, acc, -1e9)
                logits[w] = acc
            m = _tree(jnp.maximum, logits)
            p = [jnp.exp2(lg - m) for lg in logits]
            inv = _recip(_tree(jnp.add, p))
            tiles = []
            done = []
            for t in range(NT):
                if PV_GATE[s] and t >= PV_GATE[s]:
                    p[0] = _after(p[0], done[t - PV_GATE[s]])
                terms = [p[w] * va[t + dup, HALO + base - DIL * w:HALO + base - DIL * w + RC, :]
                         for w in range(WIN)]
                acc = (_tree(jnp.add, terms) if PV_TREE else functools.reduce(jnp.add, terms)) * inv
                tiles.append(acc.astype(bf16))
                done.append(acc)
            deps.append(acc if DEP_END[s] else m)
            outs.append(jnp.concatenate(tiles, axis=1))
        return jnp.concatenate(outs, axis=0)

    def load_x(r, l, look):
        r0 = pl.multiple_of(jnp.minimum(r, S // RB - 1) * RB, RB)
        w0 = pl.multiple_of(r * RB, RB)

        def load(start, dep):
            rows = pl.ds(r0 + start, LC)
            lvec = _after(jnp.full((LC, 128), l, f32), dep)
            first = jnp.concatenate([lvec == 0.0] * NT, axis=1)
            xi = xin[pl.ds(r0 + start // 16 * 16, 16), :].astype(f32)[start % 16:start % 16 + LC]
            x = jnp.where(first, xi, xs2[rows, :])
            xs[pl.ds(w0 + start, LC), :] = x
            return x

        xnb[...] = _pack(_layernorm(load, RB, look))

    def row_body(r, l):
        r0 = pl.multiple_of(r * RB, RB)
        rn = jnp.minimum(r + 1, S // RB - 1)

        @pl.when(jnp.logical_and(l == 0, r == 1))
        def _():
            for cp in queue:
                cp.start()

        rows = [pl.ds(r0 + s * SB, SB) for s in range(NSUB)]
        gate = {}
        xn2 = {}
        ya = {}

        def qkv_a(s):
            xn = _unpack(xnb[s * SB // 2:(s + 1) * SB // 2, :])
            y = lax.dot_general(xn, _unpack(wan[...]), NN, preferred_element_type=f32)
            for t in range(NT):
                qa[t, s * SB:(s + 1) * SB, :] = y[:, t * 128:(t + 1) * 128]
                for dup in range(0, NDUP * NT, NT):
                    new = slice(HALO + s * SB, HALO + (s + 1) * SB)
                    ka[t + dup, new, :] = y[:, D + t * 128:D + (t + 1) * 128]
                    va[t + dup, new, :] = y[:, 2 * D + t * 128:2 * D + (t + 1) * 128]
            gate[s] = y[SB - RC:SB, GATE_COL[s] - 128:GATE_COL[s]]

        def out_a(s):
            o = local_attn(r0, s, gate[s])
            ya[s] = lax.dot_general(o, _unpack(woa[...]), NN, preferred_element_type=f32)

        def norm_b(s):
            x1 = xs[rows[s], :] + ya[s]
            xs[rows[s], :] = x1
            xn2[s] = _layernorm(lambda st, dep: x1[st:st + LC], SB, LN_LOOK[s])

        def res_only(s):
            xs[rows[s], :] = xs[rows[s], :] + ya[s]

        def norm_only(s):
            xn2[s] = _layernorm(lambda st, dep: xs[pl.ds(r0 + s * SB + st, LC), :], SB, LN_LOOK[s])

        def weights_b(_):
            @pl.when(jnp.logical_and(l == 0, r == 0))
            def _():
                wb_copy.wait()

            @pl.when(jnp.logical_and(l == 0, r + 1 < S // RB))
            def _():
                x_copy(rn).wait()

        def proj_b(arg):
            part, s, n = arg
            xn = jnp.concatenate([xn2[s + i] for i in range(n)], axis=0)
            y = lax.dot_general(xn, wb_raw[:, part * D:(part + 1) * D], NN, preferred_element_type=f32)
            cols = pl.ds(r0 + s * SB, n * SB)
            if part == 0:
                qt[:, cols] = _pack((y * QSCALE).T.astype(bf16))
            elif part == 2:
                v_t = _pack(y.T.astype(bf16))
                vt[:, cols] = v_t
                for i in range(n):
                    vbig[...] = vbig[...] | _too_large(v_t[:, i * SB:(i + 1) * SB])
            else:
                krows = pl.ds(pl.multiple_of((r0 + s * SB) // 2, SB // 2), n * SB // 2)
                y = y.astype(bf16)
                for g in range(NT):
                    kb[g, krows, :] = _pack(y[:, g * 128:(g + 1) * 128])

        steps = {"a": qkv_a, "o": out_a, "b": proj_b, "w": weights_b, "l": norm_b,
                 "r": res_only, "m": norm_only}
        for name, s in ROW_ORDER:
            if name == "h":
                ka[:, 0:HALO, :] = ka[:, RB:RB + HALO, :]
                va[:, 0:HALO, :] = va[:, RB:RB + HALO, :]
            elif name == "n":
                load_x(r + 1, l, LX_LOOK)
            else:
                steps[name](s)
        return l

    def head_weights(g, hh, q0):
        w = qt[pl.ds(pl.multiple_of(g * 64 + hh * 16, 16), 16), pl.ds(q0, TQ)]
        parts = []
        if hh > 0:
            parts.append(jnp.zeros((16 * hh, TQ), u32))
        parts.append(w)
        if hh < 3:
            parts.append(jnp.zeros((16 * (3 - hh), TQ), u32))
        return _unpack(jnp.concatenate(parts, axis=0))

    def v_rows(g, hh, c):
        rows = pl.ds(pl.multiple_of(g * 64 + hh * 16, 16), 16)
        return _unpack(vt[rows, c * KC:(c + 1) * KC])

    def finish_group(g):
        o = jnp.dot(v_rows(g, HPB - 1, NC - 1), _unpack(pp[...]), preferred_element_type=f32)
        last = (ot[3 * DH:4 * DH, :] + o) * invs[0:1, :]
        return jnp.concatenate([ot[0:3 * DH, :], last], axis=0).T.astype(bf16)

    def o_rows(q0):
        return pl.ds(pl.multiple_of(q0 // 2, TQ // 2), TQ // 2)

    def attn_fast(q0):
        def body(i, lmax):
            st = {}

            def qk(gg, hh, c):
                g = i * GPB + gg
                if c == 0:
                    st[gg, hh] = dict(w=head_weights(g, hh, q0))
                kc = _unpack(kb[g, c * KC // 2:(c + 1) * KC // 2, :])
                return jnp.dot(kc, st[gg, hh]["w"], preferred_element_type=f32)

            def pv(gg, hh, c, s):
                g = i * GPB + gg
                d = st[gg, hh]
                if c == 0:
                    d["m"] = jnp.broadcast_to(jnp.max(s[0:8], axis=0, keepdims=True), (8, TQ))
                p = jnp.exp2(s.reshape(KC // 8, 8, TQ) - d["m"][None])
                lc = jnp.sum(p, axis=0)
                d["l"] = lc if c == 0 else d["l"] + lc
                p = p.reshape(KC, TQ).astype(bf16)
                if c == NC - 1:
                    d["lsum"] = jnp.sum(d["l"], axis=0, keepdims=True)
                if gg == GPB - 1 and hh == HPB - 1 and c == NC - 1:
                    pp[...] = _pack(p)
                    ot[hh * DH:(hh + 1) * DH, :] = d["acc"]
                    invs[...] = jnp.broadcast_to(_recip(d["lsum"]), (8, TQ))
                    return
                o = jnp.dot(v_rows(g, hh, c), p, preferred_element_type=f32)
                d["acc"] = o if c == 0 else d["acc"] + o
                if c == NC - 1:
                    d["out"] = d["acc"] * _recip(d["lsum"])
                    if gg == GPB - 1:
                        ot[hh * DH:(hh + 1) * DH, :] = d["out"]
                    elif hh == HPB - 1:
                        o_t = jnp.concatenate([st[gg, k]["out"] for k in range(HPB)], axis=0)
                        ob[g, o_rows(q0), :] = _pack(o_t.T.astype(bf16))

            pend = None
            for gg in range(GPB):
                for hh in range(HPB):
                    for c in range(NC):
                        s = qk(gg, hh, c)
                        if pend is None:
                            ob[jnp.where(i == 0, NT, i * GPB - 1), o_rows(q0), :] = _pack(
                                finish_group(jnp.maximum(i * GPB - 1, 0)))
                        else:
                            pv(*pend)
                        pend = (gg, hh, c, s)
            pv(*pend)
            for d in st.values():
                lmax = jnp.maximum(lmax, d["lsum"])
            return lmax

        return lax.fori_loop(0, NT // GPB, body, jnp.zeros((1, TQ), f32))

    def attn_exact(q0):
        def group(g, carry):
            def head(hh, carry2):
                w = qt[pl.ds(pl.multiple_of(g * 64, 64), 64), pl.ds(q0, TQ)]
                row = lax.broadcasted_iota(jnp.int32, (64, TQ), 0) // 16
                w = _unpack(jnp.where(row == hh, w, jnp.zeros_like(w)))

                def scores(c):
                    kc = kb[g, pl.ds(pl.multiple_of(c * (KC // 2), KC // 2), KC // 2), :]
                    return jnp.dot(_unpack(kc), w, preferred_element_type=f32)

                def row_max(c, m):
                    return jnp.maximum(m, jnp.max(scores(c), axis=0, keepdims=True))

                m = lax.fori_loop(0, NC, row_max, jnp.full((1, TQ), -jnp.inf, f32))

                def accumulate(c, state):
                    l, acc = state
                    p = jnp.exp2(scores(c) - m)
                    v = vt[pl.ds(pl.multiple_of(g * 64 + hh * 16, 16), 16),
                           pl.ds(pl.multiple_of(c * KC, KC), KC)]
                    o = jnp.dot(_unpack(v), p.astype(bf16), preferred_element_type=f32)
                    return l + jnp.sum(p, axis=0, keepdims=True), acc + o

                l, acc = lax.fori_loop(0, NC, accumulate,
                                       (jnp.zeros((1, TQ), f32), jnp.zeros((DH, TQ), f32)))
                ot[pl.ds(pl.multiple_of(hh * DH, DH), DH), :] = acc * (1.0 / l)
                return carry2
            lax.fori_loop(0, HPB, head, 0)
            ob[g, o_rows(q0), :] = _pack(ot[...].T.astype(bf16))
            return carry
        lax.fori_loop(0, NT, group, 0)
        pp[...] = jnp.zeros(pp.shape, u32)
        invs[...] = jnp.ones(invs.shape, f32)

    def q_body(qb, l):
        q0 = pl.multiple_of(qb * TQ, TQ)

        def attempt(state):
            a, _ = state

            @pl.when(a == 0)
            def _():
                lmx[...] = jnp.broadcast_to(attn_fast(q0), (8, TQ))

            @pl.when(a == 1)
            def _():
                attn_exact(q0)

            @pl.when(jnp.logical_or(l == 1, a == 1))
            def _():
                for j in range(TQ // OC):
                    out_copy(qb, j).wait()

            kd = (NT - 1) * 128
            o = jnp.concatenate([_unpack(ob[g, o_rows(q0), :]) for g in range(NT - 1)], axis=1)
            val = {}

            def w_rows(lo, hi):
                return _unpack(wobp[lo // 2:hi // 2, :]) if WOB_PACK else wob[lo:hi, :]

            def main(j):
                val[j] = lax.dot_general(o[j * OC:(j + 1) * OC], w_rows(0, kd), NN,
                                         preferred_element_type=f32)

            def finish(_):
                val["last"] = finish_group(NT - 1)

            def rest(j):
                yj = val[j] + lax.dot_general(val["last"][j * OC:(j + 1) * OC], w_rows(kd, D), NN,
                                              preferred_element_type=f32)
                rows = pl.ds(q0 + j * OC, OC)
                x2 = xs[rows, :] + yj
                xs2[rows, :] = x2
                outb[rows, :] = x2.astype(bf16)
                out_copy(qb, j).start()

            def whole(j):
                oj = jnp.concatenate([o[j * OC:(j + 1) * OC], val["last"][j * OC:(j + 1) * OC]], axis=1)
                yj = lax.dot_general(oj, w_rows(0, D), NN, preferred_element_type=f32)
                rows = pl.ds(q0 + j * OC, OC)
                x2 = xs[rows, :] + yj
                xs2[rows, :] = x2
                outb[rows, :] = x2.astype(bf16)
                out_copy(qb, j).start()

            def check(_):
                bad = _tree(jnp.maximum, [jnp.where(lmx[:, i * 128:(i + 1) * 128] <= L_MAX, 0.0, 1.0)
                                          for i in range(TQ // 128)])
                v_ok = (vbig[...] & jnp.uint32(0x80008000)) == 0
                val["unsafe"] = jnp.max(jnp.where(v_ok, bad, 1.0))

            for name, j in T1_ORDERS[T1O]:
                {"m": main, "f": finish, "r": rest, "w": whole, "c": check}[name](j)
            unsafe = val["unsafe"]
            return a + 1, unsafe

        lax.while_loop(lambda st: jnp.logical_or(st[0] == 0, jnp.logical_and(st[0] == 1, st[1] > 0.5)),
                       attempt, (jnp.int32(0), jnp.float32(0)))
        return l

    def layer_pair(l, carry):
        ka[:, 0:HALO, :] = jnp.zeros((NDUP * NT, HALO, 128), f32)
        va[:, 0:HALO, :] = jnp.zeros((NDUP * NT, HALO, 128), f32)
        vbig[...] = jnp.zeros(vbig.shape, u32)

        @pl.when(l == 1)
        def _():
            load_x(0, l, 32)

        lax.fori_loop(0, S // RB, row_body, l)

        @pl.when(l == 0)
        def _():
            wob_copy.wait()
            if WOB_PACK:
                wobp[...] = _pack(wob[...])

        lax.fori_loop(0, S // TQ, q_body, l)
        return carry

    x_copy(0).wait()
    load_x(0, 0, 32)
    for i in range(NWO):
        woa_copy(i).wait()
        if i == LATE_AT:
            for cp in late:
                cp.start()
        lax.fori_loop(i * NT // NWO, (i + 1) * NT // NWO, prep_woa, 0)
    lax.fori_loop(0, 2, layer_pair, 0)
    for qb in range(S // TQ):
        for j in range(TQ // OC):
            out_copy(qb, j).wait()


@jax.jit
def pallas_interleave_layers__sliding_local_dilated__softmax_full_mha__prompt_kernel(
    A_x: jax.Array,
    A_wqkv: jax.Array,
    A_wo: jax.Array,
    B_x: jax.Array,
    B_wqkv: jax.Array,
    B_wo: jax.Array,
):
    del B_x
    x = A_x.reshape(S, D)
    hbm = pl.BlockSpec(memory_space=pl.ANY)
    out = pl.pallas_call(
        _kernel,
        out_shape=jax.ShapeDtypeStruct((S, D), bf16),
        in_specs=[hbm] * 5,
        out_specs=hbm,
        scratch_shapes=[
            pltpu.VMEM((S, D), bf16),
            pltpu.VMEM((D, 3 * D), bf16),
            pltpu.VMEM((D, D), bf16),
            pltpu.VMEM((D, 3 * D), bf16),
            pltpu.VMEM((D, D), bf16),
            pltpu.VMEM((D // 2, D), u32),
            pltpu.VMEM((S, D), bf16),
            pltpu.VMEM((3, H * PITCH, 128), f32),
            pltpu.VMEM((H * WPITCH, 128), u32),
            pltpu.VMEM((D // 2, 3 * D), u32),
            pltpu.VMEM((D // 2, D), u32),
            pltpu.VMEM((RB // 2, D), u32),
            pltpu.VMEM((S + RB, D), f32),
            pltpu.VMEM((S, D), f32),
            pltpu.VMEM((NT, RB, 128), f32),
            pltpu.VMEM((NDUP * NT, HALO + RB, 128), f32),
            pltpu.VMEM((NDUP * NT, HALO + RB, 128), f32),
            pltpu.VMEM((D // 2, S), u32),
            pltpu.VMEM((NT, S // 2, 128), u32),
            pltpu.VMEM((D // 2, S), u32),
            pltpu.VMEM((NT + 1, S // 2, 128), u32),
            pltpu.VMEM((128, TQ), f32),
            pltpu.VMEM((KC // 2, TQ), u32),
            pltpu.VMEM((8, TQ), f32),
            pltpu.VMEM((8, TQ), f32),
            pltpu.VMEM((8, 128), u32),
            pltpu.SemaphoreType.DMA((S // RB,)),
            pltpu.SemaphoreType.DMA((NT,)),
            pltpu.SemaphoreType.DMA((2 + NWO,)),
            pltpu.SemaphoreType.DMA((S // OC,)),
        ],
        compiler_params=pltpu.CompilerParams(vmem_limit_bytes=110 * 1024 * 1024),
    )(x, A_wqkv, A_wo, B_wqkv, B_wo)
    return out.reshape(1, S, D)
```

```python
import math

import jax
import jax.numpy as jnp
from jax import lax
import jax.experimental.pallas as pl
import jax.experimental.pallas.tpu as pltpu

S = 2048
D = 1024
H = 32
DH = 32
WIN = 8
DIL = 2
EPS = 1e-5
NT = D // 128
HPB = 4
HALO = 16
QSCALE = (DH ** -0.5) * math.log2(math.e)

SB = 128
NSUB = 2
RB = SB * NSUB
RC = 8
LC = 8
LOOK = (1, 2)
TILE_GATE = (2, 2)
PV_GATE = (1, 1)
LN_LOOK = (2, 1)
LX_LOOK = 1

TQ = 512
KC = 256
NC = S // KC
GPB = 2
OC = 128
L_MAX = 2.0 ** 64
V_EXP = 50

NFLIGHT = 3
WA_STARTS = (2, 1, 2, 1, 2, 1, 1, 0)
NWO = 4
XLU_TILES = (8, 8, 0)
PITCH = 40
WPITCH = 20

bf16 = jnp.bfloat16
f32 = jnp.float32
u32 = jnp.uint32

NN = (((1,), (0,)), ((), ()))
NTD = (((1,), (1,)), ((), ()))


def _pack(x):
    return pltpu.bitcast(x, u32)


def _unpack(x):
    return pltpu.bitcast(x, bf16)


def _after(value, dep):
    if dep is None:
        return value
    return jnp.maximum(value, jnp.minimum(dep, -3e38))


def _tree(op, xs):
    xs = list(xs)
    while len(xs) > 1:
        xs = [op(xs[i], xs[i + 1]) if i + 1 < len(xs) else xs[i] for i in range(0, len(xs), 2)]
    return xs[0]


def _recip(x):
    r = pl.reciprocal(x, approx=True)
    return r * (2.0 - x * r)


def _too_large(packed):
    bias = 0x8000 - ((127 + V_EXP) << 7)
    t = (packed & jnp.uint32(0x7F807F80)) + jnp.uint32(bias << 16 | bias)
    return _tree(jnp.bitwise_or, [t[i:i + 8] for i in range(0, t.shape[0], 8)])


def _layernorm(load, nrows, look):
    outs = []
    deps = []
    for c in range(nrows // LC):
        dep = deps[c - look] if c >= look else None
        x = load(c * LC, dep)
        mu = jnp.broadcast_to(jnp.sum(x, axis=-1, keepdims=True), (LC, 128)) * _after(1.0 / D, dep)
        xc = x - jnp.concatenate([mu] * NT, axis=1)
        var = jnp.sum(xc * xc, axis=-1, keepdims=True) * (1.0 / D)
        y = xc * lax.rsqrt(var + EPS)
        deps.append(y[:, D - 128:])
        outs.append(y)
    return jnp.concatenate(outs, axis=0).astype(bf16)


def _kernel(x_hbm, wa_hbm, woa_hbm, wb_hbm, wob_hbm, out_hbm,
            xin, wa_raw, woa_raw, wb_raw, wob, outb,
            stg, stw, wan, woa, xnb,
            xs, xs2, qa, ka, va, qt, kb, vt, ob, ot, pp, invs, lmx, vbig,
            sem_x, sem_wa, sem_w, sem_o):
    def x_copy(r):
        rows = pl.ds(pl.multiple_of(r * RB, RB), RB)
        return pltpu.make_async_copy(x_hbm.at[rows, :], xin.at[rows, :], sem_x.at[r])

    def wa_copy(i):
        rows = pl.ds(pl.multiple_of(i * 128, 128), 128)
        return pltpu.make_async_copy(wa_hbm.at[rows, :], wa_raw.at[rows, :], sem_wa.at[i])

    wb_copy = pltpu.make_async_copy(wb_hbm, wb_raw, sem_w.at[0])

    def woa_copy(i):
        cols = pl.ds(pl.multiple_of(i * (D // NWO), D // NWO), D // NWO)
        return pltpu.make_async_copy(woa_hbm.at[:, cols], woa_raw.at[:, cols], sem_w.at[2 + i])

    wob_copy = pltpu.make_async_copy(wob_hbm, wob, sem_w.at[1])

    def out_copy(qb, j):
        rows = pl.ds(pl.multiple_of(qb * TQ + j * OC, OC), OC)
        return pltpu.make_async_copy(outb.at[rows, :], out_hbm.at[rows, :],
                                     sem_o.at[qb * (TQ // OC) + j])

    queue = ([wa_copy(i) for i in range(NT)]
             + [x_copy(0)] + [woa_copy(i) for i in range(NWO)]
             + [x_copy(1), wb_copy]
             + [x_copy(r) for r in range(2, S // RB)] + [wob_copy])
    for cp in queue[:NFLIGHT]:
        cp.start()
    queue = queue[NFLIGHT:]

    batches = [[queue.pop(0) for _ in range(n)] for n in WA_STARTS]
    late = [queue.pop(0) for _ in range(NT + 3 + NWO - NFLIGHT - sum(WA_STARTS))]

    def transpose(w):
        ri = lax.broadcasted_iota(jnp.int32, (128, 128), 0)
        ci = lax.broadcasted_iota(jnp.int32, (128, 128), 1)
        eye = jnp.where(ri == ci, 1.0, 0.0).astype(bf16)
        return lax.dot_general(eye, w, NTD, preferred_element_type=f32)

    def prep_wa(t, carry):
        wa_copy(t).wait()
        for k, batch in enumerate(batches):
            @pl.when(t == k)
            def _():
                for cp in batch:
                    cp.start()

        rows = pl.ds(pl.multiple_of(t * 128, 128), 128)

        def forward(part):
            for j in range(NT):
                wt = transpose(wa_raw[rows, part * D + j * 128:part * D + (j + 1) * 128])
                for hh in range(HPB):
                    r = (j * HPB + hh) * PITCH
                    stg[part, r:r + DH, :] = wt[hh * DH:(hh + 1) * DH]

        def back(part):
            regrouped = jnp.concatenate([stg[part, pl.ds(d, H, stride=PITCH), :]
                                         for d in range(DH)], axis=0)
            n = XLU_TILES[part] * 128
            pieces = []
            if n > 0:
                pieces.append(regrouped[:n].T)
            if n < D:
                pieces.append(transpose(regrouped[n:].astype(bf16)))
            wan[pl.ds(pl.multiple_of(t * 64, 64), 64), part * D:(part + 1) * D] = _pack(
                jnp.concatenate(pieces, axis=1).astype(bf16))

        forward(0)
        forward(1)
        back(0)
        forward(2)
        back(1)
        back(2)
        return carry

    def prep_woa(t, carry):
        cols = pl.ds(pl.multiple_of(t * 128, 128), 128)
        w = _pack(woa_raw[:, cols])
        for h in range(H):
            stw[h * WPITCH:h * WPITCH + DH // 2, :] = w[h * (DH // 2):(h + 1) * (DH // 2)]
        lo = jnp.uint32(0xFFFF)
        for j in range(DH // 2):
            even = stw[pl.ds(j, H // 2, stride=2 * WPITCH), :]
            odd = stw[pl.ds(WPITCH + j, H // 2, stride=2 * WPITCH), :]
            woa[2 * j * 16:(2 * j + 1) * 16, cols] = (even & lo) | (odd << 16)
            woa[(2 * j + 1) * 16:(2 * j + 2) * 16, cols] = (even >> 16) | (odd & ~lo)
        return carry

    ot[...] = jnp.zeros(ot.shape, f32)
    pp[...] = jnp.zeros(pp.shape, u32)
    invs[...] = jnp.ones(invs.shape, f32)
    lax.fori_loop(0, NT, prep_wa, 0)

    def local_attn(r0, s, first_dep):
        outs = []
        deps = []
        for c in range(SB // RC):
            base = s * SB + c * RC
            window = [slice(HALO + base - DIL * w, HALO + base - DIL * w + RC) for w in range(WIN)]
            scale = _after(QSCALE, deps[c - LOOK[s]] if c >= LOOK[s] else first_dep)
            logits = [None] * WIN
            for t in range(NT):
                if t > 0 and t % TILE_GATE[s] == 0:
                    scale = _after(QSCALE, logits[WIN - 1])
                q = qa[t, base:base + RC, :] * scale
                for w in range(WIN):
                    term = q * ka[t, window[w], :]
                    logits[w] = term if t == 0 else logits[w] + term
            for w in range(WIN):
                acc = logits[w]
                acc = acc + pltpu.roll(acc, 64, 1)
                acc = acc + pltpu.roll(acc, 32, 1)
                if base < DIL * w:
                    row = r0 + base + lax.broadcasted_iota(jnp.int32, (RC, 128), 0)
                    acc = jnp.where(row >= DIL * w, acc, -1e9)
                logits[w] = acc
            m = _tree(jnp.maximum, logits)
            p = [jnp.exp2(lg - m) for lg in logits]
            inv = _recip(_tree(jnp.add, p))
            tiles = []
            done = []
            for t in range(NT):
                if t >= PV_GATE[s]:
                    p[0] = _after(p[0], done[t - PV_GATE[s]])
                acc = _tree(jnp.add, [p[w] * va[t, window[w], :] for w in range(WIN)]) * inv
                tiles.append(acc.astype(bf16))
                done.append(acc)
            deps.append(m)
            outs.append(jnp.concatenate(tiles, axis=1))
        return jnp.concatenate(outs, axis=0)

    def load_x(r, l, look):
        r0 = pl.multiple_of(jnp.minimum(r, S // RB - 1) * RB, RB)
        w0 = pl.multiple_of(r * RB, RB)

        def load(start, dep):
            rows = pl.ds(r0 + start, LC)
            lvec = _after(jnp.full((LC, 128), l, f32), dep)
            first = jnp.concatenate([lvec == 0.0] * NT, axis=1)
            xi = xin[pl.ds(r0 + start // 16 * 16, 16), :].astype(f32)[start % 16:start % 16 + LC]
            x = jnp.where(first, xi, xs2[rows, :])
            xs[pl.ds(w0 + start, LC), :] = x
            return x

        xnb[...] = _pack(_layernorm(load, RB, look))

    def row_body(r, l):
        r0 = pl.multiple_of(r * RB, RB)
        rows = [pl.ds(r0 + s * SB, SB) for s in range(NSUB)]

        @pl.when(jnp.logical_and(l == 0, r == 1))
        def _():
            for cp in queue:
                cp.start()

        def qkv_a(s):
            xn = _unpack(xnb[s * SB // 2:(s + 1) * SB // 2, :])
            y = lax.dot_general(xn, _unpack(wan[...]), NN, preferred_element_type=f32)
            new = slice(HALO + s * SB, HALO + (s + 1) * SB)
            for t in range(NT):
                qa[t, s * SB:(s + 1) * SB, :] = y[:, t * 128:(t + 1) * 128]
                ka[t, new, :] = y[:, D + t * 128:D + (t + 1) * 128]
                va[t, new, :] = y[:, 2 * D + t * 128:2 * D + (t + 1) * 128]
            return y[SB - RC:SB, 2 * D - 128:2 * D]

        def out_a(s, k_done):
            o = local_attn(r0, s, k_done)
            return lax.dot_general(o, _unpack(woa[...]), NN, preferred_element_type=f32)

        def qkv_b(s, xn):
            cols = rows[s]
            y = lax.dot_general(xn, wb_raw[:, 0:D], NN, preferred_element_type=f32)
            qt[:, cols] = _pack((y * QSCALE).T.astype(bf16))
            y = lax.dot_general(xn, wb_raw[:, 2 * D:3 * D], NN, preferred_element_type=f32)
            v_t = _pack(y.T.astype(bf16))
            vt[:, cols] = v_t
            vbig[...] = vbig[...] | _too_large(v_t)
            y = lax.dot_general(xn, wb_raw[:, D:2 * D], NN, preferred_element_type=f32).astype(bf16)
            krows = pl.ds(pl.multiple_of((r0 + s * SB) // 2, SB // 2), SB // 2)
            for g in range(NT):
                kb[g, krows, :] = _pack(y[:, g * 128:(g + 1) * 128])

        k_done = [qkv_a(s) for s in range(NSUB)]
        y0 = out_a(0, k_done[0])
        ka[:, 0:HALO, :] = ka[:, RB:RB + HALO, :]
        va[:, 0:HALO, :] = va[:, RB:RB + HALO, :]
        x0 = xs[rows[0], :] + y0
        xs[rows[0], :] = x0
        xn0 = _layernorm(lambda st, dep: x0[st:st + LC], SB, LN_LOOK[0])
        y1 = out_a(1, k_done[1])
        xs[rows[1], :] = xs[rows[1], :] + y1

        @pl.when(jnp.logical_and(l == 0, r == 0))
        def _():
            wb_copy.wait()

        @pl.when(jnp.logical_and(l == 0, r + 1 < S // RB))
        def _():
            x_copy(jnp.minimum(r + 1, S // RB - 1)).wait()

        xn1 = _layernorm(lambda st, dep: xs[pl.ds(r0 + SB + st, LC), :], SB, LN_LOOK[1])
        qkv_b(0, xn0)
        load_x(r + 1, l, LX_LOOK)
        qkv_b(1, xn1)
        return l

    def head_weights(g, hh, q0):
        w = qt[pl.ds(pl.multiple_of(g * 64 + hh * 16, 16), 16), pl.ds(q0, TQ)]
        parts = []
        if hh > 0:
            parts.append(jnp.zeros((16 * hh, TQ), u32))
        parts.append(w)
        if hh < 3:
            parts.append(jnp.zeros((16 * (3 - hh), TQ), u32))
        return _unpack(jnp.concatenate(parts, axis=0))

    def v_rows(g, hh, c):
        rows = pl.ds(pl.multiple_of(g * 64 + hh * 16, 16), 16)
        return _unpack(vt[rows, c * KC:(c + 1) * KC])

    def finish_group(g):
        o = jnp.dot(v_rows(g, HPB - 1, NC - 1), _unpack(pp[...]), preferred_element_type=f32)
        last = (ot[3 * DH:4 * DH, :] + o) * invs[0:1, :]
        return jnp.concatenate([ot[0:3 * DH, :], last], axis=0).T.astype(bf16)

    def o_rows(q0):
        return pl.ds(pl.multiple_of(q0 // 2, TQ // 2), TQ // 2)

    def attn_fast(q0):
        def body(i, lmax):
            st = {}

            def qk(gg, hh, c):
                g = i * GPB + gg
                if c == 0:
                    st[gg, hh] = dict(w=head_weights(g, hh, q0))
                kc = _unpack(kb[g, c * KC // 2:(c + 1) * KC // 2, :])
                return jnp.dot(kc, st[gg, hh]["w"], preferred_element_type=f32)

            def pv(gg, hh, c, s):
                g = i * GPB + gg
                d = st[gg, hh]
                if c == 0:
                    d["m"] = jnp.broadcast_to(jnp.max(s[0:8], axis=0, keepdims=True), (8, TQ))
                p = jnp.exp2(s.reshape(KC // 8, 8, TQ) - d["m"][None])
                lc = jnp.sum(p, axis=0)
                d["l"] = lc if c == 0 else d["l"] + lc
                p = p.reshape(KC, TQ).astype(bf16)
                if c == NC - 1:
                    d["lsum"] = jnp.sum(d["l"], axis=0, keepdims=True)
                if gg == GPB - 1 and hh == HPB - 1 and c == NC - 1:
                    pp[...] = _pack(p)
                    ot[hh * DH:(hh + 1) * DH, :] = d["acc"]
                    invs[...] = jnp.broadcast_to(_recip(d["lsum"]), (8, TQ))
                    return
                o = jnp.dot(v_rows(g, hh, c), p, preferred_element_type=f32)
                d["acc"] = o if c == 0 else d["acc"] + o
                if c == NC - 1:
                    d["out"] = d["acc"] * _recip(d["lsum"])
                    if gg == GPB - 1:
                        ot[hh * DH:(hh + 1) * DH, :] = d["out"]
                    elif hh == HPB - 1:
                        o_t = jnp.concatenate([st[gg, k]["out"] for k in range(HPB)], axis=0)
                        ob[g, o_rows(q0), :] = _pack(o_t.T.astype(bf16))

            pend = None
            for gg in range(GPB):
                for hh in range(HPB):
                    for c in range(NC):
                        s = qk(gg, hh, c)
                        if pend is None:
                            ob[jnp.where(i == 0, NT, i * GPB - 1), o_rows(q0), :] = _pack(
                                finish_group(jnp.maximum(i * GPB - 1, 0)))
                        else:
                            pv(*pend)
                        pend = (gg, hh, c, s)
            pv(*pend)
            for d in st.values():
                lmax = jnp.maximum(lmax, d["lsum"])
            return lmax

        return lax.fori_loop(0, NT // GPB, body, jnp.zeros((1, TQ), f32))

    def attn_exact(q0):
        def group(g, carry):
            def head(hh, carry2):
                w = qt[pl.ds(pl.multiple_of(g * 64, 64), 64), pl.ds(q0, TQ)]
                row = lax.broadcasted_iota(jnp.int32, (64, TQ), 0) // 16
                w = _unpack(jnp.where(row == hh, w, jnp.zeros_like(w)))

                def scores(c):
                    kc = kb[g, pl.ds(pl.multiple_of(c * (KC // 2), KC // 2), KC // 2), :]
                    return jnp.dot(_unpack(kc), w, preferred_element_type=f32)

                def row_max(c, m):
                    return jnp.maximum(m, jnp.max(scores(c), axis=0, keepdims=True))

                m = lax.fori_loop(0, NC, row_max, jnp.full((1, TQ), -jnp.inf, f32))

                def accumulate(c, state):
                    l, acc = state
                    p = jnp.exp2(scores(c) - m)
                    v = vt[pl.ds(pl.multiple_of(g * 64 + hh * 16, 16), 16),
                           pl.ds(pl.multiple_of(c * KC, KC), KC)]
                    o = jnp.dot(_unpack(v), p.astype(bf16), preferred_element_type=f32)
                    return l + jnp.sum(p, axis=0, keepdims=True), acc + o

                l, acc = lax.fori_loop(0, NC, accumulate,
                                       (jnp.zeros((1, TQ), f32), jnp.zeros((DH, TQ), f32)))
                ot[pl.ds(pl.multiple_of(hh * DH, DH), DH), :] = acc * (1.0 / l)
                return carry2
            lax.fori_loop(0, HPB, head, 0)
            ob[g, o_rows(q0), :] = _pack(ot[...].T.astype(bf16))
            return carry
        lax.fori_loop(0, NT, group, 0)
        pp[...] = jnp.zeros(pp.shape, u32)
        invs[...] = jnp.ones(invs.shape, f32)

    def q_body(qb, l):
        q0 = pl.multiple_of(qb * TQ, TQ)

        def attempt(state):
            a, _ = state

            @pl.when(a == 0)
            def _():
                lmx[...] = jnp.broadcast_to(attn_fast(q0), (8, TQ))

            @pl.when(a == 1)
            def _():
                attn_exact(q0)

            @pl.when(jnp.logical_or(l == 1, a == 1))
            def _():
                for j in range(TQ // OC):
                    out_copy(qb, j).wait()

            o = jnp.concatenate([_unpack(ob[g, o_rows(q0), :]) for g in range(NT - 1)]
                                + [finish_group(NT - 1)], axis=1)
            for j in range(TQ // OC):
                if j == 2:
                    bad = _tree(jnp.maximum,
                                [jnp.where(lmx[:, i * 128:(i + 1) * 128] <= L_MAX, 0.0, 1.0)
                                 for i in range(TQ // 128)])
                    v_ok = (vbig[...] & jnp.uint32(0x80008000)) == 0
                    unsafe = jnp.max(jnp.where(v_ok, bad, 1.0))
                rows = pl.ds(q0 + j * OC, OC)
                x2 = xs[rows, :] + lax.dot_general(o[j * OC:(j + 1) * OC], wob[...], NN,
                                                   preferred_element_type=f32)
                xs2[rows, :] = x2
                outb[rows, :] = x2.astype(bf16)
                out_copy(qb, j).start()
            return a + 1, unsafe

        lax.while_loop(lambda st: jnp.logical_or(st[0] == 0, jnp.logical_and(st[0] == 1, st[1] > 0.5)),
                       attempt, (jnp.int32(0), jnp.float32(0)))
        return l

    def layer_pair(l, carry):
        ka[:, 0:HALO, :] = jnp.zeros((NT, HALO, 128), f32)
        va[:, 0:HALO, :] = jnp.zeros((NT, HALO, 128), f32)
        vbig[...] = jnp.zeros(vbig.shape, u32)

        @pl.when(l == 1)
        def _():
            load_x(0, l, RB // LC)

        lax.fori_loop(0, S // RB, row_body, l)

        @pl.when(l == 0)
        def _():
            wob_copy.wait()

        lax.fori_loop(0, S // TQ, q_body, l)
        return carry

    x_copy(0).wait()
    load_x(0, 0, RB // LC)
    for i in range(NWO):
        woa_copy(i).wait()
        if i == NWO - 1:
            for cp in late:
                cp.start()
        lax.fori_loop(i * NT // NWO, (i + 1) * NT // NWO, prep_woa, 0)
    lax.fori_loop(0, 2, layer_pair, 0)
    for qb in range(S // TQ):
        for j in range(TQ // OC):
            out_copy(qb, j).wait()


@jax.jit
def pallas_interleave_layers__sliding_local_dilated__softmax_full_mha__prompt_kernel(
    A_x: jax.Array,
    A_wqkv: jax.Array,
    A_wo: jax.Array,
    B_x: jax.Array,
    B_wqkv: jax.Array,
    B_wo: jax.Array,
):
    del B_x
    x = A_x.reshape(S, D)
    hbm = pl.BlockSpec(memory_space=pl.ANY)
    out = pl.pallas_call(
        _kernel,
        out_shape=jax.ShapeDtypeStruct((S, D), bf16),
        in_specs=[hbm] * 5,
        out_specs=hbm,
        scratch_shapes=[
            pltpu.VMEM((S, D), bf16),
            pltpu.VMEM((D, 3 * D), bf16),
            pltpu.VMEM((D, D), bf16),
            pltpu.VMEM((D, 3 * D), bf16),
            pltpu.VMEM((D, D), bf16),
            pltpu.VMEM((S, D), bf16),
            pltpu.VMEM((3, H * PITCH, 128), f32),
            pltpu.VMEM((H * WPITCH, 128), u32),
            pltpu.VMEM((D // 2, 3 * D), u32),
            pltpu.VMEM((D // 2, D), u32),
            pltpu.VMEM((RB // 2, D), u32),
            pltpu.VMEM((S + RB, D), f32),
            pltpu.VMEM((S, D), f32),
            pltpu.VMEM((NT, RB, 128), f32),
            pltpu.VMEM((NT, HALO + RB, 128), f32),
            pltpu.VMEM((NT, HALO + RB, 128), f32),
            pltpu.VMEM((D // 2, S), u32),
            pltpu.VMEM((NT, S // 2, 128), u32),
            pltpu.VMEM((D // 2, S), u32),
            pltpu.VMEM((NT + 1, S // 2, 128), u32),
            pltpu.VMEM((128, TQ), f32),
            pltpu.VMEM((KC // 2, TQ), u32),
            pltpu.VMEM((8, TQ), f32),
            pltpu.VMEM((8, TQ), f32),
            pltpu.VMEM((8, 128), u32),
            pltpu.SemaphoreType.DMA((S // RB,)),
            pltpu.SemaphoreType.DMA((NT,)),
            pltpu.SemaphoreType.DMA((2 + NWO,)),
            pltpu.SemaphoreType.DMA((S // OC,)),
        ],
        compiler_params=pltpu.CompilerParams(vmem_limit_bytes=110 * 1024 * 1024),
    )(x, A_wqkv, A_wo, B_wqkv, B_wo)
    return out.reshape(1, S, D)
```

```python
import math

import jax
import jax.numpy as jnp
from jax import lax
import jax.experimental.pallas as pl
import jax.experimental.pallas.tpu as pltpu

S = 2048
D = 1024
H = 32
DH = 32
WIN = 8
DIL = 2
EPS = 1e-5
NT = D // 128
HPB = 4
HALO = 16
QSCALE = (DH ** -0.5) * math.log2(math.e)

SB = 128
NSUB = 2
RB = SB * NSUB
RC = 8
LC = 8
LOOK = (1, 2)
TILE_GATE = (2, 2)
PV_GATE = (1, 1)
LN_LOOK = (2, 1)
LX_LOOK = 1

TQ = 512
KC = 256
NC = S // KC
GPB = 2
OC = 128
L_MAX = 2.0 ** 64
V_EXP = 50

NFLIGHT = 3
WA_STARTS = (2, 1, 2, 1, 2, 1, 1, 0)
NWO = 4
XLU_TILES = (8, 8, 0)
PITCH = 40
WPITCH = 17

bf16 = jnp.bfloat16
f32 = jnp.float32
u32 = jnp.uint32

NN = (((1,), (0,)), ((), ()))
NTD = (((1,), (1,)), ((), ()))


def _pack(x):
    return pltpu.bitcast(x, u32)


def _unpack(x):
    return pltpu.bitcast(x, bf16)


def _after(value, dep):
    if dep is None:
        return value
    return jnp.maximum(value, jnp.minimum(dep, -3e38))


def _tree(op, xs):
    xs = list(xs)
    while len(xs) > 1:
        xs = [op(xs[i], xs[i + 1]) if i + 1 < len(xs) else xs[i] for i in range(0, len(xs), 2)]
    return xs[0]


def _recip(x):
    r = pl.reciprocal(x, approx=True)
    return r * (2.0 - x * r)


def _too_large(packed):
    bias = 0x8000 - ((127 + V_EXP) << 7)
    t = (packed & jnp.uint32(0x7F807F80)) + jnp.uint32(bias << 16 | bias)
    return _tree(jnp.bitwise_or, [t[i:i + 8] for i in range(0, t.shape[0], 8)])


def _layernorm(load, nrows, look):
    outs = []
    deps = []
    for c in range(nrows // LC):
        dep = deps[c - look] if c >= look else None
        x = load(c * LC, dep)
        mu = jnp.broadcast_to(jnp.sum(x, axis=-1, keepdims=True), (LC, 128)) * _after(1.0 / D, dep)
        xc = x - jnp.concatenate([mu] * NT, axis=1)
        var = jnp.sum(xc * xc, axis=-1, keepdims=True) * (1.0 / D)
        y = xc * lax.rsqrt(var + EPS)
        deps.append(y[:, D - 128:])
        outs.append(y)
    return jnp.concatenate(outs, axis=0).astype(bf16)


def _kernel(x_hbm, wa_hbm, woa_hbm, wb_hbm, wob_hbm, out_hbm,
            xin, wa_raw, woa_raw, wb_raw, wob, outb,
            stg, stw, wan, woa, xnb,
            xs, xs2, qa, ka, va, qt, kb, vt, ob, ot, pp, invs, lmx, vbig,
            sem_x, sem_wa, sem_w, sem_o):
    def x_copy(r):
        rows = pl.ds(pl.multiple_of(r * RB, RB), RB)
        return pltpu.make_async_copy(x_hbm.at[rows, :], xin.at[rows, :], sem_x.at[r])

    def wa_copy(i):
        rows = pl.ds(pl.multiple_of(i * 128, 128), 128)
        return pltpu.make_async_copy(wa_hbm.at[rows, :], wa_raw.at[rows, :], sem_wa.at[i])

    wb_copy = pltpu.make_async_copy(wb_hbm, wb_raw, sem_w.at[0])

    def woa_copy(i):
        cols = pl.ds(pl.multiple_of(i * (D // NWO), D // NWO), D // NWO)
        return pltpu.make_async_copy(woa_hbm.at[:, cols], woa_raw.at[:, cols], sem_w.at[2 + i])

    wob_copy = pltpu.make_async_copy(wob_hbm, wob, sem_w.at[1])

    def out_copy(qb, j):
        rows = pl.ds(pl.multiple_of(qb * TQ + j * OC, OC), OC)
        return pltpu.make_async_copy(outb.at[rows, :], out_hbm.at[rows, :],
                                     sem_o.at[qb * (TQ // OC) + j])

    queue = ([wa_copy(i) for i in range(NT)]
             + [x_copy(0)] + [woa_copy(i) for i in range(NWO)]
             + [x_copy(1), wb_copy]
             + [x_copy(r) for r in range(2, S // RB)] + [wob_copy])
    for cp in queue[:NFLIGHT]:
        cp.start()
    queue = queue[NFLIGHT:]

    batches = [[queue.pop(0) for _ in range(n)] for n in WA_STARTS]
    late = [queue.pop(0) for _ in range(NT + 3 + NWO - NFLIGHT - sum(WA_STARTS))]

    def transpose(w):
        ri = lax.broadcasted_iota(jnp.int32, (128, 128), 0)
        ci = lax.broadcasted_iota(jnp.int32, (128, 128), 1)
        eye = jnp.where(ri == ci, 1.0, 0.0).astype(bf16)
        return lax.dot_general(eye, w, NTD, preferred_element_type=f32)

    def prep_wa(t, carry):
        wa_copy(t).wait()
        for k, batch in enumerate(batches):
            @pl.when(t == k)
            def _():
                for cp in batch:
                    cp.start()

        rows = pl.ds(pl.multiple_of(t * 128, 128), 128)

        def forward(part):
            for j in range(NT):
                wt = transpose(wa_raw[rows, part * D + j * 128:part * D + (j + 1) * 128])
                for hh in range(HPB):
                    r = (j * HPB + hh) * PITCH
                    stg[part, r:r + DH, :] = wt[hh * DH:(hh + 1) * DH]

        def back(part):
            regrouped = jnp.concatenate([stg[part, pl.ds(d, H, stride=PITCH), :]
                                         for d in range(DH)], axis=0)
            n = XLU_TILES[part] * 128
            pieces = []
            if n > 0:
                pieces.append(regrouped[:n].T)
            if n < D:
                pieces.append(transpose(regrouped[n:].astype(bf16)))
            wan[pl.ds(pl.multiple_of(t * 64, 64), 64), part * D:(part + 1) * D] = _pack(
                jnp.concatenate(pieces, axis=1).astype(bf16))

        forward(0)
        forward(1)
        back(0)
        forward(2)
        back(1)
        back(2)
        return carry

    def prep_woa(t, carry):
        cols = pl.ds(pl.multiple_of(t * 128, 128), 128)
        w = _pack(woa_raw[:, cols])
        for h in range(H):
            stw[h * WPITCH:h * WPITCH + DH // 2, :] = w[h * (DH // 2):(h + 1) * (DH // 2)]
        lo = jnp.uint32(0xFFFF)
        for j in range(DH // 2):
            even = stw[pl.ds(j, H // 2, stride=2 * WPITCH), :]
            odd = stw[pl.ds(WPITCH + j, H // 2, stride=2 * WPITCH), :]
            woa[2 * j * 16:(2 * j + 1) * 16, cols] = (even & lo) | (odd << 16)
            woa[(2 * j + 1) * 16:(2 * j + 2) * 16, cols] = (even >> 16) | (odd & ~lo)
        return carry

    ot[...] = jnp.zeros(ot.shape, f32)
    pp[...] = jnp.zeros(pp.shape, u32)
    invs[...] = jnp.ones(invs.shape, f32)
    lax.fori_loop(0, NT, prep_wa, 0)

    def local_attn(r0, s, first_dep):
        outs = []
        deps = []
        for c in range(SB // RC):
            base = s * SB + c * RC
            window = [slice(HALO + base - DIL * w, HALO + base - DIL * w + RC) for w in range(WIN)]
            scale = _after(QSCALE, deps[c - LOOK[s]] if c >= LOOK[s] else first_dep)
            logits = [None] * WIN
            for t in range(NT):
                if t > 0 and t % TILE_GATE[s] == 0:
                    scale = _after(QSCALE, logits[WIN - 1])
                q = qa[t, base:base + RC, :] * scale
                for w in range(WIN):
                    term = q * ka[t, window[w], :]
                    logits[w] = term if t == 0 else logits[w] + term
            for w in range(WIN):
                acc = logits[w]
                acc = acc + pltpu.roll(acc, 64, 1)
                acc = acc + pltpu.roll(acc, 32, 1)
                if base < DIL * w:
                    row = r0 + base + lax.broadcasted_iota(jnp.int32, (RC, 128), 0)
                    acc = jnp.where(row >= DIL * w, acc, -1e9)
                logits[w] = acc
            m = _tree(jnp.maximum, logits)
            p = [jnp.exp2(lg - m) for lg in logits]
            inv = _recip(_tree(jnp.add, p))
            tiles = []
            done = []
            for t in range(NT):
                if t >= PV_GATE[s]:
                    p[0] = _after(p[0], done[t - PV_GATE[s]])
                acc = _tree(jnp.add, [p[w] * va[t, window[w], :] for w in range(WIN)]) * inv
                tiles.append(acc.astype(bf16))
                done.append(acc)
            deps.append(m)
            outs.append(jnp.concatenate(tiles, axis=1))
        return jnp.concatenate(outs, axis=0)

    def load_x(r, l, look):
        r0 = pl.multiple_of(jnp.minimum(r, S // RB - 1) * RB, RB)
        w0 = pl.multiple_of(r * RB, RB)

        def load(start, dep):
            def from_input():
                x16 = xin[pl.ds(r0 + start // 16 * 16, 16), :].astype(f32)
                return x16[start % 16:start % 16 + LC]

            def from_layer_b():
                return xs2[pl.ds(r0 + start, LC), :]

            if isinstance(l, int):
                x = from_input() if l == 0 else from_layer_b()
            else:
                lvec = _after(jnp.full((LC, 128), l, f32), dep)
                first = jnp.concatenate([lvec == 0.0] * NT, axis=1)
                x = jnp.where(first, from_input(), from_layer_b())
            xs[pl.ds(w0 + start, LC), :] = x
            return x

        xnb[...] = _pack(_layernorm(load, RB, look))

    def row_body(r, l):
        r0 = pl.multiple_of(r * RB, RB)
        rows = [pl.ds(r0 + s * SB, SB) for s in range(NSUB)]

        @pl.when(jnp.logical_and(l == 0, r == 1))
        def _():
            for cp in queue:
                cp.start()

        def qkv_a(s):
            xn = _unpack(xnb[s * SB // 2:(s + 1) * SB // 2, :])
            y = lax.dot_general(xn, _unpack(wan[...]), NN, preferred_element_type=f32)
            new = slice(HALO + s * SB, HALO + (s + 1) * SB)
            for t in range(NT):
                qa[t, s * SB:(s + 1) * SB, :] = y[:, t * 128:(t + 1) * 128]
                ka[t, new, :] = y[:, D + t * 128:D + (t + 1) * 128]
                va[t, new, :] = y[:, 2 * D + t * 128:2 * D + (t + 1) * 128]
            return y[SB - RC:SB, 2 * D - 128:2 * D]

        def out_a(s, k_done):
            o = local_attn(r0, s, k_done)
            return lax.dot_general(o, _unpack(woa[...]), NN, preferred_element_type=f32)

        def qkv_b(s, xn):
            cols = rows[s]
            y = lax.dot_general(xn, wb_raw[:, 0:D], NN, preferred_element_type=f32)
            qt[:, cols] = _pack((y * QSCALE).T.astype(bf16))
            y = lax.dot_general(xn, wb_raw[:, 2 * D:3 * D], NN, preferred_element_type=f32)
            v_t = _pack(y.T.astype(bf16))
            vt[:, cols] = v_t
            vbig[...] = vbig[...] | _too_large(v_t)
            y = lax.dot_general(xn, wb_raw[:, D:2 * D], NN, preferred_element_type=f32).astype(bf16)
            krows = pl.ds(pl.multiple_of((r0 + s * SB) // 2, SB // 2), SB // 2)
            for g in range(NT):
                kb[g, krows, :] = _pack(y[:, g * 128:(g + 1) * 128])

        k_done = [qkv_a(s) for s in range(NSUB)]
        y0 = out_a(0, k_done[0])
        ka[:, 0:HALO, :] = ka[:, RB:RB + HALO, :]
        va[:, 0:HALO, :] = va[:, RB:RB + HALO, :]
        x0 = xs[rows[0], :] + y0
        xs[rows[0], :] = x0
        xn0 = _layernorm(lambda st, dep: x0[st:st + LC], SB, LN_LOOK[0])
        y1 = out_a(1, k_done[1])
        xs[rows[1], :] = xs[rows[1], :] + y1

        @pl.when(jnp.logical_and(l == 0, r == 0))
        def _():
            wb_copy.wait()

        @pl.when(jnp.logical_and(l == 0, r + 1 < S // RB))
        def _():
            x_copy(jnp.minimum(r + 1, S // RB - 1)).wait()

        xn1 = _layernorm(lambda st, dep: xs[pl.ds(r0 + SB + st, LC), :], SB, LN_LOOK[1])
        qkv_b(0, xn0)
        load_x(r + 1, l, LX_LOOK)
        qkv_b(1, xn1)
        return l

    def head_weights(g, hh, q0):
        w = qt[pl.ds(pl.multiple_of(g * 64 + hh * 16, 16), 16), pl.ds(q0, TQ)]
        parts = []
        if hh > 0:
            parts.append(jnp.zeros((16 * hh, TQ), u32))
        parts.append(w)
        if hh < 3:
            parts.append(jnp.zeros((16 * (3 - hh), TQ), u32))
        return _unpack(jnp.concatenate(parts, axis=0))

    def v_rows(g, hh, c):
        rows = pl.ds(pl.multiple_of(g * 64 + hh * 16, 16), 16)
        return _unpack(vt[rows, c * KC:(c + 1) * KC])

    def finish_group(g):
        o = jnp.dot(v_rows(g, HPB - 1, NC - 1), _unpack(pp[...]), preferred_element_type=f32)
        last = (ot[3 * DH:4 * DH, :] + o) * invs[0:1, :]
        return jnp.concatenate([ot[0:3 * DH, :], last], axis=0).T.astype(bf16)

    def o_rows(q0):
        return pl.ds(pl.multiple_of(q0 // 2, TQ // 2), TQ // 2)

    def attn_fast(q0):
        def body(i, lmax):
            st = {}

            def qk(gg, hh, c):
                g = i * GPB + gg
                if c == 0:
                    st[gg, hh] = dict(w=head_weights(g, hh, q0))
                kc = _unpack(kb[g, c * KC // 2:(c + 1) * KC // 2, :])
                return jnp.dot(kc, st[gg, hh]["w"], preferred_element_type=f32)

            def pv(gg, hh, c, s):
                g = i * GPB + gg
                d = st[gg, hh]
                if c == 0:
                    d["m"] = jnp.broadcast_to(jnp.max(s[0:8], axis=0, keepdims=True), (8, TQ))
                p = jnp.exp2(s.reshape(KC // 8, 8, TQ) - d["m"][None])
                lc = jnp.sum(p, axis=0)
                d["l"] = lc if c == 0 else d["l"] + lc
                p = p.reshape(KC, TQ).astype(bf16)
                if c == NC - 1:
                    d["lsum"] = jnp.sum(d["l"], axis=0, keepdims=True)
                if gg == GPB - 1 and hh == HPB - 1 and c == NC - 1:
                    pp[...] = _pack(p)
                    ot[hh * DH:(hh + 1) * DH, :] = d["acc"]
                    invs[...] = jnp.broadcast_to(_recip(d["lsum"]), (8, TQ))
                    return
                o = jnp.dot(v_rows(g, hh, c), p, preferred_element_type=f32)
                d["acc"] = o if c == 0 else d["acc"] + o
                if c == NC - 1:
                    d["out"] = d["acc"] * _recip(d["lsum"])
                    if gg == GPB - 1:
                        ot[hh * DH:(hh + 1) * DH, :] = d["out"]
                    elif hh == HPB - 1:
                        o_t = jnp.concatenate([st[gg, k]["out"] for k in range(HPB)], axis=0)
                        ob[g, o_rows(q0), :] = _pack(o_t.T.astype(bf16))

            pend = None
            for gg in range(GPB):
                for hh in range(HPB):
                    for c in range(NC):
                        s = qk(gg, hh, c)
                        if pend is None:
                            ob[jnp.where(i == 0, NT, i * GPB - 1), o_rows(q0), :] = _pack(
                                finish_group(jnp.maximum(i * GPB - 1, 0)))
                        else:
                            pv(*pend)
                        pend = (gg, hh, c, s)
            pv(*pend)
            for d in st.values():
                lmax = jnp.maximum(lmax, d["lsum"])
            return lmax

        return lax.fori_loop(0, NT // GPB, body, jnp.zeros((1, TQ), f32))

    def attn_exact(q0):
        def group(g, carry):
            def head(hh, carry2):
                w = qt[pl.ds(pl.multiple_of(g * 64, 64), 64), pl.ds(q0, TQ)]
                row = lax.broadcasted_iota(jnp.int32, (64, TQ), 0) // 16
                w = _unpack(jnp.where(row == hh, w, jnp.zeros_like(w)))

                def scores(c):
                    kc = kb[g, pl.ds(pl.multiple_of(c * (KC // 2), KC // 2), KC // 2), :]
                    return jnp.dot(_unpack(kc), w, preferred_element_type=f32)

                def row_max(c, m):
                    return jnp.maximum(m, jnp.max(scores(c), axis=0, keepdims=True))

                m = lax.fori_loop(0, NC, row_max, jnp.full((1, TQ), -jnp.inf, f32))

                def accumulate(c, state):
                    l, acc = state
                    p = jnp.exp2(scores(c) - m)
                    v = vt[pl.ds(pl.multiple_of(g * 64 + hh * 16, 16), 16),
                           pl.ds(pl.multiple_of(c * KC, KC), KC)]
                    o = jnp.dot(_unpack(v), p.astype(bf16), preferred_element_type=f32)
                    return l + jnp.sum(p, axis=0, keepdims=True), acc + o

                l, acc = lax.fori_loop(0, NC, accumulate,
                                       (jnp.zeros((1, TQ), f32), jnp.zeros((DH, TQ), f32)))
                ot[pl.ds(pl.multiple_of(hh * DH, DH), DH), :] = acc * (1.0 / l)
                return carry2
            lax.fori_loop(0, HPB, head, 0)
            ob[g, o_rows(q0), :] = _pack(ot[...].T.astype(bf16))
            return carry
        lax.fori_loop(0, NT, group, 0)
        pp[...] = jnp.zeros(pp.shape, u32)
        invs[...] = jnp.ones(invs.shape, f32)

    def q_body(qb, l):
        q0 = pl.multiple_of(qb * TQ, TQ)

        def attempt(state):
            a, _ = state

            @pl.when(a == 0)
            def _():
                lmx[...] = jnp.broadcast_to(attn_fast(q0), (8, TQ))

            @pl.when(a == 1)
            def _():
                attn_exact(q0)

            @pl.when(jnp.logical_or(l == 1, a == 1))
            def _():
                for j in range(TQ // OC):
                    out_copy(qb, j).wait()

            o = jnp.concatenate([_unpack(ob[g, o_rows(q0), :]) for g in range(NT - 1)]
                                + [finish_group(NT - 1)], axis=1)
            for j in range(TQ // OC):
                if j == 2:
                    bad = _tree(jnp.maximum,
                                [jnp.where(lmx[:, i * 128:(i + 1) * 128] <= L_MAX, 0.0, 1.0)
                                 for i in range(TQ // 128)])
                    v_ok = (vbig[...] & jnp.uint32(0x80008000)) == 0
                    unsafe = jnp.max(jnp.where(v_ok, bad, 1.0))
                rows = pl.ds(q0 + j * OC, OC)
                x2 = xs[rows, :] + lax.dot_general(o[j * OC:(j + 1) * OC], wob[...], NN,
                                                   preferred_element_type=f32)
                xs2[rows, :] = x2
                outb[rows, :] = x2.astype(bf16)
                out_copy(qb, j).start()
            return a + 1, unsafe

        lax.while_loop(lambda st: jnp.logical_or(st[0] == 0, jnp.logical_and(st[0] == 1, st[1] > 0.5)),
                       attempt, (jnp.int32(0), jnp.float32(0)))
        return l

    def layer_pair(l, carry):
        ka[:, 0:HALO, :] = jnp.zeros((NT, HALO, 128), f32)
        va[:, 0:HALO, :] = jnp.zeros((NT, HALO, 128), f32)
        vbig[...] = jnp.zeros(vbig.shape, u32)

        @pl.when(l == 1)
        def _():
            load_x(0, l, RB // LC)

        lax.fori_loop(0, S // RB, row_body, l)

        @pl.when(l == 0)
        def _():
            wob_copy.wait()

        lax.fori_loop(0, S // TQ, q_body, l)
        return carry

    x_copy(0).wait()
    load_x(0, 0, RB // LC)
    for i in range(NWO):
        woa_copy(i).wait()
        if i == NWO - 1:
            for cp in late:
                cp.start()
        lax.fori_loop(i * NT // NWO, (i + 1) * NT // NWO, prep_woa, 0)
    lax.fori_loop(0, 2, layer_pair, 0)
    for qb in range(S // TQ):
        for j in range(TQ // OC):
            out_copy(qb, j).wait()


@jax.jit
def pallas_interleave_layers__sliding_local_dilated__softmax_full_mha__prompt_kernel(
    A_x: jax.Array,
    A_wqkv: jax.Array,
    A_wo: jax.Array,
    B_x: jax.Array,
    B_wqkv: jax.Array,
    B_wo: jax.Array,
):
    del B_x
    x = A_x.reshape(S, D)
    hbm = pl.BlockSpec(memory_space=pl.ANY)
    out = pl.pallas_call(
        _kernel,
        out_shape=jax.ShapeDtypeStruct((S, D), bf16),
        in_specs=[hbm] * 5,
        out_specs=hbm,
        scratch_shapes=[
            pltpu.VMEM((S, D), bf16),
            pltpu.VMEM((D, 3 * D), bf16),
            pltpu.VMEM((D, D), bf16),
            pltpu.VMEM((D, 3 * D), bf16),
            pltpu.VMEM((D, D), bf16),
            pltpu.VMEM((S, D), bf16),
            pltpu.VMEM((3, (H + 1) * PITCH, 128), f32),
            pltpu.VMEM(((H + 2) * WPITCH, 128), u32),
            pltpu.VMEM((D // 2, 3 * D), u32),
            pltpu.VMEM((D // 2, D), u32),
            pltpu.VMEM((RB // 2, D), u32),
            pltpu.VMEM((S + RB, D), f32),
            pltpu.VMEM((S, D), f32),
            pltpu.VMEM((NT, RB, 128), f32),
            pltpu.VMEM((NT, HALO + RB, 128), f32),
            pltpu.VMEM((NT, HALO + RB, 128), f32),
            pltpu.VMEM((D // 2, S), u32),
            pltpu.VMEM((NT, S // 2, 128), u32),
            pltpu.VMEM((D // 2, S), u32),
            pltpu.VMEM((NT + 1, S // 2, 128), u32),
            pltpu.VMEM((128, TQ), f32),
            pltpu.VMEM((KC // 2, TQ), u32),
            pltpu.VMEM((8, TQ), f32),
            pltpu.VMEM((8, TQ), f32),
            pltpu.VMEM((8, 128), u32),
            pltpu.SemaphoreType.DMA((S // RB,)),
            pltpu.SemaphoreType.DMA((NT,)),
            pltpu.SemaphoreType.DMA((2 + NWO,)),
            pltpu.SemaphoreType.DMA((S // OC,)),
        ],
        compiler_params=pltpu.CompilerParams(vmem_limit_bytes=110 * 1024 * 1024),
    )(x, A_wqkv, A_wo, B_wqkv, B_wo)
    return out.reshape(1, S, D)
```

```python
import math

import jax
import jax.numpy as jnp
from jax import lax
import jax.experimental.pallas as pl
import jax.experimental.pallas.tpu as pltpu

S = 2048
D = 1024
H = 32
DH = 32
WIN = 8
DIL = 2
EPS = 1e-5
NT = D // 128
HPB = 4
HALO = 16
QSCALE = (DH ** -0.5) * math.log2(math.e)

SB = 128
NSUB = 2
RB = SB * NSUB
RC = 8
LC = 8
LOOK = (1, 2)
TILE_GATE = (2, 2)
PV_GATE = (1, 1)
LN_LOOK = (2, 1)
LX_LOOK = 1

TQ = 512
KC = 256
NC = S // KC
GPB = 2
OC = 128
L_MAX = 2.0 ** 64
V_EXP = 50

NFLIGHT = 3
WA_STARTS = (2, 1, 2, 1, 2, 1, 1, 0)
NWO = 4
XLU_TILES = (8, 8, 0)
PITCH = 40
WPITCH = 17

bf16 = jnp.bfloat16
f32 = jnp.float32
u32 = jnp.uint32

NN = (((1,), (0,)), ((), ()))
NTD = (((1,), (1,)), ((), ()))


def _pack(x):
    return pltpu.bitcast(x, u32)


def _unpack(x):
    return pltpu.bitcast(x, bf16)


def _after(value, dep):
    if dep is None:
        return value
    return jnp.maximum(value, jnp.minimum(dep, -3e38))


def _tree(op, xs):
    xs = list(xs)
    while len(xs) > 1:
        xs = [op(xs[i], xs[i + 1]) if i + 1 < len(xs) else xs[i] for i in range(0, len(xs), 2)]
    return xs[0]


def _recip(x):
    r = pl.reciprocal(x, approx=True)
    return r * (2.0 - x * r)


def _too_large(packed):
    bias = 0x8000 - ((127 + V_EXP) << 7)
    t = (packed & jnp.uint32(0x7F807F80)) + jnp.uint32(bias << 16 | bias)
    return _tree(jnp.bitwise_or, [t[i:i + 8] for i in range(0, t.shape[0], 8)])


def _layernorm(load, nrows, look):
    outs = []
    deps = []
    for c in range(nrows // LC):
        dep = deps[c - look] if c >= look else None
        x = load(c * LC, dep)
        mu = jnp.broadcast_to(jnp.sum(x, axis=-1, keepdims=True), (LC, 128)) * _after(1.0 / D, dep)
        xc = x - jnp.concatenate([mu] * NT, axis=1)
        var = jnp.sum(xc * xc, axis=-1, keepdims=True) * (1.0 / D)
        y = xc * lax.rsqrt(var + EPS)
        deps.append(y[:, D - 128:])
        outs.append(y)
    return jnp.concatenate(outs, axis=0).astype(bf16)


def _kernel(x_hbm, wa_hbm, woa_hbm, wb_hbm, wob_hbm, out_hbm,
            xin, wa_raw, woa_raw, wb_raw, wob, outb,
            stg, stw, wan, woa, wb0, xnb,
            xs, xs2, qa, ka, va, qt, kb, vt, ob, ot, pp, invs, lmx, vbig,
            sem_x, sem_wa, sem_w, sem_o):
    def x_copy(r):
        rows = pl.ds(pl.multiple_of(r * RB, RB), RB)
        return pltpu.make_async_copy(x_hbm.at[rows, :], xin.at[rows, :], sem_x.at[r])

    def wa_copy(i):
        rows = pl.ds(pl.multiple_of(i * 128, 128), 128)
        return pltpu.make_async_copy(wa_hbm.at[rows, :], wa_raw.at[rows, :], sem_wa.at[i])

    wb_copy = pltpu.make_async_copy(wb_hbm, wb_raw, sem_w.at[0])

    def woa_copy(i):
        cols = pl.ds(pl.multiple_of(i * (D // NWO), D // NWO), D // NWO)
        return pltpu.make_async_copy(woa_hbm.at[:, cols], woa_raw.at[:, cols], sem_w.at[2 + i])

    wob_copy = pltpu.make_async_copy(wob_hbm, wob, sem_w.at[1])

    def out_copy(qb, j):
        rows = pl.ds(pl.multiple_of(qb * TQ + j * OC, OC), OC)
        return pltpu.make_async_copy(outb.at[rows, :], out_hbm.at[rows, :],
                                     sem_o.at[qb * (TQ // OC) + j])

    queue = ([wa_copy(i) for i in range(NT)]
             + [x_copy(0)] + [woa_copy(i) for i in range(NWO)]
             + [x_copy(1), wb_copy]
             + [x_copy(r) for r in range(2, S // RB)] + [wob_copy])
    for cp in queue[:NFLIGHT]:
        cp.start()
    queue = queue[NFLIGHT:]

    batches = [[queue.pop(0) for _ in range(n)] for n in WA_STARTS]
    late = [queue.pop(0) for _ in range(NT + 3 + NWO - NFLIGHT - sum(WA_STARTS))]

    def transpose(w):
        ri = lax.broadcasted_iota(jnp.int32, (128, 128), 0)
        ci = lax.broadcasted_iota(jnp.int32, (128, 128), 1)
        eye = jnp.where(ri == ci, 1.0, 0.0).astype(bf16)
        return lax.dot_general(eye, w, NTD, preferred_element_type=f32)

    def prep_wa(t, carry):
        wa_copy(t).wait()
        for k, batch in enumerate(batches):
            @pl.when(t == k)
            def _():
                for cp in batch:
                    cp.start()

        rows = pl.ds(pl.multiple_of(t * 128, 128), 128)

        def forward(part):
            for j in range(NT):
                wt = transpose(wa_raw[rows, part * D + j * 128:part * D + (j + 1) * 128])
                for hh in range(HPB):
                    r = (j * HPB + hh) * PITCH
                    stg[part, r:r + DH, :] = wt[hh * DH:(hh + 1) * DH]

        def back(part):
            regrouped = jnp.concatenate([stg[part, pl.ds(d, H, stride=PITCH), :]
                                         for d in range(DH)], axis=0)
            n = XLU_TILES[part] * 128
            pieces = []
            if n > 0:
                pieces.append(regrouped[:n].T)
            if n < D:
                pieces.append(transpose(regrouped[n:].astype(bf16)))
            wan[pl.ds(pl.multiple_of(t * 64, 64), 64), part * D:(part + 1) * D] = _pack(
                jnp.concatenate(pieces, axis=1).astype(bf16))

        forward(0)
        forward(1)
        back(0)
        forward(2)
        back(1)
        back(2)
        return carry

    def prep_woa(t, carry):
        cols = pl.ds(pl.multiple_of(t * 128, 128), 128)
        w = _pack(woa_raw[:, cols])
        for h in range(H):
            stw[h * WPITCH:h * WPITCH + DH // 2, :] = w[h * (DH // 2):(h + 1) * (DH // 2)]
        lo = jnp.uint32(0xFFFF)
        for j in range(DH // 2):
            even = stw[pl.ds(j, H // 2, stride=2 * WPITCH), :]
            odd = stw[pl.ds(WPITCH + j, H // 2, stride=2 * WPITCH), :]
            woa[2 * j * 16:(2 * j + 1) * 16, cols] = (even & lo) | (odd << 16)
            woa[(2 * j + 1) * 16:(2 * j + 2) * 16, cols] = (even >> 16) | (odd & ~lo)
        return carry

    ot[...] = jnp.zeros(ot.shape, f32)
    pp[...] = jnp.zeros(pp.shape, u32)
    invs[...] = jnp.ones(invs.shape, f32)
    lax.fori_loop(0, NT, prep_wa, 0)

    def local_attn(r0, s, first_dep):
        outs = []
        deps = []
        for c in range(SB // RC):
            base = s * SB + c * RC
            window = [slice(HALO + base - DIL * w, HALO + base - DIL * w + RC) for w in range(WIN)]
            scale = _after(QSCALE, deps[c - LOOK[s]] if c >= LOOK[s] else first_dep)
            logits = [None] * WIN
            for t in range(NT):
                if t > 0 and t % TILE_GATE[s] == 0:
                    scale = _after(QSCALE, logits[WIN - 1])
                q = qa[t, base:base + RC, :] * scale
                for w in range(WIN):
                    term = q * ka[t, window[w], :]
                    logits[w] = term if t == 0 else logits[w] + term
            for w in range(WIN):
                acc = logits[w]
                acc = acc + pltpu.roll(acc, 64, 1)
                acc = acc + pltpu.roll(acc, 32, 1)
                if base < DIL * w:
                    row = r0 + base + lax.broadcasted_iota(jnp.int32, (RC, 128), 0)
                    acc = jnp.where(row >= DIL * w, acc, -1e9)
                logits[w] = acc
            m = _tree(jnp.maximum, logits)
            p = [jnp.exp2(lg - m) for lg in logits]
            inv = _recip(_tree(jnp.add, p))
            tiles = []
            done = []
            for t in range(NT):
                if t >= PV_GATE[s]:
                    p[0] = _after(p[0], done[t - PV_GATE[s]])
                acc = _tree(jnp.add, [p[w] * va[t, window[w], :] for w in range(WIN)]) * inv
                tiles.append(acc.astype(bf16))
                done.append(acc)
            deps.append(m)
            outs.append(jnp.concatenate(tiles, axis=1))
        return jnp.concatenate(outs, axis=0)

    def load_x(r, l, look):
        r0 = pl.multiple_of(jnp.minimum(r, S // RB - 1) * RB, RB)
        w0 = pl.multiple_of(r * RB, RB)

        def load(start, dep):
            def from_input():
                x16 = xin[pl.ds(r0 + start // 16 * 16, 16), :].astype(f32)
                return x16[start % 16:start % 16 + LC]

            def from_layer_b():
                return xs2[pl.ds(r0 + start, LC), :]

            if isinstance(l, int):
                x = from_input() if l == 0 else from_layer_b()
            else:
                lvec = _after(jnp.full((LC, 128), l, f32), dep)
                first = jnp.concatenate([lvec == 0.0] * NT, axis=1)
                x = jnp.where(first, from_input(), from_layer_b())
            xs[pl.ds(w0 + start, LC), :] = x
            return x

        xnb[...] = _pack(_layernorm(load, RB, look))

    def row_body(r, l):
        r0 = pl.multiple_of(r * RB, RB)
        rows = [pl.ds(r0 + s * SB, SB) for s in range(NSUB)]

        @pl.when(jnp.logical_and(l == 0, r == 1))
        def _():
            for cp in queue:
                cp.start()

        def qkv_a(s):
            xn = _unpack(xnb[s * SB // 2:(s + 1) * SB // 2, :])
            y = lax.dot_general(xn, _unpack(wan[...]), NN, preferred_element_type=f32)
            new = slice(HALO + s * SB, HALO + (s + 1) * SB)
            for t in range(NT):
                qa[t, s * SB:(s + 1) * SB, :] = y[:, t * 128:(t + 1) * 128]
                ka[t, new, :] = y[:, D + t * 128:D + (t + 1) * 128]
                va[t, new, :] = y[:, 2 * D + t * 128:2 * D + (t + 1) * 128]
            return y[SB - RC:SB, 2 * D - 128:2 * D]

        def out_a(s, k_done):
            o = local_attn(r0, s, k_done)
            return lax.dot_general(o, _unpack(woa[...]), NN, preferred_element_type=f32)

        def qkv_b(s, xn):
            cols = rows[s]
            if s == 0:
                y = jnp.concatenate(
                    [lax.dot_general(xn, _unpack(wb0[...]), NN, preferred_element_type=f32),
                     lax.dot_general(xn, wb_raw[:, 128:D], NN, preferred_element_type=f32)], axis=1)
            else:
                y = lax.dot_general(xn, wb_raw[:, 0:D], NN, preferred_element_type=f32)
            qt[:, cols] = _pack((y * QSCALE).T.astype(bf16))
            y = lax.dot_general(xn, wb_raw[:, 2 * D:3 * D], NN, preferred_element_type=f32)
            v_t = _pack(y.T.astype(bf16))
            vt[:, cols] = v_t
            vbig[...] = vbig[...] | _too_large(v_t)
            y = lax.dot_general(xn, wb_raw[:, D:2 * D], NN, preferred_element_type=f32).astype(bf16)
            krows = pl.ds(pl.multiple_of((r0 + s * SB) // 2, SB // 2), SB // 2)
            for g in range(NT):
                kb[g, krows, :] = _pack(y[:, g * 128:(g + 1) * 128])

        k_done = [qkv_a(s) for s in range(NSUB)]
        y0 = out_a(0, k_done[0])
        ka[:, 0:HALO, :] = ka[:, RB:RB + HALO, :]
        va[:, 0:HALO, :] = va[:, RB:RB + HALO, :]
        x0 = xs[rows[0], :] + y0
        xs[rows[0], :] = x0
        xn0 = _layernorm(lambda st, dep: x0[st:st + LC], SB, LN_LOOK[0])
        y1 = out_a(1, k_done[1])
        xs[rows[1], :] = xs[rows[1], :] + y1

        @pl.when(jnp.logical_and(l == 0, r + 1 < S // RB))
        def _():
            x_copy(jnp.minimum(r + 1, S // RB - 1)).wait()

        @pl.when(jnp.logical_and(l == 0, r == 0))
        def _():
            wb_copy.wait()
            wb0[...] = _pack(wb_raw[:, 0:128])

        xn1 = _layernorm(lambda st, dep: xs[pl.ds(r0 + SB + st, LC), :], SB, LN_LOOK[1])
        qkv_b(0, xn0)
        load_x(r + 1, l, LX_LOOK)
        qkv_b(1, xn1)
        return l

    def head_weights(g, hh, q0):
        w = qt[pl.ds(pl.multiple_of(g * 64 + hh * 16, 16), 16), pl.ds(q0, TQ)]
        parts = []
        if hh > 0:
            parts.append(jnp.zeros((16 * hh, TQ), u32))
        parts.append(w)
        if hh < 3:
            parts.append(jnp.zeros((16 * (3 - hh), TQ), u32))
        return _unpack(jnp.concatenate(parts, axis=0))

    def v_rows(g, hh, c):
        rows = pl.ds(pl.multiple_of(g * 64 + hh * 16, 16), 16)
        return _unpack(vt[rows, c * KC:(c + 1) * KC])

    def finish_group(g):
        o = jnp.dot(v_rows(g, HPB - 1, NC - 1), _unpack(pp[...]), preferred_element_type=f32)
        last = (ot[3 * DH:4 * DH, :] + o) * invs[0:1, :]
        return jnp.concatenate([ot[0:3 * DH, :], last], axis=0).T.astype(bf16)

    def o_rows(q0):
        return pl.ds(pl.multiple_of(q0 // 2, TQ // 2), TQ // 2)

    def attn_fast(q0):
        def body(i, lmax):
            st = {}

            def qk(gg, hh, c):
                g = i * GPB + gg
                if c == 0:
                    st[gg, hh] = dict(w=head_weights(g, hh, q0))
                kc = _unpack(kb[g, c * KC // 2:(c + 1) * KC // 2, :])
                return jnp.dot(kc, st[gg, hh]["w"], preferred_element_type=f32)

            def pv(gg, hh, c, s):
                g = i * GPB + gg
                d = st[gg, hh]
                if c == 0:
                    d["m"] = jnp.broadcast_to(jnp.max(s[0:8], axis=0, keepdims=True), (8, TQ))
                p = jnp.exp2(s.reshape(KC // 8, 8, TQ) - d["m"][None])
                lc = jnp.sum(p, axis=0)
                d["l"] = lc if c == 0 else d["l"] + lc
                p = p.reshape(KC, TQ).astype(bf16)
                if c == NC - 1:
                    d["lsum"] = jnp.sum(d["l"], axis=0, keepdims=True)
                if gg == GPB - 1 and hh == HPB - 1 and c == NC - 1:
                    pp[...] = _pack(p)
                    ot[hh * DH:(hh + 1) * DH, :] = d["acc"]
                    invs[...] = jnp.broadcast_to(_recip(d["lsum"]), (8, TQ))
                    return
                o = jnp.dot(v_rows(g, hh, c), p, preferred_element_type=f32)
                d["acc"] = o if c == 0 else d["acc"] + o
                if c == NC - 1:
                    d["out"] = d["acc"] * _recip(d["lsum"])
                    if gg == GPB - 1:
                        ot[hh * DH:(hh + 1) * DH, :] = d["out"]
                    elif hh == HPB - 1:
                        o_t = jnp.concatenate([st[gg, k]["out"] for k in range(HPB)], axis=0)
                        ob[g, o_rows(q0), :] = _pack(o_t.T.astype(bf16))

            pend = None
            for gg in range(GPB):
                for hh in range(HPB):
                    for c in range(NC):
                        s = qk(gg, hh, c)
                        if pend is None:
                            ob[jnp.where(i == 0, NT, i * GPB - 1), o_rows(q0), :] = _pack(
                                finish_group(jnp.maximum(i * GPB - 1, 0)))
                        else:
                            pv(*pend)
                        pend = (gg, hh, c, s)
            pv(*pend)
            for d in st.values():
                lmax = jnp.maximum(lmax, d["lsum"])
            return lmax

        return lax.fori_loop(0, NT // GPB, body, jnp.zeros((1, TQ), f32))

    def attn_exact(q0):
        def group(g, carry):
            def head(hh, carry2):
                w = qt[pl.ds(pl.multiple_of(g * 64, 64), 64), pl.ds(q0, TQ)]
                row = lax.broadcasted_iota(jnp.int32, (64, TQ), 0) // 16
                w = _unpack(jnp.where(row == hh, w, jnp.zeros_like(w)))

                def scores(c):
                    kc = kb[g, pl.ds(pl.multiple_of(c * (KC // 2), KC // 2), KC // 2), :]
                    return jnp.dot(_unpack(kc), w, preferred_element_type=f32)

                def row_max(c, m):
                    return jnp.maximum(m, jnp.max(scores(c), axis=0, keepdims=True))

                m = lax.fori_loop(0, NC, row_max, jnp.full((1, TQ), -jnp.inf, f32))

                def accumulate(c, state):
                    l, acc = state
                    p = jnp.exp2(scores(c) - m)
                    v = vt[pl.ds(pl.multiple_of(g * 64 + hh * 16, 16), 16),
                           pl.ds(pl.multiple_of(c * KC, KC), KC)]
                    o = jnp.dot(_unpack(v), p.astype(bf16), preferred_element_type=f32)
                    return l + jnp.sum(p, axis=0, keepdims=True), acc + o

                l, acc = lax.fori_loop(0, NC, accumulate,
                                       (jnp.zeros((1, TQ), f32), jnp.zeros((DH, TQ), f32)))
                ot[pl.ds(pl.multiple_of(hh * DH, DH), DH), :] = acc * (1.0 / l)
                return carry2
            lax.fori_loop(0, HPB, head, 0)
            ob[g, o_rows(q0), :] = _pack(ot[...].T.astype(bf16))
            return carry
        lax.fori_loop(0, NT, group, 0)
        pp[...] = jnp.zeros(pp.shape, u32)
        invs[...] = jnp.ones(invs.shape, f32)

    def q_body(qb, l):
        q0 = pl.multiple_of(qb * TQ, TQ)

        def attempt(state):
            a, _ = state

            @pl.when(a == 0)
            def _():
                lmx[...] = jnp.broadcast_to(attn_fast(q0), (8, TQ))

            @pl.when(a == 1)
            def _():
                attn_exact(q0)

            @pl.when(jnp.logical_or(l == 1, a == 1))
            def _():
                for j in range(TQ // OC):
                    out_copy(qb, j).wait()

            o = jnp.concatenate([_unpack(ob[g, o_rows(q0), :]) for g in range(NT - 1)]
                                + [finish_group(NT - 1)], axis=1)
            for j in range(TQ // OC):
                if j == 2:
                    bad = _tree(jnp.maximum,
                                [jnp.where(lmx[:, i * 128:(i + 1) * 128] <= L_MAX, 0.0, 1.0)
                                 for i in range(TQ // 128)])
                    v_ok = (vbig[...] & jnp.uint32(0x80008000)) == 0
                    unsafe = jnp.max(jnp.where(v_ok, bad, 1.0))
                rows = pl.ds(q0 + j * OC, OC)
                x2 = xs[rows, :] + lax.dot_general(o[j * OC:(j + 1) * OC], wob[...], NN,
                                                   preferred_element_type=f32)
                xs2[rows, :] = x2
                outb[rows, :] = x2.astype(bf16)
                out_copy(qb, j).start()
            return a + 1, unsafe

        lax.while_loop(lambda st: jnp.logical_or(st[0] == 0, jnp.logical_and(st[0] == 1, st[1] > 0.5)),
                       attempt, (jnp.int32(0), jnp.float32(0)))
        return l

    def layer_pair(l, carry):
        ka[:, 0:HALO, :] = jnp.zeros((NT, HALO, 128), f32)
        va[:, 0:HALO, :] = jnp.zeros((NT, HALO, 128), f32)
        vbig[...] = jnp.zeros(vbig.shape, u32)

        @pl.when(l == 1)
        def _():
            load_x(0, l, RB // LC)

        lax.fori_loop(0, S // RB, row_body, l)

        @pl.when(l == 0)
        def _():
            wob_copy.wait()

        lax.fori_loop(0, S // TQ, q_body, l)
        return carry

    x_copy(0).wait()
    load_x(0, 0, RB // LC)
    for i in range(NWO):
        woa_copy(i).wait()
        if i == NWO - 1:
            for cp in late:
                cp.start()
        lax.fori_loop(i * NT // NWO, (i + 1) * NT // NWO, prep_woa, 0)
    lax.fori_loop(0, 2, layer_pair, 0)
    for qb in range(S // TQ):
        for j in range(TQ // OC):
            out_copy(qb, j).wait()


@jax.jit
def pallas_interleave_layers__sliding_local_dilated__softmax_full_mha__prompt_kernel(
    A_x: jax.Array,
    A_wqkv: jax.Array,
    A_wo: jax.Array,
    B_x: jax.Array,
    B_wqkv: jax.Array,
    B_wo: jax.Array,
):
    del B_x
    x = A_x.reshape(S, D)
    hbm = pl.BlockSpec(memory_space=pl.ANY)
    out = pl.pallas_call(
        _kernel,
        out_shape=jax.ShapeDtypeStruct((S, D), bf16),
        in_specs=[hbm] * 5,
        out_specs=hbm,
        scratch_shapes=[
            pltpu.VMEM((S, D), bf16),
            pltpu.VMEM((D, 3 * D), bf16),
            pltpu.VMEM((D, D), bf16),
            pltpu.VMEM((D, 3 * D), bf16),
            pltpu.VMEM((D, D), bf16),
            pltpu.VMEM((S, D), bf16),
            pltpu.VMEM((3, (H + 1) * PITCH, 128), f32),
            pltpu.VMEM(((H + 2) * WPITCH, 128), u32),
            pltpu.VMEM((D // 2, 3 * D), u32),
            pltpu.VMEM((D // 2, D), u32),
            pltpu.VMEM((D // 2, 128), u32),
            pltpu.VMEM((RB // 2, D), u32),
            pltpu.VMEM((S + RB, D), f32),
            pltpu.VMEM((S, D), f32),
            pltpu.VMEM((NT, RB, 128), f32),
            pltpu.VMEM((NT, HALO + RB, 128), f32),
            pltpu.VMEM((NT, HALO + RB, 128), f32),
            pltpu.VMEM((D // 2, S), u32),
            pltpu.VMEM((NT, S // 2, 128), u32),
            pltpu.VMEM((D // 2, S), u32),
            pltpu.VMEM((NT + 1, S // 2, 128), u32),
            pltpu.VMEM((128, TQ), f32),
            pltpu.VMEM((KC // 2, TQ), u32),
            pltpu.VMEM((8, TQ), f32),
            pltpu.VMEM((8, TQ), f32),
            pltpu.VMEM((8, 128), u32),
            pltpu.SemaphoreType.DMA((S // RB,)),
            pltpu.SemaphoreType.DMA((NT,)),
            pltpu.SemaphoreType.DMA((2 + NWO,)),
            pltpu.SemaphoreType.DMA((S // OC,)),
        ],
        compiler_params=pltpu.CompilerParams(vmem_limit_bytes=110 * 1024 * 1024),
    )(x, A_wqkv, A_wo, B_wqkv, B_wo)
    return out.reshape(1, S, D)
```

```python
import math

import jax
import jax.numpy as jnp
from jax import lax
import jax.experimental.pallas as pl
import jax.experimental.pallas.tpu as pltpu

S = 2048
D = 1024
H = 32
DH = 32
WIN = 8
DIL = 2
EPS = 1e-5
NT = D // 128
HPB = 4
HD = D // 2
HALO = 16
QSCALE = (DH ** -0.5) * math.log2(math.e)

SB = 128
NSUB = 2
RB = SB * NSUB
RC = 8
LC = 8
LOOK = (1, 2)
TILE_GATE = (2, 2)
PV_GATE = (1, 1)
LN_LOOK = (2, 1)
LX_LOOK = 3
B_ORDER = (5, 3, 4, 'n', 2, 1, 7, 6)
T1_ORDER = (3, 6, 4, 5, 1, 7, 2)

TQ = 512
KC = 256
NC = S // KC
GPB = 2
OC = 128
L_MAX = 2.0 ** 64
V_EXP = 50

NFLIGHT = 3
WA_STARTS = (2, 1, 2, 1, 2, 1, 1, 0)
NWO = 4
XLU_TILES = (8, 8, 0)
PITCH = 40
WPITCH = 17

bf16 = jnp.bfloat16
f32 = jnp.float32
u32 = jnp.uint32

NN = (((1,), (0,)), ((), ()))
NTD = (((1,), (1,)), ((), ()))


def _pack(x):
    return pltpu.bitcast(x, u32)


def _unpack(x):
    return pltpu.bitcast(x, bf16)


def _after(value, dep):
    if dep is None:
        return value
    return jnp.maximum(value, jnp.minimum(dep, -3e38))


def _tree(op, xs):
    xs = list(xs)
    while len(xs) > 1:
        xs = [op(xs[i], xs[i + 1]) if i + 1 < len(xs) else xs[i] for i in range(0, len(xs), 2)]
    return xs[0]


def _recip(x):
    r = pl.reciprocal(x, approx=True)
    return r * (2.0 - x * r)


def _too_large(packed):
    bias = 0x8000 - ((127 + V_EXP) << 7)
    t = (packed & jnp.uint32(0x7F807F80)) + jnp.uint32(bias << 16 | bias)
    return _tree(jnp.bitwise_or, [t[i:i + 8] for i in range(0, t.shape[0], 8)])


def _layernorm(load, nrows, look):
    outs = []
    deps = []
    for c in range(nrows // LC):
        dep = deps[c - look] if c >= look else None
        x = load(c * LC, dep)
        mu = jnp.broadcast_to(jnp.sum(x, axis=-1, keepdims=True), (LC, 128)) * _after(1.0 / D, dep)
        xc = x - jnp.concatenate([mu] * NT, axis=1)
        var = jnp.sum(xc * xc, axis=-1, keepdims=True) * (1.0 / D)
        y = xc * lax.rsqrt(var + EPS)
        deps.append(y[:, D - 128:])
        outs.append(y)
    return jnp.concatenate(outs, axis=0)


def _strassen_lhs(a11, a12, a21, a22):
    return {
        1: lambda: (a11() + a22()).astype(bf16),
        2: lambda: (a21() + a22()).astype(bf16),
        3: lambda: a11().astype(bf16),
        4: lambda: a22().astype(bf16),
        5: lambda: (a11() + a12()).astype(bf16),
        6: lambda: (a21() - a11()).astype(bf16),
        7: lambda: (a12() - a22()).astype(bf16),
    }


def _strassen_rhs(b11, b12, b21, b22):
    return [b11 + b22, b11, b12 - b22, b21 - b11, b22, b11 + b12, b21 + b22]


def _kernel(x_hbm, wa_hbm, woa_hbm, wb_hbm, wob_hbm, out_hbm,
            xin, wa_raw, woa_raw, wb_raw, wob, outb,
            stg, stw, wan, woa, wbs, wos, xnb,
            xs, xs2, qa, ka, va, qt, kb, vt, ob, ot, pp, invs, lmx, vbig,
            sem_x, sem_wa, sem_w, sem_o):
    def x_copy(r):
        rows = pl.ds(pl.multiple_of(r * RB, RB), RB)
        return pltpu.make_async_copy(x_hbm.at[rows, :], xin.at[rows, :], sem_x.at[r])

    def wa_copy(i):
        rows = pl.ds(pl.multiple_of(i * 128, 128), 128)
        return pltpu.make_async_copy(wa_hbm.at[rows, :], wa_raw.at[rows, :], sem_wa.at[i])

    wb_copy = pltpu.make_async_copy(wb_hbm, wb_raw, sem_w.at[0])

    def woa_copy(i):
        cols = pl.ds(pl.multiple_of(i * (D // NWO), D // NWO), D // NWO)
        return pltpu.make_async_copy(woa_hbm.at[:, cols], woa_raw.at[:, cols], sem_w.at[2 + i])

    wob_copy = pltpu.make_async_copy(wob_hbm, wob, sem_w.at[1])

    def out_copy(qb, j):
        rows = pl.ds(pl.multiple_of(qb * TQ + j * OC, OC), OC)
        return pltpu.make_async_copy(outb.at[rows, :], out_hbm.at[rows, :],
                                     sem_o.at[qb * (TQ // OC) + j])

    queue = ([wa_copy(i) for i in range(NT)]
             + [x_copy(0)] + [woa_copy(i) for i in range(NWO)]
             + [x_copy(1), wb_copy]
             + [x_copy(r) for r in range(2, S // RB)] + [wob_copy])
    for cp in queue[:NFLIGHT]:
        cp.start()
    queue = queue[NFLIGHT:]

    batches = [[queue.pop(0) for _ in range(n)] for n in WA_STARTS]
    late = [queue.pop(0) for _ in range(NT + 3 + NWO - NFLIGHT - sum(WA_STARTS))]

    def transpose(w):
        ri = lax.broadcasted_iota(jnp.int32, (128, 128), 0)
        ci = lax.broadcasted_iota(jnp.int32, (128, 128), 1)
        eye = jnp.where(ri == ci, 1.0, 0.0).astype(bf16)
        return lax.dot_general(eye, w, NTD, preferred_element_type=f32)

    def prep_wa(t, carry):
        wa_copy(t).wait()
        for k, batch in enumerate(batches):
            @pl.when(t == k)
            def _():
                for cp in batch:
                    cp.start()

        rows = pl.ds(pl.multiple_of(t * 128, 128), 128)

        def forward(part):
            for j in range(NT):
                wt = transpose(wa_raw[rows, part * D + j * 128:part * D + (j + 1) * 128])
                for hh in range(HPB):
                    r = (j * HPB + hh) * PITCH
                    stg[part, r:r + DH, :] = wt[hh * DH:(hh + 1) * DH]

        def back(part):
            regrouped = jnp.concatenate([stg[part, pl.ds(d, H, stride=PITCH), :]
                                         for d in range(DH)], axis=0)
            n = XLU_TILES[part] * 128
            pieces = []
            if n > 0:
                pieces.append(regrouped[:n].T)
            if n < D:
                pieces.append(transpose(regrouped[n:].astype(bf16)))
            wan[pl.ds(pl.multiple_of(t * 64, 64), 64), part * D:(part + 1) * D] = _pack(
                jnp.concatenate(pieces, axis=1).astype(bf16))

        forward(0)
        forward(1)
        back(0)
        forward(2)
        back(1)
        back(2)
        return carry

    def prep_woa(t, carry):
        cols = pl.ds(pl.multiple_of(t * 128, 128), 128)
        w = _pack(woa_raw[:, cols])
        for h in range(H):
            stw[h * WPITCH:h * WPITCH + DH // 2, :] = w[h * (DH // 2):(h + 1) * (DH // 2)]
        lo = jnp.uint32(0xFFFF)
        for j in range(DH // 2):
            even = stw[pl.ds(j, H // 2, stride=2 * WPITCH), :]
            odd = stw[pl.ds(WPITCH + j, H // 2, stride=2 * WPITCH), :]
            woa[2 * j * 16:(2 * j + 1) * 16, cols] = (even & lo) | (odd << 16)
            woa[(2 * j + 1) * 16:(2 * j + 2) * 16, cols] = (even >> 16) | (odd & ~lo)
        return carry

    def prep_wb(i, carry):
        def halves(rows):
            w = wb_raw[rows, :].astype(f32)
            return w[:, 0:3 * HD], jnp.concatenate([w[:, 2 * D:], w[:, 3 * HD:2 * D]], axis=1)
        b11, b12 = halves(pl.ds(pl.multiple_of(i * 16, 16), 16))
        b21, b22 = halves(pl.ds(pl.multiple_of(HD + i * 16, 16), 16))
        for k, w in enumerate(_strassen_rhs(b11, b12, b21, b22)):
            wbs[k, pl.ds(pl.multiple_of(i * 8, 8), 8), :] = _pack(w.astype(bf16))
        return carry

    def prep_wob(i, carry):
        top = wob[pl.ds(pl.multiple_of(i * 32, 32), 32), :].astype(f32)
        bot = wob[pl.ds(pl.multiple_of(HD + i * 32, 32), 32), :].astype(f32)
        for k, w in enumerate(_strassen_rhs(top[:, :HD], top[:, HD:], bot[:, :HD], bot[:, HD:])):
            wos[k, pl.ds(pl.multiple_of(i * 16, 16), 16), :] = _pack(w.astype(bf16))
        return carry

    ot[...] = jnp.zeros(ot.shape, f32)
    pp[...] = jnp.zeros(pp.shape, u32)
    invs[...] = jnp.ones(invs.shape, f32)
    lax.fori_loop(0, NT, prep_wa, 0)

    def local_attn(r0, s, first_dep):
        outs = []
        deps = []
        for c in range(SB // RC):
            base = s * SB + c * RC
            window = [slice(HALO + base - DIL * w, HALO + base - DIL * w + RC) for w in range(WIN)]
            scale = _after(QSCALE, deps[c - LOOK[s]] if c >= LOOK[s] else first_dep)
            logits = [None] * WIN
            for t in range(NT):
                if t > 0 and t % TILE_GATE[s] == 0:
                    scale = _after(QSCALE, logits[WIN - 1])
                q = qa[t, base:base + RC, :] * scale
                for w in range(WIN):
                    term = q * ka[t, window[w], :]
                    logits[w] = term if t == 0 else logits[w] + term
            for w in range(WIN):
                acc = logits[w]
                acc = acc + pltpu.roll(acc, 64, 1)
                acc = acc + pltpu.roll(acc, 32, 1)
                if base < DIL * w:
                    row = r0 + base + lax.broadcasted_iota(jnp.int32, (RC, 128), 0)
                    acc = jnp.where(row >= DIL * w, acc, -1e9)
                logits[w] = acc
            m = _tree(jnp.maximum, logits)
            p = [jnp.exp2(lg - m) for lg in logits]
            inv = _recip(_tree(jnp.add, p))
            tiles = []
            done = []
            for t in range(NT):
                if t >= PV_GATE[s]:
                    p[0] = _after(p[0], done[t - PV_GATE[s]])
                acc = _tree(jnp.add, [p[w] * va[t, window[w], :] for w in range(WIN)]) * inv
                tiles.append(acc.astype(bf16))
                done.append(acc)
            deps.append(m)
            outs.append(jnp.concatenate(tiles, axis=1))
        return jnp.concatenate(outs, axis=0)

    def load_x(r, l, look):
        r0 = pl.multiple_of(jnp.minimum(r, S // RB - 1) * RB, RB)
        w0 = pl.multiple_of(r * RB, RB)

        def load(start, dep):
            def from_input():
                x16 = xin[pl.ds(r0 + start // 16 * 16, 16), :].astype(f32)
                return x16[start % 16:start % 16 + LC]

            def from_layer_b():
                return xs2[pl.ds(r0 + start, LC), :]

            if isinstance(l, int):
                x = from_input() if l == 0 else from_layer_b()
            else:
                lvec = _after(jnp.full((LC, 128), l, f32), dep)
                first = jnp.concatenate([lvec == 0.0] * NT, axis=1)
                x = jnp.where(first, from_input(), from_layer_b())
            xs[pl.ds(w0 + start, LC), :] = x
            return x

        xnb[...] = _pack(_layernorm(load, RB, look).astype(bf16))

    def row_body(r, l):
        r0 = pl.multiple_of(r * RB, RB)
        rows = [pl.ds(r0 + s * SB, SB) for s in range(NSUB)]

        @pl.when(jnp.logical_and(l == 0, r == 1))
        def _():
            for cp in queue:
                cp.start()

        def qkv_a(s):
            xn = _unpack(xnb[s * SB // 2:(s + 1) * SB // 2, :])
            y = lax.dot_general(xn, _unpack(wan[...]), NN, preferred_element_type=f32)
            new = slice(HALO + s * SB, HALO + (s + 1) * SB)
            for t in range(NT):
                qa[t, s * SB:(s + 1) * SB, :] = y[:, t * 128:(t + 1) * 128]
                ka[t, new, :] = y[:, D + t * 128:D + (t + 1) * 128]
                va[t, new, :] = y[:, 2 * D + t * 128:2 * D + (t + 1) * 128]
            return y[SB - RC:SB, 2 * D - 128:2 * D]

        def out_a(s, k_done):
            o = local_attn(r0, s, k_done)
            return lax.dot_general(o, _unpack(woa[...]), NN, preferred_element_type=f32)

        def put_first(s, y):
            qt[:, rows[s]] = _pack((y[:, 0:D] * QSCALE).T.astype(bf16))
            put_k(s, y[:, D:], 0)

        def put_second(s, y):
            v_t = _pack(y[:, 0:D].T.astype(bf16))
            vt[:, rows[s]] = v_t
            vbig[...] = vbig[...] | _too_large(v_t)
            put_k(s, y[:, D:], NT // 2)

        def put_k(s, y, g0):
            krows = pl.ds(pl.multiple_of((r0 + s * SB) // 2, SB // 2), SB // 2)
            y = y.astype(bf16)
            for g in range(NT // 2):
                kb[g0 + g, krows, :] = _pack(y[:, g * 128:(g + 1) * 128])

        k_done = [qkv_a(s) for s in range(NSUB)]
        y0 = out_a(0, k_done[0])
        ka[:, 0:HALO, :] = ka[:, RB:RB + HALO, :]
        va[:, 0:HALO, :] = va[:, RB:RB + HALO, :]
        x0 = xs[rows[0], :] + y0
        xs[rows[0], :] = x0
        xn0 = _layernorm(lambda st, dep: x0[st:st + LC], SB, LN_LOOK[0])
        y1 = out_a(1, k_done[1])
        xs[rows[1], :] = xs[rows[1], :] + y1

        @pl.when(jnp.logical_and(l == 0, r + 1 < S // RB))
        def _():
            x_copy(jnp.minimum(r + 1, S // RB - 1)).wait()

        @pl.when(jnp.logical_and(l == 0, r == 0))
        def _():
            wb_copy.wait()
            lax.fori_loop(0, HD // 16, prep_wb, 0)

        xn1 = _layernorm(lambda st, dep: xs[pl.ds(r0 + SB + st, LC), :], SB, LN_LOOK[1])
        lhs = _strassen_lhs(lambda: xn0[:, :HD], lambda: xn0[:, HD:], lambda: xn1[:, :HD], lambda: xn1[:, HD:])
        m = {}
        for step in B_ORDER:
            if step in ("n", 0):
                load_x(r + 1, l, LX_LOOK)
                continue
            m[step] = lax.dot_general(lhs[step](), _unpack(wbs[step - 1]), NN, preferred_element_type=f32)
            if "c12" not in m and 3 in m and 5 in m:
                m["c12"] = put_second(0, m[3] + m[5])
            if "c21" not in m and 2 in m and 4 in m:
                m["c21"] = put_first(1, m[2] + m[4])
            if "c11" not in m and all(k in m for k in (1, 4, 5, 7)):
                m["c11"] = put_first(0, (m[4] - m[5]) + m[1] + m[7])
            if "c22" not in m and all(k in m for k in (1, 2, 3, 6)):
                m["c22"] = put_second(1, (m[3] - m[2]) + m[1] + m[6])
        return l

    def head_weights(g, hh, q0):
        w = qt[pl.ds(pl.multiple_of(g * 64 + hh * 16, 16), 16), pl.ds(q0, TQ)]
        parts = []
        if hh > 0:
            parts.append(jnp.zeros((16 * hh, TQ), u32))
        parts.append(w)
        if hh < 3:
            parts.append(jnp.zeros((16 * (3 - hh), TQ), u32))
        return _unpack(jnp.concatenate(parts, axis=0))

    def v_rows(g, hh, c):
        rows = pl.ds(pl.multiple_of(g * 64 + hh * 16, 16), 16)
        return _unpack(vt[rows, c * KC:(c + 1) * KC])

    def finish_group(g):
        o = jnp.dot(v_rows(g, HPB - 1, NC - 1), _unpack(pp[...]), preferred_element_type=f32)
        last = (ot[3 * DH:4 * DH, :] + o) * invs[0:1, :]
        return jnp.concatenate([ot[0:3 * DH, :], last], axis=0).T.astype(bf16)

    def o_rows(q0):
        return pl.ds(pl.multiple_of(q0 // 2, TQ // 2), TQ // 2)

    def attn_fast(q0):
        def body(i, lmax):
            st = {}

            def qk(gg, hh, c):
                g = i * GPB + gg
                if c == 0:
                    st[gg, hh] = dict(w=head_weights(g, hh, q0))
                kc = _unpack(kb[g, c * KC // 2:(c + 1) * KC // 2, :])
                return jnp.dot(kc, st[gg, hh]["w"], preferred_element_type=f32)

            def pv(gg, hh, c, s):
                g = i * GPB + gg
                d = st[gg, hh]
                if c == 0:
                    d["m"] = jnp.broadcast_to(jnp.max(s[0:8], axis=0, keepdims=True), (8, TQ))
                p = jnp.exp2(s.reshape(KC // 8, 8, TQ) - d["m"][None])
                lc = jnp.sum(p, axis=0)
                d["l"] = lc if c == 0 else d["l"] + lc
                p = p.reshape(KC, TQ).astype(bf16)
                if c == NC - 1:
                    d["lsum"] = jnp.sum(d["l"], axis=0, keepdims=True)
                if gg == GPB - 1 and hh == HPB - 1 and c == NC - 1:
                    pp[...] = _pack(p)
                    ot[hh * DH:(hh + 1) * DH, :] = d["acc"]
                    invs[...] = jnp.broadcast_to(_recip(d["lsum"]), (8, TQ))
                    return
                o = jnp.dot(v_rows(g, hh, c), p, preferred_element_type=f32)
                d["acc"] = o if c == 0 else d["acc"] + o
                if c == NC - 1:
                    d["out"] = d["acc"] * _recip(d["lsum"])
                    if gg == GPB - 1:
                        ot[hh * DH:(hh + 1) * DH, :] = d["out"]
                    elif hh == HPB - 1:
                        o_t = jnp.concatenate([st[gg, k]["out"] for k in range(HPB)], axis=0)
                        ob[g, o_rows(q0), :] = _pack(o_t.T.astype(bf16))

            pend = None
            for gg in range(GPB):
                for hh in range(HPB):
                    for c in range(NC):
                        s = qk(gg, hh, c)
                        if pend is None:
                            ob[jnp.where(i == 0, NT, i * GPB - 1), o_rows(q0), :] = _pack(
                                finish_group(jnp.maximum(i * GPB - 1, 0)))
                        else:
                            pv(*pend)
                        pend = (gg, hh, c, s)
            pv(*pend)
            for d in st.values():
                lmax = jnp.maximum(lmax, d["lsum"])
            return lmax

        return lax.fori_loop(0, NT // GPB, body, jnp.zeros((1, TQ), f32))

    def attn_exact(q0):
        def group(g, carry):
            def head(hh, carry2):
                w = qt[pl.ds(pl.multiple_of(g * 64, 64), 64), pl.ds(q0, TQ)]
                row = lax.broadcasted_iota(jnp.int32, (64, TQ), 0) // 16
                w = _unpack(jnp.where(row == hh, w, jnp.zeros_like(w)))

                def scores(c):
                    kc = kb[g, pl.ds(pl.multiple_of(c * (KC // 2), KC // 2), KC // 2), :]
                    return jnp.dot(_unpack(kc), w, preferred_element_type=f32)

                def row_max(c, m):
                    return jnp.maximum(m, jnp.max(scores(c), axis=0, keepdims=True))

                m = lax.fori_loop(0, NC, row_max, jnp.full((1, TQ), -jnp.inf, f32))

                def accumulate(c, state):
                    l, acc = state
                    p = jnp.exp2(scores(c) - m)
                    v = vt[pl.ds(pl.multiple_of(g * 64 + hh * 16, 16), 16),
                           pl.ds(pl.multiple_of(c * KC, KC), KC)]
                    o = jnp.dot(_unpack(v), p.astype(bf16), preferred_element_type=f32)
                    return l + jnp.sum(p, axis=0, keepdims=True), acc + o

                l, acc = lax.fori_loop(0, NC, accumulate,
                                       (jnp.zeros((1, TQ), f32), jnp.zeros((DH, TQ), f32)))
                ot[pl.ds(pl.multiple_of(hh * DH, DH), DH), :] = acc * (1.0 / l)
                return carry2
            lax.fori_loop(0, HPB, head, 0)
            ob[g, o_rows(q0), :] = _pack(ot[...].T.astype(bf16))
            return carry
        lax.fori_loop(0, NT, group, 0)
        pp[...] = jnp.zeros(pp.shape, u32)
        invs[...] = jnp.ones(invs.shape, f32)

    def q_body(qb, l):
        q0 = pl.multiple_of(qb * TQ, TQ)

        def attempt(state):
            a, _ = state

            @pl.when(a == 0)
            def _():
                lmx[...] = jnp.broadcast_to(attn_fast(q0), (8, TQ))

            @pl.when(a == 1)
            def _():
                attn_exact(q0)

            @pl.when(jnp.logical_or(l == 1, a == 1))
            def _():
                for j in range(TQ // OC):
                    out_copy(qb, j).wait()

            o = jnp.concatenate([_unpack(ob[g, o_rows(q0), :]) for g in range(NT - 1)]
                                + [finish_group(NT - 1)], axis=1)
            hq = TQ // 2
            lhs = _strassen_lhs(lambda: o[:hq, :HD].astype(f32), lambda: o[:hq, HD:].astype(f32),
                                lambda: o[hq:, :HD].astype(f32), lambda: o[hq:, HD:].astype(f32))
            lhs[3] = lambda: o[:hq, :HD]
            lhs[4] = lambda: o[hq:, HD:]

            def emit(j, y):
                rows = pl.ds(q0 + j * OC, OC)
                x2 = xs[rows, :] + y
                xs2[rows, :] = x2
                outb[rows, :] = x2.astype(bf16)
                out_copy(qb, j).start()

            m = {}
            for step in T1_ORDER[:-1]:
                m[step] = lax.dot_general(lhs[step](), _unpack(wos[step - 1]), NN, preferred_element_type=f32)
                if step == T1_ORDER[2]:
                    bad = _tree(jnp.maximum,
                                [jnp.where(lmx[:, i * 128:(i + 1) * 128] <= L_MAX, 0.0, 1.0)
                                 for i in range(TQ // 128)])
                    v_ok = (vbig[...] & jnp.uint32(0x80008000)) == 0
                    unsafe = jnp.max(jnp.where(v_ok, bad, 1.0))
            top = jnp.concatenate([(m[4] - m[5]) + m[1] + m[7], m[3] + m[5]], axis=1)
            for j in range(hq // OC):
                emit(j, top[j * OC:(j + 1) * OC])
            rest22 = (m[3] + m[6]) + m[1]
            l2 = lhs[2]()
            for j in range(hq // OC):
                part = slice(j * OC, (j + 1) * OC)
                m2 = lax.dot_general(l2[part], _unpack(wos[1]), NN, preferred_element_type=f32)
                emit(hq // OC + j, jnp.concatenate([m2 + m[4][part], rest22[part] - m2], axis=1))
            return a + 1, unsafe

        lax.while_loop(lambda st: jnp.logical_or(st[0] == 0, jnp.logical_and(st[0] == 1, st[1] > 0.5)),
                       attempt, (jnp.int32(0), jnp.float32(0)))
        return l

    def layer_pair(l, carry):
        ka[:, 0:HALO, :] = jnp.zeros((NT, HALO, 128), f32)
        va[:, 0:HALO, :] = jnp.zeros((NT, HALO, 128), f32)
        vbig[...] = jnp.zeros(vbig.shape, u32)

        @pl.when(l == 1)
        def _():
            load_x(0, l, RB // LC)

        lax.fori_loop(0, S // RB, row_body, l)

        @pl.when(l == 0)
        def _():
            wob_copy.wait()
            lax.fori_loop(0, HD // 32, prep_wob, 0)

        lax.fori_loop(0, S // TQ, q_body, l)
        return carry

    x_copy(0).wait()
    load_x(0, 0, RB // LC)
    for i in range(NWO):
        woa_copy(i).wait()
        if i == NWO - 1:
            for cp in late:
                cp.start()
        lax.fori_loop(i * NT // NWO, (i + 1) * NT // NWO, prep_woa, 0)
    lax.fori_loop(0, 2, layer_pair, 0)
    for qb in range(S // TQ):
        for j in range(TQ // OC):
            out_copy(qb, j).wait()


@jax.jit
def pallas_interleave_layers__sliding_local_dilated__softmax_full_mha__prompt_kernel(
    A_x: jax.Array,
    A_wqkv: jax.Array,
    A_wo: jax.Array,
    B_x: jax.Array,
    B_wqkv: jax.Array,
    B_wo: jax.Array,
):
    del B_x
    x = A_x.reshape(S, D)
    hbm = pl.BlockSpec(memory_space=pl.ANY)
    out = pl.pallas_call(
        _kernel,
        out_shape=jax.ShapeDtypeStruct((S, D), bf16),
        in_specs=[hbm] * 5,
        out_specs=hbm,
        scratch_shapes=[
            pltpu.VMEM((S, D), bf16),
            pltpu.VMEM((D, 3 * D), bf16),
            pltpu.VMEM((D, D), bf16),
            pltpu.VMEM((D, 3 * D), bf16),
            pltpu.VMEM((D, D), bf16),
            pltpu.VMEM((S, D), bf16),
            pltpu.VMEM((3, (H + 1) * PITCH, 128), f32),
            pltpu.VMEM(((H + 2) * WPITCH, 128), u32),
            pltpu.VMEM((D // 2, 3 * D), u32),
            pltpu.VMEM((D // 2, D), u32),
            pltpu.VMEM((7, HD // 2, 3 * HD), u32),
            pltpu.VMEM((7, HD // 2, HD), u32),
            pltpu.VMEM((RB // 2, D), u32),
            pltpu.VMEM((S + RB, D), f32),
            pltpu.VMEM((S, D), f32),
            pltpu.VMEM((NT, RB, 128), f32),
            pltpu.VMEM((NT, HALO + RB, 128), f32),
            pltpu.VMEM((NT, HALO + RB, 128), f32),
            pltpu.VMEM((D // 2, S), u32),
            pltpu.VMEM((NT, S // 2, 128), u32),
            pltpu.VMEM((D // 2, S), u32),
            pltpu.VMEM((NT + 1, S // 2, 128), u32),
            pltpu.VMEM((128, TQ), f32),
            pltpu.VMEM((KC // 2, TQ), u32),
            pltpu.VMEM((8, TQ), f32),
            pltpu.VMEM((8, TQ), f32),
            pltpu.VMEM((8, 128), u32),
            pltpu.SemaphoreType.DMA((S // RB,)),
            pltpu.SemaphoreType.DMA((NT,)),
            pltpu.SemaphoreType.DMA((2 + NWO,)),
            pltpu.SemaphoreType.DMA((S // OC,)),
        ],
        compiler_params=pltpu.CompilerParams(vmem_limit_bytes=110 * 1024 * 1024),
    )(x, A_wqkv, A_wo, B_wqkv, B_wo)
    return out.reshape(1, S, D)
```

```python
import functools
import math

import jax
import jax.numpy as jnp
from jax import lax
import jax.experimental.pallas as pl
import jax.experimental.pallas.tpu as pltpu

S = 2048
D = 1024
H = 32
DH = 32
WIN = 8
DIL = 2
EPS = 1e-5
NT = D // 128
HPB = 4
HD = D // 2
HALO = 16
QSCALE = (DH ** -0.5) * math.log2(math.e)

SB = 128
NSUB = 2
RB = SB * NSUB
RC = 8
LC = 8
LOOK = (1, 2)
TILE_GATE = (2, 2)
PV_GATE = (1, 1)
LN_LOOK = (2, 1)
LX_LOOK = 5

LQK = 2
LV = 2
LO = 2
B_ORDER = [("qk", 5), ("qk", 3), ("v", 5), ("v", 3), ("next", 0), ("v", 4), ("v", 2), ("v", 1),
           ("v", 7), ("v", 6), ("qk", 4), ("qk", 2), ("qk", 1), ("qk", 7), ("qk", 6)]
SUB_B = (5, 3, 4, 2, 7, 1, 6)
SUB_T = (1, 4, 5, 7, 3, 2, 6)
PU = 4
T1_ORDER = (3, 6, 5, 4, 1, 7, 2)

TQ = 512
KC = 256
NC = S // KC
GPB = 2
OC = 128
L_MAX = 2.0 ** 64
V_EXP = 50

NFLIGHT = 3
WA_STARTS = (2, 1, 2, 1, 2, 1, 1, 0)
NWO = 4
XLU_TILES = (8, 8, 0)
PITCH = 40
WPITCH = 17

bf16 = jnp.bfloat16
f32 = jnp.float32
u32 = jnp.uint32

NN = (((1,), (0,)), ((), ()))
NTD = (((1,), (1,)), ((), ()))


def _pack(x):
    return pltpu.bitcast(x, u32)


def _unpack(x):
    return pltpu.bitcast(x, bf16)


def _after(value, dep):
    if dep is None:
        return value
    return jnp.maximum(value, jnp.minimum(dep, -3e38))


def _tree(op, xs):
    xs = list(xs)
    while len(xs) > 1:
        xs = [op(xs[i], xs[i + 1]) if i + 1 < len(xs) else xs[i] for i in range(0, len(xs), 2)]
    return xs[0]


def _recip(x):
    r = pl.reciprocal(x, approx=True)
    return r * (2.0 - x * r)


def _too_large(packed):
    bias = 0x8000 - ((127 + V_EXP) << 7)
    t = (packed & jnp.uint32(0x7F807F80)) + jnp.uint32(bias << 16 | bias)
    return _tree(jnp.bitwise_or, [t[i:i + 8] for i in range(0, t.shape[0], 8)])


def _layernorm(load, nrows, look):
    outs = []
    deps = []
    for c in range(nrows // LC):
        dep = deps[c - look] if c >= look else None
        x = load(c * LC, dep)
        mu = jnp.broadcast_to(jnp.sum(x, axis=-1, keepdims=True), (LC, 128)) * _after(1.0 / D, dep)
        xc = x - jnp.concatenate([mu] * NT, axis=1)
        var = jnp.sum(xc * xc, axis=-1, keepdims=True) * (1.0 / D)
        y = xc * lax.rsqrt(var + EPS)
        deps.append(y[:, D - 128:])
        outs.append(y)
    return jnp.concatenate(outs, axis=0)


def _strassen_lhs(k, a11, a12, a21, a22):
    if k == 1:
        return a11() + a22()
    if k == 2:
        return a21() + a22()
    if k == 3:
        return a11()
    if k == 4:
        return a22()
    if k == 5:
        return a11() + a12()
    if k == 6:
        return a21() - a11()
    return a12() - a22()


def _strassen_rhs(b11, b12, b21, b22):
    return [b11 + b22, b11, b12 - b22, b21 - b11, b22, b11 + b12, b21 + b22]


def _rhs_operands(chunks, level):
    if level == 0:
        return chunks
    h = len(chunks) // 2
    n = chunks[0].shape[1] // 2
    per_chunk = [_strassen_rhs(chunks[i][:, :n], chunks[i][:, n:], chunks[h + i][:, :n], chunks[h + i][:, n:])
                 for i in range(h)]
    out = []
    for k in range(7):
        out += _rhs_operands([per_chunk[i][k] for i in range(h)], level - 1)
    return out


def _product(a, w_ref, index, level, order):
    if level == 0:
        return lax.dot_general(a.astype(bf16), _unpack(w_ref[index]), NN, preferred_element_type=f32)
    m2, k2 = a.shape[0] // 2, a.shape[1] // 2
    blocks = (lambda: a[:m2, :k2], lambda: a[:m2, k2:], lambda: a[m2:, :k2], lambda: a[m2:, k2:])
    m = {k: _product(_strassen_lhs(k, *blocks), w_ref, index * 7 + k - 1, level - 1, order) for k in order}
    top = jnp.concatenate([(m[4] - m[5]) + m[1] + m[7], m[3] + m[5]], axis=1)
    bot = jnp.concatenate([m[2] + m[4], (m[3] - m[2]) + m[1] + m[6]], axis=1)
    return jnp.concatenate([top, bot], axis=0)


def _kernel(x_hbm, wa_hbm, woa_hbm, wb_hbm, wob_hbm, out_hbm,
            xin, wa_raw, woa_raw, wb_raw, wob, outb,
            stg, stw, wan, woa, wqk, wv, wos, xnb,
            xs, xs2, qa, ka, va, qt, kb, vt, ob, ot, pp, invs, lmx, vbig,
            sem_x, sem_wa, sem_w, sem_o):
    def x_copy(r):
        rows = pl.ds(pl.multiple_of(r * RB, RB), RB)
        return pltpu.make_async_copy(x_hbm.at[rows, :], xin.at[rows, :], sem_x.at[r])

    def wa_copy(i):
        rows = pl.ds(pl.multiple_of(i * 128, 128), 128)
        return pltpu.make_async_copy(wa_hbm.at[rows, :], wa_raw.at[rows, :], sem_wa.at[i])

    wb_copy = pltpu.make_async_copy(wb_hbm, wb_raw, sem_w.at[0])

    def woa_copy(i):
        cols = pl.ds(pl.multiple_of(i * (D // NWO), D // NWO), D // NWO)
        return pltpu.make_async_copy(woa_hbm.at[:, cols], woa_raw.at[:, cols], sem_w.at[2 + i])

    wob_copy = pltpu.make_async_copy(wob_hbm, wob, sem_w.at[1])

    def out_copy(qb, j):
        rows = pl.ds(pl.multiple_of(qb * TQ + j * OC, OC), OC)
        return pltpu.make_async_copy(outb.at[rows, :], out_hbm.at[rows, :],
                                     sem_o.at[qb * (TQ // OC) + j])

    queue = ([wa_copy(i) for i in range(NT)]
             + [x_copy(0)] + [woa_copy(i) for i in range(NWO)]
             + [x_copy(1), wb_copy]
             + [x_copy(r) for r in range(2, S // RB)] + [wob_copy])
    for cp in queue[:NFLIGHT]:
        cp.start()
    queue = queue[NFLIGHT:]

    batches = [[queue.pop(0) for _ in range(n)] for n in WA_STARTS]
    late = [queue.pop(0) for _ in range(NT + 3 + NWO - NFLIGHT - sum(WA_STARTS))]

    def transpose(w):
        ri = lax.broadcasted_iota(jnp.int32, (128, 128), 0)
        ci = lax.broadcasted_iota(jnp.int32, (128, 128), 1)
        eye = jnp.where(ri == ci, 1.0, 0.0).astype(bf16)
        return lax.dot_general(eye, w, NTD, preferred_element_type=f32)

    def prep_wa(t, carry):
        wa_copy(t).wait()
        for k, batch in enumerate(batches):
            @pl.when(t == k)
            def _():
                for cp in batch:
                    cp.start()

        rows = pl.ds(pl.multiple_of(t * 128, 128), 128)

        def forward(part):
            for j in range(NT):
                wt = transpose(wa_raw[rows, part * D + j * 128:part * D + (j + 1) * 128])
                for hh in range(HPB):
                    r = (j * HPB + hh) * PITCH
                    stg[part, r:r + DH, :] = wt[hh * DH:(hh + 1) * DH]

        def back(part):
            regrouped = jnp.concatenate([stg[part, pl.ds(d, H, stride=PITCH), :]
                                         for d in range(DH)], axis=0)
            n = XLU_TILES[part] * 128
            pieces = []
            if n > 0:
                pieces.append(regrouped[:n].T)
            if n < D:
                pieces.append(transpose(regrouped[n:].astype(bf16)))
            wan[pl.ds(pl.multiple_of(t * 64, 64), 64), part * D:(part + 1) * D] = _pack(
                jnp.concatenate(pieces, axis=1).astype(bf16))

        forward(0)
        forward(1)
        back(0)
        forward(2)
        back(1)
        back(2)
        return carry

    def prep_woa(t, carry):
        cols = pl.ds(pl.multiple_of(t * 128, 128), 128)
        w = _pack(woa_raw[:, cols])
        for h in range(H):
            stw[h * WPITCH:h * WPITCH + DH // 2, :] = w[h * (DH // 2):(h + 1) * (DH // 2)]
        lo = jnp.uint32(0xFFFF)
        for j in range(DH // 2):
            even = stw[pl.ds(j, H // 2, stride=2 * WPITCH), :]
            odd = stw[pl.ds(WPITCH + j, H // 2, stride=2 * WPITCH), :]
            woa[2 * j * 16:(2 * j + 1) * 16, cols] = (even & lo) | (odd << 16)
            woa[(2 * j + 1) * 16:(2 * j + 2) * 16, cols] = (even >> 16) | (odd & ~lo)
        return carry

    def rhs_step(src, c0, c1, dst, level, i, tile):
        nb = D >> level
        wb = (c1 - c0) >> level

        def rows(j):
            rs = pl.ds(pl.multiple_of(j * nb + i * 16, 16), 16)
            w = jnp.concatenate(
                [_pack(src[rs, c0 + q * wb + tile * 128:c0 + q * wb + (tile + 1) * 128])
                 for q in range(1 << level)], axis=1)
            return jnp.concatenate(
                [pltpu.unpack_elementwise(w, index=k, packed_dtype=bf16, unpacked_dtype=f32)
                 for k in range(2)], axis=0)

        out_rows = pl.ds(pl.multiple_of(i * 8, 8), 8)
        out_cols = slice(tile * 128, (tile + 1) * 128)
        for k, w in enumerate(_rhs_operands([rows(j) for j in range(1 << level)], level)):
            dst[k, out_rows, out_cols] = pltpu.pack_elementwise(
                [w[0:8], w[8:16]], packed_dtype=bf16).astype(u32)

    def prep_rhs(src, c0, c1, dst, level):
        for tile in range(((c1 - c0) >> level) // 128):
            def step(n, carry):
                for u in range(PU):
                    rhs_step(src, c0, c1, dst, level, n * PU + u, tile)
                return carry

            lax.fori_loop(0, (D >> level) // (16 * PU), step, 0)

    ot[...] = jnp.zeros(ot.shape, f32)
    pp[...] = jnp.zeros(pp.shape, u32)
    invs[...] = jnp.ones(invs.shape, f32)
    lax.fori_loop(0, NT, prep_wa, 0)

    def local_attn(r0, s, first_dep):
        outs = []
        deps = []
        for c in range(SB // RC):
            base = s * SB + c * RC
            window = [slice(HALO + base - DIL * w, HALO + base - DIL * w + RC) for w in range(WIN)]
            scale = _after(QSCALE, deps[c - LOOK[s]] if c >= LOOK[s] else first_dep)
            logits = [None] * WIN
            for t in range(NT):
                if t > 0 and t % TILE_GATE[s] == 0:
                    scale = _after(QSCALE, logits[WIN - 1])
                q = qa[t, base:base + RC, :] * scale
                for w in range(WIN):
                    term = q * ka[t, window[w], :]
                    logits[w] = term if t == 0 else logits[w] + term
            for w in range(WIN):
                acc = logits[w]
                acc = acc + pltpu.roll(acc, 64, 1)
                acc = acc + pltpu.roll(acc, 32, 1)
                if base < DIL * w:
                    row = r0 + base + lax.broadcasted_iota(jnp.int32, (RC, 128), 0)
                    acc = jnp.where(row >= DIL * w, acc, -1e9)
                logits[w] = acc
            m = _tree(jnp.maximum, logits)
            p = [jnp.exp2(lg - m) for lg in logits]
            inv = _recip(_tree(jnp.add, p))
            tiles = []
            done = []
            for t in range(NT):
                if t >= PV_GATE[s]:
                    p[0] = _after(p[0], done[t - PV_GATE[s]])
                acc = _tree(jnp.add, [p[w] * va[t, window[w], :] for w in range(WIN)]) * inv
                tiles.append(acc.astype(bf16))
                done.append(acc)
            deps.append(m)
            outs.append(jnp.concatenate(tiles, axis=1))
        return jnp.concatenate(outs, axis=0)

    def load_x(r, l, look):
        r0 = pl.multiple_of(jnp.minimum(r, S // RB - 1) * RB, RB)
        w0 = pl.multiple_of(r * RB, RB)

        def load(start, dep):
            def from_input():
                x16 = xin[pl.ds(r0 + start // 16 * 16, 16), :].astype(f32)
                return x16[start % 16:start % 16 + LC]

            def from_layer_b():
                return xs2[pl.ds(r0 + start, LC), :]

            if isinstance(l, int):
                x = from_input() if l == 0 else from_layer_b()
            else:
                lvec = _after(jnp.full((LC, 128), l, f32), dep)
                first = jnp.concatenate([lvec == 0.0] * NT, axis=1)
                x = jnp.where(first, from_input(), from_layer_b())
            xs[pl.ds(w0 + start, LC), :] = x
            return x

        xnb[...] = _pack(_layernorm(load, RB, look).astype(bf16))

    def row_body(r, l):
        r0 = pl.multiple_of(r * RB, RB)
        rows = [pl.ds(r0 + s * SB, SB) for s in range(NSUB)]

        @pl.when(jnp.logical_and(l == 0, r == 1))
        def _():
            for cp in queue:
                cp.start()

        def qkv_a(s):
            xn = _unpack(xnb[s * SB // 2:(s + 1) * SB // 2, :])
            y = lax.dot_general(xn, _unpack(wan[...]), NN, preferred_element_type=f32)
            new = slice(HALO + s * SB, HALO + (s + 1) * SB)
            for t in range(NT):
                qa[t, s * SB:(s + 1) * SB, :] = y[:, t * 128:(t + 1) * 128]
                ka[t, new, :] = y[:, D + t * 128:D + (t + 1) * 128]
                va[t, new, :] = y[:, 2 * D + t * 128:2 * D + (t + 1) * 128]
            return y[SB - RC:SB, 2 * D - 128:2 * D]

        def out_a(s, k_done):
            o = local_attn(r0, s, k_done)
            return lax.dot_general(o, _unpack(woa[...]), NN, preferred_element_type=f32)

        def put_q(s, y):
            qt[:, rows[s]] = _pack((y * QSCALE).T.astype(bf16))

        def put_k(s, y):
            krows = pl.ds(pl.multiple_of((r0 + s * SB) // 2, SB // 2), SB // 2)
            y = y.astype(bf16)
            for g in range(NT):
                kb[g, krows, :] = _pack(y[:, g * 128:(g + 1) * 128])

        def put_v(half, s, y):
            v_t = _pack(y.T.astype(bf16))
            vt[half * HD // 2:(half + 1) * HD // 2, rows[s]] = v_t
            vbig[...] = vbig[...] | _too_large(v_t)

        k_done = [qkv_a(s) for s in range(NSUB)]
        y0 = out_a(0, k_done[0])
        ka[:, 0:HALO, :] = ka[:, RB:RB + HALO, :]
        va[:, 0:HALO, :] = va[:, RB:RB + HALO, :]
        x0 = xs[rows[0], :] + y0
        xs[rows[0], :] = x0
        xn0 = _layernorm(lambda st, dep: x0[st:st + LC], SB, LN_LOOK[0])
        y1 = out_a(1, k_done[1])
        xs[rows[1], :] = xs[rows[1], :] + y1

        @pl.when(jnp.logical_and(l == 0, r + 1 < S // RB))
        def _():
            x_copy(jnp.minimum(r + 1, S // RB - 1)).wait()

        @pl.when(jnp.logical_and(l == 0, r == 0))
        def _():
            wb_copy.wait()
            prep_rhs(wb_raw, 0, 2 * D, wqk, LQK)
            prep_rhs(wb_raw, 2 * D, 3 * D, wv, LV)

        xn1 = _layernorm(lambda st, dep: xs[pl.ds(r0 + SB + st, LC), :], SB, LN_LOOK[1])
        blocks = (lambda: xn0[:, :HD], lambda: xn0[:, HD:], lambda: xn1[:, :HD], lambda: xn1[:, HD:])
        lhs = {}
        ms = {"qk": {}, "v": {}}
        puts = {"qk": (put_q, put_k), "v": (functools.partial(put_v, 0), functools.partial(put_v, 1))}
        for inst, step in B_ORDER:
            if inst == "next":
                load_x(r + 1, l, LX_LOOK)
                continue
            if step not in lhs:
                lhs[step] = _strassen_lhs(step, *blocks)
            m = ms[inst]
            first, second = puts[inst]
            m[step] = _product(lhs[step], wqk if inst == "qk" else wv, step - 1,
                               (LQK if inst == "qk" else LV) - 1, SUB_B)
            if "c12" not in m and 3 in m and 5 in m:
                m["c12"] = second(0, m[3] + m[5])
            if "c21" not in m and 2 in m and 4 in m:
                m["c21"] = first(1, m[2] + m[4])
            if "c11" not in m and all(k in m for k in (1, 4, 5, 7)):
                m["c11"] = first(0, (m[4] - m[5]) + m[1] + m[7])
            if "c22" not in m and all(k in m for k in (1, 2, 3, 6)):
                m["c22"] = second(1, (m[3] - m[2]) + m[1] + m[6])
        return l

    def head_weights(g, hh, q0):
        w = qt[pl.ds(pl.multiple_of(g * 64 + hh * 16, 16), 16), pl.ds(q0, TQ)]
        parts = []
        if hh > 0:
            parts.append(jnp.zeros((16 * hh, TQ), u32))
        parts.append(w)
        if hh < 3:
            parts.append(jnp.zeros((16 * (3 - hh), TQ), u32))
        return _unpack(jnp.concatenate(parts, axis=0))

    def v_rows(g, hh, c):
        rows = pl.ds(pl.multiple_of(g * 64 + hh * 16, 16), 16)
        return _unpack(vt[rows, c * KC:(c + 1) * KC])

    def finish_group(g):
        o = jnp.dot(v_rows(g, HPB - 1, NC - 1), _unpack(pp[...]), preferred_element_type=f32)
        last = (ot[3 * DH:4 * DH, :] + o) * invs[0:1, :]
        return jnp.concatenate([ot[0:3 * DH, :], last], axis=0).T.astype(bf16)

    def o_rows(q0):
        return pl.ds(pl.multiple_of(q0 // 2, TQ // 2), TQ // 2)

    def attn_fast(q0):
        def body(i, lmax):
            st = {}

            def qk(gg, hh, c):
                g = i * GPB + gg
                if c == 0:
                    st[gg, hh] = dict(w=head_weights(g, hh, q0))
                kc = _unpack(kb[g, c * KC // 2:(c + 1) * KC // 2, :])
                return jnp.dot(kc, st[gg, hh]["w"], preferred_element_type=f32)

            def pv(gg, hh, c, s):
                g = i * GPB + gg
                d = st[gg, hh]
                if c == 0:
                    d["m"] = jnp.broadcast_to(jnp.max(s[0:8], axis=0, keepdims=True), (8, TQ))
                p = jnp.exp2(s.reshape(KC // 8, 8, TQ) - d["m"][None])
                lc = jnp.sum(p, axis=0)
                d["l"] = lc if c == 0 else d["l"] + lc
                p = p.reshape(KC, TQ).astype(bf16)
                if c == NC - 1:
                    d["lsum"] = jnp.sum(d["l"], axis=0, keepdims=True)
                if gg == GPB - 1 and hh == HPB - 1 and c == NC - 1:
                    pp[...] = _pack(p)
                    ot[hh * DH:(hh + 1) * DH, :] = d["acc"]
                    invs[...] = jnp.broadcast_to(_recip(d["lsum"]), (8, TQ))
                    return
                o = jnp.dot(v_rows(g, hh, c), p, preferred_element_type=f32)
                d["acc"] = o if c == 0 else d["acc"] + o
                if c == NC - 1:
                    d["out"] = d["acc"] * _recip(d["lsum"])
                    if gg == GPB - 1:
                        ot[hh * DH:(hh + 1) * DH, :] = d["out"]
                    elif hh == HPB - 1:
                        o_t = jnp.concatenate([st[gg, k]["out"] for k in range(HPB)], axis=0)
                        ob[g, o_rows(q0), :] = _pack(o_t.T.astype(bf16))

            pend = None
            for gg in range(GPB):
                for hh in range(HPB):
                    for c in range(NC):
                        s = qk(gg, hh, c)
                        if pend is None:
                            ob[jnp.where(i == 0, NT, i * GPB - 1), o_rows(q0), :] = _pack(
                                finish_group(jnp.maximum(i * GPB - 1, 0)))
                        else:
                            pv(*pend)
                        pend = (gg, hh, c, s)
            pv(*pend)
            for d in st.values():
                lmax = jnp.maximum(lmax, d["lsum"])
            return lmax

        return lax.fori_loop(0, NT // GPB, body, jnp.zeros((1, TQ), f32))

    def attn_exact(q0):
        def group(g, carry):
            def head(hh, carry2):
                w = qt[pl.ds(pl.multiple_of(g * 64, 64), 64), pl.ds(q0, TQ)]
                row = lax.broadcasted_iota(jnp.int32, (64, TQ), 0) // 16
                w = _unpack(jnp.where(row == hh, w, jnp.zeros_like(w)))

                def scores(c):
                    kc = kb[g, pl.ds(pl.multiple_of(c * (KC // 2), KC // 2), KC // 2), :]
                    return jnp.dot(_unpack(kc), w, preferred_element_type=f32)

                def row_max(c, m):
                    return jnp.maximum(m, jnp.max(scores(c), axis=0, keepdims=True))

                m = lax.fori_loop(0, NC, row_max, jnp.full((1, TQ), -jnp.inf, f32))

                def accumulate(c, state):
                    l, acc = state
                    p = jnp.exp2(scores(c) - m)
                    v = vt[pl.ds(pl.multiple_of(g * 64 + hh * 16, 16), 16),
                           pl.ds(pl.multiple_of(c * KC, KC), KC)]
                    o = jnp.dot(_unpack(v), p.astype(bf16), preferred_element_type=f32)
                    return l + jnp.sum(p, axis=0, keepdims=True), acc + o

                l, acc = lax.fori_loop(0, NC, accumulate,
                                       (jnp.zeros((1, TQ), f32), jnp.zeros((DH, TQ), f32)))
                ot[pl.ds(pl.multiple_of(hh * DH, DH), DH), :] = acc * (1.0 / l)
                return carry2
            lax.fori_loop(0, HPB, head, 0)
            ob[g, o_rows(q0), :] = _pack(ot[...].T.astype(bf16))
            return carry
        lax.fori_loop(0, NT, group, 0)
        pp[...] = jnp.zeros(pp.shape, u32)
        invs[...] = jnp.ones(invs.shape, f32)

    def q_body(qb, l):
        q0 = pl.multiple_of(qb * TQ, TQ)

        def attempt(state):
            a, _ = state

            @pl.when(a == 0)
            def _():
                lmx[...] = jnp.broadcast_to(attn_fast(q0), (8, TQ))

            @pl.when(a == 1)
            def _():
                attn_exact(q0)

            @pl.when(jnp.logical_or(l == 1, a == 1))
            def _():
                for j in range(TQ // OC):
                    out_copy(qb, j).wait()

            o = jnp.concatenate([_unpack(ob[g, o_rows(q0), :]) for g in range(NT - 1)]
                                + [finish_group(NT - 1)], axis=1)
            hq = TQ // 2
            blocks = (lambda: o[:hq, :HD].astype(f32), lambda: o[:hq, HD:].astype(f32),
                      lambda: o[hq:, :HD].astype(f32), lambda: o[hq:, HD:].astype(f32))

            def emit(j, y):
                rows = pl.ds(q0 + j * OC, OC)
                x2 = xs[rows, :] + y
                xs2[rows, :] = x2
                outb[rows, :] = x2.astype(bf16)
                out_copy(qb, j).start()

            m = {}
            for step in T1_ORDER[:-1]:
                m[step] = _product(_strassen_lhs(step, *blocks), wos, step - 1, LO - 1, SUB_T)
                if step == T1_ORDER[2]:
                    bad = _tree(jnp.maximum,
                                [jnp.where(lmx[:, i * 128:(i + 1) * 128] <= L_MAX, 0.0, 1.0)
                                 for i in range(TQ // 128)])
                    v_ok = (vbig[...] & jnp.uint32(0x80008000)) == 0
                    unsafe = jnp.max(jnp.where(v_ok, bad, 1.0))
            top = jnp.concatenate([(m[4] - m[5]) + m[1] + m[7], m[3] + m[5]], axis=1)
            for j in range(hq // OC):
                emit(j, top[j * OC:(j + 1) * OC])
            rest22 = (m[3] + m[6]) + m[1]
            m2 = _product(_strassen_lhs(2, *blocks), wos, 1, LO - 1, SUB_T)
            bot = jnp.concatenate([m2 + m[4], rest22 - m2], axis=1)
            for j in range(hq // OC):
                emit(hq // OC + j, bot[j * OC:(j + 1) * OC])
            return a + 1, unsafe

        lax.while_loop(lambda st: jnp.logical_or(st[0] == 0, jnp.logical_and(st[0] == 1, st[1] > 0.5)),
                       attempt, (jnp.int32(0), jnp.float32(0)))
        return l

    def layer_pair(l, carry):
        ka[:, 0:HALO, :] = jnp.zeros((NT, HALO, 128), f32)
        va[:, 0:HALO, :] = jnp.zeros((NT, HALO, 128), f32)
        vbig[...] = jnp.zeros(vbig.shape, u32)

        @pl.when(l == 1)
        def _():
            load_x(0, l, RB // LC)

        lax.fori_loop(0, S // RB, row_body, l)

        @pl.when(l == 0)
        def _():
            wob_copy.wait()
            prep_rhs(wob, 0, D, wos, LO)

        lax.fori_loop(0, S // TQ, q_body, l)
        return carry

    x_copy(0).wait()
    load_x(0, 0, RB // LC)
    for i in range(NWO):
        woa_copy(i).wait()
        if i == NWO - 1:
            for cp in late:
                cp.start()
        lax.fori_loop(i * NT // NWO, (i + 1) * NT // NWO, prep_woa, 0)
    lax.fori_loop(0, 2, layer_pair, 0)
    for qb in range(S // TQ):
        for j in range(TQ // OC):
            out_copy(qb, j).wait()


@jax.jit
def pallas_interleave_layers__sliding_local_dilated__softmax_full_mha__prompt_kernel(
    A_x: jax.Array,
    A_wqkv: jax.Array,
    A_wo: jax.Array,
    B_x: jax.Array,
    B_wqkv: jax.Array,
    B_wo: jax.Array,
):
    del B_x
    x = A_x.reshape(S, D)
    hbm = pl.BlockSpec(memory_space=pl.ANY)
    out = pl.pallas_call(
        _kernel,
        out_shape=jax.ShapeDtypeStruct((S, D), bf16),
        in_specs=[hbm] * 5,
        out_specs=hbm,
        scratch_shapes=[
            pltpu.VMEM((S, D), bf16),
            pltpu.VMEM((D, 3 * D), bf16),
            pltpu.VMEM((D, D), bf16),
            pltpu.VMEM((D, 3 * D), bf16),
            pltpu.VMEM((D, D), bf16),
            pltpu.VMEM((S, D), bf16),
            pltpu.VMEM((3, (H + 1) * PITCH, 128), f32),
            pltpu.VMEM(((H + 2) * WPITCH, 128), u32),
            pltpu.VMEM((D // 2, 3 * D), u32),
            pltpu.VMEM((D // 2, D), u32),
            pltpu.VMEM((7 ** LQK, D >> LQK + 1, 2 * D >> LQK), u32),
            pltpu.VMEM((7 ** LV, D >> LV + 1, D >> LV), u32),
            pltpu.VMEM((7 ** LO, D >> LO + 1, D >> LO), u32),
            pltpu.VMEM((RB // 2, D), u32),
            pltpu.VMEM((S + RB, D), f32),
            pltpu.VMEM((S, D), f32),
            pltpu.VMEM((NT, RB, 128), f32),
            pltpu.VMEM((NT, HALO + RB, 128), f32),
            pltpu.VMEM((NT, HALO + RB, 128), f32),
            pltpu.VMEM((D // 2, S), u32),
            pltpu.VMEM((NT, S // 2, 128), u32),
            pltpu.VMEM((D // 2, S), u32),
            pltpu.VMEM((NT + 1, S // 2, 128), u32),
            pltpu.VMEM((128, TQ), f32),
            pltpu.VMEM((KC // 2, TQ), u32),
            pltpu.VMEM((8, TQ), f32),
            pltpu.VMEM((8, TQ), f32),
            pltpu.VMEM((8, 128), u32),
            pltpu.SemaphoreType.DMA((S // RB,)),
            pltpu.SemaphoreType.DMA((NT,)),
            pltpu.SemaphoreType.DMA((2 + NWO,)),
            pltpu.SemaphoreType.DMA((S // OC,)),
        ],
        compiler_params=pltpu.CompilerParams(vmem_limit_bytes=120 * 1024 * 1024),
    )(x, A_wqkv, A_wo, B_wqkv, B_wo)
    return out.reshape(1, S, D)
```

```python
import functools
import math

import jax
import jax.numpy as jnp
from jax import lax
import jax.experimental.pallas as pl
import jax.experimental.pallas.tpu as pltpu

S = 2048
D = 1024
H = 32
DH = 32
WIN = 8
DIL = 2
EPS = 1e-5
NT = D // 128
HPB = 4
HD = D // 2
HALO = 16
QSCALE = (DH ** -0.5) * math.log2(math.e)

SB = 128
NSUB = 2
RB = SB * NSUB
RC = 8
LC = 8
LOOK = (1, 2)
TILE_GATE = (2, 2)
PV_GATE = (1, 1)
LN_LOOK = (2, 1)
LX_LOOK = 5

LQK = 2
LV = 2
LO = 2
B_ORDER = [("qk", 5), ("qk", 3), ("v", 5), ("v", 3), ("next", 0), ("v", 4), ("v", 2), ("v", 1),
           ("v", 7), ("v", 6), ("qk", 4), ("qk", 2), ("qk", 1), ("qk", 7), ("qk", 6)]
SUB_B = (5, 3, 4, 2, 7, 1, 6)
SUB_T = (1, 4, 5, 7, 3, 2, 6)
T1_ORDER = (6, 5, 4, 3, 1, 7, 2)

TQ = 512
KC = 256
NC = S // KC
GPB = 2
OC = 128
L_MAX = 2.0 ** 64
V_EXP = 50

NFLIGHT = 3
WA_STARTS = (2, 1, 2, 1, 2, 1, 1, 0)
NWO = 4
XLU_TILES = (8, 8, 0)
PITCH = 40
WPITCH = 17

bf16 = jnp.bfloat16
f32 = jnp.float32
u32 = jnp.uint32

NN = (((1,), (0,)), ((), ()))
NTD = (((1,), (1,)), ((), ()))


def _pack(x):
    return pltpu.bitcast(x, u32)


def _unpack(x):
    return pltpu.bitcast(x, bf16)


def _after(value, dep):
    if dep is None:
        return value
    return jnp.maximum(value, jnp.minimum(dep, -3e38))


def _tree(op, xs):
    xs = list(xs)
    while len(xs) > 1:
        xs = [op(xs[i], xs[i + 1]) if i + 1 < len(xs) else xs[i] for i in range(0, len(xs), 2)]
    return xs[0]


def _recip(x):
    r = pl.reciprocal(x, approx=True)
    return r * (2.0 - x * r)


def _too_large(packed):
    bias = 0x8000 - ((127 + V_EXP) << 7)
    t = (packed & jnp.uint32(0x7F807F80)) + jnp.uint32(bias << 16 | bias)
    return _tree(jnp.bitwise_or, [t[i:i + 8] for i in range(0, t.shape[0], 8)])


def _layernorm(load, nrows, look):
    outs = []
    deps = []
    for c in range(nrows // LC):
        dep = deps[c - look] if c >= look else None
        x = load(c * LC, dep)
        mu = jnp.broadcast_to(jnp.sum(x, axis=-1, keepdims=True), (LC, 128)) * _after(1.0 / D, dep)
        xc = x - jnp.concatenate([mu] * NT, axis=1)
        var = jnp.sum(xc * xc, axis=-1, keepdims=True) * (1.0 / D)
        y = xc * lax.rsqrt(var + EPS)
        deps.append(y[:, D - 128:])
        outs.append(y)
    return jnp.concatenate(outs, axis=0)


def _strassen_lhs(k, a11, a12, a21, a22):
    if k == 1:
        return a11() + a22()
    if k == 2:
        return a21() + a22()
    if k == 3:
        return a11()
    if k == 4:
        return a22()
    if k == 5:
        return a11() + a12()
    if k == 6:
        return a21() - a11()
    return a12() - a22()


def _strassen_rhs(b11, b12, b21, b22):
    return [b11 + b22, b11, b12 - b22, b21 - b11, b22, b11 + b12, b21 + b22]


def _rhs_operands(chunks, level):
    if level == 0:
        return chunks
    h = len(chunks) // 2
    n = chunks[0].shape[1] // 2
    per_chunk = [_strassen_rhs(chunks[i][:, :n], chunks[i][:, n:], chunks[h + i][:, :n], chunks[h + i][:, n:])
                 for i in range(h)]
    out = []
    for k in range(7):
        out += _rhs_operands([per_chunk[i][k] for i in range(h)], level - 1)
    return out


def _product(a, w_ref, index, level, order):
    if level == 0:
        return lax.dot_general(a.astype(bf16), _unpack(w_ref[index]), NN, preferred_element_type=f32)
    m2, k2 = a.shape[0] // 2, a.shape[1] // 2
    blocks = (lambda: a[:m2, :k2], lambda: a[:m2, k2:], lambda: a[m2:, :k2], lambda: a[m2:, k2:])
    m = {k: _product(_strassen_lhs(k, *blocks), w_ref, index * 7 + k - 1, level - 1, order) for k in order}
    top = jnp.concatenate([(m[4] - m[5]) + m[1] + m[7], m[3] + m[5]], axis=1)
    bot = jnp.concatenate([m[2] + m[4], (m[3] - m[2]) + m[1] + m[6]], axis=1)
    return jnp.concatenate([top, bot], axis=0)


def _kernel(x_hbm, wa_hbm, woa_hbm, wb_hbm, wob_hbm, out_hbm,
            xin, wa_raw, woa_raw, wb_raw, wob, outb,
            stg, stw, wan, woa, wqk, wv, wos, xnb,
            xs, xs2, qa, ka, va, qt, kb, vt, ob, ot, pp, invs, lmx, vbig,
            sem_x, sem_wa, sem_w, sem_o):
    def x_copy(r):
        rows = pl.ds(pl.multiple_of(r * RB, RB), RB)
        return pltpu.make_async_copy(x_hbm.at[rows, :], xin.at[rows, :], sem_x.at[r])

    def wa_copy(i):
        rows = pl.ds(pl.multiple_of(i * 128, 128), 128)
        return pltpu.make_async_copy(wa_hbm.at[rows, :], wa_raw.at[rows, :], sem_wa.at[i])

    wb_copy = pltpu.make_async_copy(wb_hbm, wb_raw, sem_w.at[0])

    def woa_copy(i):
        cols = pl.ds(pl.multiple_of(i * (D // NWO), D // NWO), D // NWO)
        return pltpu.make_async_copy(woa_hbm.at[:, cols], woa_raw.at[:, cols], sem_w.at[2 + i])

    wob_copy = pltpu.make_async_copy(wob_hbm, wob, sem_w.at[1])

    def out_copy(qb, j):
        rows = pl.ds(pl.multiple_of(qb * TQ + j * OC, OC), OC)
        return pltpu.make_async_copy(outb.at[rows, :], out_hbm.at[rows, :],
                                     sem_o.at[qb * (TQ // OC) + j])

    queue = ([wa_copy(i) for i in range(NT)]
             + [x_copy(0)] + [woa_copy(i) for i in range(NWO)]
             + [x_copy(1), wb_copy]
             + [x_copy(r) for r in range(2, S // RB)] + [wob_copy])
    for cp in queue[:NFLIGHT]:
        cp.start()
    queue = queue[NFLIGHT:]

    batches = [[queue.pop(0) for _ in range(n)] for n in WA_STARTS]
    late = [queue.pop(0) for _ in range(NT + 3 + NWO - NFLIGHT - sum(WA_STARTS))]

    def transpose(w):
        ri = lax.broadcasted_iota(jnp.int32, (128, 128), 0)
        ci = lax.broadcasted_iota(jnp.int32, (128, 128), 1)
        eye = jnp.where(ri == ci, 1.0, 0.0).astype(bf16)
        return lax.dot_general(eye, w, NTD, preferred_element_type=f32)

    def prep_wa(t, carry):
        wa_copy(t).wait()
        for k, batch in enumerate(batches):
            @pl.when(t == k)
            def _():
                for cp in batch:
                    cp.start()

        rows = pl.ds(pl.multiple_of(t * 128, 128), 128)

        def forward(part):
            for j in range(NT):
                wt = transpose(wa_raw[rows, part * D + j * 128:part * D + (j + 1) * 128])
                for hh in range(HPB):
                    r = (j * HPB + hh) * PITCH
                    stg[part, r:r + DH, :] = wt[hh * DH:(hh + 1) * DH]

        def back(part):
            regrouped = jnp.concatenate([stg[part, pl.ds(d, H, stride=PITCH), :]
                                         for d in range(DH)], axis=0)
            n = XLU_TILES[part] * 128
            pieces = []
            if n > 0:
                pieces.append(regrouped[:n].T)
            if n < D:
                pieces.append(transpose(regrouped[n:].astype(bf16)))
            wan[pl.ds(pl.multiple_of(t * 64, 64), 64), part * D:(part + 1) * D] = _pack(
                jnp.concatenate(pieces, axis=1).astype(bf16))

        forward(0)
        forward(1)
        back(0)
        forward(2)
        back(1)
        back(2)
        return carry

    def prep_woa(t, carry):
        cols = pl.ds(pl.multiple_of(t * 128, 128), 128)
        w = _pack(woa_raw[:, cols])
        for h in range(H):
            stw[h * WPITCH:h * WPITCH + DH // 2, :] = w[h * (DH // 2):(h + 1) * (DH // 2)]
        lo = jnp.uint32(0xFFFF)
        for j in range(DH // 2):
            even = stw[pl.ds(j, H // 2, stride=2 * WPITCH), :]
            odd = stw[pl.ds(WPITCH + j, H // 2, stride=2 * WPITCH), :]
            woa[2 * j * 16:(2 * j + 1) * 16, cols] = (even & lo) | (odd << 16)
            woa[(2 * j + 1) * 16:(2 * j + 2) * 16, cols] = (even >> 16) | (odd & ~lo)
        return carry

    def rhs_step(src, c0, c1, dst, level, i, tile, odd):
        nb = D >> level
        wb = (c1 - c0) >> level

        def rows(j):
            rs = pl.ds(pl.multiple_of(j * nb + i * 16, 16), 16)
            w = _pack(jnp.concatenate(
                [src[rs, c0 + q * wb + tile * 128:c0 + q * wb + (tile + 1) * 128]
                 for q in range(1 << level)], axis=1))
            return pltpu.bitcast(jnp.concatenate([w << 16, w & jnp.uint32(0xFFFF0000)], axis=0), f32)

        out_rows = pl.ds(pl.multiple_of(i * 8, 8), 8)
        out_cols = slice(tile * 128, (tile + 1) * 128)
        for k, w in enumerate(_rhs_operands([rows(j) for j in range(1 << level)], level)):
            u = pltpu.bitcast(w, u32) + jnp.uint32(0x8000)
            dst[k, out_rows, out_cols] = _pack(jnp.where(odd, _unpack(u[8:16]), _unpack(u[0:8] >> 16)))

    def prep_rhs(src, c0, c1, dst, level):
        odd = lax.broadcasted_iota(jnp.int32, (16, 128), 0) % 2 == 1
        for tile in range(((c1 - c0) >> level) // 128):
            def step(i, carry):
                rhs_step(src, c0, c1, dst, level, i, tile, odd)
                return carry

            lax.fori_loop(0, (D >> level) // 16, step, 0)

    ot[...] = jnp.zeros(ot.shape, f32)
    pp[...] = jnp.zeros(pp.shape, u32)
    invs[...] = jnp.ones(invs.shape, f32)
    lax.fori_loop(0, NT, prep_wa, 0)

    def local_attn(r0, s, first_dep):
        outs = []
        deps = []
        for c in range(SB // RC):
            base = s * SB + c * RC
            window = [slice(HALO + base - DIL * w, HALO + base - DIL * w + RC) for w in range(WIN)]
            scale = _after(QSCALE, deps[c - LOOK[s]] if c >= LOOK[s] else first_dep)
            logits = [None] * WIN
            for t in range(NT):
                if t > 0 and t % TILE_GATE[s] == 0:
                    scale = _after(QSCALE, logits[WIN - 1])
                q = qa[t, base:base + RC, :] * scale
                for w in range(WIN):
                    term = q * ka[t, window[w], :]
                    logits[w] = term if t == 0 else logits[w] + term
            for w in range(WIN):
                acc = logits[w]
                acc = acc + pltpu.roll(acc, 64, 1)
                acc = acc + pltpu.roll(acc, 32, 1)
                if base < DIL * w:
                    row = r0 + base + lax.broadcasted_iota(jnp.int32, (RC, 128), 0)
                    acc = jnp.where(row >= DIL * w, acc, -1e9)
                logits[w] = acc
            m = _tree(jnp.maximum, logits)
            p = [jnp.exp2(lg - m) for lg in logits]
            inv = _recip(_tree(jnp.add, p))
            tiles = []
            done = []
            for t in range(NT):
                if t >= PV_GATE[s]:
                    p[0] = _after(p[0], done[t - PV_GATE[s]])
                acc = _tree(jnp.add, [p[w] * va[t, window[w], :] for w in range(WIN)]) * inv
                tiles.append(acc.astype(bf16))
                done.append(acc)
            deps.append(m)
            outs.append(jnp.concatenate(tiles, axis=1))
        return jnp.concatenate(outs, axis=0)

    def load_x(r, l, look):
        r0 = pl.multiple_of(jnp.minimum(r, S // RB - 1) * RB, RB)
        w0 = pl.multiple_of(r * RB, RB)

        def load(start, dep):
            def from_input():
                x16 = xin[pl.ds(r0 + start // 16 * 16, 16), :].astype(f32)
                return x16[start % 16:start % 16 + LC]

            def from_layer_b():
                return xs2[pl.ds(r0 + start, LC), :]

            if isinstance(l, int):
                x = from_input() if l == 0 else from_layer_b()
            else:
                lvec = _after(jnp.full((LC, 128), l, f32), dep)
                first = jnp.concatenate([lvec == 0.0] * NT, axis=1)
                x = jnp.where(first, from_input(), from_layer_b())
            xs[pl.ds(w0 + start, LC), :] = x
            return x

        xnb[...] = _pack(_layernorm(load, RB, look).astype(bf16))

    def row_body(r, l):
        r0 = pl.multiple_of(r * RB, RB)
        rows = [pl.ds(r0 + s * SB, SB) for s in range(NSUB)]

        @pl.when(jnp.logical_and(l == 0, r == 1))
        def _():
            for cp in queue:
                cp.start()

        def qkv_a(s):
            xn = _unpack(xnb[s * SB // 2:(s + 1) * SB // 2, :])
            y = lax.dot_general(xn, _unpack(wan[...]), NN, preferred_element_type=f32)
            new = slice(HALO + s * SB, HALO + (s + 1) * SB)
            for t in range(NT):
                qa[t, s * SB:(s + 1) * SB, :] = y[:, t * 128:(t + 1) * 128]
                ka[t, new, :] = y[:, D + t * 128:D + (t + 1) * 128]
                va[t, new, :] = y[:, 2 * D + t * 128:2 * D + (t + 1) * 128]
            return y[SB - RC:SB, 2 * D - 128:2 * D]

        def out_a(s, k_done):
            o = local_attn(r0, s, k_done)
            return lax.dot_general(o, _unpack(woa[...]), NN, preferred_element_type=f32)

        def put_q(s, y):
            qt[:, rows[s]] = _pack((y * QSCALE).T.astype(bf16))

        def put_k(s, y):
            krows = pl.ds(pl.multiple_of((r0 + s * SB) // 2, SB // 2), SB // 2)
            y = y.astype(bf16)
            for g in range(NT):
                kb[g, krows, :] = _pack(y[:, g * 128:(g + 1) * 128])

        def put_v(half, s, y):
            v_t = _pack(y.T.astype(bf16))
            vt[half * HD // 2:(half + 1) * HD // 2, rows[s]] = v_t
            vbig[...] = vbig[...] | _too_large(v_t)

        k_done = [qkv_a(s) for s in range(NSUB)]
        y0 = out_a(0, k_done[0])
        ka[:, 0:HALO, :] = ka[:, RB:RB + HALO, :]
        va[:, 0:HALO, :] = va[:, RB:RB + HALO, :]
        x0 = xs[rows[0], :] + y0
        xs[rows[0], :] = x0
        xn0 = _layernorm(lambda st, dep: x0[st:st + LC], SB, LN_LOOK[0])
        y1 = out_a(1, k_done[1])
        xs[rows[1], :] = xs[rows[1], :] + y1

        @pl.when(jnp.logical_and(l == 0, r + 1 < S // RB))
        def _():
            x_copy(jnp.minimum(r + 1, S // RB - 1)).wait()

        @pl.when(jnp.logical_and(l == 0, r == 0))
        def _():
            wb_copy.wait()
            prep_rhs(wb_raw, 0, 2 * D, wqk, LQK)
            prep_rhs(wb_raw, 2 * D, 3 * D, wv, LV)

        xn1 = _layernorm(lambda st, dep: xs[pl.ds(r0 + SB + st, LC), :], SB, LN_LOOK[1])
        blocks = (lambda: xn0[:, :HD], lambda: xn0[:, HD:], lambda: xn1[:, :HD], lambda: xn1[:, HD:])
        lhs = {}
        ms = {"qk": {}, "v": {}}
        puts = {"qk": (put_q, put_k), "v": (functools.partial(put_v, 0), functools.partial(put_v, 1))}
        for inst, step in B_ORDER:
            if inst == "next":
                load_x(r + 1, l, LX_LOOK)
                continue
            if step not in lhs:
                lhs[step] = _strassen_lhs(step, *blocks)
            m = ms[inst]
            first, second = puts[inst]
            m[step] = _product(lhs[step], wqk if inst == "qk" else wv, step - 1,
                               (LQK if inst == "qk" else LV) - 1, SUB_B)
            if "c12" not in m and 3 in m and 5 in m:
                m["c12"] = second(0, m[3] + m[5])
            if "c21" not in m and 2 in m and 4 in m:
                m["c21"] = first(1, m[2] + m[4])
            if "c11" not in m and all(k in m for k in (1, 4, 5, 7)):
                m["c11"] = first(0, (m[4] - m[5]) + m[1] + m[7])
            if "c22" not in m and all(k in m for k in (1, 2, 3, 6)):
                m["c22"] = second(1, (m[3] - m[2]) + m[1] + m[6])
        return l

    def head_weights(g, hh, q0):
        w = qt[pl.ds(pl.multiple_of(g * 64 + hh * 16, 16), 16), pl.ds(q0, TQ)]
        parts = []
        if hh > 0:
            parts.append(jnp.zeros((16 * hh, TQ), u32))
        parts.append(w)
        if hh < 3:
            parts.append(jnp.zeros((16 * (3 - hh), TQ), u32))
        return _unpack(jnp.concatenate(parts, axis=0))

    def v_rows(g, hh, c):
        rows = pl.ds(pl.multiple_of(g * 64 + hh * 16, 16), 16)
        return _unpack(vt[rows, c * KC:(c + 1) * KC])

    def finish_group(g):
        o = jnp.dot(v_rows(g, HPB - 1, NC - 1), _unpack(pp[...]), preferred_element_type=f32)
        last = (ot[3 * DH:4 * DH, :] + o) * invs[0:1, :]
        return jnp.concatenate([ot[0:3 * DH, :], last], axis=0).T.astype(bf16)

    def o_rows(q0):
        return pl.ds(pl.multiple_of(q0 // 2, TQ // 2), TQ // 2)

    def attn_fast(q0):
        def body(i, lmax):
            st = {}

            def qk(gg, hh, c):
                g = i * GPB + gg
                if c == 0:
                    st[gg, hh] = dict(w=head_weights(g, hh, q0))
                kc = _unpack(kb[g, c * KC // 2:(c + 1) * KC // 2, :])
                return jnp.dot(kc, st[gg, hh]["w"], preferred_element_type=f32)

            def pv(gg, hh, c, s):
                g = i * GPB + gg
                d = st[gg, hh]
                if c == 0:
                    d["m"] = jnp.broadcast_to(jnp.max(s[0:8], axis=0, keepdims=True), (8, TQ))
                p = jnp.exp2(s.reshape(KC // 8, 8, TQ) - d["m"][None])
                lc = jnp.sum(p, axis=0)
                d["l"] = lc if c == 0 else d["l"] + lc
                p = p.reshape(KC, TQ).astype(bf16)
                if c == NC - 1:
                    d["lsum"] = jnp.sum(d["l"], axis=0, keepdims=True)
                if gg == GPB - 1 and hh == HPB - 1 and c == NC - 1:
                    pp[...] = _pack(p)
                    ot[hh * DH:(hh + 1) * DH, :] = d["acc"]
                    invs[...] = jnp.broadcast_to(_recip(d["lsum"]), (8, TQ))
                    return
                o = jnp.dot(v_rows(g, hh, c), p, preferred_element_type=f32)
                d["acc"] = o if c == 0 else d["acc"] + o
                if c == NC - 1:
                    d["out"] = d["acc"] * _recip(d["lsum"])
                    if gg == GPB - 1:
                        ot[hh * DH:(hh + 1) * DH, :] = d["out"]
                    elif hh == HPB - 1:
                        o_t = jnp.concatenate([st[gg, k]["out"] for k in range(HPB)], axis=0)
                        ob[g, o_rows(q0), :] = _pack(o_t.T.astype(bf16))

            pend = None
            for gg in range(GPB):
                for hh in range(HPB):
                    for c in range(NC):
                        s = qk(gg, hh, c)
                        if pend is None:
                            ob[jnp.where(i == 0, NT, i * GPB - 1), o_rows(q0), :] = _pack(
                                finish_group(jnp.maximum(i * GPB - 1, 0)))
                        else:
                            pv(*pend)
                        pend = (gg, hh, c, s)
            pv(*pend)
            for d in st.values():
                lmax = jnp.maximum(lmax, d["lsum"])
            return lmax

        return lax.fori_loop(0, NT // GPB, body, jnp.zeros((1, TQ), f32))

    def attn_exact(q0):
        def group(g, carry):
            def head(hh, carry2):
                w = qt[pl.ds(pl.multiple_of(g * 64, 64), 64), pl.ds(q0, TQ)]
                row = lax.broadcasted_iota(jnp.int32, (64, TQ), 0) // 16
                w = _unpack(jnp.where(row == hh, w, jnp.zeros_like(w)))

                def scores(c):
                    kc = kb[g, pl.ds(pl.multiple_of(c * (KC // 2), KC // 2), KC // 2), :]
                    return jnp.dot(_unpack(kc), w, preferred_element_type=f32)

                def row_max(c, m):
                    return jnp.maximum(m, jnp.max(scores(c), axis=0, keepdims=True))

                m = lax.fori_loop(0, NC, row_max, jnp.full((1, TQ), -jnp.inf, f32))

                def accumulate(c, state):
                    l, acc = state
                    p = jnp.exp2(scores(c) - m)
                    v = vt[pl.ds(pl.multiple_of(g * 64 + hh * 16, 16), 16),
                           pl.ds(pl.multiple_of(c * KC, KC), KC)]
                    o = jnp.dot(_unpack(v), p.astype(bf16), preferred_element_type=f32)
                    return l + jnp.sum(p, axis=0, keepdims=True), acc + o

                l, acc = lax.fori_loop(0, NC, accumulate,
                                       (jnp.zeros((1, TQ), f32), jnp.zeros((DH, TQ), f32)))
                ot[pl.ds(pl.multiple_of(hh * DH, DH), DH), :] = acc * (1.0 / l)
                return carry2
            lax.fori_loop(0, HPB, head, 0)
            ob[g, o_rows(q0), :] = _pack(ot[...].T.astype(bf16))
            return carry
        lax.fori_loop(0, NT, group, 0)
        pp[...] = jnp.zeros(pp.shape, u32)
        invs[...] = jnp.ones(invs.shape, f32)

    def q_body(qb, l):
        q0 = pl.multiple_of(qb * TQ, TQ)

        def attempt(state):
            a, _ = state

            @pl.when(a == 0)
            def _():
                lmx[...] = jnp.broadcast_to(attn_fast(q0), (8, TQ))

            @pl.when(a == 1)
            def _():
                attn_exact(q0)

            @pl.when(jnp.logical_or(l == 1, a == 1))
            def _():
                for j in range(TQ // OC):
                    out_copy(qb, j).wait()

            o = jnp.concatenate([_unpack(ob[g, o_rows(q0), :]) for g in range(NT - 1)]
                                + [finish_group(NT - 1)], axis=1)
            hq = TQ // 2
            blocks = (lambda: o[:hq, :HD].astype(f32), lambda: o[:hq, HD:].astype(f32),
                      lambda: o[hq:, :HD].astype(f32), lambda: o[hq:, HD:].astype(f32))

            def emit(j, y):
                rows = pl.ds(q0 + j * OC, OC)
                x2 = xs[rows, :] + y
                xs2[rows, :] = x2
                outb[rows, :] = x2.astype(bf16)
                out_copy(qb, j).start()

            m = {}
            for step in T1_ORDER[:-1]:
                m[step] = _product(_strassen_lhs(step, *blocks), wos, step - 1, LO - 1, SUB_T)
                if step == T1_ORDER[2]:
                    bad = _tree(jnp.maximum,
                                [jnp.where(lmx[:, i * 128:(i + 1) * 128] <= L_MAX, 0.0, 1.0)
                                 for i in range(TQ // 128)])
                    v_ok = (vbig[...] & jnp.uint32(0x80008000)) == 0
                    unsafe = jnp.max(jnp.where(v_ok, bad, 1.0))
            top = jnp.concatenate([(m[4] - m[5]) + m[1] + m[7], m[3] + m[5]], axis=1)
            for j in range(hq // OC):
                emit(j, top[j * OC:(j + 1) * OC])
            rest22 = (m[3] + m[6]) + m[1]
            m2 = _product(_strassen_lhs(2, *blocks), wos, 1, LO - 1, SUB_T)
            bot = jnp.concatenate([m2 + m[4], rest22 - m2], axis=1)
            for j in range(hq // OC):
                emit(hq // OC + j, bot[j * OC:(j + 1) * OC])
            return a + 1, unsafe

        lax.while_loop(lambda st: jnp.logical_or(st[0] == 0, jnp.logical_and(st[0] == 1, st[1] > 0.5)),
                       attempt, (jnp.int32(0), jnp.float32(0)))
        return l

    def layer_pair(l, carry):
        ka[:, 0:HALO, :] = jnp.zeros((NT, HALO, 128), f32)
        va[:, 0:HALO, :] = jnp.zeros((NT, HALO, 128), f32)
        vbig[...] = jnp.zeros(vbig.shape, u32)

        @pl.when(l == 1)
        def _():
            load_x(0, l, RB // LC)

        lax.fori_loop(0, S // RB, row_body, l)

        @pl.when(l == 0)
        def _():
            wob_copy.wait()
            prep_rhs(wob, 0, D, wos, LO)

        lax.fori_loop(0, S // TQ, q_body, l)
        return carry

    x_copy(0).wait()
    load_x(0, 0, RB // LC)
    for i in range(NWO):
        woa_copy(i).wait()
        if i == NWO - 1:
            for cp in late:
                cp.start()
        lax.fori_loop(i * NT // NWO, (i + 1) * NT // NWO, prep_woa, 0)
    lax.fori_loop(0, 2, layer_pair, 0)
    for qb in range(S // TQ):
        for j in range(TQ // OC):
            out_copy(qb, j).wait()


@jax.jit
def pallas_interleave_layers__sliding_local_dilated__softmax_full_mha__prompt_kernel(
    A_x: jax.Array,
    A_wqkv: jax.Array,
    A_wo: jax.Array,
    B_x: jax.Array,
    B_wqkv: jax.Array,
    B_wo: jax.Array,
):
    del B_x
    x = A_x.reshape(S, D)
    hbm = pl.BlockSpec(memory_space=pl.ANY)
    out = pl.pallas_call(
        _kernel,
        out_shape=jax.ShapeDtypeStruct((S, D), bf16),
        in_specs=[hbm] * 5,
        out_specs=hbm,
        scratch_shapes=[
            pltpu.VMEM((S, D), bf16),
            pltpu.VMEM((D, 3 * D), bf16),
            pltpu.VMEM((D, D), bf16),
            pltpu.VMEM((D, 3 * D), bf16),
            pltpu.VMEM((D, D), bf16),
            pltpu.VMEM((S, D), bf16),
            pltpu.VMEM((3, (H + 1) * PITCH, 128), f32),
            pltpu.VMEM(((H + 2) * WPITCH, 128), u32),
            pltpu.VMEM((D // 2, 3 * D), u32),
            pltpu.VMEM((D // 2, D), u32),
            pltpu.VMEM((7 ** LQK, D >> LQK + 1, 2 * D >> LQK), u32),
            pltpu.VMEM((7 ** LV, D >> LV + 1, D >> LV), u32),
            pltpu.VMEM((7 ** LO, D >> LO + 1, D >> LO), u32),
            pltpu.VMEM((RB // 2, D), u32),
            pltpu.VMEM((S + RB, D), f32),
            pltpu.VMEM((S, D), f32),
            pltpu.VMEM((NT, RB, 128), f32),
            pltpu.VMEM((NT, HALO + RB, 128), f32),
            pltpu.VMEM((NT, HALO + RB, 128), f32),
            pltpu.VMEM((D // 2, S), u32),
            pltpu.VMEM((NT, S // 2, 128), u32),
            pltpu.VMEM((D // 2, S), u32),
            pltpu.VMEM((NT + 1, S // 2, 128), u32),
            pltpu.VMEM((128, TQ), f32),
            pltpu.VMEM((KC // 2, TQ), u32),
            pltpu.VMEM((8, TQ), f32),
            pltpu.VMEM((8, TQ), f32),
            pltpu.VMEM((8, 128), u32),
            pltpu.SemaphoreType.DMA((S // RB,)),
            pltpu.SemaphoreType.DMA((NT,)),
            pltpu.SemaphoreType.DMA((2 + NWO,)),
            pltpu.SemaphoreType.DMA((S // OC,)),
        ],
        compiler_params=pltpu.CompilerParams(vmem_limit_bytes=120 * 1024 * 1024),
    )(x, A_wqkv, A_wo, B_wqkv, B_wo)
    return out.reshape(1, S, D)
```

```python
import functools
import math

import jax
import jax.numpy as jnp
from jax import lax
import jax.experimental.pallas as pl
import jax.experimental.pallas.tpu as pltpu

S = 2048
D = 1024
H = 32
DH = 32
WIN = 8
DIL = 2
EPS = 1e-5
NT = D // 128
HPB = 4
HD = D // 2
HALO = 16
QSCALE = (DH ** -0.5) * math.log2(math.e)

SB = 128
NSUB = 2
RB = SB * NSUB
RC = 8
LC = 8
LOOK = (1, 2)
TILE_GATE = (2, 2)
PV_GATE = (1, 1)
LN_LOOK = (2, 1)
LX_LOOK = 8

LQK = 2
LV = 2
LO = 2
B_ORDER = (15, 13, 25, 23, 0, 24, 22, 11, 14, 12, 27, 26, 21, 17, 16)
SUB_B = (4, 2, 3, 5, 1, 7, 6)
SUB_T = (3, 1, 4, 5, 7, 2, 6)
T1_ORDER = (6, 5, 4, 3, 1, 7, 2)

TQ = 512
KC = 256
NC = S // KC
GPB = 2
OC = 128
L_MAX = 2.0 ** 64
V_EXP = 50

NFLIGHT = 3
WA_STARTS = (2, 1, 2, 1, 2, 1, 1, 0)
NWO = 4
XLU_TILES = (8, 8, 0)
PITCH = 40
WPITCH = 17

bf16 = jnp.bfloat16
f32 = jnp.float32
u32 = jnp.uint32

NN = (((1,), (0,)), ((), ()))
NTD = (((1,), (1,)), ((), ()))


def _pack(x):
    return pltpu.bitcast(x, u32)


def _unpack(x):
    return pltpu.bitcast(x, bf16)


def _after(value, dep):
    if dep is None:
        return value
    return jnp.maximum(value, jnp.minimum(dep, -3e38))


def _tree(op, xs):
    xs = list(xs)
    while len(xs) > 1:
        xs = [op(xs[i], xs[i + 1]) if i + 1 < len(xs) else xs[i] for i in range(0, len(xs), 2)]
    return xs[0]


def _recip(x):
    r = pl.reciprocal(x, approx=True)
    return r * (2.0 - x * r)


def _too_large(packed):
    bias = 0x8000 - ((127 + V_EXP) << 7)
    t = (packed & jnp.uint32(0x7F807F80)) + jnp.uint32(bias << 16 | bias)
    return _tree(jnp.bitwise_or, [t[i:i + 8] for i in range(0, t.shape[0], 8)])


def _layernorm(load, nrows, look):
    outs = []
    deps = []
    for c in range(nrows // LC):
        dep = deps[c - look] if c >= look else None
        x = load(c * LC, dep)
        mu = jnp.broadcast_to(jnp.sum(x, axis=-1, keepdims=True), (LC, 128)) * _after(1.0 / D, dep)
        xc = x - jnp.concatenate([mu] * NT, axis=1)
        var = jnp.sum(xc * xc, axis=-1, keepdims=True) * (1.0 / D)
        y = xc * lax.rsqrt(var + EPS)
        deps.append(y[:, D - 128:])
        outs.append(y)
    return jnp.concatenate(outs, axis=0)


def _strassen_lhs(k, a11, a12, a21, a22):
    if k == 1:
        return a11() + a22()
    if k == 2:
        return a21() + a22()
    if k == 3:
        return a11()
    if k == 4:
        return a22()
    if k == 5:
        return a11() + a12()
    if k == 6:
        return a21() - a11()
    return a12() - a22()


def _strassen_rhs(b11, b12, b21, b22):
    return [b11 + b22, b11, b12 - b22, b21 - b11, b22, b11 + b12, b21 + b22]


def _rhs_operands(chunks, level):
    if level == 0:
        return chunks
    h = len(chunks) // 2
    n = chunks[0].shape[1] // 2
    per_chunk = [_strassen_rhs(chunks[i][:, :n], chunks[i][:, n:], chunks[h + i][:, :n], chunks[h + i][:, n:])
                 for i in range(h)]
    out = []
    for k in range(7):
        out += _rhs_operands([per_chunk[i][k] for i in range(h)], level - 1)
    return out


def _product(a, w_ref, index, level, order):
    if level == 0:
        return lax.dot_general(a.astype(bf16), _unpack(w_ref[index]), NN, preferred_element_type=f32)
    m2, k2 = a.shape[0] // 2, a.shape[1] // 2
    blocks = (lambda: a[:m2, :k2], lambda: a[:m2, k2:], lambda: a[m2:, :k2], lambda: a[m2:, k2:])
    m = {k: _product(_strassen_lhs(k, *blocks), w_ref, index * 7 + k - 1, level - 1, order) for k in order}
    top = jnp.concatenate([(m[4] - m[5]) + m[1] + m[7], m[3] + m[5]], axis=1)
    bot = jnp.concatenate([m[2] + m[4], (m[3] - m[2]) + m[1] + m[6]], axis=1)
    return jnp.concatenate([top, bot], axis=0)


def _kernel(x_hbm, wa_hbm, woa_hbm, wb_hbm, wob_hbm, out_hbm,
            xin, wa_raw, woa_raw, wb_raw, wob, outb,
            stg, stw, wan, woa, wqk, wv, wos, xnb,
            xs, xs2, qa, ka, va, qt, kb, vt, ob, ot, pp, invs, lmx, vbig,
            sem_x, sem_wa, sem_w, sem_o):
    def x_copy(r):
        rows = pl.ds(pl.multiple_of(r * RB, RB), RB)
        return pltpu.make_async_copy(x_hbm.at[rows, :], xin.at[rows, :], sem_x.at[r])

    def wa_copy(i):
        rows = pl.ds(pl.multiple_of(i * 128, 128), 128)
        return pltpu.make_async_copy(wa_hbm.at[rows, :], wa_raw.at[rows, :], sem_wa.at[i])

    wb_copy = pltpu.make_async_copy(wb_hbm, wb_raw, sem_w.at[0])

    def woa_copy(i):
        cols = pl.ds(pl.multiple_of(i * (D // NWO), D // NWO), D // NWO)
        return pltpu.make_async_copy(woa_hbm.at[:, cols], woa_raw.at[:, cols], sem_w.at[2 + i])

    wob_copy = pltpu.make_async_copy(wob_hbm, wob, sem_w.at[1])

    def out_copy(qb, j):
        rows = pl.ds(pl.multiple_of(qb * TQ + j * OC, OC), OC)
        return pltpu.make_async_copy(outb.at[rows, :], out_hbm.at[rows, :],
                                     sem_o.at[qb * (TQ // OC) + j])

    queue = ([wa_copy(i) for i in range(NT)]
             + [x_copy(0)] + [woa_copy(i) for i in range(NWO)]
             + [x_copy(1), wb_copy]
             + [x_copy(r) for r in range(2, S // RB)] + [wob_copy])
    for cp in queue[:NFLIGHT]:
        cp.start()
    queue = queue[NFLIGHT:]

    batches = [[queue.pop(0) for _ in range(n)] for n in WA_STARTS]
    late = [queue.pop(0) for _ in range(NT + 3 + NWO - NFLIGHT - sum(WA_STARTS))]

    def transpose(w):
        ri = lax.broadcasted_iota(jnp.int32, (128, 128), 0)
        ci = lax.broadcasted_iota(jnp.int32, (128, 128), 1)
        eye = jnp.where(ri == ci, 1.0, 0.0).astype(bf16)
        return lax.dot_general(eye, w, NTD, preferred_element_type=f32)

    def prep_wa(t, carry):
        wa_copy(t).wait()
        for k, batch in enumerate(batches):
            @pl.when(t == k)
            def _():
                for cp in batch:
                    cp.start()

        rows = pl.ds(pl.multiple_of(t * 128, 128), 128)

        def forward(part):
            for j in range(NT):
                wt = transpose(wa_raw[rows, part * D + j * 128:part * D + (j + 1) * 128])
                for hh in range(HPB):
                    r = (j * HPB + hh) * PITCH
                    stg[part, r:r + DH, :] = wt[hh * DH:(hh + 1) * DH]

        def back(part):
            regrouped = jnp.concatenate([stg[part, pl.ds(d, H, stride=PITCH), :]
                                         for d in range(DH)], axis=0)
            n = XLU_TILES[part] * 128
            pieces = []
            if n > 0:
                pieces.append(regrouped[:n].T)
            if n < D:
                pieces.append(transpose(regrouped[n:].astype(bf16)))
            wan[pl.ds(pl.multiple_of(t * 64, 64), 64), part * D:(part + 1) * D] = _pack(
                jnp.concatenate(pieces, axis=1).astype(bf16))

        forward(0)
        forward(1)
        back(0)
        forward(2)
        back(1)
        back(2)
        return carry

    def prep_woa(t, carry):
        cols = pl.ds(pl.multiple_of(t * 128, 128), 128)
        w = _pack(woa_raw[:, cols])
        for h in range(H):
            stw[h * WPITCH:h * WPITCH + DH // 2, :] = w[h * (DH // 2):(h + 1) * (DH // 2)]
        lo = jnp.uint32(0xFFFF)
        for j in range(DH // 2):
            even = stw[pl.ds(j, H // 2, stride=2 * WPITCH), :]
            odd = stw[pl.ds(WPITCH + j, H // 2, stride=2 * WPITCH), :]
            woa[2 * j * 16:(2 * j + 1) * 16, cols] = (even & lo) | (odd << 16)
            woa[(2 * j + 1) * 16:(2 * j + 2) * 16, cols] = (even >> 16) | (odd & ~lo)
        return carry

    def rhs_step(src, c0, c1, dst, level, i, tile, odd):
        nb = D >> level
        wb = (c1 - c0) >> level

        def rows(j):
            rs = pl.ds(pl.multiple_of(j * nb + i * 16, 16), 16)
            w = _pack(jnp.concatenate(
                [src[rs, c0 + q * wb + tile * 128:c0 + q * wb + (tile + 1) * 128]
                 for q in range(1 << level)], axis=1))
            return pltpu.bitcast(jnp.concatenate([w << 16, w & jnp.uint32(0xFFFF0000)], axis=0), f32)

        out_rows = pl.ds(pl.multiple_of(i * 8, 8), 8)
        out_cols = slice(tile * 128, (tile + 1) * 128)
        for k, w in enumerate(_rhs_operands([rows(j) for j in range(1 << level)], level)):
            u = pltpu.bitcast(w, u32) + jnp.uint32(0x8000)
            dst[k, out_rows, out_cols] = _pack(jnp.where(odd, _unpack(u[8:16]), _unpack(u[0:8] >> 16)))

    def prep_rhs(src, c0, c1, dst, level):
        odd = lax.broadcasted_iota(jnp.int32, (16, 128), 0) % 2 == 1
        for tile in range(((c1 - c0) >> level) // 128):
            def step(i, carry):
                rhs_step(src, c0, c1, dst, level, i, tile, odd)
                return carry

            lax.fori_loop(0, (D >> level) // 16, step, 0)

    ot[...] = jnp.zeros(ot.shape, f32)
    pp[...] = jnp.zeros(pp.shape, u32)
    invs[...] = jnp.ones(invs.shape, f32)
    lax.fori_loop(0, NT, prep_wa, 0)

    def local_attn(r0, s, first_dep):
        outs = []
        deps = []
        for c in range(SB // RC):
            base = s * SB + c * RC
            window = [slice(HALO + base - DIL * w, HALO + base - DIL * w + RC) for w in range(WIN)]
            scale = _after(QSCALE, deps[c - LOOK[s]] if c >= LOOK[s] else first_dep)
            logits = [None] * WIN
            for t in range(NT):
                if t > 0 and t % TILE_GATE[s] == 0:
                    scale = _after(QSCALE, logits[WIN - 1])
                q = qa[t, base:base + RC, :] * scale
                for w in range(WIN):
                    term = q * ka[t, window[w], :]
                    logits[w] = term if t == 0 else logits[w] + term
            for w in range(WIN):
                acc = logits[w]
                acc = acc + pltpu.roll(acc, 64, 1)
                acc = acc + pltpu.roll(acc, 32, 1)
                if base < DIL * w:
                    row = r0 + base + lax.broadcasted_iota(jnp.int32, (RC, 128), 0)
                    acc = jnp.where(row >= DIL * w, acc, -1e9)
                logits[w] = acc
            m = _tree(jnp.maximum, logits)
            p = [jnp.exp2(lg - m) for lg in logits]
            inv = _recip(_tree(jnp.add, p))
            tiles = []
            done = []
            for t in range(NT):
                if t >= PV_GATE[s]:
                    p[0] = _after(p[0], done[t - PV_GATE[s]])
                acc = _tree(jnp.add, [p[w] * va[t, window[w], :] for w in range(WIN)]) * inv
                tiles.append(acc.astype(bf16))
                done.append(acc)
            deps.append(m)
            outs.append(jnp.concatenate(tiles, axis=1))
        return jnp.concatenate(outs, axis=0)

    def load_x(r, l, look):
        r0 = pl.multiple_of(jnp.minimum(r, S // RB - 1) * RB, RB)
        w0 = pl.multiple_of(r * RB, RB)

        def load(start, dep):
            def from_input():
                x16 = xin[pl.ds(r0 + start // 16 * 16, 16), :].astype(f32)
                return x16[start % 16:start % 16 + LC]

            def from_layer_b():
                return xs2[pl.ds(r0 + start, LC), :]

            if isinstance(l, int):
                x = from_input() if l == 0 else from_layer_b()
            else:
                lvec = _after(jnp.full((LC, 128), l, f32), dep)
                first = jnp.concatenate([lvec == 0.0] * NT, axis=1)
                x = jnp.where(first, from_input(), from_layer_b())
            xs[pl.ds(w0 + start, LC), :] = x
            return x

        xnb[...] = _pack(_layernorm(load, RB, look).astype(bf16))

    def row_body(r, l):
        r0 = pl.multiple_of(r * RB, RB)
        rows = [pl.ds(r0 + s * SB, SB) for s in range(NSUB)]

        @pl.when(jnp.logical_and(l == 0, r == 1))
        def _():
            for cp in queue:
                cp.start()

        def qkv_a(s):
            xn = _unpack(xnb[s * SB // 2:(s + 1) * SB // 2, :])
            y = lax.dot_general(xn, _unpack(wan[...]), NN, preferred_element_type=f32)
            new = slice(HALO + s * SB, HALO + (s + 1) * SB)
            for t in range(NT):
                qa[t, s * SB:(s + 1) * SB, :] = y[:, t * 128:(t + 1) * 128]
                ka[t, new, :] = y[:, D + t * 128:D + (t + 1) * 128]
                va[t, new, :] = y[:, 2 * D + t * 128:2 * D + (t + 1) * 128]
            return y[SB - RC:SB, 2 * D - 128:2 * D]

        def out_a(s, k_done):
            o = local_attn(r0, s, k_done)
            return lax.dot_general(o, _unpack(woa[...]), NN, preferred_element_type=f32)

        def put_q(s, y):
            qt[:, rows[s]] = _pack((y * QSCALE).T.astype(bf16))

        def put_k(s, y):
            krows = pl.ds(pl.multiple_of((r0 + s * SB) // 2, SB // 2), SB // 2)
            y = y.astype(bf16)
            for g in range(NT):
                kb[g, krows, :] = _pack(y[:, g * 128:(g + 1) * 128])

        def put_v(half, s, y):
            v_t = _pack(y.T.astype(bf16))
            vt[half * HD // 2:(half + 1) * HD // 2, rows[s]] = v_t
            vbig[...] = vbig[...] | _too_large(v_t)

        k_done = [qkv_a(s) for s in range(NSUB)]
        y0 = out_a(0, k_done[0])
        ka[:, 0:HALO, :] = ka[:, RB:RB + HALO, :]
        va[:, 0:HALO, :] = va[:, RB:RB + HALO, :]
        x0 = xs[rows[0], :] + y0
        xs[rows[0], :] = x0
        xn0 = _layernorm(lambda st, dep: x0[st:st + LC], SB, LN_LOOK[0])
        y1 = out_a(1, k_done[1])
        xs[rows[1], :] = xs[rows[1], :] + y1

        @pl.when(jnp.logical_and(l == 0, r + 1 < S // RB))
        def _():
            x_copy(jnp.minimum(r + 1, S // RB - 1)).wait()

        @pl.when(jnp.logical_and(l == 0, r == 0))
        def _():
            wb_copy.wait()
            prep_rhs(wb_raw, 0, 2 * D, wqk, LQK)
            prep_rhs(wb_raw, 2 * D, 3 * D, wv, LV)

        xn1 = _layernorm(lambda st, dep: xs[pl.ds(r0 + SB + st, LC), :], SB, LN_LOOK[1])
        blocks = (lambda: xn0[:, :HD], lambda: xn0[:, HD:], lambda: xn1[:, :HD], lambda: xn1[:, HD:])
        lhs = {}
        ms = {"qk": {}, "v": {}}
        puts = {"qk": (put_q, put_k), "v": (functools.partial(put_v, 0), functools.partial(put_v, 1))}
        for item in B_ORDER:
            if item == 0:
                load_x(r + 1, l, LX_LOOK)
                continue
            inst, step = ("qk" if item < 20 else "v"), item % 10
            if step not in lhs:
                lhs[step] = _strassen_lhs(step, *blocks)
            m = ms[inst]
            first, second = puts[inst]
            m[step] = _product(lhs[step], wqk if inst == "qk" else wv, step - 1,
                               (LQK if inst == "qk" else LV) - 1, SUB_B)
            if "c12" not in m and 3 in m and 5 in m:
                m["c12"] = second(0, m[3] + m[5])
            if "c21" not in m and 2 in m and 4 in m:
                m["c21"] = first(1, m[2] + m[4])
            if "c11" not in m and all(k in m for k in (1, 4, 5, 7)):
                m["c11"] = first(0, (m[4] - m[5]) + m[1] + m[7])
            if "c22" not in m and all(k in m for k in (1, 2, 3, 6)):
                m["c22"] = second(1, (m[3] - m[2]) + m[1] + m[6])
        return l

    def head_weights(g, hh, q0):
        w = qt[pl.ds(pl.multiple_of(g * 64 + hh * 16, 16), 16), pl.ds(q0, TQ)]
        parts = []
        if hh > 0:
            parts.append(jnp.zeros((16 * hh, TQ), u32))
        parts.append(w)
        if hh < 3:
            parts.append(jnp.zeros((16 * (3 - hh), TQ), u32))
        return _unpack(jnp.concatenate(parts, axis=0))

    def v_rows(g, hh, c):
        rows = pl.ds(pl.multiple_of(g * 64 + hh * 16, 16), 16)
        return _unpack(vt[rows, c * KC:(c + 1) * KC])

    def finish_group(g):
        o = jnp.dot(v_rows(g, HPB - 1, NC - 1), _unpack(pp[...]), preferred_element_type=f32)
        last = (ot[3 * DH:4 * DH, :] + o) * invs[0:1, :]
        return jnp.concatenate([ot[0:3 * DH, :], last], axis=0).T.astype(bf16)

    def o_rows(q0):
        return pl.ds(pl.multiple_of(q0 // 2, TQ // 2), TQ // 2)

    def attn_fast(q0):
        def body(i, lmax):
            st = {}

            def qk(gg, hh, c):
                g = i * GPB + gg
                if c == 0:
                    st[gg, hh] = dict(w=head_weights(g, hh, q0))
                kc = _unpack(kb[g, c * KC // 2:(c + 1) * KC // 2, :])
                return jnp.dot(kc, st[gg, hh]["w"], preferred_element_type=f32)

            def pv(gg, hh, c, s):
                g = i * GPB + gg
                d = st[gg, hh]
                if c == 0:
                    d["m"] = jnp.broadcast_to(jnp.max(s[0:8], axis=0, keepdims=True), (8, TQ))
                p = jnp.exp2(s.reshape(KC // 8, 8, TQ) - d["m"][None])
                lc = jnp.sum(p, axis=0)
                d["l"] = lc if c == 0 else d["l"] + lc
                p = p.reshape(KC, TQ).astype(bf16)
                if c == NC - 1:
                    d["lsum"] = jnp.sum(d["l"], axis=0, keepdims=True)
                if gg == GPB - 1 and hh == HPB - 1 and c == NC - 1:
                    pp[...] = _pack(p)
                    ot[hh * DH:(hh + 1) * DH, :] = d["acc"]
                    invs[...] = jnp.broadcast_to(_recip(d["lsum"]), (8, TQ))
                    return
                o = jnp.dot(v_rows(g, hh, c), p, preferred_element_type=f32)
                d["acc"] = o if c == 0 else d["acc"] + o
                if c == NC - 1:
                    d["out"] = d["acc"] * _recip(d["lsum"])
                    if gg == GPB - 1:
                        ot[hh * DH:(hh + 1) * DH, :] = d["out"]
                    elif hh == HPB - 1:
                        o_t = jnp.concatenate([st[gg, k]["out"] for k in range(HPB)], axis=0)
                        ob[g, o_rows(q0), :] = _pack(o_t.T.astype(bf16))

            pend = None
            for gg in range(GPB):
                for hh in range(HPB):
                    for c in range(NC):
                        s = qk(gg, hh, c)
                        if pend is None:
                            ob[jnp.where(i == 0, NT, i * GPB - 1), o_rows(q0), :] = _pack(
                                finish_group(jnp.maximum(i * GPB - 1, 0)))
                        else:
                            pv(*pend)
                        pend = (gg, hh, c, s)
            pv(*pend)
            for d in st.values():
                lmax = jnp.maximum(lmax, d["lsum"])
            return lmax

        return lax.fori_loop(0, NT // GPB, body, jnp.zeros((1, TQ), f32))

    def attn_exact(q0):
        def group(g, carry):
            def head(hh, carry2):
                w = qt[pl.ds(pl.multiple_of(g * 64, 64), 64), pl.ds(q0, TQ)]
                row = lax.broadcasted_iota(jnp.int32, (64, TQ), 0) // 16
                w = _unpack(jnp.where(row == hh, w, jnp.zeros_like(w)))

                def scores(c):
                    kc = kb[g, pl.ds(pl.multiple_of(c * (KC // 2), KC // 2), KC // 2), :]
                    return jnp.dot(_unpack(kc), w, preferred_element_type=f32)

                def row_max(c, m):
                    return jnp.maximum(m, jnp.max(scores(c), axis=0, keepdims=True))

                m = lax.fori_loop(0, NC, row_max, jnp.full((1, TQ), -jnp.inf, f32))

                def accumulate(c, state):
                    l, acc = state
                    p = jnp.exp2(scores(c) - m)
                    v = vt[pl.ds(pl.multiple_of(g * 64 + hh * 16, 16), 16),
                           pl.ds(pl.multiple_of(c * KC, KC), KC)]
                    o = jnp.dot(_unpack(v), p.astype(bf16), preferred_element_type=f32)
                    return l + jnp.sum(p, axis=0, keepdims=True), acc + o

                l, acc = lax.fori_loop(0, NC, accumulate,
                                       (jnp.zeros((1, TQ), f32), jnp.zeros((DH, TQ), f32)))
                ot[pl.ds(pl.multiple_of(hh * DH, DH), DH), :] = acc * (1.0 / l)
                return carry2
            lax.fori_loop(0, HPB, head, 0)
            ob[g, o_rows(q0), :] = _pack(ot[...].T.astype(bf16))
            return carry
        lax.fori_loop(0, NT, group, 0)
        pp[...] = jnp.zeros(pp.shape, u32)
        invs[...] = jnp.ones(invs.shape, f32)

    def q_body(qb, l):
        q0 = pl.multiple_of(qb * TQ, TQ)

        def attempt(state):
            a, _ = state

            @pl.when(a == 0)
            def _():
                lmx[...] = jnp.broadcast_to(attn_fast(q0), (8, TQ))

            @pl.when(a == 1)
            def _():
                attn_exact(q0)

            @pl.when(jnp.logical_or(l == 1, a == 1))
            def _():
                for j in range(TQ // OC):
                    out_copy(qb, j).wait()

            o = jnp.concatenate([_unpack(ob[g, o_rows(q0), :]) for g in range(NT - 1)]
                                + [finish_group(NT - 1)], axis=1)
            hq = TQ // 2
            blocks = (lambda: o[:hq, :HD].astype(f32), lambda: o[:hq, HD:].astype(f32),
                      lambda: o[hq:, :HD].astype(f32), lambda: o[hq:, HD:].astype(f32))

            def emit(j, y):
                rows = pl.ds(q0 + j * OC, OC)
                x2 = xs[rows, :] + y
                xs2[rows, :] = x2
                outb[rows, :] = x2.astype(bf16)
                out_copy(qb, j).start()

            m = {}
            for step in T1_ORDER[:-1]:
                m[step] = _product(_strassen_lhs(step, *blocks), wos, step - 1, LO - 1, SUB_T)
                if step == T1_ORDER[2]:
                    bad = _tree(jnp.maximum,
                                [jnp.where(lmx[:, i * 128:(i + 1) * 128] <= L_MAX, 0.0, 1.0)
                                 for i in range(TQ // 128)])
                    v_ok = (vbig[...] & jnp.uint32(0x80008000)) == 0
                    unsafe = jnp.max(jnp.where(v_ok, bad, 1.0))
            top = jnp.concatenate([(m[4] - m[5]) + m[1] + m[7], m[3] + m[5]], axis=1)
            for j in range(hq // OC):
                emit(j, top[j * OC:(j + 1) * OC])
            rest22 = (m[3] + m[6]) + m[1]
            m2 = _product(_strassen_lhs(2, *blocks), wos, 1, LO - 1, SUB_T)
            bot = jnp.concatenate([m2 + m[4], rest22 - m2], axis=1)
            for j in range(hq // OC):
                emit(hq // OC + j, bot[j * OC:(j + 1) * OC])
            return a + 1, unsafe

        lax.while_loop(lambda st: jnp.logical_or(st[0] == 0, jnp.logical_and(st[0] == 1, st[1] > 0.5)),
                       attempt, (jnp.int32(0), jnp.float32(0)))
        return l

    def layer_pair(l, carry):
        ka[:, 0:HALO, :] = jnp.zeros((NT, HALO, 128), f32)
        va[:, 0:HALO, :] = jnp.zeros((NT, HALO, 128), f32)
        vbig[...] = jnp.zeros(vbig.shape, u32)

        @pl.when(l == 1)
        def _():
            load_x(0, l, RB // LC)

        lax.fori_loop(0, S // RB, row_body, l)

        @pl.when(l == 0)
        def _():
            wob_copy.wait()
            prep_rhs(wob, 0, D, wos, LO)

        lax.fori_loop(0, S // TQ, q_body, l)
        return carry

    x_copy(0).wait()
    load_x(0, 0, RB // LC)
    for i in range(NWO):
        woa_copy(i).wait()
        if i == NWO - 1:
            for cp in late:
                cp.start()
        lax.fori_loop(i * NT // NWO, (i + 1) * NT // NWO, prep_woa, 0)
    lax.fori_loop(0, 2, layer_pair, 0)
    for qb in range(S // TQ):
        for j in range(TQ // OC):
            out_copy(qb, j).wait()


@jax.jit
def pallas_interleave_layers__sliding_local_dilated__softmax_full_mha__prompt_kernel(
    A_x: jax.Array,
    A_wqkv: jax.Array,
    A_wo: jax.Array,
    B_x: jax.Array,
    B_wqkv: jax.Array,
    B_wo: jax.Array,
):
    del B_x
    x = A_x.reshape(S, D)
    hbm = pl.BlockSpec(memory_space=pl.ANY)
    out = pl.pallas_call(
        _kernel,
        out_shape=jax.ShapeDtypeStruct((S, D), bf16),
        in_specs=[hbm] * 5,
        out_specs=hbm,
        scratch_shapes=[
            pltpu.VMEM((S, D), bf16),
            pltpu.VMEM((D, 3 * D), bf16),
            pltpu.VMEM((D, D), bf16),
            pltpu.VMEM((D, 3 * D), bf16),
            pltpu.VMEM((D, D), bf16),
            pltpu.VMEM((S, D), bf16),
            pltpu.VMEM((3, (H + 1) * PITCH, 128), f32),
            pltpu.VMEM(((H + 2) * WPITCH, 128), u32),
            pltpu.VMEM((D // 2, 3 * D), u32),
            pltpu.VMEM((D // 2, D), u32),
            pltpu.VMEM((7 ** LQK, D >> LQK + 1, 2 * D >> LQK), u32),
            pltpu.VMEM((7 ** LV, D >> LV + 1, D >> LV), u32),
            pltpu.VMEM((7 ** LO, D >> LO + 1, D >> LO), u32),
            pltpu.VMEM((RB // 2, D), u32),
            pltpu.VMEM((S + RB, D), f32),
            pltpu.VMEM((S, D), f32),
            pltpu.VMEM((NT, RB, 128), f32),
            pltpu.VMEM((NT, HALO + RB, 128), f32),
            pltpu.VMEM((NT, HALO + RB, 128), f32),
            pltpu.VMEM((D // 2, S), u32),
            pltpu.VMEM((NT, S // 2, 128), u32),
            pltpu.VMEM((D // 2, S), u32),
            pltpu.VMEM((NT + 1, S // 2, 128), u32),
            pltpu.VMEM((128, TQ), f32),
            pltpu.VMEM((KC // 2, TQ), u32),
            pltpu.VMEM((8, TQ), f32),
            pltpu.VMEM((8, TQ), f32),
            pltpu.VMEM((8, 128), u32),
            pltpu.SemaphoreType.DMA((S // RB,)),
            pltpu.SemaphoreType.DMA((NT,)),
            pltpu.SemaphoreType.DMA((2 + NWO,)),
            pltpu.SemaphoreType.DMA((S // OC,)),
        ],
        compiler_params=pltpu.CompilerParams(vmem_limit_bytes=120 * 1024 * 1024),
    )(x, A_wqkv, A_wo, B_wqkv, B_wo)
    return out.reshape(1, S, D)
```

```python
import math

import jax
import jax.numpy as jnp
from jax import lax
import jax.experimental.pallas as pl
import jax.experimental.pallas.tpu as pltpu

S = 2048
D = 1024
H = 32
DH = 32
WIN = 8
DIL = 2
EPS = 1e-5
NT = D // 128
HPB = 4
HD = D // 2
HALO = 16
QSCALE = (DH ** -0.5) * math.log2(math.e)

SB = 128
NSUB = 2
RB = SB * NSUB
RC = 8
LC = 8
LOOK = (1, 3)
TILE_GATE = (2, 3)
PV_GATE = (1, 2)
LN_LOOK = (2, 1)
LX_LOOK = 3

LB = 2
B_TILES = ([t + u for t in (0, 2, 4, 6) for u in (0, 1, 2 * NT, 2 * NT + 1)], list(range(NT, 2 * NT)))
LO = 2
B_ORDER = (15, 13, 25, 23, 22, 14, 17, 12, 21, 24, 0, 11, 16, 27, 26)
SUB_B = (3, 2, 4, 5, 1, 7, 6)
SUB_T = (3, 1, 4, 5, 7, 2, 6)
T1_ORDER = (6, 5, 4, 3, 1, 7, 2)

TQ = 512
KC = 256
NC = S // KC
GPB = 2
OC = 128
L_MAX = 2.0 ** 64
V_EXP = 50

NFLIGHT = 3
WA_STARTS = (2, 1, 2, 1, 2, 1, 1, 0)
NWO = 4
XLU_TILES = (8, 8, 0)
PITCH = 40
WPITCH = 17

bf16 = jnp.bfloat16
f32 = jnp.float32
u32 = jnp.uint32

NN = (((1,), (0,)), ((), ()))
NTD = (((1,), (1,)), ((), ()))


def _pack(x):
    return pltpu.bitcast(x, u32)


def _unpack(x):
    return pltpu.bitcast(x, bf16)


def _after(value, dep):
    if dep is None:
        return value
    return jnp.maximum(value, jnp.minimum(dep, -3e38))


def _tree(op, xs):
    xs = list(xs)
    while len(xs) > 1:
        xs = [op(xs[i], xs[i + 1]) if i + 1 < len(xs) else xs[i] for i in range(0, len(xs), 2)]
    return xs[0]


def _recip(x):
    r = pl.reciprocal(x, approx=True)
    return r * (2.0 - x * r)


def _too_large(packed):
    bias = 0x8000 - ((127 + V_EXP) << 7)
    t = (packed & jnp.uint32(0x7F807F80)) + jnp.uint32(bias << 16 | bias)
    return _tree(jnp.bitwise_or, [t[i:i + 8] for i in range(0, t.shape[0], 8)])


def _layernorm(load, nrows, look):
    outs = []
    deps = []
    for c in range(nrows // LC):
        dep = deps[c - look] if c >= look else None
        x = load(c * LC, dep)
        mu = jnp.broadcast_to(jnp.sum(x, axis=-1, keepdims=True), (LC, 128)) * _after(1.0 / D, dep)
        xc = x - jnp.concatenate([mu] * NT, axis=1)
        var = jnp.sum(xc * xc, axis=-1, keepdims=True) * (1.0 / D)
        y = xc * lax.rsqrt(var + EPS)
        deps.append(y[:, D - 128:])
        outs.append(y)
    return jnp.concatenate(outs, axis=0)


def _strassen_lhs(k, a11, a12, a21, a22):
    if k == 1:
        return a11() + a22()
    if k == 2:
        return a21() + a22()
    if k == 3:
        return a11()
    if k == 4:
        return a22()
    if k == 5:
        return a11() + a12()
    if k == 6:
        return a21() - a11()
    return a12() - a22()


def _strassen_rhs(b11, b12, b21, b22):
    return [b11 + b22, b11, b12 - b22, b21 - b11, b22, b11 + b12, b21 + b22]


def _rhs_operands(chunks, level):
    if level == 0:
        return chunks
    h = len(chunks) // 2
    n = chunks[0].shape[1] // 2
    per_chunk = [_strassen_rhs(chunks[i][:, :n], chunks[i][:, n:], chunks[h + i][:, :n], chunks[h + i][:, n:])
                 for i in range(h)]
    out = []
    for k in range(7):
        out += _rhs_operands([per_chunk[i][k] for i in range(h)], level - 1)
    return out


def _product(a, w_ref, index, level, order):
    if level == 0:
        return lax.dot_general(a.astype(bf16), _unpack(w_ref[index]), NN, preferred_element_type=f32)
    m2, k2 = a.shape[0] // 2, a.shape[1] // 2
    blocks = (lambda: a[:m2, :k2], lambda: a[:m2, k2:], lambda: a[m2:, :k2], lambda: a[m2:, k2:])
    m = {k: _product(_strassen_lhs(k, *blocks), w_ref, index * 7 + k - 1, level - 1, order) for k in order}
    top = jnp.concatenate([(m[4] - m[5]) + m[1] + m[7], m[3] + m[5]], axis=1)
    bot = jnp.concatenate([m[2] + m[4], (m[3] - m[2]) + m[1] + m[6]], axis=1)
    return jnp.concatenate([top, bot], axis=0)


def _kernel(x_hbm, wa_hbm, woa_hbm, wb_hbm, wob_hbm, out_hbm,
            xin, wa_raw, woa_raw, wb_raw, wob, outb,
            stg, stw, wan, woa, wb1, wb2, wos, xnb,
            xs, xs2, qa, ka, va, qt, kb, vt, ob, ot, pp, invs, lmx, vbig,
            sem_x, sem_wa, sem_w, sem_o):
    def x_copy(r):
        rows = pl.ds(pl.multiple_of(r * RB, RB), RB)
        return pltpu.make_async_copy(x_hbm.at[rows, :], xin.at[rows, :], sem_x.at[r])

    def wa_copy(i):
        rows = pl.ds(pl.multiple_of(i * 128, 128), 128)
        return pltpu.make_async_copy(wa_hbm.at[rows, :], wa_raw.at[rows, :], sem_wa.at[i])

    wb_copy = pltpu.make_async_copy(wb_hbm, wb_raw, sem_w.at[0])

    def woa_copy(i):
        cols = pl.ds(pl.multiple_of(i * (D // NWO), D // NWO), D // NWO)
        return pltpu.make_async_copy(woa_hbm.at[:, cols], woa_raw.at[:, cols], sem_w.at[2 + i])

    wob_copy = pltpu.make_async_copy(wob_hbm, wob, sem_w.at[1])

    def out_copy(qb, j):
        rows = pl.ds(pl.multiple_of(qb * TQ + j * OC, OC), OC)
        return pltpu.make_async_copy(outb.at[rows, :], out_hbm.at[rows, :],
                                     sem_o.at[qb * (TQ // OC) + j])

    queue = ([wa_copy(i) for i in range(NT)]
             + [x_copy(0)] + [woa_copy(i) for i in range(NWO)]
             + [x_copy(1), wb_copy]
             + [x_copy(r) for r in range(2, S // RB)] + [wob_copy])
    for cp in queue[:NFLIGHT]:
        cp.start()
    queue = queue[NFLIGHT:]

    batches = [[queue.pop(0) for _ in range(n)] for n in WA_STARTS]
    late = [queue.pop(0) for _ in range(NT + 3 + NWO - NFLIGHT - sum(WA_STARTS))]

    def transpose(w):
        ri = lax.broadcasted_iota(jnp.int32, (128, 128), 0)
        ci = lax.broadcasted_iota(jnp.int32, (128, 128), 1)
        eye = jnp.where(ri == ci, 1.0, 0.0).astype(bf16)
        return lax.dot_general(eye, w, NTD, preferred_element_type=f32)

    def prep_wa(t, carry):
        wa_copy(t).wait()
        for k, batch in enumerate(batches):
            @pl.when(t == k)
            def _():
                for cp in batch:
                    cp.start()

        rows = pl.ds(pl.multiple_of(t * 128, 128), 128)

        def forward(part):
            for j in range(NT):
                wt = transpose(wa_raw[rows, part * D + j * 128:part * D + (j + 1) * 128])
                for hh in range(HPB):
                    r = (j * HPB + hh) * PITCH
                    stg[part, r:r + DH, :] = wt[hh * DH:(hh + 1) * DH]

        def back(part):
            regrouped = jnp.concatenate([stg[part, pl.ds(d, H, stride=PITCH), :]
                                         for d in range(DH)], axis=0)
            n = XLU_TILES[part] * 128
            pieces = []
            if n > 0:
                pieces.append(regrouped[:n].T)
            if n < D:
                pieces.append(transpose(regrouped[n:].astype(bf16)))
            wan[pl.ds(pl.multiple_of(t * 64, 64), 64), part * D:(part + 1) * D] = _pack(
                jnp.concatenate(pieces, axis=1).astype(bf16))

        forward(0)
        forward(1)
        back(0)
        forward(2)
        back(1)
        back(2)
        return carry

    def prep_woa(t, carry):
        cols = pl.ds(pl.multiple_of(t * 128, 128), 128)
        w = _pack(woa_raw[:, cols])
        for h in range(H):
            stw[h * WPITCH:h * WPITCH + DH // 2, :] = w[h * (DH // 2):(h + 1) * (DH // 2)]
        lo = jnp.uint32(0xFFFF)
        for j in range(DH // 2):
            even = stw[pl.ds(j, H // 2, stride=2 * WPITCH), :]
            odd = stw[pl.ds(WPITCH + j, H // 2, stride=2 * WPITCH), :]
            woa[2 * j * 16:(2 * j + 1) * 16, cols] = (even & lo) | (odd << 16)
            woa[(2 * j + 1) * 16:(2 * j + 2) * 16, cols] = (even >> 16) | (odd & ~lo)
        return carry

    def rhs_step(src, tiles, dst, level, i, tile, odd):
        nb = D >> level
        wb = len(tiles) >> level

        def rows(j):
            rs = pl.ds(pl.multiple_of(j * nb + i * 16, 16), 16)
            w = _pack(jnp.concatenate(
                [src[rs, tiles[q * wb + tile] * 128:(tiles[q * wb + tile] + 1) * 128]
                 for q in range(1 << level)], axis=1))
            return pltpu.bitcast(jnp.concatenate([w << 16, w & jnp.uint32(0xFFFF0000)], axis=0), f32)

        out_rows = pl.ds(pl.multiple_of(i * 8, 8), 8)
        out_cols = slice(tile * 128, (tile + 1) * 128)
        for k, w in enumerate(_rhs_operands([rows(j) for j in range(1 << level)], level)):
            u = pltpu.bitcast(w, u32) + jnp.uint32(0x8000)
            dst[k, out_rows, out_cols] = _pack(jnp.where(odd, _unpack(u[8:16]), _unpack(u[0:8] >> 16)))

    def prep_rhs(src, tiles, dst, level):
        odd = lax.broadcasted_iota(jnp.int32, (16, 128), 0) % 2 == 1
        for tile in range(len(tiles) >> level):
            def step(i, carry):
                rhs_step(src, tiles, dst, level, i, tile, odd)
                return carry

            lax.fori_loop(0, (D >> level) // 16, step, 0)

    ot[...] = jnp.zeros(ot.shape, f32)
    pp[...] = jnp.zeros(pp.shape, u32)
    invs[...] = jnp.ones(invs.shape, f32)
    lax.fori_loop(0, NT, prep_wa, 0)

    def local_attn(r0, s, first_dep):
        outs = []
        deps = []
        for c in range(SB // RC):
            base = s * SB + c * RC
            window = [slice(HALO + base - DIL * w, HALO + base - DIL * w + RC) for w in range(WIN)]
            scale = _after(QSCALE, deps[c - LOOK[s]] if c >= LOOK[s] else first_dep)
            logits = [None] * WIN
            for t in range(NT):
                if t > 0 and t % TILE_GATE[s] == 0:
                    scale = _after(QSCALE, logits[WIN - 1])
                q = qa[t, base:base + RC, :] * scale
                for w in range(WIN):
                    term = q * ka[t, window[w], :]
                    logits[w] = term if t == 0 else logits[w] + term
            for w in range(WIN):
                acc = logits[w]
                acc = acc + pltpu.roll(acc, 64, 1)
                acc = acc + pltpu.roll(acc, 32, 1)
                if base < DIL * w:
                    row = r0 + base + lax.broadcasted_iota(jnp.int32, (RC, 128), 0)
                    acc = jnp.where(row >= DIL * w, acc, -1e9)
                logits[w] = acc
            m = _tree(jnp.maximum, logits)
            p = [jnp.exp2(lg - m) for lg in logits]
            inv = _recip(_tree(jnp.add, p))
            tiles = []
            done = []
            for t in range(NT):
                if t >= PV_GATE[s]:
                    p[0] = _after(p[0], done[t - PV_GATE[s]])
                acc = _tree(jnp.add, [p[w] * va[t, window[w], :] for w in range(WIN)]) * inv
                tiles.append(acc.astype(bf16))
                done.append(acc)
            deps.append(m)
            outs.append(jnp.concatenate(tiles, axis=1))
        return jnp.concatenate(outs, axis=0)

    def load_x(r, l, look):
        r0 = pl.multiple_of(jnp.minimum(r, S // RB - 1) * RB, RB)
        w0 = pl.multiple_of(r * RB, RB)

        def load(start, dep):
            def from_input():
                x16 = xin[pl.ds(r0 + start // 16 * 16, 16), :].astype(f32)
                return x16[start % 16:start % 16 + LC]

            def from_layer_b():
                return xs2[pl.ds(r0 + start, LC), :]

            if isinstance(l, int):
                x = from_input() if l == 0 else from_layer_b()
            else:
                lvec = _after(jnp.full((LC, 128), l, f32), dep)
                first = jnp.concatenate([lvec == 0.0] * NT, axis=1)
                x = jnp.where(first, from_input(), from_layer_b())
            xs[pl.ds(w0 + start, LC), :] = x
            return x

        xnb[...] = _pack(_layernorm(load, RB, look).astype(bf16))

    def row_body(r, l):
        r0 = pl.multiple_of(r * RB, RB)
        rows = [pl.ds(r0 + s * SB, SB) for s in range(NSUB)]

        @pl.when(jnp.logical_and(l == 0, r == 1))
        def _():
            for cp in queue:
                cp.start()

        def qkv_a(s):
            xn = _unpack(xnb[s * SB // 2:(s + 1) * SB // 2, :])
            y = lax.dot_general(xn, _unpack(wan[...]), NN, preferred_element_type=f32)
            new = slice(HALO + s * SB, HALO + (s + 1) * SB)
            for t in range(NT):
                qa[t, s * SB:(s + 1) * SB, :] = y[:, t * 128:(t + 1) * 128]
                ka[t, new, :] = y[:, D + t * 128:D + (t + 1) * 128]
                va[t, new, :] = y[:, 2 * D + t * 128:2 * D + (t + 1) * 128]
            return y[SB - RC:SB, 2 * D - 128:2 * D]

        def out_a(s, k_done):
            o = local_attn(r0, s, k_done)
            return lax.dot_general(o, _unpack(woa[...]), NN, preferred_element_type=f32)

        def put(tiles, s, y):
            krows = pl.ds(pl.multiple_of((r0 + s * SB) // 2, SB // 2), SB // 2)
            for j in range(0, len(tiles), 2):
                part, g = divmod(tiles[j], NT)
                yj = y[:, j * 128:(j + 2) * 128]
                if part == 0:
                    qt[g * 64:(g + 2) * 64, rows[s]] = _pack((yj * QSCALE).T.astype(bf16))
                elif part == 1:
                    yj = yj.astype(bf16)
                    kb[g, krows, :] = _pack(yj[:, :128])
                    kb[g + 1, krows, :] = _pack(yj[:, 128:])
                else:
                    v_t = _pack(yj.T.astype(bf16))
                    vt[g * 64:(g + 2) * 64, rows[s]] = v_t
                    vbig[...] = vbig[...] | _too_large(v_t)

        k_done = [qkv_a(s) for s in range(NSUB)]
        y0 = out_a(0, k_done[0])
        ka[:, 0:HALO, :] = ka[:, RB:RB + HALO, :]
        va[:, 0:HALO, :] = va[:, RB:RB + HALO, :]
        x0 = xs[rows[0], :] + y0
        xs[rows[0], :] = x0
        xn0 = _layernorm(lambda st, dep: x0[st:st + LC], SB, LN_LOOK[0])
        y1 = out_a(1, k_done[1])
        xs[rows[1], :] = xs[rows[1], :] + y1

        @pl.when(jnp.logical_and(l == 0, r + 1 < S // RB))
        def _():
            x_copy(jnp.minimum(r + 1, S // RB - 1)).wait()

        @pl.when(jnp.logical_and(l == 0, r == 0))
        def _():
            wb_copy.wait()
            prep_rhs(wb_raw, B_TILES[0], wb1, LB)
            prep_rhs(wb_raw, B_TILES[1], wb2, LB)

        xn1 = _layernorm(lambda st, dep: xs[pl.ds(r0 + SB + st, LC), :], SB, LN_LOOK[1])
        blocks = (lambda: xn0[:, :HD], lambda: xn0[:, HD:], lambda: xn1[:, :HD], lambda: xn1[:, HD:])
        lhs = {}
        ms = [{}, {}]
        for item in B_ORDER:
            if item == 0:
                load_x(r + 1, l, LX_LOOK)
                continue
            inst, step = item // 10 - 1, item % 10
            if step not in lhs:
                lhs[step] = _strassen_lhs(step, *blocks)
            m = ms[inst]
            tiles = B_TILES[inst]
            first, second = tiles[:len(tiles) // 2], tiles[len(tiles) // 2:]
            m[step] = _product(lhs[step], (wb1, wb2)[inst], step - 1, LB - 1, SUB_B)
            if "c12" not in m and 3 in m and 5 in m:
                m["c12"] = put(second, 0, m[3] + m[5])
            if "c21" not in m and 2 in m and 4 in m:
                m["c21"] = put(first, 1, m[2] + m[4])
            if "c11" not in m and all(k in m for k in (1, 4, 5, 7)):
                m["c11"] = put(first, 0, (m[4] - m[5]) + m[1] + m[7])
            if "c22" not in m and all(k in m for k in (1, 2, 3, 6)):
                m["c22"] = put(second, 1, (m[3] - m[2]) + m[1] + m[6])
        return l

    def head_weights(g, hh, q0):
        w = qt[pl.ds(pl.multiple_of(g * 64 + hh * 16, 16), 16), pl.ds(q0, TQ)]
        parts = []
        if hh > 0:
            parts.append(jnp.zeros((16 * hh, TQ), u32))
        parts.append(w)
        if hh < 3:
            parts.append(jnp.zeros((16 * (3 - hh), TQ), u32))
        return _unpack(jnp.concatenate(parts, axis=0))

    def v_rows(g, hh, c):
        rows = pl.ds(pl.multiple_of(g * 64 + hh * 16, 16), 16)
        return _unpack(vt[rows, c * KC:(c + 1) * KC])

    def finish_group(g):
        o = jnp.dot(v_rows(g, HPB - 1, NC - 1), _unpack(pp[...]), preferred_element_type=f32)
        last = (ot[3 * DH:4 * DH, :] + o) * invs[0:1, :]
        return jnp.concatenate([ot[0:3 * DH, :], last], axis=0).T.astype(bf16)

    def o_rows(q0):
        return pl.ds(pl.multiple_of(q0 // 2, TQ // 2), TQ // 2)

    def attn_fast(q0):
        def body(i, lmax):
            st = {}

            def qk(gg, hh, c):
                g = i * GPB + gg
                if c == 0:
                    st[gg, hh] = dict(w=head_weights(g, hh, q0))
                kc = _unpack(kb[g, c * KC // 2:(c + 1) * KC // 2, :])
                return jnp.dot(kc, st[gg, hh]["w"], preferred_element_type=f32)

            def pv(gg, hh, c, s):
                g = i * GPB + gg
                d = st[gg, hh]
                if c == 0:
                    d["m"] = jnp.broadcast_to(jnp.max(s[0:8], axis=0, keepdims=True), (8, TQ))
                p = jnp.exp2(s.reshape(KC // 8, 8, TQ) - d["m"][None])
                lc = jnp.sum(p, axis=0)
                d["l"] = lc if c == 0 else d["l"] + lc
                p = p.reshape(KC, TQ).astype(bf16)
                if c == NC - 1:
                    d["lsum"] = jnp.sum(d["l"], axis=0, keepdims=True)
                if gg == GPB - 1 and hh == HPB - 1 and c == NC - 1:
                    pp[...] = _pack(p)
                    ot[hh * DH:(hh + 1) * DH, :] = d["acc"]
                    invs[...] = jnp.broadcast_to(_recip(d["lsum"]), (8, TQ))
                    return
                o = jnp.dot(v_rows(g, hh, c), p, preferred_element_type=f32)
                d["acc"] = o if c == 0 else d["acc"] + o
                if c == NC - 1:
                    d["out"] = d["acc"] * _recip(d["lsum"])
                    if gg == GPB - 1:
                        ot[hh * DH:(hh + 1) * DH, :] = d["out"]
                    elif hh == HPB - 1:
                        o_t = jnp.concatenate([st[gg, k]["out"] for k in range(HPB)], axis=0)
                        ob[g, o_rows(q0), :] = _pack(o_t.T.astype(bf16))

            pend = None
            for gg in range(GPB):
                for hh in range(HPB):
                    for c in range(NC):
                        s = qk(gg, hh, c)
                        if pend is None:
                            ob[jnp.where(i == 0, NT, i * GPB - 1), o_rows(q0), :] = _pack(
                                finish_group(jnp.maximum(i * GPB - 1, 0)))
                        else:
                            pv(*pend)
                        pend = (gg, hh, c, s)
            pv(*pend)
            for d in st.values():
                lmax = jnp.maximum(lmax, d["lsum"])
            return lmax

        return lax.fori_loop(0, NT // GPB, body, jnp.zeros((1, TQ), f32))

    def attn_exact(q0):
        def group(g, carry):
            def head(hh, carry2):
                w = qt[pl.ds(pl.multiple_of(g * 64, 64), 64), pl.ds(q0, TQ)]
                row = lax.broadcasted_iota(jnp.int32, (64, TQ), 0) // 16
                w = _unpack(jnp.where(row == hh, w, jnp.zeros_like(w)))

                def scores(c):
                    kc = kb[g, pl.ds(pl.multiple_of(c * (KC // 2), KC // 2), KC // 2), :]
                    return jnp.dot(_unpack(kc), w, preferred_element_type=f32)

                def row_max(c, m):
                    return jnp.maximum(m, jnp.max(scores(c), axis=0, keepdims=True))

                m = lax.fori_loop(0, NC, row_max, jnp.full((1, TQ), -jnp.inf, f32))

                def accumulate(c, state):
                    l, acc = state
                    p = jnp.exp2(scores(c) - m)
                    v = vt[pl.ds(pl.multiple_of(g * 64 + hh * 16, 16), 16),
                           pl.ds(pl.multiple_of(c * KC, KC), KC)]
                    o = jnp.dot(_unpack(v), p.astype(bf16), preferred_element_type=f32)
                    return l + jnp.sum(p, axis=0, keepdims=True), acc + o

                l, acc = lax.fori_loop(0, NC, accumulate,
                                       (jnp.zeros((1, TQ), f32), jnp.zeros((DH, TQ), f32)))
                ot[pl.ds(pl.multiple_of(hh * DH, DH), DH), :] = acc * (1.0 / l)
                return carry2
            lax.fori_loop(0, HPB, head, 0)
            ob[g, o_rows(q0), :] = _pack(ot[...].T.astype(bf16))
            return carry
        lax.fori_loop(0, NT, group, 0)
        pp[...] = jnp.zeros(pp.shape, u32)
        invs[...] = jnp.ones(invs.shape, f32)

    def q_body(qb, l):
        q0 = pl.multiple_of(qb * TQ, TQ)

        def attempt(state):
            a, _ = state

            @pl.when(a == 0)
            def _():
                lmx[...] = jnp.broadcast_to(attn_fast(q0), (8, TQ))

            @pl.when(a == 1)
            def _():
                attn_exact(q0)

            @pl.when(jnp.logical_or(l == 1, a == 1))
            def _():
                for j in range(TQ // OC):
                    out_copy(qb, j).wait()

            o = jnp.concatenate([_unpack(ob[g, o_rows(q0), :]) for g in range(NT - 1)]
                                + [finish_group(NT - 1)], axis=1)
            hq = TQ // 2
            blocks = (lambda: o[:hq, :HD].astype(f32), lambda: o[:hq, HD:].astype(f32),
                      lambda: o[hq:, :HD].astype(f32), lambda: o[hq:, HD:].astype(f32))

            def emit(j, y):
                rows = pl.ds(q0 + j * OC, OC)
                x2 = xs[rows, :] + y
                xs2[rows, :] = x2
                outb[rows, :] = x2.astype(bf16)
                out_copy(qb, j).start()

            m = {}
            for step in T1_ORDER[:-1]:
                m[step] = _product(_strassen_lhs(step, *blocks), wos, step - 1, LO - 1, SUB_T)
                if step == T1_ORDER[2]:
                    bad = _tree(jnp.maximum,
                                [jnp.where(lmx[:, i * 128:(i + 1) * 128] <= L_MAX, 0.0, 1.0)
                                 for i in range(TQ // 128)])
                    v_ok = (vbig[...] & jnp.uint32(0x80008000)) == 0
                    unsafe = jnp.max(jnp.where(v_ok, bad, 1.0))
            top = jnp.concatenate([(m[4] - m[5]) + m[1] + m[7], m[3] + m[5]], axis=1)
            for j in range(hq // OC):
                emit(j, top[j * OC:(j + 1) * OC])
            rest22 = (m[3] + m[6]) + m[1]
            m2 = _product(_strassen_lhs(2, *blocks), wos, 1, LO - 1, SUB_T)
            bot = jnp.concatenate([m2 + m[4], rest22 - m2], axis=1)
            for j in range(hq // OC):
                emit(hq // OC + j, bot[j * OC:(j + 1) * OC])
            return a + 1, unsafe

        lax.while_loop(lambda st: jnp.logical_or(st[0] == 0, jnp.logical_and(st[0] == 1, st[1] > 0.5)),
                       attempt, (jnp.int32(0), jnp.float32(0)))
        return l

    def layer_pair(l, carry):
        ka[:, 0:HALO, :] = jnp.zeros((NT, HALO, 128), f32)
        va[:, 0:HALO, :] = jnp.zeros((NT, HALO, 128), f32)
        vbig[...] = jnp.zeros(vbig.shape, u32)

        @pl.when(l == 1)
        def _():
            load_x(0, l, RB // LC)

        lax.fori_loop(0, S // RB, row_body, l)

        @pl.when(l == 0)
        def _():
            wob_copy.wait()
            prep_rhs(wob, list(range(NT)), wos, LO)

        lax.fori_loop(0, S // TQ, q_body, l)
        return carry

    x_copy(0).wait()
    load_x(0, 0, RB // LC)
    for i in range(NWO):
        woa_copy(i).wait()
        if i == NWO - 1:
            for cp in late:
                cp.start()
        lax.fori_loop(i * NT // NWO, (i + 1) * NT // NWO, prep_woa, 0)
    lax.fori_loop(0, 2, layer_pair, 0)
    for qb in range(S // TQ):
        for j in range(TQ // OC):
            out_copy(qb, j).wait()


@jax.jit
def pallas_interleave_layers__sliding_local_dilated__softmax_full_mha__prompt_kernel(
    A_x: jax.Array,
    A_wqkv: jax.Array,
    A_wo: jax.Array,
    B_x: jax.Array,
    B_wqkv: jax.Array,
    B_wo: jax.Array,
):
    del B_x
    x = A_x.reshape(S, D)
    hbm = pl.BlockSpec(memory_space=pl.ANY)
    out = pl.pallas_call(
        _kernel,
        out_shape=jax.ShapeDtypeStruct((S, D), bf16),
        in_specs=[hbm] * 5,
        out_specs=hbm,
        scratch_shapes=[
            pltpu.VMEM((S, D), bf16),
            pltpu.VMEM((D, 3 * D), bf16),
            pltpu.VMEM((D, D), bf16),
            pltpu.VMEM((D, 3 * D), bf16),
            pltpu.VMEM((D, D), bf16),
            pltpu.VMEM((S, D), bf16),
            pltpu.VMEM((3, (H + 1) * PITCH, 128), f32),
            pltpu.VMEM(((H + 2) * WPITCH, 128), u32),
            pltpu.VMEM((D // 2, 3 * D), u32),
            pltpu.VMEM((D // 2, D), u32),
            pltpu.VMEM((7 ** LB, D >> LB + 1, 2 * D >> LB), u32),
            pltpu.VMEM((7 ** LB, D >> LB + 1, D >> LB), u32),
            pltpu.VMEM((7 ** LO, D >> LO + 1, D >> LO), u32),
            pltpu.VMEM((RB // 2, D), u32),
            pltpu.VMEM((S + RB, D), f32),
            pltpu.VMEM((S, D), f32),
            pltpu.VMEM((NT, RB, 128), f32),
            pltpu.VMEM((NT, HALO + RB, 128), f32),
            pltpu.VMEM((NT, HALO + RB, 128), f32),
            pltpu.VMEM((D // 2, S), u32),
            pltpu.VMEM((NT, S // 2, 128), u32),
            pltpu.VMEM((D // 2, S), u32),
            pltpu.VMEM((NT + 1, S // 2, 128), u32),
            pltpu.VMEM((128, TQ), f32),
            pltpu.VMEM((KC // 2, TQ), u32),
            pltpu.VMEM((8, TQ), f32),
            pltpu.VMEM((8, TQ), f32),
            pltpu.VMEM((8, 128), u32),
            pltpu.SemaphoreType.DMA((S // RB,)),
            pltpu.SemaphoreType.DMA((NT,)),
            pltpu.SemaphoreType.DMA((2 + NWO,)),
            pltpu.SemaphoreType.DMA((S // OC,)),
        ],
        compiler_params=pltpu.CompilerParams(vmem_limit_bytes=120 * 1024 * 1024),
    )(x, A_wqkv, A_wo, B_wqkv, B_wo)
    return out.reshape(1, S, D)
```
